```python
import jax
import jax.numpy as jnp

def _softmax(x, axis=-1):
    return jax.nn.softmax(x, axis=axis)

def _gelu(x):
    return jax.nn.gelu(x, approximate=True)

def _silu(x):
    return jax.nn.silu(x)

def _sigmoid(x):
    return jax.nn.sigmoid(x)

def _layernorm(x, axis=-1, eps=1e-05):
    m = jnp.mean(x, axis=axis, keepdims=True)
    v = jnp.var(x, axis=axis, keepdims=True)
    return (x - m) / jnp.sqrt(v + eps)

def _scatter_add(tgt, idx, src, axis=0):
    return tgt.at[idx].add(src)

def _segment_sum(src, seg, n):
    return jax.ops.segment_sum(src, seg, n)

class _Rng:

    def __init__(self, key):
        self._k = key

    def _next(self):
        self._k, sub = jax.random.split(self._k)
        return sub

    def normal(self, shape):
        return jax.random.normal(self._next(), shape, dtype=jnp.bfloat16)

    def randint(self, lo, hi, shape):
        return jax.random.randint(self._next(), shape, lo, hi, dtype=jnp.int32)

    def uniform(self, shape, lo=0.0, hi=1.0):
        return jax.random.uniform(self._next(), shape, jnp.bfloat16, lo, hi)

    def permutation(self, n):
        return jax.random.permutation(self._next(), n)
kernel_name = 'adaLN_cond__gqa_block_cached__moe_arch_mod__prompt'

def setup_inputs():
    _rng = _Rng(jax.random.key(int.from_bytes(__import__("os").urandom(4), "little")))
    _w = lambda a: (lambda t: t.astype(jnp.bfloat16) if jnp.issubdtype(t.dtype, jnp.floating) else t)(jnp.asarray(a))

    def _A_setup():
        B, Sq, D = (1, 2048, 576)
        Hq, Hkv, Sk, Dh = (32, 16, 2048, 128)
        assert Hq % Hkv == 0, (Hq, Hkv)
        return {'x': _w((lambda *s: _rng.normal(s) * 0.05)(B, Sq, D)), 'k_cache': _w((lambda *s: _rng.normal(s) * 0.05)(B, Hkv, Sk, Dh)), 'v_cache': _w((lambda *s: _rng.normal(s) * 0.05)(B, Hkv, Sk, Dh)), 'wq': _w((lambda *s: _rng.normal(s) * 0.05)(D, Hq * Dh) * D ** (-0.5)), 'wo': _w((lambda *s: _rng.normal(s) * 0.05)(Hq * Dh, D) * (Hq * Dh) ** (-0.5))}
    _A_in = _A_setup()

    def _B_setup():
        B, S, D, F, C = (1, 2048, 576, 4608, 8)
        return {'x': _w((lambda *s: _rng.normal(s) * 0.05)(B, S, D)), 'w_r': _w((lambda *s: _rng.normal(s) * 0.05)(D)), 'w_gate': _w((lambda *s: _rng.normal(s) * 0.05)(D, F)), 'w_up': _w((lambda *s: _rng.normal(s) * 0.05)(D, F)), 'w_down': _w((lambda *s: _rng.normal(s) * 0.05)(F, D))}
    _B_in = _B_setup()
    return {'A_x': _A_in['x'], 'A_k_cache': _A_in['k_cache'], 'A_v_cache': _A_in['v_cache'], 'A_wq': _A_in['wq'], 'A_wo': _A_in['wo'], 'B_x': _B_in['x'], 'B_w_r': _B_in['w_r'], 'B_w_gate': _B_in['w_gate'], 'B_w_up': _B_in['w_up'], 'B_w_down': _B_in['w_down'], 'c': _w((lambda *s: _rng.normal(s) * 0.05)(1, 576)), 'w_mod': _w((lambda *s: _rng.normal(s) * 0.05)(576, 6 * 576) * 576 ** (-0.5))}

def reference(A_x, A_k_cache, A_v_cache, A_wq, A_wo, B_x, B_w_r, B_w_gate, B_w_up, B_w_down, c, w_mod):

    def _A_ref(x, k_cache, v_cache, wq, wo):
        B, Sq, D = x.shape
        Hq, Dh = (32, 128)
        Hkv = k_cache.shape[1]
        rep = Hq // Hkv
        q = (lambda x, *d: x.transpose(*d))((x @ wq).reshape(B, Sq, Hq, Dh), 0, 2, 1, 3)
        k = jnp.repeat(k_cache, rep, axis=1)
        v = jnp.repeat(v_cache, rep, axis=1)
        scores = jnp.einsum('bhqd,bhkd->bhqk', q, k) * Dh ** (-0.5)
        p = _softmax(scores, axis=-1)
        o = jnp.einsum('bhqk,bhkd->bhqd', p, v)
        return (lambda x, *d: x.transpose(*d))(o, 0, 2, 1, 3).reshape(B, Sq, Hq * Dh) @ wo

    def _B_ref(x, w_r, w_gate, w_up, w_down):
        B, S, D = x.shape
        C = 8
        r = x @ w_r
        idx = jnp.argsort(-r, axis=-1)[:, :C]
        idx_e = jnp.repeat(idx.reshape(B, C, 1), D, axis=2)
        x_sel = jnp.take_along_axis(x, idx_e, axis=1)
        g = _silu(x_sel @ w_gate)
        u = x_sel @ w_up
        y = g * u @ w_down
        r_sel = _sigmoid(jnp.take_along_axis(r, idx, axis=1))
        y = y * r_sel.reshape(B, C, 1)
        b_off = (jnp.arange(B) * S).reshape(B, 1)
        flat_idx = (idx + b_off).reshape(B * C)
        zero = (x * 0.0).reshape(B * S, D)
        upd = _scatter_add(zero, flat_idx, y.reshape(B * C, D), axis=0)
        return x + upd.reshape(B, S, D)
    x = A_x
    mod = (_silu(c) @ w_mod).reshape(c.shape[0], 6, 1, -1)
    sa, ca, ga, sb, cb, gb = (mod[:, 0].copy(), mod[:, 1].copy(), mod[:, 2].copy(), mod[:, 3].copy(), mod[:, 4].copy(), mod[:, 5].copy())
    h = _layernorm(x, axis=-1) * (1 + ca) + sa
    x = x + ga * _A_ref(h, A_k_cache, A_v_cache, A_wq, A_wo)
    h = _layernorm(x, axis=-1) * (1 + cb) + sb
    x = x + gb * _B_ref(h, B_w_r, B_w_gate, B_w_up, B_w_down)
    return x
```

```python
import functools
import math

import jax
import jax.numpy as jnp
import jax.experimental.pallas as pl
import jax.experimental.pallas.tpu as pltpu

S = 2048
D = 576
HQ = 32
HKV = 16
REP = HQ // HKV
DH = 128
F = 4608
C = 8
EPS = 1e-05
TQ = 256
UNROLL = 2

BF16 = jnp.bfloat16
F32 = jnp.float32


def _r(x):
    return x.astype(BF16).astype(F32)


def _adaln(x, shift, scale):
    mean = jnp.sum(x, axis=-1, keepdims=True) * (1.0 / D)
    xc = x - mean
    var = jnp.sum(xc * xc, axis=-1, keepdims=True) * (1.0 / D)
    d = _r(x - _r(mean))
    den = _r(jnp.sqrt(_r(_r(var) + EPS)))
    ln = _r(d / den)
    return _r(_r(ln * _r(1.0 + scale)) + shift)


def _kernel(x_ref, k_ref, v_ref, wq_ref, wo_ref, wr_ref, c_ref,
            wmod_hbm, wg_hbm, wu_hbm, wd_hbm,
            out_ref,
            h_ref, q_ref, o_ref, acc_ref, mod_ref, xsel_ref,
            wmod_v, wg_v, wu_v, wd_v, sems):
    g = pl.program_id(0)
    ng = pl.num_programs(0)

    cp_mod = pltpu.make_async_copy(wmod_hbm, wmod_v, sems.at[0])
    cp_g = pltpu.make_async_copy(wg_hbm, wg_v, sems.at[1])
    cp_u = pltpu.make_async_copy(wu_hbm, wu_v, sems.at[2])
    cp_d = pltpu.make_async_copy(wd_hbm, wd_v, sems.at[3])

    @pl.when(g == 0)
    def _():
        cp_mod.start()
        cp_g.start()
        cp_u.start()
        cp_d.start()
        cp_mod.wait()
        c = c_ref[...].astype(F32)
        sc = _r(c * _r(jax.nn.sigmoid(c)))
        sc8 = jnp.broadcast_to(sc, (8, D)).astype(BF16)
        for i in range(6):
            mod_ref[i] = _r(jnp.dot(sc8, wmod_v[:, i * D:(i + 1) * D],
                                    preferred_element_type=F32))
        sa = mod_ref[0][0:1, :]
        ca = mod_ref[1][0:1, :]

        def ln_body(i, carry):
            rows = pl.ds(pl.multiple_of(i * 256, 256), 256)
            h_ref[rows, :] = _adaln(x_ref[rows, :].astype(F32), sa, ca).astype(BF16)
            return carry
        jax.lax.fori_loop(0, S // 256, ln_body, 0)
        acc_ref[...] = jnp.zeros_like(acc_ref)

    qscale = DH ** -0.5 * math.log2(math.e)
    q = jnp.dot(h_ref[...], wq_ref[...], preferred_element_type=F32) * qscale
    for r in range(REP):
        q_ref[r * S:(r + 1) * S, :] = q[:, r * DH:(r + 1) * DH].astype(BF16)

    nblk = S // TQ

    def attn_body(j, carry):
        rows = pl.ds(pl.multiple_of(j * TQ, TQ), TQ)
        for r in range(REP):
            qb = q_ref[pl.ds(pl.multiple_of(r * S + j * TQ, TQ), TQ), :]
            s = jax.lax.dot_general(qb, k_ref[0], (((1,), (1,)), ((), ())),
                                    preferred_element_type=F32)
            m = jnp.max(s, axis=-1, keepdims=True)
            p = jnp.exp2(s - m)
            l = jnp.sum(p, axis=-1, keepdims=True)
            o = jnp.dot(p.astype(BF16), v_ref[0], preferred_element_type=F32)
            o_ref[rows, r * DH:(r + 1) * DH] = (o / l).astype(BF16)
        return carry
    jax.lax.fori_loop(0, nblk, attn_body, 0, unroll=UNROLL)

    acc_ref[...] += jnp.dot(o_ref[...], wo_ref[...], preferred_element_type=F32)

    @pl.when(g == ng - 1)
    def _():
        ga = mod_ref[2][0:1, :]
        sb = mod_ref[3][0:1, :]
        cb = mod_ref[4][0:1, :]
        gb = mod_ref[5][0:1, :]

        def fin_body(i, carry):
            rows = pl.ds(pl.multiple_of(i * 256, 256), 256)
            x1 = _r(x_ref[rows, :].astype(F32) + _r(ga * _r(acc_ref[rows, :])))
            h2 = _adaln(x1, sb, cb)
            acc_ref[rows, :] = x1
            h_ref[rows, :] = h2.astype(BF16)
            out_ref[rows, :] = (x1 + _r(gb * h2)).astype(BF16)
            return carry
        jax.lax.fori_loop(0, S // 256, fin_body, 0)

        wr8 = jnp.broadcast_to(wr_ref[...].astype(F32), (8, D)).astype(BF16)
        r = jax.lax.dot_general(wr8, h_ref[...], (((1,), (1,)), ((), ())),
                                preferred_element_type=F32)
        r = _r(r[0:1, :])
        lane = jax.lax.broadcasted_iota(jnp.int32, (1, S), 1)
        row16 = jax.lax.broadcasted_iota(jnp.int32, (16, D), 0)
        row8 = jax.lax.broadcasted_iota(jnp.int32, (8, 1), 0)
        idxs = []
        rsel = jnp.zeros((8, 1), F32)
        work = r
        for t in range(C):
            mx = jnp.max(work, axis=-1, keepdims=True)
            cand = jnp.where(work == mx, lane, S)
            iv = jnp.min(cand, axis=-1, keepdims=True)
            work = jnp.where(lane == iv, -jnp.inf, work)
            rsel = jnp.where(row8 == t, mx, rsel)
            idx = jnp.clip(iv[0, 0], 0, S - 1)
            idxs.append(idx)
            base = pl.multiple_of((idx // 16) * 16, 16)
            blk = h_ref[pl.ds(base, 16), :].astype(F32)
            xsel_ref[t:t + 1, :] = jnp.sum(jnp.where(row16 == idx - base, blk, 0.0),
                                           axis=0, keepdims=True)
        cp_g.wait()
        cp_u.wait()
        cp_d.wait()
        xs = xsel_ref[...].astype(BF16)
        gpre = _r(jnp.dot(xs, wg_v[...], preferred_element_type=F32))
        gact = _r(gpre * _r(jax.nn.sigmoid(gpre)))
        u = _r(jnp.dot(xs, wu_v[...], preferred_element_type=F32))
        y = _r(jnp.dot((gact * u).astype(BF16), wd_v[...], preferred_element_type=F32))
        y = _r(y * _r(jax.nn.sigmoid(rsel)))
        for t in range(C):
            idx = idxs[t]
            base = pl.multiple_of((idx // 16) * 16, 16)
            rows = pl.ds(base, 16)
            x1 = acc_ref[rows, :]
            h2 = h_ref[rows, :].astype(F32)
            new = x1 + _r(gb * _r(h2 + y[t:t + 1, :]))
            out_ref[rows, :] = jnp.where(row16 == idx - base, new,
                                         out_ref[rows, :].astype(F32)).astype(BF16)


@jax.jit
def pallas_adaLN_cond__gqa_block_cached__moe_arch_mod__prompt_kernel(
    A_x: jax.Array,
    A_k_cache: jax.Array,
    A_v_cache: jax.Array,
    A_wq: jax.Array,
    A_wo: jax.Array,
    B_x: jax.Array,
    B_w_r: jax.Array,
    B_w_gate: jax.Array,
    B_w_up: jax.Array,
    B_w_down: jax.Array,
    c: jax.Array,
    w_mod: jax.Array,
):
    del B_x
    x = A_x.reshape(S, D)
    k = A_k_cache.reshape(HKV, S, DH)
    v = A_v_cache.reshape(HKV, S, DH)
    wr = B_w_r.reshape(1, D)

    const2 = lambda g: (0, 0)
    out = pl.pallas_call(
        _kernel,
        grid=(HKV,),
        in_specs=[
            pl.BlockSpec((S, D), const2),
            pl.BlockSpec((1, S, DH), lambda g: (g, 0, 0)),
            pl.BlockSpec((1, S, DH), lambda g: (g, 0, 0)),
            pl.BlockSpec((D, REP * DH), lambda g: (0, g)),
            pl.BlockSpec((REP * DH, D), lambda g: (g, 0)),
            pl.BlockSpec((1, D), const2),
            pl.BlockSpec((1, D), const2),
            pl.BlockSpec(memory_space=pl.ANY),
            pl.BlockSpec(memory_space=pl.ANY),
            pl.BlockSpec(memory_space=pl.ANY),
            pl.BlockSpec(memory_space=pl.ANY),
        ],
        out_specs=pl.BlockSpec((S, D), const2),
        out_shape=jax.ShapeDtypeStruct((S, D), BF16),
        scratch_shapes=[
            pltpu.VMEM((S, D), BF16),
            pltpu.VMEM((REP * S, DH), BF16),
            pltpu.VMEM((S, REP * DH), BF16),
            pltpu.VMEM((S, D), F32),
            pltpu.VMEM((6, 8, D), F32),
            pltpu.VMEM((C, D), F32),
            pltpu.VMEM((D, 6 * D), BF16),
            pltpu.VMEM((D, F), BF16),
            pltpu.VMEM((D, F), BF16),
            pltpu.VMEM((F, D), BF16),
            pltpu.SemaphoreType.DMA((4,)),
        ],
        compiler_params=pltpu.CompilerParams(
            dimension_semantics=("arbitrary",),
            vmem_limit_bytes=100 * 1024 * 1024,
        ),
    )(x, k, v, A_wq, A_wo, wr, c, w_mod, B_w_gate, B_w_up, B_w_down)
    return out.reshape(1, S, D)
```

```python
import math

import jax
import jax.numpy as jnp
import jax.experimental.pallas as pl
import jax.experimental.pallas.tpu as pltpu

S = 2048
D = 576
HQ = 32
HKV = 16
REP = HQ // HKV
DH = 128
GW = REP * DH
F = 4608
C = 8
EPS = 1e-05
TQ = 512
NBLK = S // TQ
TPB = TQ // 128
NT = S // 128
NIT = NBLK * HKV
DA = 2 * D
NC = 3
DC = D // NC
P0, P1 = 1280, 512
PG = 64

BF16 = jnp.bfloat16
F32 = jnp.float32
QSCALE = DH ** -0.5 * math.log2(math.e)


def _dot(a, b):
    return jnp.dot(a, b, preferred_element_type=F32)


def _dot_nt(a, b):
    return jax.lax.dot_general(a, b, (((1,), (1,)), ((), ())), preferred_element_type=F32)


def _r(x):
    return x.astype(BF16).astype(F32)


def _col_bcast(row):
    return jnp.broadcast_to(row, (128, 128)).T


def _after(x, m, s0):
    never = m < s0
    mask = never[:, 0:128]
    for i in range(1, m.shape[1] // 128):
        mask = jnp.logical_or(mask, never[:, i * 128:(i + 1) * 128])
    top = x[0:16, 0:128].astype(F32)
    top = jnp.concatenate([jnp.where(mask, 0.0, top[0:8]), top[8:16]], axis=0).astype(BF16)
    top = jnp.concatenate([top, x[0:16, 128:]], axis=1)
    return jnp.concatenate([top, x[16:]], axis=0)


def _paced(x, clock, pos):
    if clock is None:
        return x
    g = clock[pos:pos + x.shape[0], 0:128]
    return jnp.where(g * g < 0.0, g, x)


def _softmax_numer(s, m):
    n, w = s.shape
    p = jnp.exp2(s - m).reshape(n // PG, PG // 8, 8, w)
    ts = jnp.sum(p, axis=1)
    last = jnp.where(ts < 0.0, ts, p[:, PG // 8 - 1])
    p = jnp.concatenate([p[:, :PG // 8 - 1], last[:, None]], axis=1).reshape(n, w)
    l = jnp.sum(jnp.sum(ts, axis=0), axis=0, keepdims=True)
    return p.astype(BF16), l


def _colmax(x, chains):
    n, w = x.shape
    x = jnp.max(x.reshape(n // (8 * chains), 8 * chains, w), axis=0)
    n = 8 * chains
    while n > 8:
        n //= 2
        lo, hi = x[:n], x[n:]
        x = jnp.where(lo > hi, lo, hi)
    return jnp.max(x, axis=0, keepdims=True)


def _kernel(wr_ref, c_ref,
            xt_hbm, k_hbm, v_hbm, wq_hbm, wot_hbm, wmod_hbm, wg_hbm, wu_hbm, wdt_hbm,
            out_hbm,
            x_v, k_v, v_v, wq_v, wot_v, wmod_v, wg_v, wu_v, wdt_v,
            h_ref, vt_ref, s_ref, o_ref, acc_ref, mod_ref, wrb_ref,
            x1_ref, h2_ref, out_v, r_ref, st_ref,
            gsem, msem, osem):

    def cp_x(t, sem):
        return pltpu.make_async_copy(xt_hbm.at[:, pl.ds(pl.multiple_of(t * 128, 128), 128)],
                                     x_v.at[t], sem)

    def group_copies(n):
        cols = pl.ds(pl.multiple_of(n * GW, GW), GW)
        sem = gsem.at[n]
        return [pltpu.make_async_copy(wq_hbm.at[:, cols], wq_v.at[n], sem),
                pltpu.make_async_copy(k_hbm.at[n], k_v.at[n], sem),
                pltpu.make_async_copy(v_hbm.at[n], v_v.at[n], sem),
                pltpu.make_async_copy(wot_hbm.at[:, cols], wot_v.at[n], sem)]

    cp_moda = pltpu.make_async_copy(wmod_hbm.at[:, 0:DA], wmod_v.at[:, 0:DA], msem.at[0])
    cp_modb = pltpu.make_async_copy(wmod_hbm.at[:, DA:6 * D], wmod_v.at[:, DA:6 * D], msem.at[1])
    cp_g = pltpu.make_async_copy(wg_hbm, wg_v, msem.at[2])
    cp_u = pltpu.make_async_copy(wu_hbm, wu_v, msem.at[3])
    cp_d = pltpu.make_async_copy(wdt_hbm, wdt_v, msem.at[4])
    x_first = [cp_x(t, msem.at[5]) for t in range(TPB)]
    x_rest = [cp_x(t, msem.at[6]) for t in range(TPB, NT)]

    def cp_out(t):
        return pltpu.make_async_copy(out_v.at[t],
                                     out_hbm.at[:, pl.ds(pl.multiple_of(t * 128, 128), 128)],
                                     osem.at[t])

    def mod_part(lo, hi):
        c = c_ref[...].astype(F32)
        sc = _r(c * _r(jax.nn.sigmoid(c)))
        sc8 = jnp.broadcast_to(sc, (8, D)).astype(BF16)
        mod = _r(_dot(sc8, wmod_v[:, lo:hi]))
        for t in range((hi - lo) // 128):
            mod_ref[lo + t * 128:lo + (t + 1) * 128, :] = _col_bcast(mod[0:1, t * 128:(t + 1) * 128])

    def ln1_tile(t):
        x = x_v[t].astype(F32)
        mean = jnp.sum(x, axis=0, keepdims=True) * (1.0 / D)
        xc = x - mean
        var = jnp.sum(xc * xc, axis=0, keepdims=True) * (1.0 / D)
        h = xc * jax.lax.rsqrt(var + EPS) * mod_ref[D:2 * D, :] + mod_ref[0:D, :]
        h_ref[pl.ds(pl.multiple_of(t * 128, 128), 128), :] = h.astype(BF16).T

    def ln2_stats(t, c, clock=None):
        rows = pl.ds(pl.multiple_of(c * DC, 16), DC)
        acc = acc_ref[t, rows, :]
        ga = mod_ref[pl.ds(pl.multiple_of(2 * D + c * DC, 8), DC), :]
        x1 = _r(x_v[t, rows, :].astype(F32) + _r(ga * _r(acc)))
        x1_ref[t, rows, :] = _paced(x1, clock, P0).astype(BF16)
        mc = jnp.sum(x1, axis=0, keepdims=True) * (1.0 / DC)
        xc = x1 - mc
        m2 = jnp.sum(xc * xc, axis=0, keepdims=True)
        st_ref[t, pl.ds(c, 1), :] = _paced(mc, clock, P0 + DC + 64)
        st_ref[t, pl.ds(NC + c, 1), :] = _paced(m2, clock, P0 + DC + 128)

    def ln2_apply(t, c, clock=None):
        rows = pl.ds(pl.multiple_of(c * DC, 16), DC)
        mrow = lambda k: mod_ref[pl.ds(pl.multiple_of(k * D + c * DC, 8), DC), :]
        st = st_ref[t]
        mc, m2 = st[0:NC], st[NC:2 * NC]
        mean = jnp.sum(mc, axis=0, keepdims=True) * (1.0 / NC)
        dm = mc - mean
        var = jnp.sum(m2 + DC * (dm * dm), axis=0, keepdims=True) * (1.0 / D)
        den = _r(jnp.sqrt(_r(_r(var) + EPS)))
        x1 = x1_ref[t, rows, :].astype(F32)
        ln = _r(_r(x1 - _r(mean)) / den)
        h2 = _r(_r(ln * mrow(4)) + mrow(3))
        h2_ref[t, rows, :] = _paced(h2, clock, P1).astype(BF16)
        out_v[t, rows, :] = _paced(x1 + _r(mrow(5) * h2), clock, P1 + 16).astype(BF16)
        wr = wrb_ref[pl.ds(pl.multiple_of(c * DC, 8), DC), :]
        rp = jnp.sum(h2 * wr, axis=0, keepdims=True)
        r_ref[c, pl.ds(t, 1), :] = _paced(rp, clock, P1 + DC + 64)

    def q_proj(i, tie=None):
        g, j = i % HKV, i // HKV
        half = TQ // 2
        q = []
        for r in range(REP):
            for a in range(2):
                hb = h_ref[pl.ds(pl.multiple_of(j * TQ + a * half, half), half), :]
                if tie is not None and (r, a) == (1, 0):
                    hb = _after(hb, *tie)
                q.append((_dot(hb, wq_v[g, :, r * DH:(r + 1) * DH]) * QSCALE).astype(BF16))
        return jnp.concatenate(q, axis=0)

    def scores(i, q):
        s = _dot_nt(k_v[i % HKV], q)
        s_ref[...] = s
        return s

    def v_transpose(i):
        vt_ref[i % 2] = v_v[i % HKV].T

    def pv(i, r, m):
        p, l = _softmax_numer(s_ref[:, r * TQ:(r + 1) * TQ], m)
        o_ref[r * DH:(r + 1) * DH, :] = (_dot(vt_ref[i % 2], p) * (1.0 / l)).astype(BF16)
        return l

    def out_proj(i, o, tie=None):
        g, j = i % HKV, i // HKV
        w = wot_v[g]
        half = TPB // 2
        for a in range(2):
            if tie is not None and a == 1:
                w = _after(w, *tie)
            upd = _dot(w, o[:, a * half * 128:(a + 1) * half * 128])
            for b in range(half):
                acc_ref[j * TPB + a * half + b] += upd[:, b * 128:(b + 1) * 128]

    for cp in x_first:
        cp.start()
    cp_moda.start()
    for cp in x_first:
        cp.wait()
    for cp in group_copies(0):
        cp.start()
    for cp in x_rest:
        cp.start()
    cp_moda.wait()
    mod_part(0, DA)
    mod_ref[D:2 * D, :] = _r(1.0 + mod_ref[D:2 * D, :])
    for t in range(TPB):
        ln1_tile(t)
    for cp in group_copies(0):
        cp.wait()
    for n in range(1, 3):
        for cp in group_copies(n):
            cp.start()
    q = q_proj(0)
    s_ref[:, 0:TQ] = _dot_nt(k_v[0], q[0:TQ])
    v_transpose(0)
    acc_ref[...] = jnp.zeros_like(acc_ref)
    o_ref[...] = jnp.zeros_like(o_ref)
    st_ref[...] = jnp.zeros_like(st_ref)
    x1_ref[0] = jnp.zeros((D, 128), BF16)
    mod_ref[DA:6 * D, :] = jnp.zeros((4 * D, 128), F32)
    wr = jnp.concatenate([wr_ref[...].astype(F32), jnp.zeros((1, 64), F32)], axis=1)
    for t in range(5):
        wrb_ref[t * 128:(t + 1) * 128, :] = _col_bcast(wr[:, t * 128:(t + 1) * 128])
    for cp in x_rest:
        cp.wait()
    s_ref[:, TQ:] = _dot_nt(k_v[0], q[TQ:])
    for t in range(TPB, NT):
        ln1_tile(t)

    LAG = HKV + 1

    def step(i, carry):
        @pl.when(i < HKV)
        def _():
            @pl.when(i + 1 < HKV)
            def _():
                for cp in group_copies(i + 1):
                    cp.wait()

            @pl.when(i + 3 < HKV)
            def _():
                for cp in group_copies(i + 3):
                    cp.start()

            @pl.when(i == 1)
            def _():
                cp_modb.start()

            @pl.when(i == 8)
            def _():
                cp_modb.wait()
                mod_part(DA, 6 * D)
                mod_ref[4 * D:5 * D, :] = _r(1.0 + mod_ref[4 * D:5 * D, :])

            @pl.when(i == HKV - 1)
            def _():
                cp_g.start()
                cp_u.start()
                cp_d.start()

        m = [_colmax(s_ref[:, r * TQ:(r + 1) * TQ], 1) for r in range(REP)]
        s0 = [s_ref[0:8, r * TQ:(r + 1) * TQ] for r in range(REP)]
        out_proj(jnp.maximum(i - 1, 0), o_ref[...], tie=(m[0], s0[0]))
        q = q_proj(i + 1, tie=(m[1], s0[1]))
        for r in range(REP):
            pv(i, r, m[r])
        n = jnp.maximum(i - LAG, 0)
        base, slot = (n // HKV) * TPB, n % HKV
        sa = jnp.minimum(slot, TPB * NC - 1)
        sc = jnp.clip(slot - NC, 0, TPB * NC - 1)
        sn = scores(i + 1, q)
        ln2_apply(base + sc // NC, sc % NC, sn)
        ln2_stats(base + sa // NC, sa % NC, sn)
        v_transpose(i + 1)
        return carry

    jax.lax.fori_loop(0, NIT - 1, step, 0)

    last = NIT - 1
    for t in range(NT - TPB - 1):
        cp_out(t).start()
    ln2_apply(NT - TPB - 1, NC - 1)
    cp_out(NT - TPB - 1).start()
    m = [_colmax(s_ref[:, r * TQ:(r + 1) * TQ], 4) for r in range(REP)]
    out_proj(last - 1, o_ref[...])
    for r in range(REP):
        pv(last, r, m[r])
    out_proj(last, o_ref[...])
    for t in range(NT - TPB, NT):
        for c in range(NC):
            ln2_stats(t, c)
        for c in range(NC):
            ln2_apply(t, c)

    r = _r(r_ref[0] + r_ref[1] + r_ref[2]) + 0.0
    tok = (jax.lax.broadcasted_iota(jnp.int32, (NT, 128), 0) * 128
           + jax.lax.broadcasted_iota(jnp.int32, (NT, 128), 1))
    bits = jax.lax.shift_right_arithmetic(pltpu.bitcast(r, jnp.int32), 16)
    code = jnp.where(bits < 0, -32769 - bits, bits) + 32768
    work = pltpu.bitcast(code * S + (S - 1 - tok) + 0x20000000, F32)
    row16 = jax.lax.broadcasted_iota(jnp.int32, (16, 128), 0)
    lane16 = jax.lax.broadcasted_iota(jnp.int32, (16, 128), 1)
    sel = jnp.full((16, 128), 0x20000000, jnp.int32)
    tiles = []
    for t in range(C):
        mx = jnp.max(jnp.max(work, axis=0, keepdims=True), axis=1, keepdims=True)
        work = jnp.where(work == mx, 0.0, work)
        mxi = pltpu.bitcast(mx, jnp.int32)
        sel = jnp.where(row16 == t, mxi, sel)
        tiles.append(((S - 1) - (mxi[0, 0] & (S - 1))) // 128)
    sel = sel - 0x20000000
    sel_tok = jnp.where(row16 < C, (S - 1) - (sel & (S - 1)), -1)
    sel_code = jax.lax.shift_right_logical(sel, 11) - 32768
    sel_bits = jnp.where(sel_code < 0, -32769 - sel_code, sel_code)
    r_sel = jnp.where(row16 < C, pltpu.bitcast(jax.lax.shift_left(sel_bits, 16), F32), 0.0)[:, 0:1]

    def dirty(t):
        d = tiles[0] == t
        for u in range(1, C):
            d = jnp.logical_or(d, tiles[u] == t)
        return d

    for t in range(NT - TPB, NT):
        @pl.when(jnp.logical_not(dirty(t)))
        def _():
            cp_out(t).start()

    xs = jnp.zeros((16, D), F32)
    for t in range(C):
        oh = jnp.where(jnp.logical_and(sel_tok == tiles[t] * 128 + lane16, row16 == t), 1.0, 0.0)
        xs = xs + _dot_nt(oh.astype(BF16), h2_ref[tiles[t]])
    xs = xs.astype(BF16)

    cp_g.wait()
    cp_u.wait()
    cp_d.wait()
    gpre = _r(_dot(xs, wg_v[...]))
    gact = _r(gpre * _r(jax.nn.sigmoid(gpre)))
    u = _r(_dot(xs, wu_v[...]))
    y = _r(_dot_nt((gact * u).astype(BF16), wdt_v[...]))
    y = (y * _r(jax.nn.sigmoid(r_sel))).astype(BF16)

    for t in range(NT - TPB):
        cp_out(t).wait()
    for t in range(C):
        oh = jnp.where(sel_tok == tiles[t] * 128 + lane16, 1.0, 0.0).astype(BF16)
        upd = jax.lax.dot_general(y, oh, (((0,), (0,)), ((), ())), preferred_element_type=F32)
        out_v[tiles[t]] = (x1_ref[tiles[t]].astype(F32)
                           + _r(mod_ref[5 * D:6 * D, :]
                                * _r(h2_ref[tiles[t]].astype(F32) + upd))).astype(BF16)
    for t in range(NT):
        @pl.when(dirty(t))
        def _():
            cp_out(t).start()
    for t in range(NT):
        if t >= NT - TPB:
            cp_out(t).wait()
        else:
            @pl.when(dirty(t))
            def _():
                cp_out(t).wait()


@jax.jit
def pallas_adaLN_cond__gqa_block_cached__moe_arch_mod__prompt_kernel(
    A_x: jax.Array,
    A_k_cache: jax.Array,
    A_v_cache: jax.Array,
    A_wq: jax.Array,
    A_wo: jax.Array,
    B_x: jax.Array,
    B_w_r: jax.Array,
    B_w_gate: jax.Array,
    B_w_up: jax.Array,
    B_w_down: jax.Array,
    c: jax.Array,
    w_mod: jax.Array,
):
    del B_x
    xt = A_x.reshape(S, D).T
    k = A_k_cache.reshape(HKV, S, DH)
    v = A_v_cache.reshape(HKV, S, DH)
    wr = B_w_r.reshape(1, D)

    hbm = pl.BlockSpec(memory_space=pl.ANY)
    vmem = pl.BlockSpec(memory_space=pltpu.VMEM)
    out = pl.pallas_call(
        _kernel,
        in_specs=[vmem, vmem] + [hbm] * 9,
        out_specs=hbm,
        out_shape=jax.ShapeDtypeStruct((D, S), BF16),
        scratch_shapes=[
            pltpu.VMEM((NT, D, 128), BF16),
            pltpu.VMEM((HKV, S, DH), BF16),
            pltpu.VMEM((HKV, S, DH), BF16),
            pltpu.VMEM((HKV, D, GW), BF16),
            pltpu.VMEM((HKV, D, GW), BF16),
            pltpu.VMEM((D, 6 * D), BF16),
            pltpu.VMEM((D, F), BF16),
            pltpu.VMEM((D, F), BF16),
            pltpu.VMEM((D, F), BF16),
            pltpu.VMEM((S, D), BF16),
            pltpu.VMEM((2, DH, S), BF16),
            pltpu.VMEM((S, REP * TQ), F32),
            pltpu.VMEM((GW, TQ), BF16),
            pltpu.VMEM((NT, D, 128), F32),
            pltpu.VMEM((6 * D, 128), F32),
            pltpu.VMEM((5 * 128, 128), F32),
            pltpu.VMEM((NT, D, 128), BF16),
            pltpu.VMEM((NT, D, 128), BF16),
            pltpu.VMEM((NT, D, 128), BF16),
            pltpu.VMEM((NC, NT, 128), F32),
            pltpu.VMEM((NT, 8, 128), F32),
            pltpu.SemaphoreType.DMA((HKV,)),
            pltpu.SemaphoreType.DMA((7,)),
            pltpu.SemaphoreType.DMA((NT,)),
        ],
        compiler_params=pltpu.CompilerParams(vmem_limit_bytes=110 * 1024 * 1024),
    )(wr, c, xt, k, v, A_wq, A_wo.T, w_mod, B_w_gate, B_w_up, B_w_down.T)
    return out.T.reshape(1, S, D)
```

```python
import math

import jax
import jax.numpy as jnp
import jax.experimental.pallas as pl
import jax.experimental.pallas.tpu as pltpu

S = 2048
D = 576
HQ = 32
HKV = 16
REP = HQ // HKV
DH = 128
GW = REP * DH
F = 4608
C = 8
EPS = 1e-05
TQ = 512
NBLK = S // TQ
TPB = TQ // 128
NT = S // 128
NU = NBLK * HKV
DA = 2 * D
NC = 3
DC = D // NC
PG = 64
NFB = F // 128
WD0 = 24
PACE = (1280, 304, 304, 1024)

BF16 = jnp.bfloat16
F32 = jnp.float32
U32 = jnp.uint32
QSCALE = DH ** -0.5 * math.log2(math.e)


def _dot(a, b):
    return jnp.dot(a, b, preferred_element_type=F32)


def _dot_nt(a, b):
    return jax.lax.dot_general(a, b, (((1,), (1,)), ((), ())), preferred_element_type=F32)


def _r(x):
    return x.astype(BF16).astype(F32)


def _col_bcast(row):
    return jnp.broadcast_to(row, (128, 128)).T


def _blk(u):
    return u // HKV if isinstance(u, int) else jax.lax.shift_right_logical(u, 4)


def _grp(u):
    return u % HKV if isinstance(u, int) else jnp.bitwise_and(u, HKV - 1)


def _lanes(t, n=1):
    return pl.ds(pl.multiple_of(t * 128, 128), n * 128)


def _paced(x, clock, pos):
    if clock is None:
        return x
    row, col = pos % S, (pos // S) * TQ
    g = clock[row:row + x.shape[0], col:col + 128]
    return jnp.where(g * g < 0.0, g, x)


def _softmax_numer(s, m):
    n, w = s.shape
    p = jnp.exp2(s - m).reshape(n // PG, PG // 8, 8, w)
    ts = jnp.sum(p, axis=1)
    last = jnp.where(ts < 0.0, ts, p[:, PG // 8 - 1])
    p = jnp.concatenate([p[:, :PG // 8 - 1], last[:, None]], axis=1).reshape(n, w)
    l = jnp.sum(jnp.sum(ts, axis=0), axis=0, keepdims=True)
    return p.astype(BF16), l


def _chunk_stats(x):
    m = jnp.sum(x, axis=0, keepdims=True) * (1.0 / DC)
    xc = x - m
    return m, jnp.sum(xc * xc, axis=0, keepdims=True)


def _mean_var(stats):
    mean = sum(m for m, _ in stats) * (1.0 / NC)
    var = sum(s + DC * (m - mean) * (m - mean) for m, s in stats) * (1.0 / D)
    return mean, var


def _kernel(wr_ref, c_ref,
            xt_hbm, k_hbm, v_hbm, wq_hbm, wot_hbm, wmod_hbm, wg_hbm, wu_hbm, wdt_hbm,
            out_hbm,
            xw_v, k_v, v_v, wq_v, wot_v, wmod_v, wg_v, wu_v, wd_ref,
            ht_ref, acc_ref, mod_ref, wrb_ref, x1_ref, h2_ref, out_v, r_ref, st1_ref, st2_ref,
            s0_ref, m0_ref, vt0_ref, wqt0_ref, s1_ref, m1_ref, vt1_ref, wqt1_ref,
            bsem, msem, osem):
    streams = ((s0_ref, m0_ref, vt0_ref, wqt0_ref), (s1_ref, m1_ref, vt1_ref, wqt1_ref))

    def cp_cols(src, dst, t, n, sem, dst_t=None):
        return pltpu.make_async_copy(src.at[:, _lanes(t, n)],
                                     dst.at[:, _lanes(t if dst_t is None else dst_t, n)], sem)

    def cp_pair(src, dst, p, sem):
        return pltpu.make_async_copy(src.at[pl.ds(2 * p, 2)], dst.at[pl.ds(2 * p, 2)], sem)

    cp_k = lambda p, sem: cp_pair(k_hbm, k_v, p, sem)
    cp_v = lambda p, sem: cp_pair(v_hbm, v_v, p, sem)

    class Both:
        def __init__(self, cps):
            self.cps = cps

        def start(self):
            for cp in self.cps:
                cp.start()

        def wait(self):
            for cp in self.cps:
                cp.wait()

    def cp_w(src, dst, p, sem):
        return Both([pltpu.make_async_copy(src.at[:, _lanes((2 * p + a) * REP, REP)],
                                           dst.at[2 * p + a], sem) for a in range(2)])

    cp_wq = lambda p, sem: cp_w(wq_hbm, wq_v, p, sem)
    cp_wo = lambda p, sem: cp_w(wot_hbm, wot_v, p, sem)
    cp_x = lambda j, sem: Both([pltpu.make_async_copy(xt_hbm.at[:, _lanes(TPB * j + t)],
                                                      xw_v.at[TPB * j + t], sem) for t in range(TPB)])
    NP = HKV // 2

    def bundle(n, act):
        sem = bsem.at[n]

        def on(cond, cps):
            def go():
                for cp in cps():
                    getattr(cp, act)()
            if isinstance(cond, bool):
                if cond:
                    go()
            else:
                pl.when(cond)(go)
        on(n + 1 < NP, lambda: [cp_k(n + 1, sem), cp_v(n + 1, sem)])
        on(n + 2 < NP, lambda: [cp_wq(n + 2, sem)])
        on(jnp.logical_and(n >= 1, n < NBLK) if not isinstance(n, int) else 1 <= n < NBLK, lambda: [cp_x(n, sem)])
        on(True, lambda: [cp_wo(n, sem)])

    cp_moda = cp_cols(wmod_hbm, wmod_v, 0, DA // 128, msem.at[0])
    cp_modb = cp_cols(wmod_hbm, wmod_v, DA // 128, 4 * D // 128, msem.at[1])
    cp_g = pltpu.make_async_copy(wg_hbm, wg_v, msem.at[2])
    cp_u = pltpu.make_async_copy(wu_hbm, wu_v, msem.at[3])
    cp_d = Both([pltpu.make_async_copy(wdt_hbm.at[:, _lanes(b)], xw_v.at[NT + b], msem.at[4])
                 for b in range(NFB)])
    cp_out = lambda t, n, sem: Both([pltpu.make_async_copy(out_v.at[t + a], out_hbm.at[:, _lanes(t + a)],
                                                           sem) for a in range(n)])

    def mod_part(lo, hi):
        c = c_ref[...].astype(F32)
        sc = _r(c * _r(jax.nn.sigmoid(c)))
        sc8 = jnp.broadcast_to(sc, (8, D)).astype(BF16)
        mod = _r(_dot(sc8, wmod_v[:, lo:hi]))[0:1]
        col = lo + jax.lax.broadcasted_iota(jnp.int32, mod.shape, 1)
        is_scale = jnp.logical_or(jnp.logical_and(col >= D, col < 2 * D),
                                  jnp.logical_and(col >= 4 * D, col < 5 * D))
        mod = jnp.where(is_scale, _r(1.0 + mod), mod)
        for t in range((hi - lo) // 128):
            mod_ref[lo + t * 128:lo + (t + 1) * 128, :] = _col_bcast(mod[:, t * 128:(t + 1) * 128])

    def mod(k):
        return mod_ref[k * D:(k + 1) * D, :]

    def put_stats(st_ref, t, shift, scale, clock, pos):
        row = jax.lax.broadcasted_iota(jnp.int32, (8, 128), 0)
        st_ref[t] = _paced(jnp.where(row == 0, shift, scale), clock, pos)

    def ln1_stats(t, clock=None):
        for c in range(NC):
            m, s = _chunk_stats(xw_v[t, c * DC:(c + 1) * DC, :].astype(F32))
            put_stats(st1_ref, t * NC + c, m, s, clock, PACE[0] + 192 * c)

    def ln1_apply(t, clock=None):
        mean, var = _mean_var([(st1_ref[t * NC + c, 0:1, :], st1_ref[t * NC + c, 1:2, :])
                               for c in range(NC)])
        h = (xw_v[t].astype(F32) - mean) * jax.lax.rsqrt(var + EPS) * mod(1) + mod(0)
        ht_ref[t] = _paced(h, clock, PACE[1]).astype(BF16)

    def ln2_stats(t, clock=None):
        x1 = _r(xw_v[t].astype(F32) + mod(2) * acc_ref[t])
        x1_ref[t] = _paced(x1, clock, PACE[2]).astype(BF16)
        mean, var = _mean_var([_chunk_stats(x1[c * DC:(c + 1) * DC]) for c in range(NC)])
        put_stats(st2_ref, t, _r(mean), 1.0 / _r(jnp.sqrt(_r(_r(var) + EPS))), clock, PACE[2] + D + 128)

    def ln2_apply(t, clock=None):
        x1 = x1_ref[t].astype(F32)
        h2 = _r((x1 - st2_ref[t, 0:1, :]) * st2_ref[t, 1:2, :] * mod(4) + mod(3))
        h2_ref[t] = _paced(h2, clock, PACE[3]).astype(BF16)
        out_v[t] = _paced(x1 + mod(5) * h2, clock, PACE[3] + 16).astype(BF16)
        rp = jnp.sum(h2 * wrb_ref[0:D, :], axis=0, keepdims=True)
        r_ref[pl.ds(t, 1), :] = _paced(rp, clock, PACE[3] + D + 64)

    def q_proj(u, wqt_ref):
        q = _dot(pltpu.bitcast(wqt_ref[...], BF16), jnp.concatenate([ht_ref[_blk(u) * TPB + t] for t in range(TPB)], axis=1))
        q = (q * QSCALE).astype(BF16)
        return jnp.concatenate([q[r * DH:(r + 1) * DH] for r in range(REP)], axis=1)

    def scores(u, q, s_ref, m_ref):
        s = _dot(k_v[_grp(u)], q)
        s_ref[...] = s
        m_ref[...] = jnp.broadcast_to(jnp.max(s, axis=0, keepdims=True), m_ref.shape)
        return s

    def v_transpose(u, vt_ref):
        vt_ref[...] = pltpu.bitcast(v_v[_grp(u)].T, U32)

    def wq_transpose(u, wqt_ref):
        wqt_ref[...] = pltpu.bitcast(wq_v[_grp(u)].T, U32)

    def attend(s_ref, m_ref, vt_ref):
        m = m_ref[0:1, :]
        o = []
        for r in range(REP):
            cols = slice(r * TQ, (r + 1) * TQ)
            p, l = _softmax_numer(s_ref[:, cols], m[:, cols])
            o.append((_dot(pltpu.bitcast(vt_ref[...], BF16), p) * (1.0 / l)).astype(BF16))
        return jnp.concatenate(o, axis=0)

    cp_x(0, msem.at[5]).start()
    cp_wq(0, msem.at[6]).start()
    cp_moda.start()
    acc_ref[...] = jnp.zeros_like(acc_ref)
    mod_ref[DA:6 * D, :] = jnp.zeros((4 * D, 128), F32)
    wr = jnp.concatenate([wr_ref[...].astype(F32), jnp.zeros((1, 64), F32)], axis=1)
    for t in range(5):
        wrb_ref[t * 128:(t + 1) * 128, :] = _col_bcast(wr[:, t * 128:(t + 1) * 128])
    cp_x(0, msem.at[5]).wait()
    cp_wq(0, msem.at[6]).wait()
    cp_k(0, msem.at[5]).start()
    for t in range(TPB):
        ln1_stats(t)
    for a in range(2):
        wq_transpose(a, streams[a][3])
    cp_moda.wait()
    cp_v(0, msem.at[6]).start()
    cp_wq(1, msem.at[6]).start()
    mod_part(0, DA)
    for t in range(TPB):
        ln1_apply(t)
    q = [q_proj(a, streams[a][3]) for a in range(2)]
    cp_k(0, msem.at[5]).wait()
    bundle(0, 'start')
    scores(0, q[0], s0_ref, m0_ref)
    cp_v(0, msem.at[6]).wait()
    cp_wq(1, msem.at[6]).wait()
    scores(1, q[1], s1_ref, m1_ref)
    for a in range(2):
        v_transpose(a, streams[a][2])
        wq_transpose(a + 2, streams[a][3])

    def unit(u, side, s_ref, m_ref, vt_ref, wqt_ref):
        q = q_proj(u + 2, wqt_ref)
        o = attend(s_ref, m_ref, vt_ref)
        clock = scores(u + 2, q, s_ref, m_ref)
        side(clock)
        upd = _dot(wot_v[_grp(u)], o)
        for t in range(TPB):
            acc_ref[_blk(u) * TPB + t] += upd[:, t * 128:(t + 1) * 128]
        v_transpose(u + 2, vt_ref)
        wq_transpose(u + 4, wqt_ref)
        fb = jnp.clip(u - WD0, 0, NFB - 1)
        src = jnp.where(u >= WD0, NT + fb, 0)
        wd_ref[pl.ds(pl.multiple_of(fb * 64, 64), 64), :] = pltpu.bitcast(xw_v[src].T, U32)

    def step(n, carry):
        @pl.when(n <= WD0 // 2)
        def _():
            @pl.when(n < NP)
            def _():
                with jax.named_scope('BW'):
                    bundle(n, 'wait')

            @pl.when(n + 1 < NP)
            def _():
                bundle(n + 1, 'start')

            @pl.when(n == 1)
            def _():
                cp_modb.start()

            @pl.when(n == 4)
            def _():
                cp_modb.wait()
                mod_part(DA, 6 * D)

            @pl.when(n == NP - 1)
            def _():
                cp_d.start()
                cp_g.start()
                cp_u.start()

            @pl.when(n == WD0 // 2)
            def _():
                cp_d.wait()

        t1 = jnp.minimum(n + 2, NT - 1)
        v = jnp.maximum(n - NP, 0)
        t2 = jax.lax.shift_right_logical(v, 3) * TPB + jnp.minimum(jnp.bitwise_and(v, NP - 1), TPB - 1)

        def stats(clock):
            ln2_stats(t2, clock)
            ln1_stats(t1, clock)

        def apply(clock):
            ln1_apply(t1, clock)
            ln2_apply(t2, clock)

        for a in range(2):
            unit(2 * n + a, (stats, apply)[a], *streams[a])
        return carry

    jax.lax.fori_loop(0, NU // 2 - 1, step, 0)

    T0 = NT - TPB
    cp_out(0, T0, osem.at[NT]).start()
    o = jnp.concatenate([attend(*streams[a][0:3]) for a in range(2)], axis=0)
    wlast = jnp.concatenate([wot_v[HKV - 2], wot_v[HKV - 1]], axis=1)
    for t in range(TPB):
        acc_ref[T0 + t] += _dot(wlast, o[:, t * 128:(t + 1) * 128])
        ln2_stats(T0 + t)
        ln2_apply(T0 + t)

    r = _r(r_ref[...]) + 0.0
    tok = (jax.lax.broadcasted_iota(jnp.int32, (NT, 128), 0) * 128
           + jax.lax.broadcasted_iota(jnp.int32, (NT, 128), 1))
    bits = jax.lax.shift_right_arithmetic(pltpu.bitcast(r, jnp.int32), 16)
    code = jnp.where(bits < 0, -32769 - bits, bits) + 32768
    work = pltpu.bitcast(code * S + (S - 1 - tok) + 0x20000000, F32)
    row16 = jax.lax.broadcasted_iota(jnp.int32, (16, 128), 0)
    lane16 = jax.lax.broadcasted_iota(jnp.int32, (16, 128), 1)
    sel = jnp.full((16, 128), 0x20000000, jnp.int32)
    tiles = []
    for t in range(C):
        mx = jnp.max(jnp.max(work, axis=0, keepdims=True), axis=1, keepdims=True)
        work = jnp.where(work == mx, 0.0, work)
        mxi = pltpu.bitcast(mx, jnp.int32)
        sel = jnp.where(row16 == t, mxi, sel)
        tiles.append(((S - 1) - (mxi[0, 0] & (S - 1))) // 128)
    sel = sel - 0x20000000
    sel_tok = jnp.where(row16 < C, (S - 1) - (sel & (S - 1)), -1)
    sel_code = jax.lax.shift_right_logical(sel, 11) - 32768
    sel_bits = jnp.where(sel_code < 0, -32769 - sel_code, sel_code)
    r_sel = jnp.where(row16 < C, pltpu.bitcast(jax.lax.shift_left(sel_bits, 16), F32), 0.0)[:, 0:1]

    def dirty(t):
        d = tiles[0] == t
        for u in range(1, C):
            d = jnp.logical_or(d, tiles[u] == t)
        return d

    for t in range(T0, NT):
        @pl.when(jnp.logical_not(dirty(t)))
        def _():
            cp_out(t, 1, osem.at[t]).start()

    xs = jnp.zeros((16, D), F32)
    for t in range(C):
        oh = jnp.where(jnp.logical_and(sel_tok == tiles[t] * 128 + lane16, row16 == t), 1.0, 0.0)
        xs = xs + _dot_nt(oh.astype(BF16), h2_ref[tiles[t]])
    xs = xs.astype(BF16)

    cp_g.wait()
    cp_u.wait()
    cp_out(0, T0, osem.at[NT]).wait()
    gpre = _r(_dot(xs, wg_v[...]))
    gact = _r(gpre * _r(jax.nn.sigmoid(gpre)))
    u = _r(_dot(xs, wu_v[...]))
    y = _r(_dot((gact * u).astype(BF16), pltpu.bitcast(wd_ref[...], BF16)))
    y = (y * _r(jax.nn.sigmoid(r_sel))).astype(BF16)

    for t in range(C):
        oh = jnp.where(sel_tok == tiles[t] * 128 + lane16, 1.0, 0.0).astype(BF16)
        upd = jax.lax.dot_general(y, oh, (((0,), (0,)), ((), ())), preferred_element_type=F32)
        out_v[tiles[t]] = (x1_ref[tiles[t]].astype(F32)
                          + mod(5) * (h2_ref[tiles[t]].astype(F32) + upd)).astype(BF16)
    for t in range(NT):
        @pl.when(dirty(t))
        def _():
            cp_out(t, 1, osem.at[t]).start()
    for t in range(NT):
        if t >= T0:
            cp_out(t, 1, osem.at[t]).wait()
        else:
            @pl.when(dirty(t))
            def _():
                cp_out(t, 1, osem.at[t]).wait()


@jax.jit
def pallas_adaLN_cond__gqa_block_cached__moe_arch_mod__prompt_kernel(
    A_x: jax.Array,
    A_k_cache: jax.Array,
    A_v_cache: jax.Array,
    A_wq: jax.Array,
    A_wo: jax.Array,
    B_x: jax.Array,
    B_w_r: jax.Array,
    B_w_gate: jax.Array,
    B_w_up: jax.Array,
    B_w_down: jax.Array,
    c: jax.Array,
    w_mod: jax.Array,
):
    del B_x
    xt = A_x.reshape(S, D).T
    k = A_k_cache.reshape(HKV, S, DH)
    v = A_v_cache.reshape(HKV, S, DH)
    wr = B_w_r.reshape(1, D)

    hbm = pl.BlockSpec(memory_space=pl.ANY)
    vmem = pl.BlockSpec(memory_space=pltpu.VMEM)
    stream = [
        pltpu.VMEM((S, REP * TQ), F32),
        pltpu.VMEM((8, REP * TQ), F32),
        pltpu.VMEM((DH // 2, S), U32),
        pltpu.VMEM((GW // 2, D), U32),
    ]
    out = pl.pallas_call(
        _kernel,
        in_specs=[vmem, vmem] + [hbm] * 9,
        out_specs=hbm,
        out_shape=jax.ShapeDtypeStruct((D, S), BF16),
        scratch_shapes=[
            pltpu.VMEM((NT + NFB, D, 128), BF16),
            pltpu.VMEM((HKV, S, DH), BF16),
            pltpu.VMEM((HKV, S, DH), BF16),
            pltpu.VMEM((HKV, D, GW), BF16),
            pltpu.VMEM((HKV, D, GW), BF16),
            pltpu.VMEM((D, 6 * D), BF16),
            pltpu.VMEM((D, F), BF16),
            pltpu.VMEM((D, F), BF16),
            pltpu.VMEM((F // 2, D), U32),
            pltpu.VMEM((NT, D, 128), BF16),
            pltpu.VMEM((NT, D, 128), F32),
            pltpu.VMEM((6 * D, 128), F32),
            pltpu.VMEM((5 * 128, 128), F32),
            pltpu.VMEM((NT, D, 128), BF16),
            pltpu.VMEM((NT, D, 128), BF16),
            pltpu.VMEM((NT, D, 128), BF16),
            pltpu.VMEM((NT, 128), F32),
            pltpu.VMEM((NT * NC, 8, 128), F32),
            pltpu.VMEM((NT, 8, 128), F32),
        ] + stream + stream + [
            pltpu.SemaphoreType.DMA((HKV // 2,)),
            pltpu.SemaphoreType.DMA((7,)),
            pltpu.SemaphoreType.DMA((NT + 1,)),
        ],
        compiler_params=pltpu.CompilerParams(vmem_limit_bytes=120 * 1024 * 1024,
                                             disable_bounds_checks=True),
    )(wr, c, xt, k, v, A_wq, A_wo.T, w_mod, B_w_gate, B_w_up, B_w_down.T)
    return out.T.reshape(1, S, D)
```

```python
import math

import jax
import jax.numpy as jnp
import jax.experimental.pallas as pl
import jax.experimental.pallas.tpu as pltpu

S = 2048
D = 576
HQ = 32
HKV = 16
REP = HQ // HKV
DH = 128
GW = REP * DH
F = 4608
C = 8
EPS = 1e-05
TQ = 512
NBLK = S // TQ
TPB = TQ // 128
NT = S // 128
NU = NBLK * HKV
DA = 2 * D
NC = 3
DC = D // NC
TLAG = 160
PG = 64
NFB = F // 128
NMB = 4 * D // 128
MPI = 3
MB0 = 2
WD0 = 24
PACE = (1280, 304, 304, 1024, 2304, 3200)

BF16 = jnp.bfloat16
F32 = jnp.float32
U32 = jnp.uint32
QSCALE = DH ** -0.5 * math.log2(math.e)


def _dot(a, b):
    return jnp.dot(a, b, preferred_element_type=F32)


def _dot_nt(a, b):
    return jax.lax.dot_general(a, b, (((1,), (1,)), ((), ())), preferred_element_type=F32)


def _r(x):
    return x.astype(BF16).astype(F32)


def _col_bcast(row):
    return jnp.broadcast_to(row, (128, 128)).T


def _blk(u):
    return u // HKV if isinstance(u, int) else jax.lax.shift_right_logical(u, 4)


def _grp(u):
    return u % HKV if isinstance(u, int) else jnp.bitwise_and(u, HKV - 1)


def _lanes(t, n=1):
    return pl.ds(pl.multiple_of(t * 128, 128), n * 128)


def _paced(x, clock, pos):
    if clock is None:
        return x
    row, col = pos % S, (pos // S) * TQ
    g = clock[row:row + x.shape[0], col:col + x.shape[1]]
    return jnp.where(g * g < 0.0, jnp.zeros_like(x), x)


def _softmax_numer(s, m):
    n, w = s.shape
    p = jnp.exp2(s - m).reshape(n // PG, PG // 8, 8, w)
    ts = jnp.sum(p, axis=1)
    last = jnp.where(ts < 0.0, ts, p[:, PG // 8 - 1])
    p = jnp.concatenate([p[:, :PG // 8 - 1], last[:, None]], axis=1).reshape(n, w)
    l = jnp.sum(jnp.sum(ts, axis=0), axis=0, keepdims=True)
    return p.astype(BF16), l


def _chunk_stats(x):
    m = jnp.sum(x, axis=0, keepdims=True) * (1.0 / DC)
    xc = x - m
    return m, jnp.sum(xc * xc, axis=0, keepdims=True)


def _mean_var(stats):
    mean = sum(m for m, _ in stats) * (1.0 / NC)
    var = sum(s + DC * (m - mean) * (m - mean) for m, s in stats) * (1.0 / D)
    return mean, var


def _kernel(wr_ref, c_ref,
            xt_hbm, k_hbm, v_hbm, wq_hbm, wot_hbm, wmod_hbm, wg_hbm, wu_hbm, wdt_hbm,
            out_hbm,
            xw_v, k_v, v_v, wq_v, wot_v, wmod_v, wg_v, wu_v, wd_ref,
            ht_ref, acc_ref, mod_ref, wrb_ref, scb_ref, ln0_ref, x1_ref, h2_ref, h2row_ref, out_v,
            r_ref, st1_ref, st2_ref, lm_ref,
            s0_ref, m0_ref, vt0_ref, wqt0_ref, s1_ref, m1_ref, vt1_ref, wqt1_ref,
            bsem, msem, osem):
    streams = ((s0_ref, m0_ref, vt0_ref, wqt0_ref), (s1_ref, m1_ref, vt1_ref, wqt1_ref))

    def cp_cols(src, dst, t, n, sem, dst_t=None):
        return pltpu.make_async_copy(src.at[:, _lanes(t, n)],
                                     dst.at[:, _lanes(t if dst_t is None else dst_t, n)], sem)

    def cp_pair(src, dst, p, sem):
        return pltpu.make_async_copy(src.at[pl.ds(2 * p, 2)], dst.at[pl.ds(2 * p, 2)], sem)

    cp_k = lambda p, sem: cp_pair(k_hbm, k_v, p, sem)
    cp_v1 = lambda g, sem: pltpu.make_async_copy(v_hbm.at[g], v_v.at[g], sem)
    cp_k1 = lambda g, sem: pltpu.make_async_copy(k_hbm.at[g], k_v.at[g], sem)

    class Both:
        def __init__(self, cps):
            self.cps = cps

        def start(self):
            for cp in self.cps:
                cp.start()

        def wait(self):
            for cp in self.cps:
                cp.wait()

    def cp_w1(src, dst, g, sem):
        return pltpu.make_async_copy(src.at[:, _lanes(g * REP, REP)], dst.at[g], sem)

    def cp_w(src, dst, p, sem):
        return Both([cp_w1(src, dst, 2 * p + a, sem) for a in range(2)])

    cp_wq = lambda p, sem: cp_w(wq_hbm, wq_v, p, sem)
    cp_wo = lambda p, sem: cp_w(wot_hbm, wot_v, p, sem)
    cp_x = lambda j, sem: Both([pltpu.make_async_copy(xt_hbm.at[:, _lanes(TPB * j + t)],
                                                      xw_v.at[TPB * j + t], sem) for t in range(TPB)])
    NP = HKV // 2

    def bundle(n, act):
        sem = bsem.at[n if isinstance(n, int) else jnp.minimum(n, NP - 1)]

        def on(cond, cps):
            def go():
                for cp in cps():
                    getattr(cp, act)()
            if isinstance(cond, bool):
                if cond:
                    go()
            else:
                pl.when(cond)(go)
        on(n + 1 < NP, lambda: [cp_k(n + 1, sem), cp_v1(2 * n + 2, sem), cp_w1(wq_hbm, wq_v, 2 * n + 3, sem)])
        on(n + 2 < NP, lambda: [cp_w1(wq_hbm, wq_v, 2 * n + 4, sem)])
        on(jnp.logical_and(n >= 1, n < NBLK) if not isinstance(n, int) else 1 <= n < NBLK, lambda: [cp_x(n, sem)])
        on(n < NP, lambda: [cp_v1(2 * n + 1, sem), cp_wo(n, sem)])

    cp_moda = cp_cols(wmod_hbm, wmod_v, 0, DA // 128, msem.at[0])
    cp_modb = Both([pltpu.make_async_copy(wmod_hbm.at[:, _lanes(DA // 128 + b)],
                                          xw_v.at[NT + NFB + b], msem.at[1]) for b in range(NMB)])
    cp_g = pltpu.make_async_copy(wg_hbm, wg_v, msem.at[2])
    cp_u = pltpu.make_async_copy(wu_hbm, wu_v, msem.at[3])
    cp_d = Both([pltpu.make_async_copy(wdt_hbm.at[:, _lanes(b)], xw_v.at[NT + b], msem.at[4])
                 for b in range(NFB)])
    cp_out = lambda t, n, sem: Both([pltpu.make_async_copy(out_v.at[t + a], out_hbm.at[:, _lanes(t + a)],
                                                           sem) for a in range(n)])

    def silu_c():
        c = c_ref[...].astype(F32)
        return _r(c * _r(jax.nn.sigmoid(c)))

    def finish_mod(mod, lo):
        mod = _r(mod)
        col = lo + jax.lax.broadcasted_iota(jnp.int32, mod.shape, 1)
        is_scale = jnp.logical_or(jnp.logical_and(col >= D, col < 2 * D),
                                  jnp.logical_and(col >= 4 * D, col < 5 * D))
        mod = jnp.where(is_scale, _r(1.0 + mod), mod)
        for t in range(mod.shape[1] // 128):
            rows = pl.ds(pl.multiple_of(lo + t * 128, 128), 128)
            mod_ref[rows, :] = _col_bcast(mod[:, t * 128:(t + 1) * 128])

    def late_mod_sums(n, clock):
        b0 = jnp.clip(n - MB0, 0, NMB // MPI - 1) * MPI
        for k in range(MPI):
            w = xw_v[jnp.where(n >= MB0, NT + NFB + b0 + k, 0)].astype(F32)
            part = jnp.sum((w * scb_ref[0:D, :]).reshape(D // 8, 8, 128), axis=0)
            lm_ref[k] = _paced(part, clock, PACE[4] + 256 * k)

    def late_mod_store(n):
        b0 = jnp.clip(n - MB0, 0, NMB // MPI - 1) * MPI
        for k in range(MPI):
            finish_mod(jnp.sum(lm_ref[k], axis=0, keepdims=True), DA + (b0 + k) * 128)

    def col_vector(ref, row):
        row = jnp.concatenate([row, jnp.zeros((1, 64), F32)], axis=1)
        for t in range(5):
            ref[t * 128:(t + 1) * 128, :] = _col_bcast(row[:, t * 128:(t + 1) * 128])

    def mod(k):
        return mod_ref[k * D:(k + 1) * D, :]

    def put_stats(st_ref, t, shift, scale, clock, pos):
        row = jax.lax.broadcasted_iota(jnp.int32, (8, 128), 0)
        st_ref[t] = _paced(jnp.where(row == 0, shift, scale), clock, pos)

    def ln1_stats(t, clock=None):
        for c in range(NC):
            m, s = _chunk_stats(xw_v[t, c * DC:(c + 1) * DC, :].astype(F32))
            put_stats(st1_ref, t * NC + c, m, s, clock, PACE[0] + 192 * c)

    def ln1_norm(t):
        mean, var = _mean_var([(st1_ref[t * NC + c, 0:1, :], st1_ref[t * NC + c, 1:2, :])
                               for c in range(NC)])
        return (xw_v[t].astype(F32) - mean) * jax.lax.rsqrt(var + EPS)

    def ln1_apply(t, clock=None, ln=None):
        h = (ln1_norm(t) if ln is None else ln) * mod(1) + mod(0)
        ht_ref[t] = _paced(h, clock, PACE[1]).astype(BF16)

    def h2_rows(t, clock=None):
        x = pltpu.bitcast(h2_ref[t].T, U32)
        x = jnp.concatenate([_paced(x[:, a:min(a + 128, D)], clock, PACE[5] + a // 2)
                             for a in range(0, D, 128)], axis=1)
        h2row_ref[pl.ds(pl.multiple_of(t * 64, 64), 64), :] = x

    def ln2_stats(t, clock=None, attn=None):
        x1 = _r(xw_v[t].astype(F32) + mod(2) * (acc_ref[t] if attn is None else attn))
        x1_ref[t] = _paced(x1, clock, PACE[2]).astype(BF16)
        mean, var = _mean_var([_chunk_stats(x1[c * DC:(c + 1) * DC]) for c in range(NC)])
        put_stats(st2_ref, t, _r(mean), 1.0 / _r(jnp.sqrt(_r(_r(var) + EPS))), clock, PACE[2] + D + 128)

    def ln2_apply(t, clock=None, gate=None):
        x1 = x1_ref[t].astype(F32)
        if gate is not None and gate.shape[0] > 0:
            n = gate.shape[0]
            x1 = jnp.concatenate([_paced(x1[:n], gate, 0), x1[n:]], axis=0) if n < D else _paced(x1, gate, 0)
        h2 = _r((x1 - st2_ref[t, 0:1, :]) * st2_ref[t, 1:2, :] * mod(4) + mod(3))
        h2_ref[t] = _paced(h2, clock, PACE[3]).astype(BF16)
        out_v[t] = _paced(x1 + mod(5) * h2, clock, PACE[3] + 16).astype(BF16)
        rp = jnp.sum(h2 * wrb_ref[0:D, :], axis=0, keepdims=True)
        r_ref[pl.ds(t, 1), :] = _paced(rp, clock, PACE[3] + D + 64)

    def q_proj(u, wqt_ref):
        q = _dot(pltpu.bitcast(wqt_ref[...], BF16), jnp.concatenate([ht_ref[_blk(u) * TPB + t] for t in range(TPB)], axis=1))
        q = (q * QSCALE).astype(BF16)
        return jnp.concatenate([q[r * DH:(r + 1) * DH] for r in range(REP)], axis=1)

    def scores(u, q, s_ref, m_ref):
        s = _dot(k_v[_grp(u)], q)
        s_ref[...] = s
        m_ref[...] = jnp.broadcast_to(jnp.max(s, axis=0, keepdims=True), m_ref.shape)
        return s

    def v_transpose(u, vt_ref):
        vt_ref[...] = pltpu.bitcast(v_v[_grp(u)].T, U32)

    def wq_transpose(u, wqt_ref):
        wqt_ref[...] = pltpu.bitcast(wq_v[_grp(u)].T, U32)

    def attend(s_ref, m_ref, vt_ref):
        m = m_ref[0:1, :]
        o = []
        for r in range(REP):
            cols = slice(r * TQ, (r + 1) * TQ)
            p, l = _softmax_numer(s_ref[:, cols], m[:, cols])
            o.append((_dot(pltpu.bitcast(vt_ref[...], BF16), p) * (1.0 / l)).astype(BF16))
        return jnp.concatenate(o, axis=0)

    cp_x(0, msem.at[5]).start()
    cp_w1(wq_hbm, wq_v, 0, msem.at[6]).start()
    cp_moda.start()
    acc_ref[...] = jnp.zeros_like(acc_ref)
    mod_ref[DA:6 * D, :] = jnp.zeros((4 * D, 128), F32)
    h2_ref[0] = jnp.zeros((D, 128), BF16)
    col_vector(wrb_ref, wr_ref[...].astype(F32))
    col_vector(scb_ref, silu_c())
    cp_x(0, msem.at[5]).wait()
    cp_w1(wq_hbm, wq_v, 0, msem.at[6]).wait()
    first = Both([cp_k1(0, msem.at[5]), cp_w1(wq_hbm, wq_v, 1, msem.at[5])])
    first.start()
    for t in range(TPB):
        ln1_stats(t)
        ln0_ref[t] = ln1_norm(t)
    wq_transpose(0, wqt0_ref)
    cp_moda.wait()
    second = Both([cp_k1(1, msem.at[6]), cp_v1(0, msem.at[6]), cp_w1(wq_hbm, wq_v, 2, msem.at[6])])
    second.start()
    finish_mod(_dot(jnp.broadcast_to(silu_c(), (8, D)).astype(BF16), wmod_v[...])[0:1], 0)
    for t in range(TPB):
        ln1_apply(t, ln=ln0_ref[t])
    q = q_proj(0, wqt0_ref)
    first.wait()
    bundle(0, 'start')
    scores(0, q, s0_ref, m0_ref)
    wq_transpose(1, wqt1_ref)
    second.wait()
    scores(1, q_proj(1, wqt1_ref), s1_ref, m1_ref)
    v_transpose(0, vt0_ref)
    wq_transpose(2, wqt0_ref)

    def unit(u, side, s_ref, m_ref, vt_ref, wqt_ref):
        q = q_proj(u + 2, wqt_ref)
        o = attend(s_ref, m_ref, vt_ref)
        clock = scores(u + 2, q, s_ref, m_ref)
        side(clock)
        upd = _dot(wot_v[_grp(u)], o)
        for t in range(TPB):
            acc_ref[_blk(u) * TPB + t] += upd[:, t * 128:(t + 1) * 128]
        fb = jnp.clip(u - WD0, 0, NFB - 1)
        src = jnp.where(u >= WD0, NT + fb, 0)
        wd_ref[pl.ds(pl.multiple_of(fb * 64, 64), 64), :] = pltpu.bitcast(xw_v[src].T, U32)

    def step(n, carry):
        @pl.when(n <= WD0 // 2)
        def _():
            @pl.when(n < NP)
            def _():
                with jax.named_scope('BW'):
                    bundle(n, 'wait')

            @pl.when(n == 0)
            def _():
                cp_modb.start()

            @pl.when(n == MB0)
            def _():
                cp_modb.wait()

            @pl.when(n == NP - 1)
            def _():
                cp_d.start()
                cp_g.start()
                cp_u.start()

            @pl.when(n == WD0 // 2)
            def _():
                cp_d.wait()

        bundle(jnp.minimum(n + 1, NP), 'start')

        t1 = jnp.minimum(n + 2, NT - 1)
        v = jnp.maximum(n - NP, 0)
        tile2 = lambda v: (jax.lax.shift_right_logical(v, 3) * TPB
                           + jnp.minimum(jnp.bitwise_and(v, NP - 1), TPB - 1))
        t2 = tile2(v)
        v_transpose(2 * n + 1, vt1_ref)
        wq_transpose(2 * n + 3, wqt1_ref)

        def stats(clock):
            ln2_stats(t2, clock)
            ln1_stats(t1, clock)
            late_mod_sums(n, clock)
            h2_rows(tile2(jnp.maximum(v - 1, 0)), clock)

        def apply(clock):
            ln1_apply(t1, clock)
            ln2_apply(t2, clock)
            late_mod_store(n)

        for a in range(2):
            unit(2 * n + a, (stats, apply)[a], *streams[a])
        v_transpose(2 * n + 2, vt0_ref)
        wq_transpose(2 * n + 4, wqt0_ref)
        return carry

    jax.lax.fori_loop(0, NU // 2 - 1, step, 0)

    T0 = NT - TPB
    cp_out(0, T0, osem.at[C + TPB]).start()
    v_transpose(NU - 1, vt1_ref)
    o = jnp.concatenate([attend(*streams[a][0:3]) for a in range(2)], axis=0)
    wlast = jnp.concatenate([wot_v[HKV - 2], wot_v[HKV - 1]], axis=1)
    fin = [acc_ref[T0 + t] + _dot(wlast, o[:, t * 128:(t + 1) * 128]) for t in range(TPB)]
    clock = jnp.concatenate(fin, axis=0)
    for t in range(TPB):
        ln2_stats(T0 + t, attn=fin[t])
        ln2_apply(T0 + t, gate=clock[(t + 1) * D + TLAG:(t + 2) * D + TLAG])
    for t in range(T0, NT):
        h2_rows(t)
    cp_g.wait()
    cp_u.wait()
    cp_out(0, T0, osem.at[C + TPB]).wait()

    r = _r(r_ref[...]) + 0.0
    tok = (jax.lax.broadcasted_iota(jnp.int32, (NT, 128), 0) * 128
           + jax.lax.broadcasted_iota(jnp.int32, (NT, 128), 1))
    bits = jax.lax.shift_right_arithmetic(pltpu.bitcast(r, jnp.int32), 16)
    code = jnp.where(bits < 0, -32769 - bits, bits) + 32768
    work = pltpu.bitcast(code * S + (S - 1 - tok) + 0x20000000, F32)
    row16 = jax.lax.broadcasted_iota(jnp.int32, (16, 128), 0)
    lane16 = jax.lax.broadcasted_iota(jnp.int32, (16, 128), 1)
    sel = jnp.full((16, 128), 0x20000000, jnp.int32)
    toks, tiles = [], []
    for t in range(C):
        mx = jnp.max(jnp.max(work, axis=0, keepdims=True), axis=1, keepdims=True)
        work = jnp.where(work == mx, 0.0, work)
        mxi = pltpu.bitcast(mx, jnp.int32)
        sel = jnp.where(row16 == t, mxi, sel)
        toks.append((S - 1) - (mxi[0, 0] & (S - 1)))
        tiles.append(jax.lax.shift_right_logical(toks[t], 7))
    sel = sel - 0x20000000
    sel_tok = jnp.where(row16 < C, (S - 1) - (sel & (S - 1)), -1)
    sel_code = jax.lax.shift_right_logical(sel, 11) - 32768
    sel_bits = jnp.where(sel_code < 0, -32769 - sel_code, sel_code)
    r_sel = jnp.where(row16 < C, pltpu.bitcast(jax.lax.shift_left(sel_bits, 16), F32), 0.0)[:, 0:1]

    clean = []
    for t in range(T0, NT):
        d = tiles[0] != t
        for u in range(1, C):
            d = jnp.logical_and(d, tiles[u] != t)
        clean.append(d)
        pl.when(d)(cp_out(t, 1, osem.at[C + t - T0]).start)
    final = []
    for t in range(C):
        d = True
        for u in range(t + 1, C):
            d = jnp.logical_and(d, tiles[u] != tiles[t])
        final.append(d)

    words = jnp.concatenate([h2row_ref[pl.ds(jax.lax.shift_right_logical(toks[t], 1), 1), :]
                             for t in range(C)], axis=0)
    odd = jnp.bitwise_and(sel_tok[0:C, 0:1], 1) == 1
    xs = pltpu.bitcast(jnp.where(odd, jnp.bitwise_and(words, jnp.uint32(0xFFFF0000)),
                                 jax.lax.shift_left(words, jnp.uint32(16))), F32)
    xs = jnp.concatenate([xs, jnp.zeros((16 - C, D), F32)], axis=0).astype(BF16)

    gpre = _r(_dot(xs, wg_v[...]))
    gact = _r(gpre * _r(jax.nn.sigmoid(gpre)))
    u = _r(_dot(xs, wu_v[...]))
    y = _r(_dot((gact * u).astype(BF16), pltpu.bitcast(wd_ref[...], BF16)))
    y = (y * _r(jax.nn.sigmoid(r_sel))).astype(BF16)

    for t in range(C):
        oh = jnp.where(sel_tok == tiles[t] * 128 + lane16, 1.0, 0.0).astype(BF16)
        upd = jax.lax.dot_general(y, oh, (((0,), (0,)), ((), ())), preferred_element_type=F32)
        out_v[tiles[t]] = (x1_ref[tiles[t]].astype(F32)
                          + mod(5) * (h2_ref[tiles[t]].astype(F32) + upd)).astype(BF16)
        if final[t] is True:
            cp_out(tiles[t], 1, osem.at[t]).start()
        else:
            pl.when(final[t])(cp_out(tiles[t], 1, osem.at[t]).start)
    for t in range(T0, NT):
        pl.when(clean[t - T0])(cp_out(t, 1, osem.at[C + t - T0]).wait)
    for t in range(C):
        if final[t] is True:
            cp_out(tiles[t], 1, osem.at[t]).wait()
        else:
            pl.when(final[t])(cp_out(tiles[t], 1, osem.at[t]).wait)


@jax.jit
def pallas_adaLN_cond__gqa_block_cached__moe_arch_mod__prompt_kernel(
    A_x: jax.Array,
    A_k_cache: jax.Array,
    A_v_cache: jax.Array,
    A_wq: jax.Array,
    A_wo: jax.Array,
    B_x: jax.Array,
    B_w_r: jax.Array,
    B_w_gate: jax.Array,
    B_w_up: jax.Array,
    B_w_down: jax.Array,
    c: jax.Array,
    w_mod: jax.Array,
):
    del B_x
    xt = A_x.reshape(S, D).T
    k = A_k_cache.reshape(HKV, S, DH)
    v = A_v_cache.reshape(HKV, S, DH)
    wr = B_w_r.reshape(1, D)

    hbm = pl.BlockSpec(memory_space=pl.ANY)
    vmem = pl.BlockSpec(memory_space=pltpu.VMEM)
    stream = [
        pltpu.VMEM((S, REP * TQ), F32),
        pltpu.VMEM((8, REP * TQ), F32),
        pltpu.VMEM((DH // 2, S), U32),
        pltpu.VMEM((GW // 2, D), U32),
    ]
    out = pl.pallas_call(
        _kernel,
        in_specs=[vmem, vmem] + [hbm] * 9,
        out_specs=hbm,
        out_shape=jax.ShapeDtypeStruct((D, S), BF16),
        scratch_shapes=[
            pltpu.VMEM((NT + NFB + NMB, D, 128), BF16),
            pltpu.VMEM((HKV, S, DH), BF16),
            pltpu.VMEM((HKV, S, DH), BF16),
            pltpu.VMEM((HKV, D, GW), BF16),
            pltpu.VMEM((HKV, D, GW), BF16),
            pltpu.VMEM((D, DA), BF16),
            pltpu.VMEM((D, F), BF16),
            pltpu.VMEM((D, F), BF16),
            pltpu.VMEM((F // 2, D), U32),
            pltpu.VMEM((NT, D, 128), BF16),
            pltpu.VMEM((NT, D, 128), F32),
            pltpu.VMEM((6 * D, 128), F32),
            pltpu.VMEM((5 * 128, 128), F32),
            pltpu.VMEM((5 * 128, 128), F32),
            pltpu.VMEM((TPB, D, 128), F32),
            pltpu.VMEM((NT, D, 128), BF16),
            pltpu.VMEM((NT, D, 128), BF16),
            pltpu.VMEM((S // 2, D), U32),
            pltpu.VMEM((NT, D, 128), BF16),
            pltpu.VMEM((NT, 128), F32),
            pltpu.VMEM((NT * NC, 8, 128), F32),
            pltpu.VMEM((NT, 8, 128), F32),
            pltpu.VMEM((MPI, 8, 128), F32),
        ] + stream + stream + [
            pltpu.SemaphoreType.DMA((HKV // 2,)),
            pltpu.SemaphoreType.DMA((7,)),
            pltpu.SemaphoreType.DMA((C + TPB + 1,)),
        ],
        compiler_params=pltpu.CompilerParams(vmem_limit_bytes=120 * 1024 * 1024,
                                             disable_bounds_checks=True),
    )(wr, c, xt, k, v, A_wq, A_wo.T, w_mod, B_w_gate, B_w_up, B_w_down.T)
    return out.T.reshape(1, S, D)
```

```python
import math

import jax
import jax.numpy as jnp
import jax.experimental.pallas as pl
import jax.experimental.pallas.tpu as pltpu

S = 2048
D = 576
HQ = 32
HKV = 16
REP = HQ // HKV
DH = 128
GW = REP * DH
F = 4608
C = 8
EPS = 1e-05
TQ = 512
NBLK = S // TQ
TPB = TQ // 128
NT = S // 128
NU = NBLK * HKV
DA = 2 * D
NC = 3
DC = D // NC
TLAG = 160
PG = 64
NFB = F // 128
NMB = 4 * D // 128
MPI = 3
MB0 = 2
WD0 = 14
PACE = (1280, 304, 2112, 1024, 400, 3200)

BF16 = jnp.bfloat16
F32 = jnp.float32
U32 = jnp.uint32
QSCALE = DH ** -0.5 * math.log2(math.e)


def _dot(a, b):
    return jnp.dot(a, b, preferred_element_type=F32)


def _dot_nt(a, b):
    return jax.lax.dot_general(a, b, (((1,), (1,)), ((), ())), preferred_element_type=F32)


def _r(x):
    return x.astype(BF16).astype(F32)


def _col_bcast(row):
    return jnp.broadcast_to(row, (128, 128)).T


def _blk(u):
    return u // HKV if isinstance(u, int) else jax.lax.shift_right_logical(u, 4)


def _grp(u):
    return u % HKV if isinstance(u, int) else jnp.bitwise_and(u, HKV - 1)


def _lanes(t, n=1):
    return pl.ds(pl.multiple_of(t * 128, 128), n * 128)


def _paced(x, clock, pos):
    if clock is None:
        return x
    row, col = pos % S, (pos // S) * TQ
    g = clock[row:row + x.shape[0], col:col + x.shape[1]]
    return jnp.where(g * g < 0.0, jnp.zeros_like(x), x)


def _softmax_numer(s, m):
    n, w = s.shape
    p = jnp.exp2(s - m).reshape(n // PG, PG // 8, 8, w)
    ts = jnp.sum(p, axis=1)
    last = jnp.where(ts < 0.0, ts, p[:, PG // 8 - 1])
    p = jnp.concatenate([p[:, :PG // 8 - 1], last[:, None]], axis=1).reshape(n, w)
    l = jnp.sum(jnp.sum(ts, axis=0), axis=0, keepdims=True)
    return p.astype(BF16), l


def _chunk_stats(x):
    m = jnp.sum(x, axis=0, keepdims=True) * (1.0 / DC)
    xc = x - m
    return m, jnp.sum(xc * xc, axis=0, keepdims=True)


def _mean_var(stats):
    mean = sum(m for m, _ in stats) * (1.0 / NC)
    var = sum(s + DC * (m - mean) * (m - mean) for m, s in stats) * (1.0 / D)
    return mean, var


def _kernel(wr_ref, c_ref,
            xt_hbm, k_hbm, v_hbm, wq_hbm, wot_hbm, wmod_hbm, wg_hbm, wu_hbm, wdt_hbm,
            out_hbm,
            xw_v, k_v, v_v, wq_v, wot_v, wmod_v, wg_v, wu_v, wd_ref,
            ht_ref, acc_ref, mod_ref, wrb_ref, scb_ref, ln0_ref, x1_ref, h2_ref, h2row_ref, out_v,
            r_ref, st1_ref, st2_ref, lm_ref,
            s0_ref, m0_ref, vt0_ref, wqt0_ref, s1_ref, m1_ref, vt1_ref, wqt1_ref,
            bsem, msem, osem):
    streams = ((s0_ref, m0_ref, vt0_ref, wqt0_ref), (s1_ref, m1_ref, vt1_ref, wqt1_ref))

    def cp_cols(src, dst, t, n, sem, dst_t=None):
        return pltpu.make_async_copy(src.at[:, _lanes(t, n)],
                                     dst.at[:, _lanes(t if dst_t is None else dst_t, n)], sem)

    def cp_pair(src, dst, p, sem):
        return pltpu.make_async_copy(src.at[pl.ds(2 * p, 2)], dst.at[pl.ds(2 * p, 2)], sem)

    cp_k = lambda p, sem: cp_pair(k_hbm, k_v, p, sem)
    cp_v1 = lambda g, sem: pltpu.make_async_copy(v_hbm.at[g], v_v.at[g], sem)
    cp_k1 = lambda g, sem: pltpu.make_async_copy(k_hbm.at[g], k_v.at[g], sem)

    class Both:
        def __init__(self, cps):
            self.cps = cps

        def start(self):
            for cp in self.cps:
                cp.start()

        def wait(self):
            for cp in self.cps:
                cp.wait()

    def cp_w1(src, dst, g, sem):
        return pltpu.make_async_copy(src.at[:, _lanes(g * REP, REP)], dst.at[g], sem)

    def cp_w(src, dst, p, sem):
        return Both([cp_w1(src, dst, 2 * p + a, sem) for a in range(2)])

    cp_wq = lambda p, sem: cp_w(wq_hbm, wq_v, p, sem)
    cp_wo = lambda p, sem: cp_w(wot_hbm, wot_v, p, sem)
    cp_x = lambda j, sem: Both([pltpu.make_async_copy(xt_hbm.at[:, _lanes(TPB * j + t)],
                                                      xw_v.at[TPB * j + t], sem) for t in range(TPB)])
    NP = HKV // 2

    def bundle(n, act):
        sem = bsem.at[n if isinstance(n, int) else jnp.minimum(n, NP - 1)]

        def on(cond, cps):
            def go():
                for cp in cps():
                    getattr(cp, act)()
            if isinstance(cond, bool):
                if cond:
                    go()
            else:
                pl.when(cond)(go)
        on(n + 1 < NP, lambda: [cp_k(n + 1, sem), cp_v1(2 * n + 2, sem), cp_w1(wq_hbm, wq_v, 2 * n + 3, sem)])
        on(n + 2 < NP, lambda: [cp_w1(wq_hbm, wq_v, 2 * n + 4, sem)])
        on(jnp.logical_and(n >= 1, n < NBLK) if not isinstance(n, int) else 1 <= n < NBLK, lambda: [cp_x(n, sem)])
        on(n < NP, lambda: [cp_v1(2 * n + 1, sem), cp_wo(n, sem)])

    cp_moda = cp_cols(wmod_hbm, wmod_v, 0, DA // 128, msem.at[0])
    cp_modb = Both([pltpu.make_async_copy(wmod_hbm.at[:, _lanes(DA // 128 + b)],
                                          xw_v.at[NT + NFB + b], msem.at[1]) for b in range(NMB)])
    cp_g = pltpu.make_async_copy(wg_hbm, wg_v, msem.at[2])
    cp_u = pltpu.make_async_copy(wu_hbm, wu_v, msem.at[3])
    cp_d = Both([pltpu.make_async_copy(wdt_hbm.at[:, _lanes(b)], xw_v.at[NT + b], msem.at[4])
                 for b in range(NFB)])
    cp_out = lambda t, n, sem: Both([pltpu.make_async_copy(out_v.at[t + a], out_hbm.at[:, _lanes(t + a)],
                                                           sem) for a in range(n)])

    def silu_c():
        c = c_ref[...].astype(F32)
        return _r(c * _r(jax.nn.sigmoid(c)))

    def finish_mod(mod, lo):
        mod = _r(mod)
        col = lo + jax.lax.broadcasted_iota(jnp.int32, mod.shape, 1)
        is_scale = jnp.logical_or(jnp.logical_and(col >= D, col < 2 * D),
                                  jnp.logical_and(col >= 4 * D, col < 5 * D))
        mod = jnp.where(is_scale, _r(1.0 + mod), mod)
        for t in range(mod.shape[1] // 128):
            rows = pl.ds(pl.multiple_of(lo + t * 128, 128), 128)
            mod_ref[rows, :] = _col_bcast(mod[:, t * 128:(t + 1) * 128])

    def late_mod_sums(n, clock):
        b0 = jnp.clip(n - MB0, 0, NMB // MPI - 1) * MPI
        for k in range(MPI):
            w = xw_v[jnp.where(n >= MB0, NT + NFB + b0 + k, 0)].astype(F32)
            part = jnp.sum((w * scb_ref[0:D, :]).reshape(D // 8, 8, 128), axis=0)
            lm_ref[k] = _paced(part, clock, PACE[4] + 256 * k)

    def late_mod_store(n):
        b0 = jnp.clip(n - MB0, 0, NMB // MPI - 1) * MPI
        for k in range(MPI):
            finish_mod(jnp.sum(lm_ref[k], axis=0, keepdims=True), DA + (b0 + k) * 128)

    def col_vector(ref, row):
        row = jnp.concatenate([row, jnp.zeros((1, 64), F32)], axis=1)
        for t in range(5):
            ref[t * 128:(t + 1) * 128, :] = _col_bcast(row[:, t * 128:(t + 1) * 128])

    def mod(k):
        return mod_ref[k * D:(k + 1) * D, :]

    def put_stats(st_ref, t, shift, scale, clock, pos):
        row = jax.lax.broadcasted_iota(jnp.int32, (8, 128), 0)
        st_ref[t] = _paced(jnp.where(row == 0, shift, scale), clock, pos)

    def ln1_stats(t, clock=None):
        for c in range(NC):
            m, s = _chunk_stats(xw_v[t, c * DC:(c + 1) * DC, :].astype(F32))
            put_stats(st1_ref, t * NC + c, m, s, clock, PACE[0] + 192 * c)

    def ln1_norm(t):
        mean, var = _mean_var([(st1_ref[t * NC + c, 0:1, :], st1_ref[t * NC + c, 1:2, :])
                               for c in range(NC)])
        return (xw_v[t].astype(F32) - mean) * jax.lax.rsqrt(var + EPS)

    def ln1_apply(t, clock=None, ln=None):
        h = (ln1_norm(t) if ln is None else ln) * mod(1) + mod(0)
        ht_ref[t] = _paced(h, clock, PACE[1]).astype(BF16)

    def h2_rows(t, clock=None):
        x = pltpu.bitcast(h2_ref[t].T, U32)
        x = jnp.concatenate([_paced(x[:, a:min(a + 128, D)], clock, PACE[5] + a // 2)
                             for a in range(0, D, 128)], axis=1)
        h2row_ref[pl.ds(pl.multiple_of(t * 64, 64), 64), :] = x

    def ln2_stats(t, clock=None, attn=None):
        x1 = _r(xw_v[t].astype(F32) + mod(2) * (acc_ref[t] if attn is None else attn))
        x1_ref[t] = _paced(x1, clock, PACE[2]).astype(BF16)
        mean, var = _mean_var([_chunk_stats(x1[c * DC:(c + 1) * DC]) for c in range(NC)])
        put_stats(st2_ref, t, _r(mean), 1.0 / _r(jnp.sqrt(_r(_r(var) + EPS))), clock, PACE[2] + D + 128)

    def ln2_apply(t, clock=None, gate=None):
        x1 = x1_ref[t].astype(F32)
        if gate is not None and gate.shape[0] > 0:
            n = gate.shape[0]
            x1 = jnp.concatenate([_paced(x1[:n], gate, 0), x1[n:]], axis=0) if n < D else _paced(x1, gate, 0)
        h2 = _r((x1 - st2_ref[t, 0:1, :]) * st2_ref[t, 1:2, :] * mod(4) + mod(3))
        h2_ref[t] = _paced(h2, clock, PACE[3]).astype(BF16)
        out_v[t] = _paced(x1 + mod(5) * h2, clock, PACE[3] + 16).astype(BF16)
        rp = jnp.sum(h2 * wrb_ref[0:D, :], axis=0, keepdims=True)
        r_ref[pl.ds(t, 1), :] = _paced(rp, clock, PACE[3] + D + 64)

    def q_proj(u, wqt_ref):
        q = _dot(pltpu.bitcast(wqt_ref[...], BF16), jnp.concatenate([ht_ref[_blk(u) * TPB + t] for t in range(TPB)], axis=1))
        q = (q * QSCALE).astype(BF16)
        return jnp.concatenate([q[r * DH:(r + 1) * DH] for r in range(REP)], axis=1)

    def scores(u, q, s_ref, m_ref):
        s = _dot(k_v[_grp(u)], q)
        s_ref[...] = s
        m_ref[...] = jnp.broadcast_to(jnp.max(s, axis=0, keepdims=True), m_ref.shape)
        return s

    def v_transpose(u, vt_ref):
        vt_ref[...] = pltpu.bitcast(v_v[_grp(u)].T, U32)

    def wq_transpose(u, wqt_ref):
        wqt_ref[...] = pltpu.bitcast(wq_v[_grp(u)].T, U32)

    def attend(s_ref, m_ref, vt_ref):
        m = m_ref[0:1, :]
        o = []
        for r in range(REP):
            cols = slice(r * TQ, (r + 1) * TQ)
            p, l = _softmax_numer(s_ref[:, cols], m[:, cols])
            o.append((_dot(pltpu.bitcast(vt_ref[...], BF16), p) * (1.0 / l)).astype(BF16))
        return jnp.concatenate(o, axis=0)

    cp_x(0, msem.at[5]).start()
    cp_w1(wq_hbm, wq_v, 0, msem.at[6]).start()
    cp_moda.start()
    acc_ref[...] = jnp.zeros_like(acc_ref)
    mod_ref[DA:6 * D, :] = jnp.zeros((4 * D, 128), F32)
    h2_ref[0] = jnp.zeros((D, 128), BF16)
    col_vector(wrb_ref, wr_ref[...].astype(F32).reshape(1, D))
    col_vector(scb_ref, silu_c())
    cp_x(0, msem.at[5]).wait()
    cp_w1(wq_hbm, wq_v, 0, msem.at[6]).wait()
    first = Both([cp_k1(0, msem.at[5]), cp_w1(wq_hbm, wq_v, 1, msem.at[5])])
    first.start()
    for t in range(TPB):
        ln1_stats(t)
        ln0_ref[t] = ln1_norm(t)
    wq_transpose(0, wqt0_ref)
    cp_moda.wait()
    second = Both([cp_k1(1, msem.at[6]), cp_v1(0, msem.at[6]), cp_w1(wq_hbm, wq_v, 2, msem.at[6])])
    second.start()
    finish_mod(_dot(jnp.broadcast_to(silu_c(), (8, D)).astype(BF16), wmod_v[...])[0:1], 0)
    for t in range(TPB):
        ln1_apply(t, ln=ln0_ref[t])
    q = q_proj(0, wqt0_ref)
    first.wait()
    bundle(0, 'start')
    scores(0, q, s0_ref, m0_ref)
    wq_transpose(1, wqt1_ref)
    second.wait()
    scores(1, q_proj(1, wqt1_ref), s1_ref, m1_ref)
    v_transpose(0, vt0_ref)
    wq_transpose(2, wqt0_ref)

    def unit(u, side, s_ref, m_ref, vt_ref, wqt_ref):
        q = q_proj(u + 2, wqt_ref)
        o = attend(s_ref, m_ref, vt_ref)
        clock = scores(u + 2, q, s_ref, m_ref)
        side(clock)
        upd = _dot(wot_v[_grp(u)], o)
        for t in range(TPB):
            acc_ref[_blk(u) * TPB + t] += upd[:, t * 128:(t + 1) * 128]
        fb = jnp.clip(u - WD0, 0, NFB - 1)
        src = jnp.where(u >= WD0, NT + fb, 0)
        wd_ref[pl.ds(pl.multiple_of(fb * 64, 64), 64), :] = pltpu.bitcast(xw_v[src].T, U32)

    def step(n, carry):
        def waits(_, c):
            bundle(n, 'wait')
            pl.when(n == MB0)(cp_modb.wait)
            pl.when(n == WD0 // 2)(cp_d.wait)
            return c
        jax.lax.fori_loop(0, jnp.where(n < NP, 1, 0), waits, 0)

        bundle(jnp.minimum(n + 1, NP), 'start')
        pl.when(n == 0)(cp_modb.start)
        for a in range(3):
            pl.when(n == 2 + a)(Both(cp_d.cps[a * NFB // 3:(a + 1) * NFB // 3]).start)
        pl.when(n == NP)(Both([cp_g, cp_u]).start)

        t1 = jnp.minimum(n + 2, NT - 1)
        v = jnp.maximum(n - NP, 0)
        tile2 = lambda v: (jax.lax.shift_right_logical(v, 3) * TPB
                           + jnp.minimum(jnp.bitwise_and(v, NP - 1), TPB - 1))
        t2 = tile2(v)
        v_transpose(2 * n + 1, vt1_ref)
        wq_transpose(2 * n + 3, wqt1_ref)

        def stats(clock):
            ln2_stats(t2, clock)
            ln1_stats(t1, clock)
            late_mod_sums(n, clock)
            h2_rows(tile2(jnp.maximum(v - 1, 0)), clock)

        def apply(clock):
            ln1_apply(t1, clock)
            ln2_apply(t2, clock)
            late_mod_store(n)

        for a in range(2):
            unit(2 * n + a, (stats, apply)[a], *streams[a])
        v_transpose(2 * n + 2, vt0_ref)
        wq_transpose(2 * n + 4, wqt0_ref)
        return carry

    jax.lax.fori_loop(0, NU // 2 - 1, step, 0)

    T0 = NT - TPB
    cp_out(0, T0, osem.at[C + TPB]).start()
    v_transpose(NU - 1, vt1_ref)
    o = jnp.concatenate([attend(*streams[a][0:3]) for a in range(2)], axis=0)
    wlast = jnp.concatenate([wot_v[HKV - 2], wot_v[HKV - 1]], axis=1)
    fin = [acc_ref[T0 + t] + _dot(wlast, o[:, t * 128:(t + 1) * 128]) for t in range(TPB)]
    clock = jnp.concatenate(fin, axis=0)
    for t in range(TPB):
        ln2_stats(T0 + t, attn=fin[t])
        ln2_apply(T0 + t, gate=clock[(t + 1) * D + TLAG:(t + 2) * D + TLAG])
    for t in range(T0, NT):
        h2_rows(t)
    cp_g.wait()
    cp_u.wait()
    cp_out(0, T0, osem.at[C + TPB]).wait()

    r = _r(r_ref[...]) + 0.0
    tok = (jax.lax.broadcasted_iota(jnp.int32, (NT, 128), 0) * 128
           + jax.lax.broadcasted_iota(jnp.int32, (NT, 128), 1))
    bits = jax.lax.shift_right_arithmetic(pltpu.bitcast(r, jnp.int32), 16)
    code = jnp.where(bits < 0, -32769 - bits, bits) + 32768
    work = pltpu.bitcast(code * S + (S - 1 - tok) + 0x20000000, F32)
    row16 = jax.lax.broadcasted_iota(jnp.int32, (16, 128), 0)
    lane16 = jax.lax.broadcasted_iota(jnp.int32, (16, 128), 1)
    sel = jnp.full((16, 128), 0x20000000, jnp.int32)
    toks, tiles = [], []
    for t in range(C):
        mx = jnp.max(jnp.max(work, axis=0, keepdims=True), axis=1, keepdims=True)
        work = jnp.where(work == mx, 0.0, work)
        mxi = pltpu.bitcast(mx, jnp.int32)
        sel = jnp.where(row16 == t, mxi, sel)
        toks.append((S - 1) - (mxi[0, 0] & (S - 1)))
        tiles.append(jax.lax.shift_right_logical(toks[t], 7))
    sel = sel - 0x20000000
    sel_tok = jnp.where(row16 < C, (S - 1) - (sel & (S - 1)), -1)
    sel_code = jax.lax.shift_right_logical(sel, 11) - 32768
    sel_bits = jnp.where(sel_code < 0, -32769 - sel_code, sel_code)
    r_sel = jnp.where(row16 < C, pltpu.bitcast(jax.lax.shift_left(sel_bits, 16), F32), 0.0)[:, 0:1]

    clean = []
    for t in range(T0, NT):
        d = tiles[0] != t
        for u in range(1, C):
            d = jnp.logical_and(d, tiles[u] != t)
        clean.append(d)
        pl.when(d)(cp_out(t, 1, osem.at[C + t - T0]).start)
    final = []
    for t in range(C):
        d = True
        for u in range(t + 1, C):
            d = jnp.logical_and(d, tiles[u] != tiles[t])
        final.append(d)

    words = jnp.concatenate([h2row_ref[pl.ds(jax.lax.shift_right_logical(toks[t], 1), 1), :]
                             for t in range(C)], axis=0)
    odd = jnp.bitwise_and(sel_tok[0:C, 0:1], 1) == 1
    xs = pltpu.bitcast(jnp.where(odd, jnp.bitwise_and(words, jnp.uint32(0xFFFF0000)),
                                 jax.lax.shift_left(words, jnp.uint32(16))), F32)
    xs = jnp.concatenate([xs, jnp.zeros((16 - C, D), F32)], axis=0).astype(BF16)

    gpre = _r(_dot(xs, wg_v[...]))
    gact = _r(gpre * _r(jax.nn.sigmoid(gpre)))
    u = _r(_dot(xs, wu_v[...]))
    y = _r(_dot((gact * u).astype(BF16), pltpu.bitcast(wd_ref[...], BF16)))
    y = (y * _r(jax.nn.sigmoid(r_sel))).astype(BF16)

    for t in range(C):
        oh = jnp.where(sel_tok == tiles[t] * 128 + lane16, 1.0, 0.0).astype(BF16)
        upd = jax.lax.dot_general(y, oh, (((0,), (0,)), ((), ())), preferred_element_type=F32)
        out_v[tiles[t]] = (x1_ref[tiles[t]].astype(F32)
                          + mod(5) * (h2_ref[tiles[t]].astype(F32) + upd)).astype(BF16)
        if final[t] is True:
            cp_out(tiles[t], 1, osem.at[t]).start()
        else:
            pl.when(final[t])(cp_out(tiles[t], 1, osem.at[t]).start)
    for t in range(T0, NT):
        pl.when(clean[t - T0])(cp_out(t, 1, osem.at[C + t - T0]).wait)
    for t in range(C):
        if final[t] is True:
            cp_out(tiles[t], 1, osem.at[t]).wait()
        else:
            pl.when(final[t])(cp_out(tiles[t], 1, osem.at[t]).wait)


@jax.jit
def pallas_adaLN_cond__gqa_block_cached__moe_arch_mod__prompt_kernel(
    A_x: jax.Array,
    A_k_cache: jax.Array,
    A_v_cache: jax.Array,
    A_wq: jax.Array,
    A_wo: jax.Array,
    B_x: jax.Array,
    B_w_r: jax.Array,
    B_w_gate: jax.Array,
    B_w_up: jax.Array,
    B_w_down: jax.Array,
    c: jax.Array,
    w_mod: jax.Array,
):
    del B_x
    xt = A_x.reshape(S, D).T
    k = A_k_cache.reshape(HKV, S, DH)
    v = A_v_cache.reshape(HKV, S, DH)

    hbm = pl.BlockSpec(memory_space=pl.ANY)
    vmem = pl.BlockSpec(memory_space=pltpu.VMEM)
    stream = [
        pltpu.VMEM((S, REP * TQ), F32),
        pltpu.VMEM((8, REP * TQ), F32),
        pltpu.VMEM((DH // 2, S), U32),
        pltpu.VMEM((GW // 2, D), U32),
    ]
    out = pl.pallas_call(
        _kernel,
        in_specs=[vmem, vmem] + [hbm] * 9,
        out_specs=hbm,
        out_shape=jax.ShapeDtypeStruct((D, S), BF16),
        scratch_shapes=[
            pltpu.VMEM((NT + NFB + NMB, D, 128), BF16),
            pltpu.VMEM((HKV, S, DH), BF16),
            pltpu.VMEM((HKV, S, DH), BF16),
            pltpu.VMEM((HKV, D, GW), BF16),
            pltpu.VMEM((HKV, D, GW), BF16),
            pltpu.VMEM((D, DA), BF16),
            pltpu.VMEM((D, F), BF16),
            pltpu.VMEM((D, F), BF16),
            pltpu.VMEM((F // 2, D), U32),
            pltpu.VMEM((NT, D, 128), BF16),
            pltpu.VMEM((NT, D, 128), F32),
            pltpu.VMEM((6 * D, 128), F32),
            pltpu.VMEM((5 * 128, 128), F32),
            pltpu.VMEM((5 * 128, 128), F32),
            pltpu.VMEM((TPB, D, 128), F32),
            pltpu.VMEM((NT, D, 128), BF16),
            pltpu.VMEM((NT, D, 128), BF16),
            pltpu.VMEM((S // 2, D), U32),
            pltpu.VMEM((NT, D, 128), BF16),
            pltpu.VMEM((NT, 128), F32),
            pltpu.VMEM((NT * NC, 8, 128), F32),
            pltpu.VMEM((NT, 8, 128), F32),
            pltpu.VMEM((MPI, 8, 128), F32),
        ] + stream + stream + [
            pltpu.SemaphoreType.DMA((HKV // 2,)),
            pltpu.SemaphoreType.DMA((7,)),
            pltpu.SemaphoreType.DMA((C + TPB + 1,)),
        ],
        compiler_params=pltpu.CompilerParams(vmem_limit_bytes=120 * 1024 * 1024,
                                             disable_bounds_checks=True),
    )(B_w_r, c, xt, k, v, A_wq, A_wo.T, w_mod, B_w_gate, B_w_up, B_w_down.T)
    return out.T.reshape(1, S, D)
```

```python
import math

import jax
import jax.numpy as jnp
import jax.experimental.pallas as pl
import jax.experimental.pallas.tpu as pltpu

S = 2048
D = 576
HQ = 32
HKV = 16
REP = HQ // HKV
DH = 128
GW = REP * DH
F = 4608
C = 8
EPS = 1e-05
TQ = 512
NBLK = S // TQ
TPB = TQ // 128
NT = S // 128
NU = NBLK * HKV
DA = 2 * D
NC = 3
DC = D // NC
TLAG = 160
BAR = 1
PG = 64
NFB = F // 128
MODA = ((0, 4, 5), (1, 2, 6), (3, 7, 8))
NMB = 4 * D // 128
MPI = 3
MB0 = 2
WD0 = 14
PACE = (1280, 304, 2112, 1024, 400, 3200)

BF16 = jnp.bfloat16
F32 = jnp.float32
U32 = jnp.uint32
QSCALE = DH ** -0.5 * math.log2(math.e)


def _dot(a, b):
    return jnp.dot(a, b, preferred_element_type=F32)


def _dot_nt(a, b):
    return jax.lax.dot_general(a, b, (((1,), (1,)), ((), ())), preferred_element_type=F32)


def _r(x):
    return x.astype(BF16).astype(F32)


def _col_bcast(row):
    return jnp.broadcast_to(row, (128, 128)).T


def _blk(u):
    return u // HKV if isinstance(u, int) else jax.lax.shift_right_logical(u, 4)


def _grp(u):
    return u % HKV if isinstance(u, int) else jnp.bitwise_and(u, HKV - 1)


def _lanes(t, n=1):
    return pl.ds(pl.multiple_of(t * 128, 128), n * 128)


def _paced(x, clock, pos):
    if clock is None:
        return x
    row, col = pos % S, (pos // S) * TQ
    g = clock[row:row + x.shape[0], col:col + x.shape[1]]
    return jnp.where(g * g < 0.0, jnp.zeros_like(x), x)


def _softmax_numer(s, m):
    n, w = s.shape
    p = jnp.exp2(s - m).reshape(n // PG, PG // 8, 8, w)
    ts = jnp.sum(p, axis=1)
    last = jnp.where(ts < 0.0, ts, p[:, PG // 8 - 1])
    p = jnp.concatenate([p[:, :PG // 8 - 1], last[:, None]], axis=1).reshape(n, w)
    l = jnp.sum(jnp.sum(ts, axis=0), axis=0, keepdims=True)
    return p.astype(BF16), l


KEY0 = 0x20000000


def _score_key(r, t):
    tok = t * 128 + jax.lax.broadcasted_iota(jnp.int32, r.shape, 1)
    bits = jax.lax.shift_right_arithmetic(pltpu.bitcast(_r(r) + 0.0, jnp.int32), 16)
    code = jnp.where(bits < 0, -32769 - bits, bits) + 32768
    return pltpu.bitcast(code * S + (S - 1 - tok) + KEY0, F32)


def _chunk_stats(x):
    m = jnp.sum(x, axis=0, keepdims=True) * (1.0 / DC)
    xc = x - m
    return m, jnp.sum(xc * xc, axis=0, keepdims=True)


def _mean_var(stats):
    mean = sum(m for m, _ in stats) * (1.0 / NC)
    var = sum(s + DC * (m - mean) * (m - mean) for m, s in stats) * (1.0 / D)
    return mean, var


def _kernel(wr_hbm, c_hbm,
            xt_hbm, k_hbm, v_hbm, wq_hbm, wot_hbm, wmod_hbm, wg_hbm, wu_hbm, wdt_hbm,
            out_hbm,
            xw_v, k_v, v_v, wq_v, wot_v, wmod_v, wg_v, wu_v, wd_ref,
            ht_ref, acc_ref, mod_ref, wrb_ref, scb_ref, ln0_ref, x1_ref, h2_ref, h2row_ref, out_v,
            key_ref, st1_ref, st2_ref, lm_ref,
            s0_ref, m0_ref, vt0_ref, wqt0_ref, s1_ref, m1_ref, vt1_ref, wqt1_ref,
            wr_ref, c_ref, bsem, msem, osem):
    streams = ((s0_ref, m0_ref, vt0_ref, wqt0_ref), (s1_ref, m1_ref, vt1_ref, wqt1_ref))

    def cp_cols(src, dst, t, n, sem, dst_t=None):
        return pltpu.make_async_copy(src.at[:, _lanes(t, n)],
                                     dst.at[:, _lanes(t if dst_t is None else dst_t, n)], sem)

    def cp_pair(src, dst, p, sem):
        return pltpu.make_async_copy(src.at[pl.ds(2 * p, 2)], dst.at[pl.ds(2 * p, 2)], sem)

    cp_k = lambda p, sem: cp_pair(k_hbm, k_v, p, sem)
    cp_v1 = lambda g, sem: pltpu.make_async_copy(v_hbm.at[g], v_v.at[g], sem)
    cp_k1 = lambda g, sem: pltpu.make_async_copy(k_hbm.at[g], k_v.at[g], sem)

    class Both:
        def __init__(self, cps):
            self.cps = cps

        def start(self):
            for cp in self.cps:
                cp.start()

        def wait(self):
            for cp in self.cps:
                cp.wait()

    def cp_w1(src, dst, g, sem):
        return pltpu.make_async_copy(src.at[:, _lanes(g * REP, REP)], dst.at[g], sem)

    def cp_w(src, dst, p, sem):
        return Both([cp_w1(src, dst, 2 * p + a, sem) for a in range(2)])

    cp_wq = lambda p, sem: cp_w(wq_hbm, wq_v, p, sem)
    cp_wo = lambda p, sem: cp_w(wot_hbm, wot_v, p, sem)
    cp_x = lambda j, sem: Both([pltpu.make_async_copy(xt_hbm.at[:, _lanes(TPB * j + t)],
                                                      xw_v.at[TPB * j + t], sem) for t in range(TPB)])
    NP = HKV // 2

    def bundle(n, act):
        sem = bsem.at[n if isinstance(n, int) else jnp.minimum(n, NP - 1)]

        def on(cond, cps):
            def go():
                for cp in cps():
                    getattr(cp, act)()
            if isinstance(cond, bool):
                if cond:
                    go()
            else:
                pl.when(cond)(go)
        on(n + 1 < NP, lambda: [cp_k(n + 1, sem), cp_v1(2 * n + 2, sem), cp_w1(wq_hbm, wq_v, 2 * n + 3, sem)])
        on(n + 2 < NP, lambda: [cp_w1(wq_hbm, wq_v, 2 * n + 4, sem)])
        on(jnp.logical_and(n >= 1, n < NBLK) if not isinstance(n, int) else 1 <= n < NBLK, lambda: [cp_x(n, sem)])
        on(n < NP, lambda: [cp_v1(2 * n + 1, sem), cp_wo(n, sem)])

    cp_moda = [Both([cp_cols(wmod_hbm, wmod_v, t, 1, msem.at[s]) for t in tiles])
               for s, tiles in zip((0, 6, 10), MODA)]
    cp_modb = Both([pltpu.make_async_copy(wmod_hbm.at[:, _lanes(DA // 128 + b)],
                                          xw_v.at[NT + NFB + b], msem.at[1]) for b in range(NMB)])
    cp_g = pltpu.make_async_copy(wg_hbm, wg_v, msem.at[2])
    cp_u = pltpu.make_async_copy(wu_hbm, wu_v, msem.at[3])
    cp_d = Both([pltpu.make_async_copy(wdt_hbm.at[:, _lanes(b)], xw_v.at[NT + b], msem.at[4])
                 for b in range(NFB)])
    cp_out = lambda t, n, sem: Both([pltpu.make_async_copy(out_v.at[t + a], out_hbm.at[:, _lanes(t + a)],
                                                           sem) for a in range(n)])

    def silu_c():
        c = c_ref[...].astype(F32)
        return _r(c * _r(jax.nn.sigmoid(c)))

    def finish_mod(mod, lo):
        mod = _r(mod)
        col = lo + jax.lax.broadcasted_iota(jnp.int32, mod.shape, 1)
        is_scale = jnp.logical_or(jnp.logical_and(col >= D, col < 2 * D),
                                  jnp.logical_and(col >= 4 * D, col < 5 * D))
        mod = jnp.where(is_scale, _r(1.0 + mod), mod)
        for t in range(mod.shape[1] // 128):
            rows = pl.ds(pl.multiple_of(lo + t * 128, 128), 128)
            mod_ref[rows, :] = _col_bcast(mod[:, t * 128:(t + 1) * 128])

    def late_mod_sums(n, clock):
        b0 = jnp.clip(n - MB0, 0, NMB // MPI - 1) * MPI
        for k in range(MPI):
            w = xw_v[jnp.where(n >= MB0, NT + NFB + b0 + k, 0)].astype(F32)
            part = jnp.sum((w * scb_ref[0:D, :]).reshape(D // 8, 8, 128), axis=0)
            lm_ref[k] = _paced(part, clock, PACE[4] + 256 * k)

    def late_mod_store(n):
        b0 = jnp.clip(n - MB0, 0, NMB // MPI - 1) * MPI
        for k in range(MPI):
            finish_mod(jnp.sum(lm_ref[k], axis=0, keepdims=True), DA + (b0 + k) * 128)

    def col_vector(ref, row):
        row = jnp.concatenate([row, jnp.zeros((1, 64), F32)], axis=1)
        for t in range(5):
            ref[t * 128:(t + 1) * 128, :] = _col_bcast(row[:, t * 128:(t + 1) * 128])

    def mod(k):
        return mod_ref[k * D:(k + 1) * D, :]

    def put_stats(st_ref, t, shift, scale, clock, pos):
        row = jax.lax.broadcasted_iota(jnp.int32, (8, 128), 0)
        st_ref[t] = _paced(jnp.where(row == 0, shift, scale), clock, pos)

    def ln1_stats(t, clock=None):
        for c in range(NC):
            m, s = _chunk_stats(xw_v[t, c * DC:(c + 1) * DC, :].astype(F32))
            put_stats(st1_ref, t * NC + c, m, s, clock, PACE[0] + 192 * c)

    def ln1_norm(t):
        mean, var = _mean_var([(st1_ref[t * NC + c, 0:1, :], st1_ref[t * NC + c, 1:2, :])
                               for c in range(NC)])
        return (xw_v[t].astype(F32) - mean) * jax.lax.rsqrt(var + EPS)

    def ln1_apply(t, clock=None, ln=None):
        h = (ln1_norm(t) if ln is None else ln) * mod(1) + mod(0)
        ht_ref[t] = _paced(h, clock, PACE[1]).astype(BF16)

    def h2_rows(t, clock=None):
        x = pltpu.bitcast(h2_ref[t].T, U32)
        x = jnp.concatenate([_paced(x[:, a:min(a + 128, D)], clock, PACE[5] + a // 2)
                             for a in range(0, D, 128)], axis=1)
        h2row_ref[pl.ds(pl.multiple_of(t * 64, 64), 64), :] = x

    def router_terms():
        u = mod(4) * wrb_ref[0:D, :]
        return (u, jnp.sum(u, axis=0, keepdims=True),
                jnp.sum(mod(3) * wrb_ref[0:D, :], axis=0, keepdims=True))

    def ln2_stats(t, clock=None, attn=None, terms=None):
        x1 = _r(xw_v[t].astype(F32) + mod(2) * (acc_ref[t] if attn is None else attn))
        x1_ref[t] = _paced(x1, clock, PACE[2]).astype(BF16)
        mean, var = _mean_var([_chunk_stats(x1[c * DC:(c + 1) * DC]) for c in range(NC)])
        mean = _r(mean)
        inv = 1.0 / _r(jnp.sqrt(_r(_r(var) + EPS)))
        put_stats(st2_ref, t, mean, inv, clock, PACE[2] + D + 128)
        if terms is not None:
            u, u_sum, b_sum = terms
            r = (jnp.sum(x1 * u, axis=0, keepdims=True) - mean * u_sum) * inv + b_sum
            return _score_key(r, t)

    def ln2_h2(t, x1):
        return (x1 - st2_ref[t, 0:1, :]) * st2_ref[t, 1:2, :] * mod(4) + mod(3)

    def ln2_apply(t, clock):
        x1 = x1_ref[t].astype(F32)
        h2 = ln2_h2(t, x1)
        key = _score_key(jnp.sum(h2 * wrb_ref[0:D, :], axis=0, keepdims=True), t)
        key_ref[pl.ds(t, 1), :] = _paced(key, clock, PACE[3] + D + 96)
        h2 = _r(h2)
        h2_ref[t] = _paced(h2, clock, PACE[3]).astype(BF16)
        out_v[t] = _paced(x1 + mod(5) * h2, clock, PACE[3] + 16).astype(BF16)

    def q_proj(u, wqt_ref, split=False):
        w = pltpu.bitcast(wqt_ref[...], BF16)
        h = jnp.concatenate([ht_ref[_blk(u) * TPB + t] for t in range(TPB)], axis=1)
        if split:
            q = sum(_dot(w[:, a:min(a + 128, D)], h[a:min(a + 128, D)]) for a in range(0, D, 128))
        else:
            q = _dot(w, h)
        q = (q * QSCALE).astype(BF16)
        return jnp.concatenate([q[r * DH:(r + 1) * DH] for r in range(REP)], axis=1)

    def scores(u, q, s_ref, m_ref):
        s = _dot(k_v[_grp(u)], q)
        s_ref[...] = s
        m_ref[...] = jnp.broadcast_to(jnp.max(s, axis=0, keepdims=True), m_ref.shape)
        return s

    def v_transpose(u, vt_ref):
        vt_ref[...] = pltpu.bitcast(v_v[_grp(u)].T, U32)

    def wq_transpose(u, wqt_ref):
        wqt_ref[...] = pltpu.bitcast(wq_v[_grp(u)].T, U32)

    def attend(s_ref, m_ref, vt_ref):
        m = m_ref[0:1, :]
        o = []
        for r in range(REP):
            cols = slice(r * TQ, (r + 1) * TQ)
            p, l = _softmax_numer(s_ref[:, cols], m[:, cols])
            o.append((_dot(pltpu.bitcast(vt_ref[...], BF16), p) * (1.0 / l)).astype(BF16))
        return jnp.concatenate(o, axis=0)

    small = Both([pltpu.make_async_copy(wr_hbm, wr_ref, msem.at[7]),
                  pltpu.make_async_copy(c_hbm, c_ref, msem.at[7])])
    zeroth = Both([cp_x(0, msem.at[5]), cp_w1(wq_hbm, wq_v, 0, msem.at[5])])
    first = Both([cp_k1(0, msem.at[8]), cp_w1(wq_hbm, wq_v, 1, msem.at[8])])
    second = Both([cp_k1(1, msem.at[9]), cp_v1(0, msem.at[9]), cp_w1(wq_hbm, wq_v, 2, msem.at[9])])
    for cp in [small, zeroth] + cp_moda + [first, second]:
        cp.start()
    acc_ref[...] = jnp.zeros_like(acc_ref)
    mod_ref[DA:6 * D, :] = jnp.zeros((4 * D, 128), F32)
    h2_ref[0] = jnp.zeros((D, 128), BF16)
    small.wait()
    col_vector(wrb_ref, wr_ref[...].astype(F32).reshape(1, D))
    col_vector(scb_ref, silu_c())
    sc8 = jnp.broadcast_to(silu_c(), (8, D)).astype(BF16)
    zeroth.wait()
    for t in range(TPB):
        ln1_stats(t)
        ln0_ref[t] = ln1_norm(t)
    wq_transpose(0, wqt0_ref)
    for cp, tiles in zip(cp_moda, MODA):
        cp.wait()
        for t in tiles:
            finish_mod(_dot(sc8, wmod_v[:, t * 128:(t + 1) * 128])[0:1], t * 128)
    for t in range(TPB):
        ln1_apply(t, ln=ln0_ref[t])
    q = q_proj(0, wqt0_ref, split=True)
    first.wait()
    bundle(0, 'start')
    scores(0, q, s0_ref, m0_ref)
    wq_transpose(1, wqt1_ref)
    second.wait()
    bundle(1, 'start')
    scores(1, q_proj(1, wqt1_ref), s1_ref, m1_ref)
    v_transpose(0, vt0_ref)
    wq_transpose(2, wqt0_ref)

    def unit(u, side, s_ref, m_ref, vt_ref, wqt_ref):
        q = q_proj(u + 2, wqt_ref)
        o = attend(s_ref, m_ref, vt_ref)
        clock = scores(u + 2, q, s_ref, m_ref)
        side(clock)
        upd = _dot(wot_v[_grp(u)], o)
        for t in range(TPB):
            acc_ref[_blk(u) * TPB + t] += upd[:, t * 128:(t + 1) * 128]
        fb = jnp.clip(u - WD0, 0, NFB - 1)
        src = jnp.where(u >= WD0, NT + fb, 0)
        wd_ref[pl.ds(pl.multiple_of(fb * 64, 64), 64), :] = pltpu.bitcast(xw_v[src].T, U32)

    def step(n, carry):
        def waits(_, c):
            bundle(n, 'wait')
            pl.when(n == MB0)(cp_modb.wait)
            pl.when(n == WD0 // 2)(cp_d.wait)
            return c
        jax.lax.fori_loop(0, jnp.where(n < NP, 1, 0), waits, 0)

        pl.when(n == 0)(cp_modb.start)
        bundle(jnp.minimum(n + 2, NP), 'start')
        for a in range(3):
            pl.when(n == 2 + a)(Both(cp_d.cps[a * NFB // 3:(a + 1) * NFB // 3]).start)
        pl.when(n == NP)(Both([cp_g, cp_u]).start)

        t1 = jnp.minimum(n + 2, NT - 1)
        v = jnp.maximum(n - NP, 0)
        tile2 = lambda v: (jax.lax.shift_right_logical(v, 3) * TPB
                           + jnp.minimum(jnp.bitwise_and(v, NP - 1), TPB - 1))
        t2 = tile2(v)
        v_transpose(2 * n + 1, vt1_ref)
        wq_transpose(2 * n + 3, wqt1_ref)

        def stats(clock):
            ln2_stats(t2, clock)
            ln1_stats(t1, clock)
            late_mod_sums(n, clock)
            h2_rows(tile2(jnp.maximum(v - 1, 0)), clock)

        def apply(clock):
            ln1_apply(t1, clock)
            ln2_apply(t2, clock)
            late_mod_store(n)

        for a in range(2):
            unit(2 * n + a, (stats, apply)[a], *streams[a])
        v_transpose(2 * n + 2, vt0_ref)
        wq_transpose(2 * n + 4, wqt0_ref)
        return carry

    jax.lax.fori_loop(0, NU // 2 - 1, step, 0)

    T0 = NT - TPB
    cp_out(0, T0, osem.at[C + TPB]).start()
    cp_g.wait()
    v_transpose(NU - 1, vt1_ref)
    o = jnp.concatenate([attend(*streams[a][0:3]) for a in range(2)], axis=0)
    wlast = jnp.concatenate([wot_v[HKV - 2], wot_v[HKV - 1]], axis=1)
    fin = [acc_ref[T0 + t] + _dot(wlast, o[:, t * 128:(t + 1) * 128]) for t in range(TPB)]
    clock = jnp.concatenate(fin, axis=0)
    row8 = jax.lax.broadcasted_iota(jnp.int32, (C, 128), 0)
    lane8 = jax.lax.broadcasted_iota(jnp.int32, (C, 128), 1)
    work = key_ref[0:T0, :]
    lead = jnp.zeros((C, 128), F32)
    for t in range(C):
        mx = jnp.max(jnp.max(work, axis=0, keepdims=True), axis=1, keepdims=True)
        work = jnp.where(work == mx, 0.0, work)
        lead = jnp.where(row8 == t, mx, lead)

    def spread(row):
        return pltpu.roll(jnp.broadcast_to(row, (128, 128)), 0, 1, stride=1, stride_axis=0)

    def merge(lead, rows, spreads):
        cols = jnp.concatenate([lead] + spreads, axis=0)
        best = jnp.zeros((C, 128), F32)
        for row in [jnp.max(jnp.where(row8 == lane8, lead, 0.0), axis=0, keepdims=True)] + rows:
            rank = jnp.sum(jnp.where(cols > row, 1.0, 0.0), axis=0, keepdims=True)
            best = jnp.maximum(best, jnp.where(rank == row8.astype(F32), row, 0.0))
        return jnp.max(best, axis=1, keepdims=True)

    def tail_h2(t, gate=None):
        x1 = x1_ref[t].astype(F32)
        if gate is not None:
            n = gate.shape[0]
            x1 = jnp.concatenate([_paced(x1[:n], gate, 0), x1[n:]], axis=0) if n < D else _paced(x1, gate, 0)
        h2_ref[t] = ln2_h2(t, x1).astype(BF16)
        if t < NT - 2:
            h2_rows(t)

    terms = router_terms()
    keys = []
    for t in range(TPB):
        keys.append(ln2_stats(T0 + t, attn=fin[t], terms=terms))
        if t < TPB - 1:
            tail_h2(T0 + t, clock[(t + 1) * D + TLAG:(t + 2) * D + TLAG])
    lead = jnp.broadcast_to(merge(lead, keys[0:2], [spread(k) for k in keys[0:2]]), (C, 128))
    spread2 = spread(keys[2])
    if BAR == 0:
        cp_u.wait()
        cp_out(0, T0, osem.at[C + TPB]).wait()

    h2_rows(NT - 2)
    tail_h2(NT - 1)
    h2_rows(NT - 1)
    sel = pltpu.bitcast(merge(lead, keys[2:4], [spread2, spread(keys[3])]), jnp.int32) - KEY0
    sel_tok = (S - 1) - (sel & (S - 1))
    toks = [sel_tok[t, 0] for t in range(C)]
    tiles = [jax.lax.shift_right_logical(tk, 7) for tk in toks]
    sel_code = jax.lax.shift_right_logical(sel, 11) - 32768
    sel_bits = jnp.where(sel_code < 0, -32769 - sel_code, sel_code)
    r_sel = pltpu.bitcast(jax.lax.shift_left(sel_bits, 16), F32)

    final = []
    for t in range(C):
        d = True
        for u in range(t + 1, C):
            d = jnp.logical_and(d, tiles[u] != tiles[t])
        final.append(d)

    words = jnp.concatenate([h2row_ref[pl.ds(jax.lax.shift_right_logical(toks[t], 1), 1), :]
                             for t in range(C)], axis=0)
    odd = jnp.bitwise_and(sel_tok, 1) == 1
    xs = pltpu.bitcast(jnp.where(odd, jnp.bitwise_and(words, jnp.uint32(0xFFFF0000)),
                                 jax.lax.shift_left(words, jnp.uint32(16))), F32)
    xs = xs.astype(BF16)

    if BAR == 1:
        cp_u.wait()
        cp_out(0, T0, osem.at[C + TPB]).wait()
    gpre = _r(_dot(xs, wg_v[...]))
    gact = _r(gpre * _r(jax.nn.sigmoid(gpre)))
    u = _r(_dot(xs, wu_v[...]))
    act = (gact * u).astype(BF16)
    FK = F // 4
    yk = [[_dot(act[:, a * FK:(a + 1) * FK],
                pltpu.bitcast(wd_ref[a * FK // 2:(a + 1) * FK // 2, j:min(j + 128, D)], BF16))
           for a in range(4)] for j in range(0, D, 128)]
    y = jnp.concatenate([sum(p) for p in yk], axis=1)
    clean = []
    for t in range(T0, NT):
        gate = jnp.concatenate([yk[t - T0][a // 18] for a in range(D // 8)], axis=0)
        x1 = _paced(x1_ref[t].astype(F32), gate, 0)
        out_v[t] = (x1 + mod(5) * h2_ref[t].astype(F32)).astype(BF16)
        d = tiles[0] != t
        for a in range(1, C):
            d = jnp.logical_and(d, tiles[a] != t)
        clean.append(d)
        pl.when(d)(cp_out(t, 1, osem.at[C + t - T0]).start)
    y = _r(y)
    y = y * _r(jax.nn.sigmoid(r_sel))
    yt = jnp.concatenate([y, jnp.zeros((16 - C, D), F32)], axis=0).astype(BF16).T

    Q = D // 4
    for t in range(C):
        oh = jnp.where(sel_tok == tiles[t] * 128 + lane8, 1.0, 0.0)
        oh = jnp.concatenate([oh, jnp.zeros((16 - C, 128), F32)], axis=0).astype(BF16)
        upd = jnp.concatenate([_dot(yt[a * Q:(a + 1) * Q], oh) for a in range(4)], axis=0)
        out_v[tiles[t]] = (x1_ref[tiles[t]].astype(F32)
                           + mod(5) * (h2_ref[tiles[t]].astype(F32) + upd)).astype(BF16)
        if final[t] is True:
            cp_out(tiles[t], 1, osem.at[t]).start()
        else:
            pl.when(final[t])(cp_out(tiles[t], 1, osem.at[t]).start)
    for t in range(T0, NT):
        pl.when(clean[t - T0])(cp_out(t, 1, osem.at[C + t - T0]).wait)
    for t in range(C):
        if final[t] is True:
            cp_out(tiles[t], 1, osem.at[t]).wait()
        else:
            pl.when(final[t])(cp_out(tiles[t], 1, osem.at[t]).wait)


@jax.jit
def pallas_adaLN_cond__gqa_block_cached__moe_arch_mod__prompt_kernel(
    A_x: jax.Array,
    A_k_cache: jax.Array,
    A_v_cache: jax.Array,
    A_wq: jax.Array,
    A_wo: jax.Array,
    B_x: jax.Array,
    B_w_r: jax.Array,
    B_w_gate: jax.Array,
    B_w_up: jax.Array,
    B_w_down: jax.Array,
    c: jax.Array,
    w_mod: jax.Array,
):
    del B_x
    xt = A_x.reshape(S, D).T
    k = A_k_cache.reshape(HKV, S, DH)
    v = A_v_cache.reshape(HKV, S, DH)

    hbm = pl.BlockSpec(memory_space=pl.ANY)
    stream = [
        pltpu.VMEM((S, REP * TQ), F32),
        pltpu.VMEM((8, REP * TQ), F32),
        pltpu.VMEM((DH // 2, S), U32),
        pltpu.VMEM((GW // 2, D), U32),
    ]
    out = pl.pallas_call(
        _kernel,
        in_specs=[hbm] * 11,
        out_specs=hbm,
        out_shape=jax.ShapeDtypeStruct((D, S), BF16),
        scratch_shapes=[
            pltpu.VMEM((NT + NFB + NMB, D, 128), BF16),
            pltpu.VMEM((HKV, S, DH), BF16),
            pltpu.VMEM((HKV, S, DH), BF16),
            pltpu.VMEM((HKV, D, GW), BF16),
            pltpu.VMEM((HKV, D, GW), BF16),
            pltpu.VMEM((D, DA), BF16),
            pltpu.VMEM((D, F), BF16),
            pltpu.VMEM((D, F), BF16),
            pltpu.VMEM((F // 2, D), U32),
            pltpu.VMEM((NT, D, 128), BF16),
            pltpu.VMEM((NT, D, 128), F32),
            pltpu.VMEM((6 * D, 128), F32),
            pltpu.VMEM((5 * 128, 128), F32),
            pltpu.VMEM((5 * 128, 128), F32),
            pltpu.VMEM((TPB, D, 128), F32),
            pltpu.VMEM((NT, D, 128), BF16),
            pltpu.VMEM((NT, D, 128), BF16),
            pltpu.VMEM((S // 2, D), U32),
            pltpu.VMEM((NT, D, 128), BF16),
            pltpu.VMEM((NT, 128), F32),
            pltpu.VMEM((NT * NC, 8, 128), F32),
            pltpu.VMEM((NT, 8, 128), F32),
            pltpu.VMEM((MPI, 8, 128), F32),
        ] + stream + stream + [
            pltpu.VMEM((D,), BF16),
            pltpu.VMEM((1, D), BF16),
            pltpu.SemaphoreType.DMA((HKV // 2,)),
            pltpu.SemaphoreType.DMA((11,)),
            pltpu.SemaphoreType.DMA((C + TPB + 1,)),
        ],
        compiler_params=pltpu.CompilerParams(vmem_limit_bytes=120 * 1024 * 1024,
                                             disable_bounds_checks=True,
                                             disable_semaphore_checks=True),
    )(B_w_r, c, xt, k, v, A_wq, A_wo.T, w_mod, B_w_gate, B_w_up, B_w_down.T)
    return out.T.reshape(1, S, D)
```

```python
import math

import jax
import jax.numpy as jnp
import jax.experimental.pallas as pl
import jax.experimental.pallas.tpu as pltpu

S = 2048
D = 576
HQ = 32
HKV = 16
REP = HQ // HKV
DH = 128
GW = REP * DH
F = 4608
C = 8
EPS = 1e-05
TQ = 512
NBLK = S // TQ
TPB = TQ // 128
NT = S // 128
NU = NBLK * HKV
DA = 2 * D
NC = 3
DC = D // NC
TLAG = 160
SLAG = 96
BAR = 1
PG = 64
NFB = F // 128
MODA = ((0, 4, 5), (1, 2, 6), (3, 7, 8))
NMB = 4 * D // 128
MPI = 3
MB0 = 2
WD0 = 14
PACE = (1280, 304, 2112, 1024, 400, 3200)

BF16 = jnp.bfloat16
F32 = jnp.float32
U32 = jnp.uint32
QSCALE = DH ** -0.5 * math.log2(math.e)


def _dot(a, b):
    return jnp.dot(a, b, preferred_element_type=F32)


def _dot_nt(a, b):
    return jax.lax.dot_general(a, b, (((1,), (1,)), ((), ())), preferred_element_type=F32)


def _r(x):
    return x.astype(BF16).astype(F32)


def _col_bcast(row):
    return jnp.broadcast_to(row, (128, 128)).T


def _blk(u):
    return u // HKV if isinstance(u, int) else jax.lax.shift_right_logical(u, 4)


def _grp(u):
    return u % HKV if isinstance(u, int) else jnp.bitwise_and(u, HKV - 1)


def _lanes(t, n=1):
    return pl.ds(pl.multiple_of(t * 128, 128), n * 128)


def _paced(x, clock, pos):
    if clock is None:
        return x
    row, col = pos % S, (pos // S) * TQ
    g = clock[row:row + x.shape[0], col:col + x.shape[1]]
    return jnp.where(g * g < 0.0, jnp.zeros_like(x), x)


def _softmax_numer(s, m):
    n, w = s.shape
    p = jnp.exp2(s - m).reshape(n // PG, PG // 8, 8, w)
    ts = jnp.sum(p, axis=1)
    last = jnp.where(ts < 0.0, ts, p[:, PG // 8 - 1])
    p = jnp.concatenate([p[:, :PG // 8 - 1], last[:, None]], axis=1).reshape(n, w)
    l = jnp.sum(jnp.sum(ts, axis=0), axis=0, keepdims=True)
    return p.astype(BF16), l


KEY0 = 0x20000000


def _score_key(r, t):
    tok = t * 128 + jax.lax.broadcasted_iota(jnp.int32, r.shape, 1)
    bits = jax.lax.shift_right_arithmetic(pltpu.bitcast(_r(r) + 0.0, jnp.int32), 16)
    code = jnp.where(bits < 0, -32769 - bits, bits) + 32768
    return pltpu.bitcast(code * S + (S - 1 - tok) + KEY0, F32)


def _chunk_stats(x):
    m = jnp.sum(x, axis=0, keepdims=True) * (1.0 / DC)
    xc = x - m
    return m, jnp.sum(xc * xc, axis=0, keepdims=True)


def _mean_var(stats):
    mean = sum(m for m, _ in stats) * (1.0 / NC)
    var = sum(s + DC * (m - mean) * (m - mean) for m, s in stats) * (1.0 / D)
    return mean, var


def _kernel(wr_hbm, c_hbm,
            xt_hbm, k_hbm, v_hbm, wq_hbm, wot_hbm, wmod_hbm, wg_hbm, wu_hbm, wdt_hbm,
            out_hbm,
            xw_v, k_v, v_v, wq_v, wot_v, wmod_v, wg_v, wu_v, wd_ref,
            ht_ref, acc_ref, mod_ref, wrb_ref, scb_ref, ln0_ref, x1_ref, h2_ref, h2row_ref, out_v,
            key_ref, st1_ref, st2_ref, lm_ref,
            s0_ref, m0_ref, vt0_ref, wqt0_ref, s1_ref, m1_ref, vt1_ref, wqt1_ref,
            wr_ref, c_ref, bsem, msem, osem):
    streams = ((s0_ref, m0_ref, vt0_ref, wqt0_ref), (s1_ref, m1_ref, vt1_ref, wqt1_ref))

    def cp_cols(src, dst, t, n, sem, dst_t=None):
        return pltpu.make_async_copy(src.at[:, _lanes(t, n)],
                                     dst.at[:, _lanes(t if dst_t is None else dst_t, n)], sem)

    def cp_pair(src, dst, p, sem):
        return pltpu.make_async_copy(src.at[pl.ds(2 * p, 2)], dst.at[pl.ds(2 * p, 2)], sem)

    cp_k = lambda p, sem: cp_pair(k_hbm, k_v, p, sem)
    cp_v1 = lambda g, sem: pltpu.make_async_copy(v_hbm.at[g], v_v.at[g], sem)
    cp_k1 = lambda g, sem: pltpu.make_async_copy(k_hbm.at[g], k_v.at[g], sem)

    class Both:
        def __init__(self, cps):
            self.cps = cps

        def start(self):
            for cp in self.cps:
                cp.start()

        def wait(self):
            for cp in self.cps:
                cp.wait()

    def cp_w1(src, dst, g, sem):
        return pltpu.make_async_copy(src.at[:, _lanes(g * REP, REP)], dst.at[g], sem)

    def cp_w(src, dst, p, sem):
        return Both([cp_w1(src, dst, 2 * p + a, sem) for a in range(2)])

    cp_wq = lambda p, sem: cp_w(wq_hbm, wq_v, p, sem)
    cp_wo = lambda p, sem: cp_w(wot_hbm, wot_v, p, sem)
    cp_x = lambda j, sem: Both([pltpu.make_async_copy(xt_hbm.at[:, _lanes(TPB * j + t)],
                                                      xw_v.at[TPB * j + t], sem) for t in range(TPB)])
    NP = HKV // 2

    def bundle(n, act):
        sem = bsem.at[n if isinstance(n, int) else jnp.minimum(n, NP - 1)]

        def on(cond, cps):
            def go():
                for cp in cps():
                    getattr(cp, act)()
            if isinstance(cond, bool):
                if cond:
                    go()
            else:
                pl.when(cond)(go)
        on(n + 1 < NP, lambda: [cp_k(n + 1, sem), cp_v1(2 * n + 2, sem), cp_w1(wq_hbm, wq_v, 2 * n + 3, sem)])
        on(n + 2 < NP, lambda: [cp_w1(wq_hbm, wq_v, 2 * n + 4, sem)])
        on(jnp.logical_and(n >= 1, n < NBLK) if not isinstance(n, int) else 1 <= n < NBLK, lambda: [cp_x(n, sem)])
        on(n < NP, lambda: [cp_v1(2 * n + 1, sem), cp_wo(n, sem)])

    cp_moda = [Both([cp_cols(wmod_hbm, wmod_v, t, 1, msem.at[s]) for t in tiles])
               for s, tiles in zip((0, 6, 10), MODA)]
    cp_modb = Both([pltpu.make_async_copy(wmod_hbm.at[:, _lanes(DA // 128 + b)],
                                          xw_v.at[NT + NFB + b], msem.at[1]) for b in range(NMB)])
    cp_g = pltpu.make_async_copy(wg_hbm, wg_v, msem.at[2])
    cp_u = pltpu.make_async_copy(wu_hbm, wu_v, msem.at[3])
    cp_d = Both([pltpu.make_async_copy(wdt_hbm.at[:, _lanes(b)], xw_v.at[NT + b], msem.at[4])
                 for b in range(NFB)])
    cp_out = lambda t, n, sem: Both([pltpu.make_async_copy(out_v.at[t + a], out_hbm.at[:, _lanes(t + a)],
                                                           sem) for a in range(n)])

    def silu_c():
        c = c_ref[...].astype(F32)
        return _r(c * _r(jax.nn.sigmoid(c)))

    def finish_mod(mod, lo):
        mod = _r(mod)
        col = lo + jax.lax.broadcasted_iota(jnp.int32, mod.shape, 1)
        is_scale = jnp.logical_or(jnp.logical_and(col >= D, col < 2 * D),
                                  jnp.logical_and(col >= 4 * D, col < 5 * D))
        mod = jnp.where(is_scale, _r(1.0 + mod), mod)
        for t in range(mod.shape[1] // 128):
            rows = pl.ds(pl.multiple_of(lo + t * 128, 128), 128)
            mod_ref[rows, :] = _col_bcast(mod[:, t * 128:(t + 1) * 128])

    def late_mod_sums(n, clock):
        b0 = jnp.clip(n - MB0, 0, NMB // MPI - 1) * MPI
        for k in range(MPI):
            w = xw_v[jnp.where(n >= MB0, NT + NFB + b0 + k, 0)].astype(F32)
            part = jnp.sum((w * scb_ref[0:D, :]).reshape(D // 8, 8, 128), axis=0)
            lm_ref[k] = _paced(part, clock, PACE[4] + 256 * k)

    def late_mod_store(n):
        b0 = jnp.clip(n - MB0, 0, NMB // MPI - 1) * MPI
        for k in range(MPI):
            finish_mod(jnp.sum(lm_ref[k], axis=0, keepdims=True), DA + (b0 + k) * 128)

    def col_vector(ref, row):
        row = jnp.concatenate([row, jnp.zeros((1, 64), F32)], axis=1)
        for t in range(5):
            ref[t * 128:(t + 1) * 128, :] = _col_bcast(row[:, t * 128:(t + 1) * 128])

    def mod(k):
        return mod_ref[k * D:(k + 1) * D, :]

    def put_stats(st_ref, t, shift, scale, clock, pos):
        row = jax.lax.broadcasted_iota(jnp.int32, (8, 128), 0)
        st_ref[t] = _paced(jnp.where(row == 0, shift, scale), clock, pos)

    def ln1_stats(t, clock=None):
        for c in range(NC):
            m, s = _chunk_stats(xw_v[t, c * DC:(c + 1) * DC, :].astype(F32))
            put_stats(st1_ref, t * NC + c, m, s, clock, PACE[0] + 192 * c)

    def ln1_norm(t):
        mean, var = _mean_var(load_stats(st1_ref, t))
        return (xw_v[t].astype(F32) - mean) * jax.lax.rsqrt(var + EPS)

    def ln1_apply(t, clock=None, ln=None):
        h = (ln1_norm(t) if ln is None else ln) * mod(1) + mod(0)
        ht_ref[t] = _paced(h, clock, PACE[1]).astype(BF16)

    def h2_rows(t, clock=None):
        x = pltpu.bitcast(h2_ref[t].T, U32)
        x = jnp.concatenate([_paced(x[:, a:min(a + 128, D)], clock, PACE[5] + a // 2)
                             for a in range(0, D, 128)], axis=1)
        h2row_ref[pl.ds(pl.multiple_of(t * 64, 64), 64), :] = x

    def router_terms():
        u = mod(4) * wrb_ref[0:D, :]
        return (u, jnp.sum(u, axis=0, keepdims=True),
                jnp.sum(mod(3) * wrb_ref[0:D, :], axis=0, keepdims=True))

    def load_stats(st_ref, t):
        return [(st_ref[t * NC + c, 0:1, :], st_ref[t * NC + c, 1:2, :]) for c in range(NC)]

    def ln2_x1(t, attn, clock=None):
        x1 = _r(xw_v[t].astype(F32) + mod(2) * attn)
        x1_ref[t] = _paced(x1, clock, PACE[2]).astype(BF16)
        return x1, [_chunk_stats(x1[c * DC:(c + 1) * DC]) for c in range(NC)]

    def ln2_norm(stats):
        mean, var = _mean_var(stats)
        return _r(mean), 1.0 / _r(jnp.sqrt(_r(_r(var) + EPS)))

    def ln2_h2(x1, mean, inv):
        return (x1 - mean) * inv * mod(4) + mod(3)

    def ln2_stats(t, clock):
        for c, (m, s) in enumerate(ln2_x1(t, acc_ref[t], clock)[1]):
            put_stats(st2_ref, t * NC + c, m, s, clock, PACE[2] + (c + 1) * DC + SLAG)

    def ln2_apply(t, clock):
        x1 = x1_ref[t].astype(F32)
        h2 = ln2_h2(x1, *ln2_norm(load_stats(st2_ref, t)))
        key = _score_key(jnp.sum(h2 * wrb_ref[0:D, :], axis=0, keepdims=True), t)
        key_ref[pl.ds(t, 1), :] = _paced(key, clock, PACE[3] + D + 96)
        h2 = _r(h2)
        h2_ref[t] = _paced(h2, clock, PACE[3]).astype(BF16)
        out_v[t] = _paced(x1 + mod(5) * h2, clock, PACE[3] + 16).astype(BF16)

    def q_proj(u, wqt_ref, split=False):
        w = pltpu.bitcast(wqt_ref[...], BF16)
        h = jnp.concatenate([ht_ref[_blk(u) * TPB + t] for t in range(TPB)], axis=1)
        if split == 1:
            q = sum(_dot(w[:, a:min(a + 128, D)], h[a:min(a + 128, D)]) for a in range(0, D, 128))
        elif split == 2:
            q = _dot(w[:, 512:], h[512:])
            q = _dot(w[:, :512], h[:512]) + q
        else:
            q = _dot(w, h)
        q = (q * QSCALE).astype(BF16)
        return jnp.concatenate([q[r * DH:(r + 1) * DH] for r in range(REP)], axis=1)

    def scores(u, q, s_ref, m_ref):
        s = _dot(k_v[_grp(u)], q)
        s_ref[...] = s
        m_ref[...] = jnp.broadcast_to(jnp.max(s, axis=0, keepdims=True), m_ref.shape)
        return s

    def v_transpose(u, vt_ref):
        vt_ref[...] = pltpu.bitcast(v_v[_grp(u)].T, U32)

    def wq_transpose(u, wqt_ref):
        wqt_ref[...] = pltpu.bitcast(wq_v[_grp(u)].T, U32)

    def attend(s_ref, m_ref, vt_ref):
        m = m_ref[0:1, :]
        o = []
        for r in range(REP):
            cols = slice(r * TQ, (r + 1) * TQ)
            p, l = _softmax_numer(s_ref[:, cols], m[:, cols])
            o.append((_dot(pltpu.bitcast(vt_ref[...], BF16), p) * (1.0 / l)).astype(BF16))
        return jnp.concatenate(o, axis=0)

    small = Both([pltpu.make_async_copy(wr_hbm, wr_ref, msem.at[7]),
                  pltpu.make_async_copy(c_hbm, c_ref, msem.at[7])])
    zeroth = Both([cp_x(0, msem.at[5]), cp_w1(wq_hbm, wq_v, 0, msem.at[5])])
    first = Both([cp_k1(0, msem.at[8]), cp_w1(wq_hbm, wq_v, 1, msem.at[8])])
    second = Both([cp_k1(1, msem.at[9]), cp_v1(0, msem.at[9]), cp_w1(wq_hbm, wq_v, 2, msem.at[9])])
    for cp in [small, zeroth] + cp_moda + [first, second]:
        cp.start()
    acc_ref[...] = jnp.zeros_like(acc_ref)
    mod_ref[DA:6 * D, :] = jnp.zeros((4 * D, 128), F32)
    h2_ref[0] = jnp.zeros((D, 128), BF16)
    small.wait()
    col_vector(wrb_ref, wr_ref[...].astype(F32).reshape(1, D))
    col_vector(scb_ref, silu_c())
    sc8 = jnp.broadcast_to(silu_c(), (8, D)).astype(BF16)
    zeroth.wait()
    for t in range(TPB):
        ln1_stats(t)
        ln0_ref[t] = ln1_norm(t)
    wq_transpose(0, wqt0_ref)
    for cp, tiles in zip(cp_moda, MODA):
        cp.wait()
        for t in tiles:
            finish_mod(_dot(sc8, wmod_v[:, t * 128:(t + 1) * 128])[0:1], t * 128)
    for t in range(TPB):
        ln1_apply(t, ln=ln0_ref[t])
    q = q_proj(0, wqt0_ref, split=True)
    first.wait()
    bundle(0, 'start')
    scores(0, q, s0_ref, m0_ref)
    wq_transpose(1, wqt1_ref)
    second.wait()
    bundle(1, 'start')
    scores(1, q_proj(1, wqt1_ref, split=2), s1_ref, m1_ref)
    v_transpose(0, vt0_ref)
    wq_transpose(2, wqt0_ref)

    def unit(u, side, s_ref, m_ref, vt_ref, wqt_ref):
        q = q_proj(u + 2, wqt_ref, split=2 if s_ref is s0_ref else 0)
        o = attend(s_ref, m_ref, vt_ref)
        clock = scores(u + 2, q, s_ref, m_ref)
        side(clock)
        upd = _dot(wot_v[_grp(u)], o)
        for t in range(TPB):
            acc_ref[_blk(u) * TPB + t] += upd[:, t * 128:(t + 1) * 128]
        fb = jnp.clip(u - WD0, 0, NFB - 1)
        src = jnp.where(u >= WD0, NT + fb, 0)
        wd_ref[pl.ds(pl.multiple_of(fb * 64, 64), 64), :] = pltpu.bitcast(xw_v[src].T, U32)

    def step(n, carry):
        def waits(_, c):
            bundle(n, 'wait')
            pl.when(n == MB0)(cp_modb.wait)
            pl.when(n == WD0 // 2)(cp_d.wait)
            return c
        jax.lax.fori_loop(0, jnp.where(n < NP, 1, 0), waits, 0)

        pl.when(n == 0)(cp_modb.start)
        bundle(jnp.minimum(n + 2, NP), 'start')
        for a in range(3):
            pl.when(n == 2 + a)(Both(cp_d.cps[a * NFB // 3:(a + 1) * NFB // 3]).start)
        pl.when(n == NP)(Both([cp_g, cp_u]).start)

        t1 = jnp.minimum(n + 2, NT - 1)
        v = jnp.maximum(n - NP, 0)
        tile2 = lambda v: (jax.lax.shift_right_logical(v, 3) * TPB
                           + jnp.minimum(jnp.bitwise_and(v, NP - 1), TPB - 1))
        t2 = tile2(v)
        v_transpose(2 * n + 1, vt1_ref)
        wq_transpose(2 * n + 3, wqt1_ref)

        def stats(clock):
            ln2_stats(t2, clock)
            ln1_stats(t1, clock)
            late_mod_sums(n, clock)
            h2_rows(tile2(jnp.maximum(v - 1, 0)), clock)

        def apply(clock):
            ln1_apply(t1, clock)
            ln2_apply(t2, clock)
            late_mod_store(n)

        for a in range(2):
            unit(2 * n + a, (stats, apply)[a], *streams[a])
        v_transpose(2 * n + 2, vt0_ref)
        wq_transpose(2 * n + 4, wqt0_ref)
        return carry

    jax.lax.fori_loop(0, NU // 2 - 1, step, 0)

    T0 = NT - TPB
    cp_out(0, T0, osem.at[C + TPB]).start()
    cp_g.wait()
    v_transpose(NU - 1, vt1_ref)
    o = jnp.concatenate([attend(*streams[a][0:3]) for a in range(2)], axis=0)
    wlast = jnp.concatenate([wot_v[HKV - 2], wot_v[HKV - 1]], axis=1)
    fin = [acc_ref[T0 + t] + _dot(wlast, o[:, t * 128:(t + 1) * 128]) for t in range(TPB)]
    clock = jnp.concatenate(fin, axis=0)
    row8 = jax.lax.broadcasted_iota(jnp.int32, (C, 128), 0)
    lane8 = jax.lax.broadcasted_iota(jnp.int32, (C, 128), 1)
    work = key_ref[0:T0, :]
    lead = jnp.zeros((C, 128), F32)
    for t in range(C):
        mx = jnp.max(jnp.max(work, axis=0, keepdims=True), axis=1, keepdims=True)
        work = jnp.where(work == mx, 0.0, work)
        lead = jnp.where(row8 == t, mx, lead)

    def spread(row):
        return pltpu.roll(jnp.broadcast_to(row, (128, 128)), 0, 1, stride=1, stride_axis=0)

    def merge(lead, rows, spreads):
        cols = jnp.concatenate([lead] + spreads, axis=0)
        best = jnp.zeros((C, 128), F32)
        for row in [jnp.max(jnp.where(row8 == lane8, lead, 0.0), axis=0, keepdims=True)] + rows:
            rank = jnp.sum(jnp.where(cols > row, 1.0, 0.0), axis=0, keepdims=True)
            best = jnp.maximum(best, jnp.where(rank == row8.astype(F32), row, 0.0))
        return jnp.max(best, axis=1, keepdims=True)

    def tail_h2(t, norm, gate=None):
        x1 = x1_ref[t].astype(F32)
        if gate is not None:
            n = gate.shape[0]
            x1 = jnp.concatenate([_paced(x1[:n], gate, 0), x1[n:]], axis=0) if n < D else _paced(x1, gate, 0)
        h2_ref[t] = ln2_h2(x1, *norm).astype(BF16)
        if t < NT - 2:
            h2_rows(t)

    u_vec, u_sum, b_sum = router_terms()
    keys = []
    for t in range(TPB):
        x1, stats = ln2_x1(T0 + t, fin[t])
        mean, inv = norm = ln2_norm(stats)
        r = (jnp.sum(x1 * u_vec, axis=0, keepdims=True) - mean * u_sum) * inv + b_sum
        keys.append(_score_key(r, T0 + t))
        if t < TPB - 1:
            tail_h2(T0 + t, norm, clock[(t + 1) * D + TLAG:(t + 2) * D + TLAG])
    lead = jnp.broadcast_to(merge(lead, keys[0:2], [spread(k) for k in keys[0:2]]), (C, 128))
    spread2 = spread(keys[2])
    if BAR == 0:
        cp_u.wait()
        cp_out(0, T0, osem.at[C + TPB]).wait()

    h2_rows(NT - 2)
    tail_h2(NT - 1, norm)
    h2_rows(NT - 1)
    sel = pltpu.bitcast(merge(lead, keys[2:4], [spread2, spread(keys[3])]), jnp.int32) - KEY0
    sel_tok = (S - 1) - (sel & (S - 1))
    toks = [sel_tok[t, 0] for t in range(C)]
    tiles = [jax.lax.shift_right_logical(tk, 7) for tk in toks]
    sel_code = jax.lax.shift_right_logical(sel, 11) - 32768
    sel_bits = jnp.where(sel_code < 0, -32769 - sel_code, sel_code)
    r_sel = pltpu.bitcast(jax.lax.shift_left(sel_bits, 16), F32)

    final = []
    for t in range(C):
        d = True
        for u in range(t + 1, C):
            d = jnp.logical_and(d, tiles[u] != tiles[t])
        final.append(d)

    words = jnp.concatenate([h2row_ref[pl.ds(jax.lax.shift_right_logical(toks[t], 1), 1), :]
                             for t in range(C)], axis=0)
    odd = jnp.bitwise_and(sel_tok, 1) == 1
    xs = pltpu.bitcast(jnp.where(odd, jnp.bitwise_and(words, jnp.uint32(0xFFFF0000)),
                                 jax.lax.shift_left(words, jnp.uint32(16))), F32)
    xs = xs.astype(BF16)

    if BAR == 1:
        cp_u.wait()
        cp_out(0, T0, osem.at[C + TPB]).wait()
    gpre = _r(_dot(xs, wg_v[...]))
    gact = _r(gpre * _r(jax.nn.sigmoid(gpre)))
    u = _r(_dot(xs, wu_v[...]))
    act = (gact * u).astype(BF16)
    FK = F // 4
    yk = [[_dot(act[:, a * FK:(a + 1) * FK],
                pltpu.bitcast(wd_ref[a * FK // 2:(a + 1) * FK // 2, j:min(j + 128, D)], BF16))
           for a in range(4)] for j in range(0, D, 128)]
    y = jnp.concatenate([sum(p) for p in yk], axis=1)
    clean = []
    for t in range(T0, NT):
        gate = jnp.concatenate([yk[t - T0][a // 18] for a in range(D // 8)], axis=0)
        x1 = _paced(x1_ref[t].astype(F32), gate, 0)
        out_v[t] = (x1 + mod(5) * h2_ref[t].astype(F32)).astype(BF16)
        d = tiles[0] != t
        for a in range(1, C):
            d = jnp.logical_and(d, tiles[a] != t)
        clean.append(d)
        pl.when(d)(cp_out(t, 1, osem.at[C + t - T0]).start)
    y = _r(y)
    y = y * _r(jax.nn.sigmoid(r_sel))
    yt = jnp.concatenate([y, jnp.zeros((16 - C, D), F32)], axis=0).astype(BF16).T

    Q = D // 4
    for t in range(C):
        oh = jnp.where(sel_tok == tiles[t] * 128 + lane8, 1.0, 0.0)
        oh = jnp.concatenate([oh, jnp.zeros((16 - C, 128), F32)], axis=0).astype(BF16)
        upd = jnp.concatenate([_dot(yt[a * Q:(a + 1) * Q], oh) for a in range(4)], axis=0)
        out_v[tiles[t]] = (x1_ref[tiles[t]].astype(F32)
                           + mod(5) * (h2_ref[tiles[t]].astype(F32) + upd)).astype(BF16)
        if final[t] is True:
            cp_out(tiles[t], 1, osem.at[t]).start()
        else:
            pl.when(final[t])(cp_out(tiles[t], 1, osem.at[t]).start)
    for t in range(T0, NT):
        pl.when(clean[t - T0])(cp_out(t, 1, osem.at[C + t - T0]).wait)
    for t in range(C):
        if final[t] is True:
            cp_out(tiles[t], 1, osem.at[t]).wait()
        else:
            pl.when(final[t])(cp_out(tiles[t], 1, osem.at[t]).wait)


@jax.jit
def pallas_adaLN_cond__gqa_block_cached__moe_arch_mod__prompt_kernel(
    A_x: jax.Array,
    A_k_cache: jax.Array,
    A_v_cache: jax.Array,
    A_wq: jax.Array,
    A_wo: jax.Array,
    B_x: jax.Array,
    B_w_r: jax.Array,
    B_w_gate: jax.Array,
    B_w_up: jax.Array,
    B_w_down: jax.Array,
    c: jax.Array,
    w_mod: jax.Array,
):
    del B_x
    xt = A_x.reshape(S, D).T
    k = A_k_cache.reshape(HKV, S, DH)
    v = A_v_cache.reshape(HKV, S, DH)

    hbm = pl.BlockSpec(memory_space=pl.ANY)
    stream = [
        pltpu.VMEM((S, REP * TQ), F32),
        pltpu.VMEM((8, REP * TQ), F32),
        pltpu.VMEM((DH // 2, S), U32),
        pltpu.VMEM((GW // 2, D), U32),
    ]
    out = pl.pallas_call(
        _kernel,
        in_specs=[hbm] * 11,
        out_specs=hbm,
        out_shape=jax.ShapeDtypeStruct((D, S), BF16),
        scratch_shapes=[
            pltpu.VMEM((NT + NFB + NMB, D, 128), BF16),
            pltpu.VMEM((HKV, S, DH), BF16),
            pltpu.VMEM((HKV, S, DH), BF16),
            pltpu.VMEM((HKV, D, GW), BF16),
            pltpu.VMEM((HKV, D, GW), BF16),
            pltpu.VMEM((D, DA), BF16),
            pltpu.VMEM((D, F), BF16),
            pltpu.VMEM((D, F), BF16),
            pltpu.VMEM((F // 2, D), U32),
            pltpu.VMEM((NT, D, 128), BF16),
            pltpu.VMEM((NT, D, 128), F32),
            pltpu.VMEM((6 * D, 128), F32),
            pltpu.VMEM((5 * 128, 128), F32),
            pltpu.VMEM((5 * 128, 128), F32),
            pltpu.VMEM((TPB, D, 128), F32),
            pltpu.VMEM((NT, D, 128), BF16),
            pltpu.VMEM((NT, D, 128), BF16),
            pltpu.VMEM((S // 2, D), U32),
            pltpu.VMEM((NT, D, 128), BF16),
            pltpu.VMEM((NT, 128), F32),
            pltpu.VMEM((NT * NC, 8, 128), F32),
            pltpu.VMEM((NT * NC, 8, 128), F32),
            pltpu.VMEM((MPI, 8, 128), F32),
        ] + stream + stream + [
            pltpu.VMEM((D,), BF16),
            pltpu.VMEM((1, D), BF16),
            pltpu.SemaphoreType.DMA((HKV // 2,)),
            pltpu.SemaphoreType.DMA((11,)),
            pltpu.SemaphoreType.DMA((C + TPB + 1,)),
        ],
        compiler_params=pltpu.CompilerParams(vmem_limit_bytes=120 * 1024 * 1024,
                                             disable_bounds_checks=True,
                                             disable_semaphore_checks=True),
    )(B_w_r, c, xt, k, v, A_wq, A_wo.T, w_mod, B_w_gate, B_w_up, B_w_down.T)
    return out.T.reshape(1, S, D)
```

```python
import math

import jax
import jax.numpy as jnp
import jax.experimental.pallas as pl
import jax.experimental.pallas.tpu as pltpu

S = 2048
D = 576
HQ = 32
HKV = 16
REP = HQ // HKV
DH = 128
GW = REP * DH
F = 4608
C = 8
EPS = 1e-05
TQ = 512
NBLK = S // TQ
TPB = TQ // 128
NT = S // 128
NU = NBLK * HKV
DA = 2 * D
NC = 3
DC = D // NC
TLAG = 160
TKS = 18
SCLAG = 2
CL2 = 0
SLAG = 96
BAR = 1
PG = 64
NFB = F // 128
MODA = ((0, 4, 5), (1, 2, 6), (3, 7, 8))
NMB = 4 * D // 128
MPI = 3
MB0 = 2
WD0 = 14
PACE = (1280, 304, 2112, 1024, 400, 3200)

BF16 = jnp.bfloat16
F32 = jnp.float32
U32 = jnp.uint32
QSCALE = DH ** -0.5 * math.log2(math.e)


def _dot(a, b):
    return jnp.dot(a, b, preferred_element_type=F32)


def _dot_nt(a, b):
    return jax.lax.dot_general(a, b, (((1,), (1,)), ((), ())), preferred_element_type=F32)


def _r(x):
    return x.astype(BF16).astype(F32)


def _col_bcast(row):
    return jnp.broadcast_to(row, (128, 128)).T


def _blk(u):
    return u // HKV if isinstance(u, int) else jax.lax.shift_right_logical(u, 4)


def _grp(u):
    return u % HKV if isinstance(u, int) else jnp.bitwise_and(u, HKV - 1)


def _lanes(t, n=1):
    return pl.ds(pl.multiple_of(t * 128, 128), n * 128)


def _paced(x, clock, pos):
    if clock is None:
        return x
    row, col = pos % S, (pos // S) * TQ
    g = clock[row:row + x.shape[0], col:col + x.shape[1]]
    return jnp.where(g * g < 0.0, jnp.zeros_like(x), x)


def _softmax_numer(s, m):
    n, w = s.shape
    p = jnp.exp2(s - m).reshape(n // PG, PG // 8, 8, w)
    ts = jnp.sum(p, axis=1)
    last = jnp.where(ts < 0.0, ts, p[:, PG // 8 - 1])
    p = jnp.concatenate([p[:, :PG // 8 - 1], last[:, None]], axis=1).reshape(n, w)
    l = jnp.sum(jnp.sum(ts, axis=0), axis=0, keepdims=True)
    return p.astype(BF16), l


KEY0 = 0x20000000


def _score_key(r, t):
    tok = t * 128 + jax.lax.broadcasted_iota(jnp.int32, r.shape, 1)
    bits = jax.lax.shift_right_arithmetic(pltpu.bitcast(_r(r) + 0.0, jnp.int32), 16)
    code = jnp.where(bits < 0, -32769 - bits, bits) + 32768
    return pltpu.bitcast(code * S + (S - 1 - tok) + KEY0, F32)


def _chunk_stats(x):
    m = jnp.sum(x, axis=0, keepdims=True) * (1.0 / DC)
    xc = x - m
    return m, jnp.sum(xc * xc, axis=0, keepdims=True)


def _mean_var(stats):
    mean = sum(m for m, _ in stats) * (1.0 / NC)
    var = sum(s + DC * (m - mean) * (m - mean) for m, s in stats) * (1.0 / D)
    return mean, var


def _kernel(wr_hbm, c_hbm,
            xt_hbm, k_hbm, v_hbm, wq_hbm, wot_hbm, wmod_hbm, wg_hbm, wu_hbm, wdt_hbm,
            out_hbm,
            xw_v, k_v, v_v, wq_v, wot_v, wmod_v, wg_v, wu_v, wd_ref,
            ht_ref, acc_ref, mod_ref, wrb_ref, scb_ref, ln0_ref, x1_ref, h2_ref, h2row_ref, out_v, fix_v,
            key_ref, st1_ref, st2_ref, lm_ref,
            s0_ref, m0_ref, vt0_ref, wqt0_ref, s1_ref, m1_ref, vt1_ref, wqt1_ref,
            wr_ref, c_ref, bsem, msem, osem):
    streams = ((s0_ref, m0_ref, vt0_ref, wqt0_ref), (s1_ref, m1_ref, vt1_ref, wqt1_ref))

    def cp_cols(src, dst, t, n, sem, dst_t=None):
        return pltpu.make_async_copy(src.at[:, _lanes(t, n)],
                                     dst.at[:, _lanes(t if dst_t is None else dst_t, n)], sem)

    def cp_pair(src, dst, p, sem):
        return pltpu.make_async_copy(src.at[pl.ds(2 * p, 2)], dst.at[pl.ds(2 * p, 2)], sem)

    cp_k = lambda p, sem: cp_pair(k_hbm, k_v, p, sem)
    cp_v1 = lambda g, sem: pltpu.make_async_copy(v_hbm.at[g], v_v.at[g], sem)
    cp_k1 = lambda g, sem: pltpu.make_async_copy(k_hbm.at[g], k_v.at[g], sem)

    class Both:
        def __init__(self, cps):
            self.cps = cps

        def start(self):
            for cp in self.cps:
                cp.start()

        def wait(self):
            for cp in self.cps:
                cp.wait()

    def cp_w1(src, dst, g, sem):
        return pltpu.make_async_copy(src.at[:, _lanes(g * REP, REP)], dst.at[g], sem)

    def cp_w(src, dst, p, sem):
        return Both([cp_w1(src, dst, 2 * p + a, sem) for a in range(2)])

    cp_wq = lambda p, sem: cp_w(wq_hbm, wq_v, p, sem)
    cp_wo = lambda p, sem: cp_w(wot_hbm, wot_v, p, sem)
    cp_x = lambda j, sem: Both([pltpu.make_async_copy(xt_hbm.at[:, _lanes(TPB * j + t)],
                                                      xw_v.at[TPB * j + t], sem) for t in range(TPB)])
    NP = HKV // 2

    def bundle(n, act):
        sem = bsem.at[n if isinstance(n, int) else jnp.minimum(n, NP - 1)]

        def on(cond, cps):
            def go():
                for cp in cps():
                    getattr(cp, act)()
            if isinstance(cond, bool):
                if cond:
                    go()
            else:
                pl.when(cond)(go)
        on(n + 1 < NP, lambda: [cp_k(n + 1, sem), cp_v1(2 * n + 2, sem), cp_w1(wq_hbm, wq_v, 2 * n + 3, sem)])
        on(n + 2 < NP, lambda: [cp_w1(wq_hbm, wq_v, 2 * n + 4, sem)])
        on(jnp.logical_and(n >= 1, n < NBLK) if not isinstance(n, int) else 1 <= n < NBLK, lambda: [cp_x(n, sem)])
        on(n < NP, lambda: [cp_v1(2 * n + 1, sem), cp_wo(n, sem)])

    cp_moda = [Both([cp_cols(wmod_hbm, wmod_v, t, 1, msem.at[s]) for t in tiles])
               for s, tiles in zip((0, 6, 10), MODA)]
    cp_modb = Both([pltpu.make_async_copy(wmod_hbm.at[:, _lanes(DA // 128 + b)],
                                          xw_v.at[NT + NFB + b], msem.at[1]) for b in range(NMB)])
    cp_g = pltpu.make_async_copy(wg_hbm, wg_v, msem.at[2])
    cp_u = pltpu.make_async_copy(wu_hbm, wu_v, msem.at[3])
    cp_d = Both([pltpu.make_async_copy(wdt_hbm.at[:, _lanes(b)], xw_v.at[NT + b], msem.at[4])
                 for b in range(NFB)])
    cp_out = lambda t, n, sem: Both([pltpu.make_async_copy(out_v.at[t + a], out_hbm.at[:, _lanes(t + a)],
                                                           sem) for a in range(n)])

    def silu_c():
        c = c_ref[...].astype(F32)
        return _r(c * _r(jax.nn.sigmoid(c)))

    def finish_mod(mod, lo):
        mod = _r(mod)
        col = lo + jax.lax.broadcasted_iota(jnp.int32, mod.shape, 1)
        is_scale = jnp.logical_or(jnp.logical_and(col >= D, col < 2 * D),
                                  jnp.logical_and(col >= 4 * D, col < 5 * D))
        mod = jnp.where(is_scale, _r(1.0 + mod), mod)
        for t in range(mod.shape[1] // 128):
            rows = pl.ds(pl.multiple_of(lo + t * 128, 128), 128)
            mod_ref[rows, :] = _col_bcast(mod[:, t * 128:(t + 1) * 128])

    def late_mod_sums(n, clock):
        b0 = jnp.clip(n - MB0, 0, NMB // MPI - 1) * MPI
        for k in range(MPI):
            w = xw_v[jnp.where(n >= MB0, NT + NFB + b0 + k, 0)].astype(F32)
            part = jnp.sum((w * scb_ref[0:D, :]).reshape(D // 8, 8, 128), axis=0)
            lm_ref[k] = _paced(part, clock, PACE[4] + 256 * k)

    def late_mod_store(n):
        b0 = jnp.clip(n - MB0, 0, NMB // MPI - 1) * MPI
        for k in range(MPI):
            finish_mod(jnp.sum(lm_ref[k], axis=0, keepdims=True), DA + (b0 + k) * 128)

    def col_vector(ref, row):
        row = jnp.concatenate([row, jnp.zeros((1, 64), F32)], axis=1)
        for t in range(5):
            ref[t * 128:(t + 1) * 128, :] = _col_bcast(row[:, t * 128:(t + 1) * 128])

    def mod(k):
        return mod_ref[k * D:(k + 1) * D, :]

    def put_stats(st_ref, t, shift, scale, clock, pos):
        row = jax.lax.broadcasted_iota(jnp.int32, (8, 128), 0)
        st_ref[t] = _paced(jnp.where(row == 0, shift, scale), clock, pos)

    def ln1_stats(t, clock=None):
        for c in range(NC):
            m, s = _chunk_stats(xw_v[t, c * DC:(c + 1) * DC, :].astype(F32))
            put_stats(st1_ref, t * NC + c, m, s, clock, PACE[0] + 192 * c)

    def ln1_norm(t):
        mean, var = _mean_var(load_stats(st1_ref, t))
        return (xw_v[t].astype(F32) - mean) * jax.lax.rsqrt(var + EPS)

    def ln1_apply(t, clock=None, ln=None):
        h = (ln1_norm(t) if ln is None else ln) * mod(1) + mod(0)
        ht_ref[t] = _paced(h, clock, PACE[1]).astype(BF16)

    def h2_rows(t, clock=None):
        x = pltpu.bitcast(h2_ref[t].T, U32)
        x = jnp.concatenate([_paced(x[:, a:min(a + 128, D)], clock, PACE[5] + a // 2)
                             for a in range(0, D, 128)], axis=1)
        h2row_ref[pl.ds(pl.multiple_of(t * 64, 64), 64), :] = x

    def router_terms():
        u = mod(4) * wrb_ref[0:D, :]
        return (u, jnp.sum(u, axis=0, keepdims=True),
                jnp.sum(mod(3) * wrb_ref[0:D, :], axis=0, keepdims=True))

    def load_stats(st_ref, t):
        return [(st_ref[t * NC + c, 0:1, :], st_ref[t * NC + c, 1:2, :]) for c in range(NC)]

    def ln2_x1(t, attn, clock=None):
        x1 = _r(xw_v[t].astype(F32) + mod(2) * attn)
        x1_ref[t] = _paced(x1, clock, PACE[2]).astype(BF16)
        return x1, [_chunk_stats(x1[c * DC:(c + 1) * DC]) for c in range(NC)]

    def ln2_norm(stats):
        mean, var = _mean_var(stats)
        return _r(mean), 1.0 / _r(jnp.sqrt(_r(_r(var) + EPS)))

    def ln2_h2(x1, mean, inv):
        return (x1 - mean) * inv * mod(4) + mod(3)

    def ln2_stats(t, clock):
        for c, (m, s) in enumerate(ln2_x1(t, acc_ref[t], clock)[1]):
            put_stats(st2_ref, t * NC + c, m, s, clock, PACE[2] + (c + 1) * DC + SLAG)

    def ln2_apply(t, clock):
        x1 = x1_ref[t].astype(F32)
        h2 = ln2_h2(x1, *ln2_norm(load_stats(st2_ref, t)))
        key = _score_key(jnp.sum(h2 * wrb_ref[0:D, :], axis=0, keepdims=True), t)
        key_ref[pl.ds(t, 1), :] = _paced(key, clock, PACE[3] + D + 96)
        h2 = _r(h2)
        h2_ref[t] = _paced(h2, clock, PACE[3]).astype(BF16)
        out_v[t] = _paced(x1 + mod(5) * h2, clock, PACE[3] + 16).astype(BF16)

    def q_proj(u, wqt_ref, split=False):
        w = pltpu.bitcast(wqt_ref[...], BF16)
        h = jnp.concatenate([ht_ref[_blk(u) * TPB + t] for t in range(TPB)], axis=1)
        if split == 1:
            q = sum(_dot(w[:, a:min(a + 128, D)], h[a:min(a + 128, D)]) for a in range(0, D, 128))
        elif split == 2:
            q = _dot(w[:, 512:], h[512:])
            q = _dot(w[:, :512], h[:512]) + q
        else:
            q = _dot(w, h)
        q = (q * QSCALE).astype(BF16)
        return jnp.concatenate([q[r * DH:(r + 1) * DH] for r in range(REP)], axis=1)

    def scores(u, q, s_ref, m_ref):
        s = _dot(k_v[_grp(u)], q)
        s_ref[...] = s
        m_ref[...] = jnp.broadcast_to(jnp.max(s, axis=0, keepdims=True), m_ref.shape)
        return s

    def v_transpose(u, vt_ref):
        vt_ref[...] = pltpu.bitcast(v_v[_grp(u)].T, U32)

    def wq_transpose(u, wqt_ref):
        wqt_ref[...] = pltpu.bitcast(wq_v[_grp(u)].T, U32)

    def attend(s_ref, m_ref, vt_ref):
        m = m_ref[0:1, :]
        o = []
        for r in range(REP):
            cols = slice(r * TQ, (r + 1) * TQ)
            p, l = _softmax_numer(s_ref[:, cols], m[:, cols])
            o.append((_dot(pltpu.bitcast(vt_ref[...], BF16), p) * (1.0 / l)).astype(BF16))
        return jnp.concatenate(o, axis=0)

    small = Both([pltpu.make_async_copy(wr_hbm, wr_ref, msem.at[7]),
                  pltpu.make_async_copy(c_hbm, c_ref, msem.at[7])])
    zeroth = Both([cp_x(0, msem.at[5]), cp_w1(wq_hbm, wq_v, 0, msem.at[5])])
    first = Both([cp_k1(0, msem.at[8]), cp_w1(wq_hbm, wq_v, 1, msem.at[8])])
    second = Both([cp_k1(1, msem.at[9]), cp_v1(0, msem.at[9]), cp_w1(wq_hbm, wq_v, 2, msem.at[9])])
    for cp in [small, zeroth] + cp_moda + [first, second]:
        cp.start()
    acc_ref[...] = jnp.zeros_like(acc_ref)
    mod_ref[DA:6 * D, :] = jnp.zeros((4 * D, 128), F32)
    h2_ref[0] = jnp.zeros((D, 128), BF16)
    small.wait()
    col_vector(wrb_ref, wr_ref[...].astype(F32).reshape(1, D))
    col_vector(scb_ref, silu_c())
    sc8 = jnp.broadcast_to(silu_c(), (8, D)).astype(BF16)
    zeroth.wait()
    for t in range(TPB):
        ln1_stats(t)
        ln0_ref[t] = ln1_norm(t)
    wq_transpose(0, wqt0_ref)
    for cp, tiles in zip(cp_moda, MODA):
        cp.wait()
        for t in tiles:
            finish_mod(_dot(sc8, wmod_v[:, t * 128:(t + 1) * 128])[0:1], t * 128)
    for t in range(TPB):
        ln1_apply(t, ln=ln0_ref[t])
    q = q_proj(0, wqt0_ref, split=True)
    first.wait()
    bundle(0, 'start')
    scores(0, q, s0_ref, m0_ref)
    wq_transpose(1, wqt1_ref)
    second.wait()
    bundle(1, 'start')
    scores(1, q_proj(1, wqt1_ref, split=2), s1_ref, m1_ref)
    v_transpose(0, vt0_ref)
    wq_transpose(2, wqt0_ref)

    def unit(u, side, s_ref, m_ref, vt_ref, wqt_ref):
        q = q_proj(u + 2, wqt_ref, split=2 if s_ref is s0_ref else 0)
        o = attend(s_ref, m_ref, vt_ref)
        clock = scores(u + 2, q, s_ref, m_ref)
        side(clock)
        upd = _dot(wot_v[_grp(u)], o)
        for t in range(TPB):
            acc_ref[_blk(u) * TPB + t] += upd[:, t * 128:(t + 1) * 128]
        fb = jnp.clip(u - WD0, 0, NFB - 1)
        src = jnp.where(u >= WD0, NT + fb, 0)
        wd_ref[pl.ds(pl.multiple_of(fb * 64, 64), 64), :] = pltpu.bitcast(xw_v[src].T, U32)

    def step(n, carry):
        def waits(_, c):
            bundle(n, 'wait')
            pl.when(n == MB0)(cp_modb.wait)
            pl.when(n == WD0 // 2)(cp_d.wait)
            return c
        jax.lax.fori_loop(0, jnp.where(n < NP, 1, 0), waits, 0)

        pl.when(n == 0)(cp_modb.start)
        bundle(jnp.minimum(n + 2, NP), 'start')
        for a in range(3):
            pl.when(n == 2 + a)(Both(cp_d.cps[a * NFB // 3:(a + 1) * NFB // 3]).start)
        pl.when(n == NP)(Both([cp_g, cp_u]).start)

        t1 = jnp.minimum(n + 2, NT - 1)
        v = jnp.maximum(n - NP, 0)
        tile2 = lambda v: (jax.lax.shift_right_logical(v, 3) * TPB
                           + jnp.minimum(jnp.bitwise_and(v, NP - 1), TPB - 1))
        t2 = tile2(v)
        v_transpose(2 * n + 1, vt1_ref)
        wq_transpose(2 * n + 3, wqt1_ref)

        def stats(clock):
            ln2_stats(t2, clock)
            ln1_stats(t1, clock)
            late_mod_sums(n, clock)
            h2_rows(tile2(jnp.maximum(v - 1, 0)), clock)

        def apply(clock):
            ln1_apply(t1, clock)
            ln2_apply(t2, clock)
            late_mod_store(n)

        for a in range(2):
            unit(2 * n + a, (stats, apply)[a], *streams[a])
        v_transpose(2 * n + 2, vt0_ref)
        wq_transpose(2 * n + 4, wqt0_ref)
        return carry

    jax.lax.fori_loop(0, NU // 2 - 1, step, 0)

    T0 = NT - TPB
    cp_out(0, T0, osem.at[C + TPB]).start()
    cp_g.wait()
    v_transpose(NU - 1, vt1_ref)
    o = jnp.concatenate([attend(*streams[a][0:3]) for a in range(2)], axis=0)
    wlast = jnp.concatenate([wot_v[HKV - 2], wot_v[HKV - 1]], axis=1)
    fin = [acc_ref[T0 + t] + _dot(wlast, o[:, t * 128:(t + 1) * 128]) for t in range(TPB)]
    clock = jnp.concatenate(fin, axis=0)
    row8 = jax.lax.broadcasted_iota(jnp.int32, (C, 128), 0)
    lane8 = jax.lax.broadcasted_iota(jnp.int32, (C, 128), 1)
    work = key_ref[0:T0, :]
    lead = jnp.zeros((C, 128), F32)
    for t in range(C):
        mx = jnp.max(jnp.max(work, axis=0, keepdims=True), axis=1, keepdims=True)
        work = jnp.where(work == mx, 0.0, work)
        lead = jnp.where(row8 == t, mx, lead)

    def spread(row):
        return pltpu.roll(jnp.broadcast_to(row, (128, 128)), 0, 1, stride=1, stride_axis=0)

    def merge(lead, rows, spreads):
        cols = jnp.concatenate([lead] + spreads, axis=0)
        best = jnp.zeros((C, 128), F32)
        for row in [jnp.max(jnp.where(row8 == lane8, lead, 0.0), axis=0, keepdims=True)] + rows:
            rank = jnp.sum(jnp.where(cols > row, 1.0, 0.0), axis=0, keepdims=True)
            best = jnp.maximum(best, jnp.where(rank == row8.astype(F32), row, 0.0))
        return jnp.max(best, axis=1, keepdims=True)

    def tail_h2(t, norm, gate=None):
        x1 = x1_ref[t].astype(F32)
        if gate is not None:
            n = gate.shape[0]
            x1 = jnp.concatenate([_paced(x1[:n], gate, 0), x1[n:]], axis=0) if n < D else _paced(x1, gate, 0)
        h2_ref[t] = ln2_h2(x1, *norm).astype(BF16)
        if t < NT - 2:
            h2_rows(t)

    u_vec, u_sum, b_sum = router_terms()
    keys = []
    for t in range(TPB):
        x1, stats = ln2_x1(T0 + t, fin[t])
        mean, inv = norm = ln2_norm(stats)
        r = (jnp.sum(x1 * u_vec, axis=0, keepdims=True) - mean * u_sum) * inv + b_sum
        keys.append(_score_key(r, T0 + t))
        if t < TPB - 1:
            tail_h2(T0 + t, norm, clock[(t + 1) * D + TLAG:(t + 2) * D + TLAG])
    lead = jnp.broadcast_to(merge(lead, keys[0:2], [spread(k) for k in keys[0:2]]), (C, 128))
    spread2 = spread(keys[2])
    if BAR == 0:
        cp_u.wait()
        cp_out(0, T0, osem.at[C + TPB]).wait()

    h2_rows(NT - 2)
    tail_h2(NT - 1, norm)
    h2_rows(NT - 1)
    sel = pltpu.bitcast(merge(lead, keys[2:4], [spread2, spread(keys[3])]), jnp.int32) - KEY0
    sel_tok = (S - 1) - (sel & (S - 1))
    toks = [sel_tok[t, 0] for t in range(C)]
    tiles = [jax.lax.shift_right_logical(tk, 7) for tk in toks]
    sel_code = jax.lax.shift_right_logical(sel, 11) - 32768
    sel_bits = jnp.where(sel_code < 0, -32769 - sel_code, sel_code)
    r_sel = pltpu.bitcast(jax.lax.shift_left(sel_bits, 16), F32)

    final = []
    for t in range(C):
        d = True
        for u in range(t + 1, C):
            d = jnp.logical_and(d, tiles[u] != tiles[t])
        final.append(d)

    words = jnp.concatenate([h2row_ref[pl.ds(jax.lax.shift_right_logical(toks[t], 1), 1), :]
                             for t in range(C)], axis=0)
    odd = jnp.bitwise_and(sel_tok, 1) == 1
    xs = pltpu.bitcast(jnp.where(odd, jnp.bitwise_and(words, jnp.uint32(0xFFFF0000)),
                                 jax.lax.shift_left(words, jnp.uint32(16))), F32)
    xs = xs.astype(BF16)

    def plain_out(t, ticks=None):
        x1 = x1_ref[t].astype(F32)
        if ticks is not None:
            gate = jnp.concatenate([ticks[a * len(ticks) // (D // 8)] for a in range(D // 8)], axis=0)
            x1 = _paced(x1, gate, 0)
        out_v[t] = (x1 + mod(5) * h2_ref[t].astype(F32)).astype(BF16)

    clean = []

    def send_clean(t):
        d = tiles[0] != t
        for a in range(1, C):
            d = jnp.logical_and(d, tiles[a] != t)
        clean.append(d)
        pl.when(d)(cp_out(t, 1, osem.at[C + t - T0]).start)

    if BAR == 1:
        cp_u.wait()
        cp_out(0, T0, osem.at[C + TPB]).wait()
    gpre = _dot(xs, wg_v[...])
    u = _dot(xs, wu_v[...])
    ticks = [z[:, a * 128:(a + 1) * 128] for z in (gpre, u) for a in range(NFB)]
    for t in range(TPB):
        plain_out(T0 + t, ticks[t * TKS:(t + 1) * TKS])
        send_clean(T0 + t)
    gpre, u = _r(gpre), _r(u)
    gact = _r(gpre * _r(jax.nn.sigmoid(gpre)))
    act = (gact * u).astype(BF16)
    gate_r = _r(jax.nn.sigmoid(r_sel))
    ohs = []
    for t in range(C):
        oh = jnp.where(sel_tok == tiles[t] * 128 + lane8, 1.0, 0.0)
        ohs.append(jnp.concatenate([oh, jnp.zeros((16 - C, 128), F32)], axis=0).astype(BF16))

    def cp_fix(t, lo, hi):
        return pltpu.make_async_copy(fix_v.at[t, lo:hi, :], out_hbm.at[lo:hi, _lanes(tiles[t])],
                                     osem.at[t])

    def guarded(cond, fn):
        if cond is True:
            fn()
        else:
            pl.when(cond)(fn)

    def scatter(j, yt, t):
        lo, hi = j * 128, min(j * 128 + 128, D)
        upd = jnp.concatenate([_dot(yt[a:a + 64], ohs[t]) for a in range(0, hi - lo, 64)], axis=0)
        fix_v[t, lo:hi, :] = (x1_ref[tiles[t], lo:hi, :].astype(F32) + mod_ref[5 * D + lo:5 * D + hi, :]
                              * (h2_ref[tiles[t], lo:hi, :].astype(F32) + upd)).astype(BF16)
        guarded(final[t], cp_fix(t, lo, hi).start)

    NJ = (D + 127) // 128
    yts = []
    for j in range(NJ):
        lo, hi = j * 128, min(j * 128 + 128, D)
        nk = 4
        FK = F // nk
        yk = []
        for a in range(nk):
            w = pltpu.bitcast(wd_ref[a * FK // 2:(a + 1) * FK // 2, lo:hi], BF16)
            yk.append(_dot(act[:, a * FK:(a + 1) * FK], w))
            if j >= SCLAG:
                for t in (2 * a, 2 * a + 1):
                    scatter(j - SCLAG, yts[j - SCLAG], t)
        y = _r(sum(yk)) * gate_r
        yts.append(jnp.concatenate([y, jnp.zeros_like(y)], axis=0).astype(BF16).T)
    for j in range(NJ - SCLAG, NJ):
        for t in range(C):
            scatter(j, yts[j], t)
    for t in range(T0, NT):
        pl.when(clean[t - T0])(cp_out(t, 1, osem.at[C + t - T0]).wait)
    for t in range(C):
        guarded(final[t], cp_fix(t, 0, D).wait)


@jax.jit
def pallas_adaLN_cond__gqa_block_cached__moe_arch_mod__prompt_kernel(
    A_x: jax.Array,
    A_k_cache: jax.Array,
    A_v_cache: jax.Array,
    A_wq: jax.Array,
    A_wo: jax.Array,
    B_x: jax.Array,
    B_w_r: jax.Array,
    B_w_gate: jax.Array,
    B_w_up: jax.Array,
    B_w_down: jax.Array,
    c: jax.Array,
    w_mod: jax.Array,
):
    del B_x
    xt = A_x.reshape(S, D).T
    k = A_k_cache.reshape(HKV, S, DH)
    v = A_v_cache.reshape(HKV, S, DH)

    hbm = pl.BlockSpec(memory_space=pl.ANY)
    stream = [
        pltpu.VMEM((S, REP * TQ), F32),
        pltpu.VMEM((8, REP * TQ), F32),
        pltpu.VMEM((DH // 2, S), U32),
        pltpu.VMEM((GW // 2, D), U32),
    ]
    out = pl.pallas_call(
        _kernel,
        in_specs=[hbm] * 11,
        out_specs=hbm,
        out_shape=jax.ShapeDtypeStruct((D, S), BF16),
        scratch_shapes=[
            pltpu.VMEM((NT + NFB + NMB, D, 128), BF16),
            pltpu.VMEM((HKV, S, DH), BF16),
            pltpu.VMEM((HKV, S, DH), BF16),
            pltpu.VMEM((HKV, D, GW), BF16),
            pltpu.VMEM((HKV, D, GW), BF16),
            pltpu.VMEM((D, DA), BF16),
            pltpu.VMEM((D, F), BF16),
            pltpu.VMEM((D, F), BF16),
            pltpu.VMEM((F // 2, D), U32),
            pltpu.VMEM((NT, D, 128), BF16),
            pltpu.VMEM((NT, D, 128), F32),
            pltpu.VMEM((6 * D, 128), F32),
            pltpu.VMEM((5 * 128, 128), F32),
            pltpu.VMEM((5 * 128, 128), F32),
            pltpu.VMEM((TPB, D, 128), F32),
            pltpu.VMEM((NT, D, 128), BF16),
            pltpu.VMEM((NT, D, 128), BF16),
            pltpu.VMEM((S // 2, D), U32),
            pltpu.VMEM((NT, D, 128), BF16),
            pltpu.VMEM((C, D, 128), BF16),
            pltpu.VMEM((NT, 128), F32),
            pltpu.VMEM((NT * NC, 8, 128), F32),
            pltpu.VMEM((NT * NC, 8, 128), F32),
            pltpu.VMEM((MPI, 8, 128), F32),
        ] + stream + stream + [
            pltpu.VMEM((D,), BF16),
            pltpu.VMEM((1, D), BF16),
            pltpu.SemaphoreType.DMA((HKV // 2,)),
            pltpu.SemaphoreType.DMA((11,)),
            pltpu.SemaphoreType.DMA((C + TPB + 1,)),
        ],
        compiler_params=pltpu.CompilerParams(vmem_limit_bytes=120 * 1024 * 1024,
                                             disable_bounds_checks=True,
                                             disable_semaphore_checks=True),
    )(B_w_r, c, xt, k, v, A_wq, A_wo.T, w_mod, B_w_gate, B_w_up, B_w_down.T)
    return out.T.reshape(1, S, D)
```

```python
import math

import jax
import jax.numpy as jnp
import jax.experimental.pallas as pl
import jax.experimental.pallas.tpu as pltpu

S = 2048
D = 576
HQ = 32
HKV = 16
REP = HQ // HKV
DH = 128
GW = REP * DH
F = 4608
C = 8
EPS = 1e-05
TQ = 512
NBLK = S // TQ
TPB = TQ // 128
NT = S // 128
NU = NBLK * HKV
DA = 2 * D
NC = 3
DC = D // NC
TLAG = 160
TKS = 18
SCLAG = 2
CL2 = 0
SLAG = 96
BAR = 1
PG = 64
NFB = F // 128
MODA = ((0, 4, 5), (1, 2, 6), (3, 7, 8))
NMB = 4 * D // 128
MPI = 3
MB0 = 2
WD0 = 14
DM = 512
KR = D - DM
NV = 2
CH = 3
QC, SC, WC = 0, 1024, 1024 + 2 * S
OUTER0, OSTEP = (SC + 0, SC + 0), 138
TABLE = 1
TAB0, TAB1 = SC + 3150, WC + 1000
TPI = 16
PACE = (SC + 3900, SC + 3150, SC + 3150, SC + 3800, WC + 400, WC + 760)

BF16 = jnp.bfloat16
F32 = jnp.float32
U32 = jnp.uint32
QSCALE = DH ** -0.5 * math.log2(math.e)


def _dot(a, b):
    return jnp.dot(a, b, preferred_element_type=F32)


def _dot_nt(a, b):
    return jax.lax.dot_general(a, b, (((1,), (1,)), ((), ())), preferred_element_type=F32)


def _r(x):
    return x.astype(BF16).astype(F32)


def _col_bcast(row):
    return jnp.broadcast_to(row, (128, 128)).T


def _blk(u):
    return u // HKV if isinstance(u, int) else jax.lax.shift_right_logical(u, 4)


def _grp(u):
    return u % HKV if isinstance(u, int) else jnp.bitwise_and(u, HKV - 1)


def _lanes(t, n=1):
    return pl.ds(pl.multiple_of(t * 128, 128), n * 128)


def _paced(x, clock, pos):
    if clock is None:
        return x
    pos = pos // 8 * 8
    g = clock[pos:pos + x.shape[0], 0:x.shape[1]]
    return jnp.where(g * g < 0.0, jnp.zeros_like(x), x)


def _softmax_numer(s, m):
    n, w = s.shape
    p = jnp.exp2(s - m).reshape(n // PG, PG // 8, 8, w)
    ts = jnp.sum(p, axis=1)
    last = jnp.where(ts < 0.0, ts, p[:, PG // 8 - 1])
    p = jnp.concatenate([p[:, :PG // 8 - 1], last[:, None]], axis=1).reshape(n, w)
    l = jnp.sum(jnp.sum(ts, axis=0), axis=0, keepdims=True)
    return p.astype(BF16), l, ts


KEY0 = 0x20000000


def _score_key(r, t):
    tok = t * 128 + jax.lax.broadcasted_iota(jnp.int32, r.shape, 1)
    bits = jax.lax.shift_right_arithmetic(pltpu.bitcast(_r(r) + 0.0, jnp.int32), 16)
    code = jnp.where(bits < 0, -32769 - bits, bits) + 32768
    return pltpu.bitcast(code * S + (S - 1 - tok) + KEY0, F32)


def _chunk_stats(x):
    m = jnp.sum(x, axis=0, keepdims=True) * (1.0 / DC)
    xc = x - m
    return m, jnp.sum(xc * xc, axis=0, keepdims=True)


def _mean_var(stats):
    mean = sum(m for m, _ in stats) * (1.0 / NC)
    var = sum(s + DC * (m - mean) * (m - mean) for m, s in stats) * (1.0 / D)
    return mean, var


def _kernel(wr_hbm, c_hbm,
            xt_hbm, k_hbm, v_hbm, wq_hbm, wot_hbm, wmod_hbm, wg_hbm, wu_hbm, wdt_hbm,
            out_hbm,
            xw_v, k_v, v_v, wq_v, wot_v, wmod_v, wg_v, wu_v, wd_ref,
            ht_ref, acc_ref, mod_ref, wrb_ref, scb_ref, x1_ref, h2_ref, h2row_ref, out_v, fix_v,
            key_ref, st1_ref, st2_ref, lm_ref,
            hb_ref, wrem_v,
            s0_ref, m0_ref, vt0_ref, wqt0_ref, qr0_ref, wf0_ref,
            s1_ref, m1_ref, vt1_ref, wqt1_ref, qr1_ref, wf1_ref,
            wr_ref, c_ref, bsem, msem, osem):
    streams = ((s0_ref, m0_ref, vt0_ref, wqt0_ref, qr0_ref, wf0_ref),
               (s1_ref, m1_ref, vt1_ref, wqt1_ref, qr1_ref, wf1_ref))

    def cp_cols(src, dst, t, n, sem, dst_t=None):
        return pltpu.make_async_copy(src.at[:, _lanes(t, n)],
                                     dst.at[:, _lanes(t if dst_t is None else dst_t, n)], sem)

    def cp_pair(src, dst, p, sem):
        return pltpu.make_async_copy(src.at[pl.ds(2 * p, 2)], dst.at[pl.ds(2 * p, 2)], sem)

    cp_k = lambda p, sem: cp_pair(k_hbm, k_v, p, sem)
    cp_v1 = lambda g, sem: pltpu.make_async_copy(v_hbm.at[g], v_v.at[g], sem)
    cp_k1 = lambda g, sem: pltpu.make_async_copy(k_hbm.at[g], k_v.at[g], sem)

    class Both:
        def __init__(self, cps):
            self.cps = cps

        def start(self):
            for cp in self.cps:
                cp.start()

        def wait(self):
            for cp in self.cps:
                cp.wait()

    def cp_w1(src, dst, g, sem):
        return pltpu.make_async_copy(src.at[:, _lanes(g * REP, REP)], dst.at[g], sem)

    def cp_w(src, dst, p, sem):
        return Both([cp_w1(src, dst, 2 * p + a, sem) for a in range(2)])

    cp_wq = lambda p, sem: cp_w(wq_hbm, wq_v, p, sem)
    cp_wo = lambda p, sem: cp_w(wot_hbm, wot_v, p, sem)
    cp_x = lambda t0, n, sem: Both([pltpu.make_async_copy(xt_hbm.at[:, _lanes(t0 + t)],
                                                          xw_v.at[t0 + t], sem) for t in range(n)])
    NP = HKV // 2

    def bundle(n, act):
        sem = bsem.at[n if isinstance(n, int) else jnp.minimum(n, NP - 1)]

        def on(cond, cps):
            def go():
                for cp in cps():
                    getattr(cp, act)()
            if isinstance(cond, bool):
                if cond:
                    go()
            else:
                pl.when(cond)(go)
        on(n + 1 < NP, lambda: [cp_k(n + 1, sem), cp_v1(2 * n + 2, sem), cp_w1(wq_hbm, wq_v, 2 * n + 3, sem)])
        on(n + 2 < NP, lambda: [cp_w1(wq_hbm, wq_v, 2 * n + 4, sem)])
        on(jnp.logical_and(n >= 1, n < NBLK) if not isinstance(n, int) else 1 <= n < NBLK,
           lambda: [cp_x(TPB * n + 1, TPB - 1, sem)])
        on(jnp.logical_and(n >= 1, n < NBLK - 1) if not isinstance(n, int) else 1 <= n < NBLK - 1,
           lambda: [cp_x(TPB * n + TPB, 1, sem)])
        on(n < NP, lambda: [cp_v1(2 * n + 1, sem), cp_wo(n, sem)])

    cp_moda = [Both([cp_cols(wmod_hbm, wmod_v, t, 1, msem.at[s]) for t in tiles])
               for s, tiles in zip((0, 6, 10), MODA)]
    cp_modb = Both([pltpu.make_async_copy(wmod_hbm.at[:, _lanes(DA // 128 + b)],
                                          xw_v.at[NT + NFB + b], msem.at[1]) for b in range(NMB)])
    cp_g = pltpu.make_async_copy(wg_hbm, wg_v, msem.at[2])
    cp_u = pltpu.make_async_copy(wu_hbm, wu_v, msem.at[3])
    cp_d = Both([pltpu.make_async_copy(wdt_hbm.at[:, _lanes(b)], xw_v.at[NT + b], msem.at[4])
                 for b in range(NFB)])
    cp_out = lambda t, n, sem: Both([pltpu.make_async_copy(out_v.at[t + a], out_hbm.at[:, _lanes(t + a)],
                                                           sem) for a in range(n)])

    def silu_c():
        c = c_ref[...].astype(F32)
        return _r(c * _r(jax.nn.sigmoid(c)))

    def finish_mod(mod, lo):
        mod = _r(mod)
        col = lo + jax.lax.broadcasted_iota(jnp.int32, mod.shape, 1)
        is_scale = jnp.logical_or(jnp.logical_and(col >= D, col < 2 * D),
                                  jnp.logical_and(col >= 4 * D, col < 5 * D))
        mod = jnp.where(is_scale, _r(1.0 + mod), mod)
        for t in range(mod.shape[1] // 128):
            rows = pl.ds(pl.multiple_of(lo + t * 128, 128), 128)
            mod_ref[rows, :] = _col_bcast(mod[:, t * 128:(t + 1) * 128])

    def late_mod_sums(n, clock):
        b0 = jnp.clip(n - MB0, 0, NMB // MPI - 1) * MPI
        for k in range(MPI):
            w = xw_v[jnp.where(n >= MB0, NT + NFB + b0 + k, 0)].astype(F32)
            part = jnp.sum((w * scb_ref[0:D, :]).reshape(D // 8, 8, 128), axis=0)
            lm_ref[k] = _paced(part, clock, PACE[4] + 192 * k)

    def late_mod_store(n):
        b0 = jnp.clip(n - MB0, 0, NMB // MPI - 1) * MPI
        for k in range(MPI):
            finish_mod(jnp.sum(lm_ref[k], axis=0, keepdims=True), DA + (b0 + k) * 128)

    def col_vector(ref, row):
        row = jnp.concatenate([row, jnp.zeros((1, 64), F32)], axis=1)
        for t in range(5):
            ref[t * 128:(t + 1) * 128, :] = _col_bcast(row[:, t * 128:(t + 1) * 128])

    def mod(k):
        return mod_ref[k * D:(k + 1) * D, :]

    def put_stats(st_ref, t, shift, scale, clock, pos):
        row = jax.lax.broadcasted_iota(jnp.int32, (8, 128), 0)
        st_ref[t] = _paced(jnp.where(row == 0, shift, scale), clock, pos)

    def ln1_stats(t, clock=None, pos=None):
        for c in range(NC):
            m, s = _chunk_stats(xw_v[t, c * DC:(c + 1) * DC, :].astype(F32))
            put_stats(st1_ref, t * NC + c, m, s, clock, (PACE[0] if pos is None else pos) + 192 * c)

    def ln1_norm(t):
        mean, var = _mean_var(load_stats(st1_ref, t))
        return (xw_v[t].astype(F32) - mean) * jax.lax.rsqrt(var + EPS)

    def ln1_apply(t, clock=None, pos=None, ln=None):
        h = (ln1_norm(t) if ln is None else ln) * mod(1) + mod(0)
        ht_ref[t] = _paced(h, clock, PACE[1] if pos is None else pos).astype(BF16)

    def h2_rows(t, clock=None):
        x = pltpu.bitcast(h2_ref[t].T, U32)
        x = jnp.concatenate([_paced(x[:, a:min(a + 128, D)], clock, PACE[5] + a // 2)
                             for a in range(0, D, 128)], axis=1)
        h2row_ref[pl.ds(pl.multiple_of(t * 64, 64), 64), :] = x

    def router_terms():
        u = mod(4) * wrb_ref[0:D, :]
        return (u, jnp.sum(u, axis=0, keepdims=True),
                jnp.sum(mod(3) * wrb_ref[0:D, :], axis=0, keepdims=True))

    def load_stats(st_ref, t):
        return [(st_ref[t * NC + c, 0:1, :], st_ref[t * NC + c, 1:2, :]) for c in range(NC)]

    def ln2_x1(t, attn, clock=None):
        x1 = _r(xw_v[t].astype(F32) + mod(2) * attn)
        x1_ref[t] = _paced(x1, clock, PACE[2]).astype(BF16)
        return x1, [_chunk_stats(x1[c * DC:(c + 1) * DC]) for c in range(NC)]

    def ln2_norm(stats):
        mean, var = _mean_var(stats)
        return _r(mean), 1.0 / _r(jnp.sqrt(_r(_r(var) + EPS)))

    def ln2_h2(x1, mean, inv):
        return (x1 - mean) * inv * mod(4) + mod(3)

    def ln2_stats(t, clock):
        for c, (m, s) in enumerate(ln2_x1(t, acc_ref[t], clock)[1]):
            put_stats(st2_ref, t * NC + c, m, s, clock, PACE[2] + (c + 1) * DC + SLAG)

    def ln2_apply(t, clock):
        x1 = x1_ref[t].astype(F32)
        h2 = ln2_h2(x1, *ln2_norm(load_stats(st2_ref, t)))
        key = _score_key(jnp.sum(h2 * wrb_ref[0:D, :], axis=0, keepdims=True), t)
        key_ref[pl.ds(t, 1), :] = _paced(key, clock, PACE[3] + D + 96)
        h2 = _r(h2)
        h2_ref[t] = _paced(h2, clock, PACE[3]).astype(BF16)
        out_v[t] = _paced(x1 + mod(5) * h2, clock, PACE[3] + 16).astype(BF16)

    def finish_q(q):
        q = (q * QSCALE).astype(BF16)
        return jnp.concatenate([q[r * DH:(r + 1) * DH] for r in range(REP)], axis=1)

    def q_proj(u, wqt_ref, qr_ref=None, split=False):
        w = pltpu.bitcast(wqt_ref[...], BF16)
        h = jnp.concatenate([ht_ref[_blk(u) * TPB + t] for t in range(TPB)], axis=1)
        if split:
            return sum(_dot(w[:, a:min(a + 128, D)], h[a:min(a + 128, D)]) for a in range(0, D, 128))
        if qr_ref is None:
            rem = _dot(w[:, DM:], h[DM:])
        else:
            rem = [qr_ref[...].T]
            if NV < TPB:
                R = GW * (TPB - NV) // 4
                rem.append(jnp.concatenate([_dot(w[a:a + R, DM:], h[DM:, NV * 128:])
                                            for a in range(0, GW, R)], axis=0))
            rem = jnp.concatenate(rem, axis=1)
        return _dot(w[:, :DM], h[:DM]) + rem

    def w_rest(u, wf_ref):
        w = wrem_v[:, _lanes(_grp(u) * REP, REP)].astype(F32)
        for r in range(REP):
            wf_ref[r] = w[:, r * DH:(r + 1) * DH]

    def outer(u, qr_ref, wf_ref, clock, start):
        base = jnp.bitwise_and(_blk(u), 1) * (NV * 16)
        cells = [(tv, r) for r in range(REP) for tv in range(NV * 16)]
        for g in range(0, len(cells), CH):
            acc = {}
            for k in range(KR):
                for tv, r in cells[g:g + CH]:
                    t = hb_ref[base + tv, k] * wf_ref[r, pl.ds(k, 8, stride=0), :]
                    acc[tv, r] = t if k == 0 else acc[tv, r] + t
            for (tv, r), a in acc.items():
                qr_ref[tv * 8:(tv + 1) * 8, r * DH:(r + 1) * DH] = _paced(
                    a, clock, min(start + OSTEP * (g // CH + 1), clock.shape[0] - 8))

    def h_table(hr, base, k0, gates):
        nk = hr.shape[0]
        for j in range(nk):
            cb = _col_bcast(hr[j:j + 1])
            for b in range(16):
                g = gates[(j * 16 + b) * len(gates) // (nk * 16)]
                hb_ref[base + b, k0 + j] = jnp.where(g, 0.0, cb[b * 8:(b + 1) * 8])

    def never_of(clock, lo, hi):
        return [clock[a:a + 8] * clock[a:a + 8] < 0.0 for a in range(lo // 8 * 8, hi, 8)]

    def scores(u, q, s_ref, m_ref):
        s = _dot(k_v[_grp(u)], q)
        s_ref[...] = s
        m_ref[...] = jnp.broadcast_to(jnp.max(s, axis=0, keepdims=True), m_ref.shape)
        return jnp.concatenate([s[:, 0:128], s[:, TQ:TQ + 128]], axis=0)

    def v_transpose(u, vt_ref):
        vt_ref[...] = pltpu.bitcast(v_v[_grp(u)].T, U32)

    def wq_transpose(u, wqt_ref):
        wqt_ref[...] = pltpu.bitcast(wq_v[_grp(u)].T, U32)

    def attend(s_ref, m_ref, vt_ref):
        m = m_ref[0:1, :]
        o, never = [], []
        for r in range(REP):
            cols = slice(r * TQ, (r + 1) * TQ)
            p, l, ts = _softmax_numer(s_ref[:, cols], m[:, cols])
            o.append((_dot(pltpu.bitcast(vt_ref[...], BF16), p) * (1.0 / l)).astype(BF16))
            never += [ts[i, :, c * 128:(c + 1) * 128] < 0.0 for c in range(TPB) for i in range(S // PG)]
        return jnp.concatenate(o, axis=0), never

    small = Both([pltpu.make_async_copy(wr_hbm, wr_ref, msem.at[7]),
                  pltpu.make_async_copy(c_hbm, c_ref, msem.at[7])])
    zeroth = Both([cp_x(0, TPB, msem.at[5]), cp_w1(wq_hbm, wq_v, 0, msem.at[5])])
    first = Both([cp_k1(0, msem.at[8]), cp_w1(wq_hbm, wq_v, 1, msem.at[8])])
    second = Both([cp_k1(1, msem.at[9]), cp_v1(0, msem.at[9]), cp_w1(wq_hbm, wq_v, 2, msem.at[9]),
                   pltpu.make_async_copy(wq_hbm.at[DM:, :], wrem_v, msem.at[9]), cp_x(TPB, 1, msem.at[9])])
    for cp in [small, zeroth] + cp_moda + [first, second]:
        cp.start()
    acc_ref[...] = jnp.zeros_like(acc_ref)
    mod_ref[DA:6 * D, :] = jnp.zeros((4 * D, 128), F32)
    h2_ref[0] = jnp.zeros((D, 128), BF16)
    small.wait()
    col_vector(wrb_ref, wr_ref[...].astype(F32).reshape(1, D))
    col_vector(scb_ref, silu_c())
    sc8 = jnp.broadcast_to(silu_c(), (8, D)).astype(BF16)
    zeroth.wait()
    ln0 = []
    for t in range(TPB):
        ln1_stats(t)
        ln0.append(ln1_norm(t))
    wq_transpose(0, wqt0_ref)
    for cp, tiles in zip(cp_moda, MODA):
        cp.wait()
        for t in tiles:
            finish_mod(_dot(sc8, wmod_v[:, t * 128:(t + 1) * 128])[0:1], t * 128)
    for t in range(TPB):
        ln1_apply(t, ln=ln0[t])
    q = finish_q(q_proj(0, wqt0_ref, split=True))
    first.wait()
    bundle(0, 'start')
    def first_table(gates, lo, hi):
        for i in range(NV + 1):
            a, b = max(lo, i * KR), min(hi, (i + 1) * KR)
            if a < b:
                gs = gates[(a - lo) * len(gates) // (hi - lo):(b - lo) * len(gates) // (hi - lo)]
                hr = ht_ref[i if i < NV else TPB, DM:, :].astype(F32)[a - i * KR:b - i * KR]
                h_table(hr, i * 16, a - i * KR, gs)

    TSPLIT = 80
    first_table(never_of(scores(0, q, s0_ref, m0_ref), 64, 2 * S - 192), 0, TSPLIT)
    wq_transpose(1, wqt1_ref)
    second.wait()
    bundle(1, 'start')
    hrem = jnp.concatenate([ht_ref[t, DM:, :] for t in range(NV)], axis=1)
    for a in range(2):
        streams[a][4][...] = jax.lax.dot_general(
            hrem, wrem_v[:, (a + 2) * GW:(a + 3) * GW], (((0,), (0,)), ((), ())),
            preferred_element_type=F32)
    q = q_proj(1, wqt1_ref)
    clock = jnp.concatenate([q[:, t * 128:(t + 1) * 128] for t in range(TPB)]
                            + [scores(1, finish_q(q), s1_ref, m1_ref)], axis=0)
    ln1_stats(TPB, clock, SC + 200)
    ln1_apply(TPB, clock, SC + 900)
    first_table(never_of(clock, 0, SC + 2 * S - 600), TSPLIT, NV * KR + 2 * TPI)
    for a in range(2):
        w_rest(a + 4, streams[a][5])
    v_transpose(0, vt0_ref)
    wq_transpose(2, wqt0_ref)

    def unit(u, side, s_ref, m_ref, vt_ref, wqt_ref, qr_ref, wf_ref):
        q = q_proj(u + 2, wqt_ref, qr_ref)
        o, _ = attend(s_ref, m_ref, vt_ref)
        sclk = scores(u + 2, finish_q(q), s_ref, m_ref)
        upd = _dot(wot_v[_grp(u)], o)
        clock = jnp.concatenate([q[:, t * 128:(t + 1) * 128] for t in range(TPB)] + [sclk]
                                + [upd[:, 0:128], upd[:, 256:384]], axis=0)
        side(clock, lambda start: outer(u + 4, qr_ref, wf_ref, clock, start))
        w_rest(u + 6, wf_ref)
        for t in range(TPB):
            acc_ref[_blk(u) * TPB + t] += upd[:, t * 128:(t + 1) * 128]
        fb = jnp.clip(u - WD0, 0, NFB - 1)
        src = jnp.where(u >= WD0, NT + fb, 0)
        wd_ref[pl.ds(pl.multiple_of(fb * 64, 64), 64), :] = pltpu.bitcast(xw_v[src].T, U32)

    def step(n, carry):
        def waits(_, c):
            bundle(n, 'wait')
            pl.when(n == MB0)(cp_modb.wait)
            pl.when(n == WD0 // 2)(cp_d.wait)
            return c
        jax.lax.fori_loop(0, jnp.where(n < NP, 1, 0), waits, 0)

        pl.when(n == 0)(cp_modb.start)
        bundle(jnp.minimum(n + 2, NP), 'start')
        for a in range(3):
            pl.when(n == 2 + a)(Both(cp_d.cps[a * NFB // 3:(a + 1) * NFB // 3]).start)
        pl.when(n == NP)(Both([cp_g, cp_u]).start)

        t1 = jnp.minimum(n + 4, NT - 1)
        v = jnp.maximum(n - NP, 0)
        tile2 = lambda v: (jax.lax.shift_right_logical(v, 3) * TPB
                           + jnp.minimum(jnp.bitwise_and(v, NP - 1), TPB - 1))
        t2 = tile2(v)
        v_transpose(2 * n + 1, vt1_ref)
        wq_transpose(2 * n + 3, wqt1_ref)

        def stats(clock, outer_at):
            ln2_stats(t2, clock)
            ln1_stats(t1, clock)
            late_mod_sums(n, clock)
            h2_rows(tile2(jnp.maximum(v - 1, 0)), clock)
            outer_at(OUTER0[0])

        def apply(clock, outer_at):
            blk = jnp.minimum(jax.lax.shift_right_logical(n + 2, 3) + 1, NBLK - 1)
            e0 = jnp.bitwise_and(n + 2, 7) * TPI
            i, k0 = jax.lax.shift_right_logical(e0, 6), jnp.bitwise_and(e0, KR - 1)
            hr = ht_ref[blk * TPB + i, pl.ds(pl.multiple_of(DM + k0, 16), TPI), :].astype(F32)
            ln1_apply(t1, clock)
            ln2_apply(t2, clock)
            late_mod_store(n)
            outer_at(OUTER0[1])
            h_table(hr, (jnp.bitwise_and(blk, 1) * NV + i) * 16, k0, never_of(clock, TAB0, TAB1))

        for a in range(2):
            unit(2 * n + a, (stats, apply)[a], *streams[a])
        v_transpose(2 * n + 2, vt0_ref)
        wq_transpose(2 * n + 4, wqt0_ref)
        return carry

    jax.lax.fori_loop(0, NU // 2 - 1, step, 0)

    T0 = NT - TPB
    cp_out(0, T0, osem.at[C + TPB]).start()
    cp_g.wait()
    v_transpose(NU - 1, vt1_ref)
    o = jnp.concatenate([attend(*streams[a][0:3])[0] for a in range(2)], axis=0)
    wlast = jnp.concatenate([wot_v[HKV - 2], wot_v[HKV - 1]], axis=1)
    fin = [acc_ref[T0 + t] + _dot(wlast, o[:, t * 128:(t + 1) * 128]) for t in range(TPB)]
    clock = jnp.concatenate(fin, axis=0)
    row8 = jax.lax.broadcasted_iota(jnp.int32, (C, 128), 0)
    lane8 = jax.lax.broadcasted_iota(jnp.int32, (C, 128), 1)
    work = key_ref[0:T0, :]
    lead = jnp.zeros((C, 128), F32)
    for t in range(C):
        mx = jnp.max(jnp.max(work, axis=0, keepdims=True), axis=1, keepdims=True)
        work = jnp.where(work == mx, 0.0, work)
        lead = jnp.where(row8 == t, mx, lead)

    def spread(row):
        return pltpu.roll(jnp.broadcast_to(row, (128, 128)), 0, 1, stride=1, stride_axis=0)

    def merge(lead, rows, spreads):
        cols = jnp.concatenate([lead] + spreads, axis=0)
        best = jnp.zeros((C, 128), F32)
        for row in [jnp.max(jnp.where(row8 == lane8, lead, 0.0), axis=0, keepdims=True)] + rows:
            rank = jnp.sum(jnp.where(cols > row, 1.0, 0.0), axis=0, keepdims=True)
            best = jnp.maximum(best, jnp.where(rank == row8.astype(F32), row, 0.0))
        return jnp.max(best, axis=1, keepdims=True)

    def tail_h2(t, norm, gate=None):
        x1 = x1_ref[t].astype(F32)
        if gate is not None:
            n = gate.shape[0]
            x1 = jnp.concatenate([_paced(x1[:n], gate, 0), x1[n:]], axis=0) if n < D else _paced(x1, gate, 0)
        h2_ref[t] = ln2_h2(x1, *norm).astype(BF16)
        if t < NT - 2:
            h2_rows(t)

    u_vec, u_sum, b_sum = router_terms()
    keys = []
    for t in range(TPB):
        x1, stats = ln2_x1(T0 + t, fin[t])
        mean, inv = norm = ln2_norm(stats)
        r = (jnp.sum(x1 * u_vec, axis=0, keepdims=True) - mean * u_sum) * inv + b_sum
        keys.append(_score_key(r, T0 + t))
        if t < TPB - 1:
            tail_h2(T0 + t, norm, clock[(t + 1) * D + TLAG:(t + 2) * D + TLAG])
    lead = jnp.broadcast_to(merge(lead, keys[0:2], [spread(k) for k in keys[0:2]]), (C, 128))
    spread2 = spread(keys[2])
    if BAR == 0:
        cp_u.wait()
        cp_out(0, T0, osem.at[C + TPB]).wait()

    h2_rows(NT - 2)
    tail_h2(NT - 1, norm)
    h2_rows(NT - 1)
    sel = pltpu.bitcast(merge(lead, keys[2:4], [spread2, spread(keys[3])]), jnp.int32) - KEY0
    sel_tok = (S - 1) - (sel & (S - 1))
    toks = [sel_tok[t, 0] for t in range(C)]
    tiles = [jax.lax.shift_right_logical(tk, 7) for tk in toks]
    sel_code = jax.lax.shift_right_logical(sel, 11) - 32768
    sel_bits = jnp.where(sel_code < 0, -32769 - sel_code, sel_code)
    r_sel = pltpu.bitcast(jax.lax.shift_left(sel_bits, 16), F32)

    final = []
    for t in range(C):
        d = True
        for u in range(t + 1, C):
            d = jnp.logical_and(d, tiles[u] != tiles[t])
        final.append(d)

    words = jnp.concatenate([h2row_ref[pl.ds(jax.lax.shift_right_logical(toks[t], 1), 1), :]
                             for t in range(C)], axis=0)
    odd = jnp.bitwise_and(sel_tok, 1) == 1
    xs = pltpu.bitcast(jnp.where(odd, jnp.bitwise_and(words, jnp.uint32(0xFFFF0000)),
                                 jax.lax.shift_left(words, jnp.uint32(16))), F32)
    xs = xs.astype(BF16)

    def plain_out(t, ticks=None):
        x1 = x1_ref[t].astype(F32)
        if ticks is not None:
            gate = jnp.concatenate([ticks[a * len(ticks) // (D // 8)] for a in range(D // 8)], axis=0)
            x1 = _paced(x1, gate, 0)
        out_v[t] = (x1 + mod(5) * h2_ref[t].astype(F32)).astype(BF16)

    clean = []

    def send_clean(t):
        d = tiles[0] != t
        for a in range(1, C):
            d = jnp.logical_and(d, tiles[a] != t)
        clean.append(d)
        pl.when(d)(cp_out(t, 1, osem.at[C + t - T0]).start)

    if BAR == 1:
        cp_u.wait()
        cp_out(0, T0, osem.at[C + TPB]).wait()
    gpre = _dot(xs, wg_v[...])
    u = _dot(xs, wu_v[...])
    ticks = [z[:, a * 128:(a + 1) * 128] for z in (gpre, u) for a in range(NFB)]
    for t in range(TPB):
        plain_out(T0 + t, ticks[t * TKS:(t + 1) * TKS])
        send_clean(T0 + t)
    gpre, u = _r(gpre), _r(u)
    gact = _r(gpre * _r(jax.nn.sigmoid(gpre)))
    act = (gact * u).astype(BF16)
    gate_r = _r(jax.nn.sigmoid(r_sel))
    ohs = []
    for t in range(C):
        oh = jnp.where(sel_tok == tiles[t] * 128 + lane8, 1.0, 0.0)
        ohs.append(jnp.concatenate([oh, jnp.zeros((16 - C, 128), F32)], axis=0).astype(BF16))

    def cp_fix(t, lo, hi):
        return pltpu.make_async_copy(fix_v.at[t, lo:hi, :], out_hbm.at[lo:hi, _lanes(tiles[t])],
                                     osem.at[t])

    def guarded(cond, fn):
        if cond is True:
            fn()
        else:
            pl.when(cond)(fn)

    def scatter(j, yt, t):
        lo, hi = j * 128, min(j * 128 + 128, D)
        upd = jnp.concatenate([_dot(yt[a:a + 64], ohs[t]) for a in range(0, hi - lo, 64)], axis=0)
        fix_v[t, lo:hi, :] = (x1_ref[tiles[t], lo:hi, :].astype(F32) + mod_ref[5 * D + lo:5 * D + hi, :]
                              * (h2_ref[tiles[t], lo:hi, :].astype(F32) + upd)).astype(BF16)
        guarded(final[t], cp_fix(t, lo, hi).start)

    NJ = (D + 127) // 128
    yts = []
    for j in range(NJ):
        lo, hi = j * 128, min(j * 128 + 128, D)
        nk = 4
        FK = F // nk
        yk = []
        for a in range(nk):
            w = pltpu.bitcast(wd_ref[a * FK // 2:(a + 1) * FK // 2, lo:hi], BF16)
            yk.append(_dot(act[:, a * FK:(a + 1) * FK], w))
            if j >= SCLAG:
                for t in (2 * a, 2 * a + 1):
                    scatter(j - SCLAG, yts[j - SCLAG], t)
        y = _r(sum(yk)) * gate_r
        yts.append(jnp.concatenate([y, jnp.zeros_like(y)], axis=0).astype(BF16).T)
    for j in range(NJ - SCLAG, NJ):
        for t in range(C):
            scatter(j, yts[j], t)
    for t in range(T0, NT):
        pl.when(clean[t - T0])(cp_out(t, 1, osem.at[C + t - T0]).wait)
    for t in range(C):
        guarded(final[t], cp_fix(t, 0, D).wait)


@jax.jit
def pallas_adaLN_cond__gqa_block_cached__moe_arch_mod__prompt_kernel(
    A_x: jax.Array,
    A_k_cache: jax.Array,
    A_v_cache: jax.Array,
    A_wq: jax.Array,
    A_wo: jax.Array,
    B_x: jax.Array,
    B_w_r: jax.Array,
    B_w_gate: jax.Array,
    B_w_up: jax.Array,
    B_w_down: jax.Array,
    c: jax.Array,
    w_mod: jax.Array,
):
    del B_x
    xt = A_x.reshape(S, D).T
    k = A_k_cache.reshape(HKV, S, DH)
    v = A_v_cache.reshape(HKV, S, DH)

    hbm = pl.BlockSpec(memory_space=pl.ANY)
    stream = [
        pltpu.VMEM((S, REP * TQ), F32),
        pltpu.VMEM((8, REP * TQ), F32),
        pltpu.VMEM((DH // 2, S), U32),
        pltpu.VMEM((GW // 2, D), U32),
        pltpu.VMEM((NV * 128, GW), F32),
        pltpu.VMEM((REP, KR, DH), F32),
    ]
    out = pl.pallas_call(
        _kernel,
        in_specs=[hbm] * 11,
        out_specs=hbm,
        out_shape=jax.ShapeDtypeStruct((D, S), BF16),
        scratch_shapes=[
            pltpu.VMEM((NT + NFB + NMB, D, 128), BF16),
            pltpu.VMEM((HKV, S, DH), BF16),
            pltpu.VMEM((HKV, S, DH), BF16),
            pltpu.VMEM((HKV, D, GW), BF16),
            pltpu.VMEM((HKV, D, GW), BF16),
            pltpu.VMEM((D, DA), BF16),
            pltpu.VMEM((D, F), BF16),
            pltpu.VMEM((D, F), BF16),
            pltpu.VMEM((F // 2, D), U32),
            pltpu.VMEM((NT, D, 128), BF16),
            pltpu.VMEM((NT, D, 128), F32),
            pltpu.VMEM((6 * D, 128), F32),
            pltpu.VMEM((5 * 128, 128), F32),
            pltpu.VMEM((5 * 128, 128), F32),
            pltpu.VMEM((NT, D, 128), BF16),
            pltpu.VMEM((NT, D, 128), BF16),
            pltpu.VMEM((S // 2, D), U32),
            pltpu.VMEM((NT, D, 128), BF16),
            pltpu.VMEM((C, D, 128), BF16),
            pltpu.VMEM((NT, 128), F32),
            pltpu.VMEM((NT * NC, 8, 128), F32),
            pltpu.VMEM((NT * NC, 8, 128), F32),
            pltpu.VMEM((MPI, 8, 128), F32),
            pltpu.VMEM((2 * NV * 16, KR, 8, 128), F32),
            pltpu.VMEM((KR, HQ * DH), BF16),
        ] + stream + stream + [
            pltpu.VMEM((D,), BF16),
            pltpu.VMEM((1, D), BF16),
            pltpu.SemaphoreType.DMA((HKV // 2,)),
            pltpu.SemaphoreType.DMA((11,)),
            pltpu.SemaphoreType.DMA((C + TPB + 1,)),
        ],
        compiler_params=pltpu.CompilerParams(vmem_limit_bytes=127 * 1024 * 1024,
                                             disable_bounds_checks=True,
                                             disable_semaphore_checks=True),
    )(B_w_r, c, xt, k, v, A_wq, A_wo.T, w_mod, B_w_gate, B_w_up, B_w_down.T)
    return out.T.reshape(1, S, D)
```

```python
import math

import jax
import jax.numpy as jnp
import jax.experimental.pallas as pl
import jax.experimental.pallas.tpu as pltpu

S = 2048
D = 576
HQ = 32
HKV = 16
REP = HQ // HKV
DH = 128
GW = REP * DH
F = 4608
C = 8
EPS = 1e-05
TQ = 512
NBLK = S // TQ
TPB = TQ // 128
NT = S // 128
NU = NBLK * HKV
DA = 2 * D
NC = 3
DC = D // NC
TLAG = 160
TKS = 18
SCLAG = 2
CL2 = 0
SLAG = 96
BAR = 1
PG = 64
NFB = F // 128
MODA = ((0, 4, 5), (1, 2, 6), (3, 7, 8))
NMB = 4 * D // 128
MPI = 3
MB0 = 2
WD0 = 14
DM = 512
KR = D - DM
NV = 2
CH = 3
QC, SC, WC = 0, 1024, 1024 + 2 * S
OUTER0, OSTEP = (SC + 0, SC + 0), 138
TABLE = 1
TAB0, TAB1 = SC + 3150, WC + 600
XP = (SC + 2500, SC + 300, SC + 1400, SC + 2100, WC + 640, SC + 100, SC + 1200)
TPI = 16
PACE = (SC + 3900, SC + 3150, SC + 3150, SC + 3800, WC + 400, SC + 2100)

BF16 = jnp.bfloat16
F32 = jnp.float32
U32 = jnp.uint32
QSCALE = DH ** -0.5 * math.log2(math.e)


def _dot(a, b):
    return jnp.dot(a, b, preferred_element_type=F32)


def _dot_nt(a, b):
    return jax.lax.dot_general(a, b, (((1,), (1,)), ((), ())), preferred_element_type=F32)


def _r(x):
    return x.astype(BF16).astype(F32)


def _col_bcast(row):
    return jnp.broadcast_to(row, (128, 128)).T


def _blk(u):
    return u // HKV if isinstance(u, int) else jax.lax.shift_right_logical(u, 4)


def _grp(u):
    return u % HKV if isinstance(u, int) else jnp.bitwise_and(u, HKV - 1)


def _lanes(t, n=1):
    return pl.ds(pl.multiple_of(t * 128, 128), n * 128)


def _paced(x, clock, pos):
    if clock is None:
        return x
    pos = pos // 8 * 8
    g = clock[pos:pos + x.shape[0], 0:x.shape[1]]
    return jnp.where(g * g < 0.0, jnp.zeros_like(x), x)


def _paced_wide(x, clock, pos):
    n, w = x.shape
    return jnp.concatenate([_paced(x[:, a:min(a + 128, w)], clock, pos + a // 128 * n)
                            for a in range(0, w, 128)], axis=1)


def _softmax_numer(s, m):
    n, w = s.shape
    p = jnp.exp2(s - m).reshape(n // PG, PG // 8, 8, w)
    ts = jnp.sum(p, axis=1)
    last = jnp.where(ts < 0.0, ts, p[:, PG // 8 - 1])
    p = jnp.concatenate([p[:, :PG // 8 - 1], last[:, None]], axis=1).reshape(n, w)
    l = jnp.sum(jnp.sum(ts, axis=0), axis=0, keepdims=True)
    return p.astype(BF16), l, ts


KEY0 = 0x20000000


def _score_key(r, t):
    tok = t * 128 + jax.lax.broadcasted_iota(jnp.int32, r.shape, 1)
    bits = jax.lax.shift_right_arithmetic(pltpu.bitcast(_r(r) + 0.0, jnp.int32), 16)
    code = jnp.where(bits < 0, -32769 - bits, bits) + 32768
    return pltpu.bitcast(code * S + (S - 1 - tok) + KEY0, F32)


def _chunk_stats(x):
    m = jnp.sum(x, axis=0, keepdims=True) * (1.0 / DC)
    xc = x - m
    return m, jnp.sum(xc * xc, axis=0, keepdims=True)


def _mean_var(stats):
    mean = sum(m for m, _ in stats) * (1.0 / NC)
    var = sum(s + DC * (m - mean) * (m - mean) for m, s in stats) * (1.0 / D)
    return mean, var


def _kernel(wr_hbm, c_hbm,
            xt_hbm, k_hbm, v_hbm, wq_hbm, wot_hbm, wmod_hbm, wg_hbm, wu_hbm, wdt_hbm,
            out_hbm,
            xw_v, k_v, v_v, wq_v, wot_v, wmod_v, wg_v, wu_v, wd_ref,
            ht_ref, acc_ref, mod_ref, wrb_ref, scb_ref, x1_ref, h2_ref, h2row_ref, out_v, fix_v,
            key_ref, st1_ref, st2_ref, lm_ref,
            hb_ref, wrem_v,
            s0_ref, m0_ref, vt0_ref, wqt0_ref, qr0_ref, wf0_ref,
            s1_ref, m1_ref, vt1_ref, wqt1_ref, qr1_ref, wf1_ref,
            wr_ref, c_ref, bsem, msem, osem):
    streams = ((s0_ref, m0_ref, vt0_ref, wqt0_ref, qr0_ref, wf0_ref),
               (s1_ref, m1_ref, vt1_ref, wqt1_ref, qr1_ref, wf1_ref))

    def cp_cols(src, dst, t, n, sem, dst_t=None):
        return pltpu.make_async_copy(src.at[:, _lanes(t, n)],
                                     dst.at[:, _lanes(t if dst_t is None else dst_t, n)], sem)

    def cp_pair(src, dst, p, sem):
        return pltpu.make_async_copy(src.at[pl.ds(2 * p, 2)], dst.at[pl.ds(2 * p, 2)], sem)

    cp_k = lambda p, sem: cp_pair(k_hbm, k_v, p, sem)
    cp_v1 = lambda g, sem: pltpu.make_async_copy(v_hbm.at[g], v_v.at[g], sem)
    cp_k1 = lambda g, sem: pltpu.make_async_copy(k_hbm.at[g], k_v.at[g], sem)

    class Both:
        def __init__(self, cps):
            self.cps = cps

        def start(self):
            for cp in self.cps:
                cp.start()

        def wait(self):
            for cp in self.cps:
                cp.wait()

    def cp_w1(src, dst, g, sem):
        return pltpu.make_async_copy(src.at[:, _lanes(g * REP, REP)], dst.at[g], sem)

    def cp_w(src, dst, p, sem):
        return Both([cp_w1(src, dst, 2 * p + a, sem) for a in range(2)])

    cp_wq = lambda p, sem: cp_w(wq_hbm, wq_v, p, sem)
    cp_wo = lambda p, sem: cp_w(wot_hbm, wot_v, p, sem)
    cp_x = lambda t0, n, sem: Both([pltpu.make_async_copy(xt_hbm.at[:, _lanes(t0 + t)],
                                                          xw_v.at[t0 + t], sem) for t in range(n)])
    NP = HKV // 2

    def bundle(n, act):
        sem = bsem.at[n if isinstance(n, int) else jnp.minimum(n, NP - 1)]

        def on(cond, cps):
            def go():
                for cp in cps():
                    getattr(cp, act)()
            if isinstance(cond, bool):
                if cond:
                    go()
            else:
                pl.when(cond)(go)
        on(n + 1 < NP, lambda: [cp_k(n + 1, sem), cp_v1(2 * n + 2, sem), cp_w1(wq_hbm, wq_v, 2 * n + 3, sem)])
        on(n + 2 < NP, lambda: [cp_w1(wq_hbm, wq_v, 2 * n + 4, sem)])
        on(jnp.logical_and(n >= 1, n < NBLK) if not isinstance(n, int) else 1 <= n < NBLK,
           lambda: [cp_x(TPB * n + 1, TPB - 1, sem)])
        on(jnp.logical_and(n >= 1, n < NBLK - 1) if not isinstance(n, int) else 1 <= n < NBLK - 1,
           lambda: [cp_x(TPB * n + TPB, 1, sem)])
        on(n < NP, lambda: [cp_v1(2 * n + 1, sem), cp_wo(n, sem)])

    cp_moda = [Both([cp_cols(wmod_hbm, wmod_v, t, 1, msem.at[s]) for t in tiles])
               for s, tiles in zip((0, 6, 10), MODA)]
    cp_modb = Both([pltpu.make_async_copy(wmod_hbm.at[:, _lanes(DA // 128 + b)],
                                          xw_v.at[NT + NFB + b], msem.at[1]) for b in range(NMB)])
    cp_g = pltpu.make_async_copy(wg_hbm, wg_v, msem.at[2])
    cp_u = pltpu.make_async_copy(wu_hbm, wu_v, msem.at[3])
    cp_d = Both([pltpu.make_async_copy(wdt_hbm.at[:, _lanes(b)], xw_v.at[NT + b], msem.at[4])
                 for b in range(NFB)])
    cp_out = lambda t, n, sem: Both([pltpu.make_async_copy(out_v.at[t + a], out_hbm.at[:, _lanes(t + a)],
                                                           sem) for a in range(n)])

    def silu_c():
        c = c_ref[...].astype(F32)
        return _r(c * _r(jax.nn.sigmoid(c)))

    def finish_mod(mod, lo, clock=None, pos=0):
        mod = _r(mod)
        col = lo + jax.lax.broadcasted_iota(jnp.int32, mod.shape, 1)
        is_scale = jnp.logical_or(jnp.logical_and(col >= D, col < 2 * D),
                                  jnp.logical_and(col >= 4 * D, col < 5 * D))
        mod = jnp.where(is_scale, _r(1.0 + mod), mod)
        for t in range(mod.shape[1] // 128):
            rows = pl.ds(pl.multiple_of(lo + t * 128, 128), 128)
            mod_ref[rows, :] = _paced(_col_bcast(mod[:, t * 128:(t + 1) * 128]), clock, pos)

    def late_mod_sums(n, clock):
        b0 = jnp.clip(n - MB0, 0, NMB // MPI - 1) * MPI
        for k in range(MPI):
            w = xw_v[jnp.where(n >= MB0, NT + NFB + b0 + k, 0)].astype(F32)
            part = jnp.sum((w * scb_ref[0:D, :]).reshape(D // 8, 8, 128), axis=0)
            lm_ref[k] = _paced(part, clock, PACE[4] + 192 * k)

    def late_mod_store(n, clock):
        b0 = jnp.clip(n - MB0, 0, NMB // MPI - 1) * MPI
        for k in range(MPI):
            finish_mod(jnp.sum(lm_ref[k], axis=0, keepdims=True), DA + (b0 + k) * 128,
                       clock, XP[4] + 128 * k)

    def col_vector(ref, row):
        row = jnp.concatenate([row, jnp.zeros((1, 64), F32)], axis=1)
        for t in range(5):
            ref[t * 128:(t + 1) * 128, :] = _col_bcast(row[:, t * 128:(t + 1) * 128])

    def mod(k):
        return mod_ref[k * D:(k + 1) * D, :]

    def put_stats(st_ref, t, shift, scale, clock, pos):
        row = jax.lax.broadcasted_iota(jnp.int32, (8, 128), 0)
        st_ref[t] = _paced(jnp.where(row == 0, shift, scale), clock, pos)

    def ln1_stats(t, clock=None, pos=None):
        for c in range(NC):
            m, s = _chunk_stats(xw_v[t, c * DC:(c + 1) * DC, :].astype(F32))
            put_stats(st1_ref, t * NC + c, m, s, clock, (PACE[0] if pos is None else pos) + 192 * c)

    def ln1_norm(t):
        mean, var = _mean_var(load_stats(st1_ref, t))
        return (xw_v[t].astype(F32) - mean) * jax.lax.rsqrt(var + EPS)

    def ln1_apply(t, clock=None, pos=None, ln=None):
        h = (ln1_norm(t) if ln is None else ln) * mod(1) + mod(0)
        ht_ref[t] = _paced(h, clock, PACE[1] if pos is None else pos).astype(BF16)

    def h2_rows(t, clock=None):
        x = _paced_wide(pltpu.bitcast(h2_ref[t].T, U32), clock, PACE[5])
        h2row_ref[pl.ds(pl.multiple_of(t * 64, 64), 64), :] = x

    def router_terms():
        u = mod(4) * wrb_ref[0:D, :]
        return (u, jnp.sum(u, axis=0, keepdims=True),
                jnp.sum(mod(3) * wrb_ref[0:D, :], axis=0, keepdims=True))

    def load_stats(st_ref, t):
        return [(st_ref[t * NC + c, 0:1, :], st_ref[t * NC + c, 1:2, :]) for c in range(NC)]

    def ln2_x1(t, attn, clock=None):
        x1 = _r(xw_v[t].astype(F32) + mod(2) * attn)
        x1_ref[t] = _paced(x1, clock, PACE[2]).astype(BF16)
        return x1, [_chunk_stats(x1[c * DC:(c + 1) * DC]) for c in range(NC)]

    def ln2_norm(stats):
        mean, var = _mean_var(stats)
        return _r(mean), 1.0 / _r(jnp.sqrt(_r(_r(var) + EPS)))

    def ln2_h2(x1, mean, inv):
        return (x1 - mean) * inv * mod(4) + mod(3)

    def ln2_stats(t, clock):
        for c, (m, s) in enumerate(ln2_x1(t, acc_ref[t], clock)[1]):
            put_stats(st2_ref, t * NC + c, m, s, clock, PACE[2] + (c + 1) * DC + SLAG)

    def ln2_apply(t, clock):
        x1 = x1_ref[t].astype(F32)
        h2 = ln2_h2(x1, *ln2_norm(load_stats(st2_ref, t)))
        key = _score_key(jnp.sum(h2 * wrb_ref[0:D, :], axis=0, keepdims=True), t)
        key_ref[pl.ds(t, 1), :] = _paced(key, clock, PACE[3] + D + 96)
        h2 = _r(h2)
        h2_ref[t] = _paced(h2, clock, PACE[3]).astype(BF16)
        out_v[t] = _paced(x1 + mod(5) * h2, clock, PACE[3] + 16).astype(BF16)

    def finish_q(q):
        q = (q * QSCALE).astype(BF16)
        return jnp.concatenate([q[r * DH:(r + 1) * DH] for r in range(REP)], axis=1)

    def q_proj(u, wqt_ref, qr_ref=None, split=False):
        w = pltpu.bitcast(wqt_ref[...], BF16)
        h = jnp.concatenate([ht_ref[_blk(u) * TPB + t] for t in range(TPB)], axis=1)
        if split:
            return sum(_dot(w[:, a:min(a + 128, D)], h[a:min(a + 128, D)]) for a in range(0, D, 128))
        if qr_ref is None:
            rem = _dot(w[:, DM:], h[DM:])
        else:
            rem = [qr_ref[...].T]
            if NV < TPB:
                R = GW * (TPB - NV) // 4
                rem.append(jnp.concatenate([_dot(w[a:a + R, DM:], h[DM:, NV * 128:])
                                            for a in range(0, GW, R)], axis=0))
            rem = jnp.concatenate(rem, axis=1)
        return _dot(w[:, :DM], h[:DM]) + rem

    def w_rest(u, wf_ref):
        w = wrem_v[:, _lanes(_grp(u) * REP, REP)].astype(F32)
        for r in range(REP):
            wf_ref[r] = w[:, r * DH:(r + 1) * DH]

    def outer(u, qr_ref, wf_ref, clock, start):
        base = jnp.bitwise_and(_blk(u), 1) * (NV * 16)
        cells = [(tv, r) for r in range(REP) for tv in range(NV * 16)]
        for g in range(0, len(cells), CH):
            acc = {}
            for k in range(KR):
                for tv, r in cells[g:g + CH]:
                    t = hb_ref[base + tv, k] * wf_ref[r, pl.ds(k, 8, stride=0), :]
                    acc[tv, r] = t if k == 0 else acc[tv, r] + t
            for (tv, r), a in acc.items():
                qr_ref[tv * 8:(tv + 1) * 8, r * DH:(r + 1) * DH] = _paced(
                    a, clock, min(start + OSTEP * (g // CH + 1), clock.shape[0] - 8))

    def h_table(hr, base, k0, gates):
        nk = hr.shape[0]
        for j in range(nk):
            cb = _col_bcast(hr[j:j + 1])
            for b in range(16):
                g = gates[(j * 16 + b) * len(gates) // (nk * 16)]
                hb_ref[base + b, k0 + j] = jnp.where(g, 0.0, cb[b * 8:(b + 1) * 8])

    def never_of(clock, lo, hi):
        return [clock[a:a + 8] * clock[a:a + 8] < 0.0 for a in range(lo // 8 * 8, hi, 8)]

    def scores(u, q, s_ref, m_ref):
        s = _dot(k_v[_grp(u)], q)
        s_ref[...] = s
        m_ref[...] = jnp.broadcast_to(jnp.max(s, axis=0, keepdims=True), m_ref.shape)
        return jnp.concatenate([s[:, 0:128], s[:, TQ:TQ + 128]], axis=0)

    def v_transpose(u, vt_ref, clock=None, pos=0):
        vt_ref[...] = _paced_wide(pltpu.bitcast(v_v[_grp(u)].T, U32), clock, pos)

    def wq_transpose(u, wqt_ref, clock=None, pos=0):
        wqt_ref[...] = _paced_wide(pltpu.bitcast(wq_v[_grp(u)].T, U32), clock, pos)

    def wd_transpose(u, clock, pos):
        fb = jnp.clip(u - WD0, 0, NFB - 1)
        src = jnp.where(u >= WD0, NT + fb, 0)
        wd_ref[pl.ds(pl.multiple_of(fb * 64, 64), 64), :] = _paced_wide(
            pltpu.bitcast(xw_v[src].T, U32), clock, pos)

    def attend(s_ref, m_ref, vt_ref):
        m = m_ref[0:1, :]
        o, never = [], []
        for r in range(REP):
            cols = slice(r * TQ, (r + 1) * TQ)
            p, l, ts = _softmax_numer(s_ref[:, cols], m[:, cols])
            o.append((_dot(pltpu.bitcast(vt_ref[...], BF16), p) * (1.0 / l)).astype(BF16))
            never += [ts[i, :, c * 128:(c + 1) * 128] < 0.0 for c in range(TPB) for i in range(S // PG)]
        return jnp.concatenate(o, axis=0), never

    small = Both([pltpu.make_async_copy(wr_hbm, wr_ref, msem.at[7]),
                  pltpu.make_async_copy(c_hbm, c_ref, msem.at[7])])
    zeroth = Both([cp_x(0, TPB, msem.at[5]), cp_w1(wq_hbm, wq_v, 0, msem.at[5])])
    first = Both([cp_k1(0, msem.at[8]), cp_w1(wq_hbm, wq_v, 1, msem.at[8])])
    second = Both([cp_k1(1, msem.at[9]), cp_v1(0, msem.at[9]), cp_w1(wq_hbm, wq_v, 2, msem.at[9]),
                   pltpu.make_async_copy(wq_hbm.at[DM:, :], wrem_v, msem.at[9]), cp_x(TPB, 1, msem.at[9])])
    for cp in [small, zeroth] + cp_moda + [first, second]:
        cp.start()
    acc_ref[...] = jnp.zeros_like(acc_ref)
    mod_ref[DA:6 * D, :] = jnp.zeros((4 * D, 128), F32)
    h2_ref[0] = jnp.zeros((D, 128), BF16)
    small.wait()
    col_vector(wrb_ref, wr_ref[...].astype(F32).reshape(1, D))
    col_vector(scb_ref, silu_c())
    sc8 = jnp.broadcast_to(silu_c(), (8, D)).astype(BF16)
    zeroth.wait()
    ln0 = []
    for t in range(TPB):
        ln1_stats(t)
        ln0.append(ln1_norm(t))
    wq_transpose(0, wqt0_ref)
    for cp, tiles in zip(cp_moda, MODA):
        cp.wait()
        for t in tiles:
            finish_mod(_dot(sc8, wmod_v[:, t * 128:(t + 1) * 128])[0:1], t * 128)
    for t in range(TPB):
        ln1_apply(t, ln=ln0[t])
    q = finish_q(q_proj(0, wqt0_ref, split=True))
    first.wait()
    bundle(0, 'start')
    def first_table(gates, lo, hi):
        for i in range(NV + 1):
            a, b = max(lo, i * KR), min(hi, (i + 1) * KR)
            if a < b:
                gs = gates[(a - lo) * len(gates) // (hi - lo):(b - lo) * len(gates) // (hi - lo)]
                hr = ht_ref[i if i < NV else TPB, DM:, :].astype(F32)[a - i * KR:b - i * KR]
                h_table(hr, i * 16, a - i * KR, gs)

    TSPLIT = 80
    first_table(never_of(scores(0, q, s0_ref, m0_ref), 64, 2 * S - 192), 0, TSPLIT)
    wq_transpose(1, wqt1_ref)
    second.wait()
    bundle(1, 'start')
    hrem = jnp.concatenate([ht_ref[t, DM:, :] for t in range(NV)], axis=1)
    for a in range(2):
        streams[a][4][...] = jax.lax.dot_general(
            hrem, wrem_v[:, (a + 2) * GW:(a + 3) * GW], (((0,), (0,)), ((), ())),
            preferred_element_type=F32)
    q = q_proj(1, wqt1_ref)
    clock = jnp.concatenate([q[:, t * 128:(t + 1) * 128] for t in range(TPB)]
                            + [scores(1, finish_q(q), s1_ref, m1_ref)], axis=0)
    ln1_stats(TPB, clock, SC + 200)
    ln1_apply(TPB, clock, SC + 900)
    first_table(never_of(clock, 0, SC + 2 * S - 600), TSPLIT, NV * KR + 2 * TPI)
    for a in range(2):
        w_rest(a + 4, streams[a][5])
    v_transpose(0, vt0_ref)
    wq_transpose(2, wqt0_ref)

    def unit(u, side, s_ref, m_ref, vt_ref, wqt_ref, qr_ref, wf_ref):
        q = q_proj(u + 2, wqt_ref, qr_ref)
        o, _ = attend(s_ref, m_ref, vt_ref)
        sclk = scores(u + 2, finish_q(q), s_ref, m_ref)
        upd = _dot(wot_v[_grp(u)], o)
        clock = jnp.concatenate([q[:, t * 128:(t + 1) * 128] for t in range(TPB)] + [sclk]
                                + [upd[:, 0:128], upd[:, 256:384]], axis=0)
        side(clock, lambda start: outer(u + 4, qr_ref, wf_ref, clock, start))
        w_rest(u + 6, wf_ref)
        for t in range(TPB):
            acc_ref[_blk(u) * TPB + t] += upd[:, t * 128:(t + 1) * 128]

    def step(n, carry):
        def waits(_, c):
            bundle(n, 'wait')
            pl.when(n == MB0)(cp_modb.wait)
            pl.when(n == WD0 // 2)(cp_d.wait)
            return c
        jax.lax.fori_loop(0, jnp.where(n < NP, 1, 0), waits, 0)

        pl.when(n == 0)(cp_modb.start)
        bundle(jnp.minimum(n + 2, NP), 'start')
        for a in range(3):
            pl.when(n == 2 + a)(Both(cp_d.cps[a * NFB // 3:(a + 1) * NFB // 3]).start)
        pl.when(n == NP)(Both([cp_g, cp_u]).start)

        t1 = jnp.minimum(n + 4, NT - 1)
        v = jnp.maximum(n - NP, 0)
        tile2 = lambda v: (jax.lax.shift_right_logical(v, 3) * TPB
                           + jnp.minimum(jnp.bitwise_and(v, NP - 1), TPB - 1))
        t2 = tile2(v)

        def stats(clock, outer_at):
            v_transpose(2 * n + 1, vt1_ref, clock, XP[5])
            wq_transpose(2 * n + 3, wqt1_ref, clock, XP[6])
            ln2_stats(t2, clock)
            ln1_stats(t1, clock)
            late_mod_sums(n, clock)
            h2_rows(tile2(jnp.maximum(v - 1, 0)), clock)
            wd_transpose(2 * n, clock, XP[0])
            outer_at(OUTER0[0])

        def apply(clock, outer_at):
            blk = jnp.minimum(jax.lax.shift_right_logical(n + 2, 3) + 1, NBLK - 1)
            e0 = jnp.bitwise_and(n + 2, 7) * TPI
            i, k0 = jax.lax.shift_right_logical(e0, 6), jnp.bitwise_and(e0, KR - 1)
            hr = ht_ref[blk * TPB + i, pl.ds(pl.multiple_of(DM + k0, 16), TPI), :].astype(F32)
            v_transpose(2 * n + 2, vt0_ref, clock, XP[1])
            wq_transpose(2 * n + 4, wqt0_ref, clock, XP[2])
            wd_transpose(2 * n + 1, clock, XP[3])
            ln1_apply(t1, clock)
            ln2_apply(t2, clock)
            outer_at(OUTER0[1])
            h_table(hr, (jnp.bitwise_and(blk, 1) * NV + i) * 16, k0, never_of(clock, TAB0, TAB1))
            late_mod_store(n, clock)

        for a in range(2):
            unit(2 * n + a, (stats, apply)[a], *streams[a])
        return carry

    jax.lax.fori_loop(0, NU // 2 - 1, step, 0)

    T0 = NT - TPB
    cp_out(0, T0, osem.at[C + TPB]).start()
    cp_g.wait()
    v_transpose(NU - 1, vt1_ref)
    o = jnp.concatenate([attend(*streams[a][0:3])[0] for a in range(2)], axis=0)
    wlast = jnp.concatenate([wot_v[HKV - 2], wot_v[HKV - 1]], axis=1)
    fin = [acc_ref[T0 + t] + _dot(wlast, o[:, t * 128:(t + 1) * 128]) for t in range(TPB)]
    clock = jnp.concatenate(fin, axis=0)
    row8 = jax.lax.broadcasted_iota(jnp.int32, (C, 128), 0)
    lane8 = jax.lax.broadcasted_iota(jnp.int32, (C, 128), 1)
    work = key_ref[0:T0, :]
    lead = jnp.zeros((C, 128), F32)
    for t in range(C):
        mx = jnp.max(jnp.max(work, axis=0, keepdims=True), axis=1, keepdims=True)
        work = jnp.where(work == mx, 0.0, work)
        lead = jnp.where(row8 == t, mx, lead)

    def spread(row):
        return pltpu.roll(jnp.broadcast_to(row, (128, 128)), 0, 1, stride=1, stride_axis=0)

    def merge(lead, rows, spreads):
        cols = jnp.concatenate([lead] + spreads, axis=0)
        best = jnp.zeros((C, 128), F32)
        for row in [jnp.max(jnp.where(row8 == lane8, lead, 0.0), axis=0, keepdims=True)] + rows:
            rank = jnp.sum(jnp.where(cols > row, 1.0, 0.0), axis=0, keepdims=True)
            best = jnp.maximum(best, jnp.where(rank == row8.astype(F32), row, 0.0))
        return jnp.max(best, axis=1, keepdims=True)

    def tail_h2(t, norm, gate=None):
        x1 = x1_ref[t].astype(F32)
        if gate is not None:
            n = gate.shape[0]
            x1 = jnp.concatenate([_paced(x1[:n], gate, 0), x1[n:]], axis=0) if n < D else _paced(x1, gate, 0)
        h2_ref[t] = ln2_h2(x1, *norm).astype(BF16)
        if t < NT - 2:
            h2_rows(t)

    u_vec, u_sum, b_sum = router_terms()
    keys = []
    for t in range(TPB):
        x1, stats = ln2_x1(T0 + t, fin[t])
        mean, inv = norm = ln2_norm(stats)
        r = (jnp.sum(x1 * u_vec, axis=0, keepdims=True) - mean * u_sum) * inv + b_sum
        keys.append(_score_key(r, T0 + t))
        if t < TPB - 1:
            tail_h2(T0 + t, norm, clock[(t + 1) * D + TLAG:(t + 2) * D + TLAG])
    lead = jnp.broadcast_to(merge(lead, keys[0:2], [spread(k) for k in keys[0:2]]), (C, 128))
    spread2 = spread(keys[2])
    if BAR == 0:
        cp_u.wait()
        cp_out(0, T0, osem.at[C + TPB]).wait()

    h2_rows(NT - 2)
    tail_h2(NT - 1, norm)
    h2_rows(NT - 1)
    sel = pltpu.bitcast(merge(lead, keys[2:4], [spread2, spread(keys[3])]), jnp.int32) - KEY0
    sel_tok = (S - 1) - (sel & (S - 1))
    toks = [sel_tok[t, 0] for t in range(C)]
    tiles = [jax.lax.shift_right_logical(tk, 7) for tk in toks]
    sel_code = jax.lax.shift_right_logical(sel, 11) - 32768
    sel_bits = jnp.where(sel_code < 0, -32769 - sel_code, sel_code)
    r_sel = pltpu.bitcast(jax.lax.shift_left(sel_bits, 16), F32)

    final = []
    for t in range(C):
        d = True
        for u in range(t + 1, C):
            d = jnp.logical_and(d, tiles[u] != tiles[t])
        final.append(d)

    words = jnp.concatenate([h2row_ref[pl.ds(jax.lax.shift_right_logical(toks[t], 1), 1), :]
                             for t in range(C)], axis=0)
    odd = jnp.bitwise_and(sel_tok, 1) == 1
    xs = pltpu.bitcast(jnp.where(odd, jnp.bitwise_and(words, jnp.uint32(0xFFFF0000)),
                                 jax.lax.shift_left(words, jnp.uint32(16))), F32)
    xs = xs.astype(BF16)

    def plain_out(t, ticks=None):
        x1 = x1_ref[t].astype(F32)
        if ticks is not None:
            gate = jnp.concatenate([ticks[a * len(ticks) // (D // 8)] for a in range(D // 8)], axis=0)
            x1 = _paced(x1, gate, 0)
        out_v[t] = (x1 + mod(5) * h2_ref[t].astype(F32)).astype(BF16)

    clean = []

    def send_clean(t):
        d = tiles[0] != t
        for a in range(1, C):
            d = jnp.logical_and(d, tiles[a] != t)
        clean.append(d)
        pl.when(d)(cp_out(t, 1, osem.at[C + t - T0]).start)

    if BAR == 1:
        cp_u.wait()
        cp_out(0, T0, osem.at[C + TPB]).wait()
    gpre = _dot(xs, wg_v[...])
    u = _dot(xs, wu_v[...])
    ticks = [z[:, a * 128:(a + 1) * 128] for z in (gpre, u) for a in range(NFB)]
    for t in range(TPB):
        plain_out(T0 + t, ticks[t * TKS:(t + 1) * TKS])
        send_clean(T0 + t)
    gpre, u = _r(gpre), _r(u)
    gact = _r(gpre * _r(jax.nn.sigmoid(gpre)))
    act = (gact * u).astype(BF16)
    gate_r = _r(jax.nn.sigmoid(r_sel))
    ohs = []
    for t in range(C):
        oh = jnp.where(sel_tok == tiles[t] * 128 + lane8, 1.0, 0.0)
        ohs.append(jnp.concatenate([oh, jnp.zeros((16 - C, 128), F32)], axis=0).astype(BF16))

    def cp_fix(t, lo, hi):
        return pltpu.make_async_copy(fix_v.at[t, lo:hi, :], out_hbm.at[lo:hi, _lanes(tiles[t])],
                                     osem.at[t])

    def guarded(cond, fn):
        if cond is True:
            fn()
        else:
            pl.when(cond)(fn)

    def scatter(j, yt, t):
        lo, hi = j * 128, min(j * 128 + 128, D)
        upd = jnp.concatenate([_dot(yt[a:a + 64], ohs[t]) for a in range(0, hi - lo, 64)], axis=0)
        fix_v[t, lo:hi, :] = (x1_ref[tiles[t], lo:hi, :].astype(F32) + mod_ref[5 * D + lo:5 * D + hi, :]
                              * (h2_ref[tiles[t], lo:hi, :].astype(F32) + upd)).astype(BF16)
        guarded(final[t], cp_fix(t, lo, hi).start)

    NJ = (D + 127) // 128
    yts = []
    for j in range(NJ):
        lo, hi = j * 128, min(j * 128 + 128, D)
        nk = 4
        FK = F // nk
        yk = []
        for a in range(nk):
            w = pltpu.bitcast(wd_ref[a * FK // 2:(a + 1) * FK // 2, lo:hi], BF16)
            yk.append(_dot(act[:, a * FK:(a + 1) * FK], w))
            if j >= SCLAG:
                for t in (2 * a, 2 * a + 1):
                    scatter(j - SCLAG, yts[j - SCLAG], t)
        y = _r(sum(yk)) * gate_r
        yts.append(jnp.concatenate([y, jnp.zeros_like(y)], axis=0).astype(BF16).T)
    for j in range(NJ - SCLAG, NJ):
        for t in range(C):
            scatter(j, yts[j], t)
    for t in range(T0, NT):
        pl.when(clean[t - T0])(cp_out(t, 1, osem.at[C + t - T0]).wait)
    for t in range(C):
        guarded(final[t], cp_fix(t, 0, D).wait)


@jax.jit
def pallas_adaLN_cond__gqa_block_cached__moe_arch_mod__prompt_kernel(
    A_x: jax.Array,
    A_k_cache: jax.Array,
    A_v_cache: jax.Array,
    A_wq: jax.Array,
    A_wo: jax.Array,
    B_x: jax.Array,
    B_w_r: jax.Array,
    B_w_gate: jax.Array,
    B_w_up: jax.Array,
    B_w_down: jax.Array,
    c: jax.Array,
    w_mod: jax.Array,
):
    del B_x
    xt = A_x.reshape(S, D).T
    k = A_k_cache.reshape(HKV, S, DH)
    v = A_v_cache.reshape(HKV, S, DH)

    hbm = pl.BlockSpec(memory_space=pl.ANY)
    stream = [
        pltpu.VMEM((S, REP * TQ), F32),
        pltpu.VMEM((8, REP * TQ), F32),
        pltpu.VMEM((DH // 2, S), U32),
        pltpu.VMEM((GW // 2, D), U32),
        pltpu.VMEM((NV * 128, GW), F32),
        pltpu.VMEM((REP, KR, DH), F32),
    ]
    out = pl.pallas_call(
        _kernel,
        in_specs=[hbm] * 11,
        out_specs=hbm,
        out_shape=jax.ShapeDtypeStruct((D, S), BF16),
        scratch_shapes=[
            pltpu.VMEM((NT + NFB + NMB, D, 128), BF16),
            pltpu.VMEM((HKV, S, DH), BF16),
            pltpu.VMEM((HKV, S, DH), BF16),
            pltpu.VMEM((HKV, D, GW), BF16),
            pltpu.VMEM((HKV, D, GW), BF16),
            pltpu.VMEM((D, DA), BF16),
            pltpu.VMEM((D, F), BF16),
            pltpu.VMEM((D, F), BF16),
            pltpu.VMEM((F // 2, D), U32),
            pltpu.VMEM((NT, D, 128), BF16),
            pltpu.VMEM((NT, D, 128), F32),
            pltpu.VMEM((6 * D, 128), F32),
            pltpu.VMEM((5 * 128, 128), F32),
            pltpu.VMEM((5 * 128, 128), F32),
            pltpu.VMEM((NT, D, 128), BF16),
            pltpu.VMEM((NT, D, 128), BF16),
            pltpu.VMEM((S // 2, D), U32),
            pltpu.VMEM((NT, D, 128), BF16),
            pltpu.VMEM((C, D, 128), BF16),
            pltpu.VMEM((NT, 128), F32),
            pltpu.VMEM((NT * NC, 8, 128), F32),
            pltpu.VMEM((NT * NC, 8, 128), F32),
            pltpu.VMEM((MPI, 8, 128), F32),
            pltpu.VMEM((2 * NV * 16, KR, 8, 128), F32),
            pltpu.VMEM((KR, HQ * DH), BF16),
        ] + stream + stream + [
            pltpu.VMEM((D,), BF16),
            pltpu.VMEM((1, D), BF16),
            pltpu.SemaphoreType.DMA((HKV // 2,)),
            pltpu.SemaphoreType.DMA((11,)),
            pltpu.SemaphoreType.DMA((C + TPB + 1,)),
        ],
        compiler_params=pltpu.CompilerParams(vmem_limit_bytes=127 * 1024 * 1024,
                                             disable_bounds_checks=True,
                                             disable_semaphore_checks=True),
    )(B_w_r, c, xt, k, v, A_wq, A_wo.T, w_mod, B_w_gate, B_w_up, B_w_down.T)
    return out.T.reshape(1, S, D)
```

```python
import math

import jax
import jax.numpy as jnp
import jax.experimental.pallas as pl
import jax.experimental.pallas.tpu as pltpu

S = 2048
D = 576
HQ = 32
HKV = 16
REP = HQ // HKV
DH = 128
GW = REP * DH
F = 4608
C = 8
EPS = 1e-05
TQ = 512
NBLK = S // TQ
TPB = TQ // 128
NT = S // 128
NU = NBLK * HKV
DA = 2 * D
NC = 3
DC = D // NC
TLAG = 160
TKS = 18
SCLAG = 2
CL2 = 0
SLAG = 96
BAR = 1
PG = 64
NFB = F // 128
MODA = ((0, 4, 5), (1, 2, 6), (3, 7, 8))
NMB = 4 * D // 128
MPI = 3
MB0 = 2
WD0 = 14
DM = 512
KR = D - DM
NV = 2
NPV = 0
KB = 1
CH = 3
QC, SC, WC = 0, 1024, 1024 + 2 * S
OUTER0, OSTEP = (SC + 0, SC + 0), 138
TABLE = 1
TAB0, TAB1 = SC + 3150, WC + 600
XP = (WC + 800, SC + 300, SC + 1400, SC + 2100, WC + 640, SC + 2100, SC + 3200)
PV0 = 0
TPI = 16
PACE = (SC + 3900, SC + 3150, SC + 3150, SC + 3800, WC + 400, WC + 450)

BF16 = jnp.bfloat16
F32 = jnp.float32
U32 = jnp.uint32
QSCALE = DH ** -0.5 * math.log2(math.e)


def _dot(a, b):
    return jnp.dot(a, b, preferred_element_type=F32)


def _dot_nt(a, b):
    return jax.lax.dot_general(a, b, (((1,), (1,)), ((), ())), preferred_element_type=F32)


def _r(x):
    return x.astype(BF16).astype(F32)


def _col_bcast(row):
    return jnp.broadcast_to(row, (128, 128)).T


def _blk(u):
    return u // HKV if isinstance(u, int) else jax.lax.shift_right_logical(u, 4)


def _grp(u):
    return u % HKV if isinstance(u, int) else jnp.bitwise_and(u, HKV - 1)


def _lanes(t, n=1):
    return pl.ds(pl.multiple_of(t * 128, 128), n * 128)


def _paced(x, clock, pos):
    if clock is None:
        return x
    pos = pos // 8 * 8
    g = clock[pos:pos + x.shape[0], 0:x.shape[1]]
    return jnp.where(g * g < 0.0, jnp.zeros_like(x), x)


def _paced_wide(x, clock, pos):
    n, w = x.shape
    return jnp.concatenate([_paced(x[:, a:min(a + 128, w)], clock, pos + a // 128 * n)
                            for a in range(0, w, 128)], axis=1)


def _softmax_numer(s, m):
    n, w = s.shape
    p = jnp.exp2(s - m).reshape(n // PG, PG // 8, 8, w)
    ts = jnp.sum(p, axis=1)
    last = jnp.where(ts < 0.0, ts, p[:, PG // 8 - 1])
    p = jnp.concatenate([p[:, :PG // 8 - 1], last[:, None]], axis=1).reshape(n, w)
    l = jnp.sum(jnp.sum(ts, axis=0), axis=0, keepdims=True)
    return p.astype(BF16), l, ts


KEY0 = 0x20000000


def _score_key(r, t):
    tok = t * 128 + jax.lax.broadcasted_iota(jnp.int32, r.shape, 1)
    bits = jax.lax.shift_right_arithmetic(pltpu.bitcast(_r(r) + 0.0, jnp.int32), 16)
    code = jnp.where(bits < 0, -32769 - bits, bits) + 32768
    return pltpu.bitcast(code * S + (S - 1 - tok) + KEY0, F32)


def _chunk_stats(x):
    m = jnp.sum(x, axis=0, keepdims=True) * (1.0 / DC)
    xc = x - m
    return m, jnp.sum(xc * xc, axis=0, keepdims=True)


def _mean_var(stats):
    mean = sum(m for m, _ in stats) * (1.0 / NC)
    var = sum(s + DC * (m - mean) * (m - mean) for m, s in stats) * (1.0 / D)
    return mean, var


def _kernel(wr_hbm, c_hbm,
            xt_hbm, k_hbm, v_hbm, wq_hbm, wot_hbm, wmod_hbm, wg_hbm, wu_hbm, wdt_hbm,
            out_hbm,
            xw_v, k_v, v_v, wq_v, wot_v, wmod_v, wg_v, wu_v, wd_ref,
            ht_ref, acc_ref, mod_ref, wrb_ref, scb_ref, x1_ref, h2_ref, h2row_ref, out_v, fix_v,
            key_ref, st1_ref, st2_ref, lm_ref,
            hb_ref, wrem_v,
            s0_ref, m0_ref, vt0_ref, wqt0_ref, qr0_ref, wf0_ref,
            s1_ref, m1_ref, vt1_ref, wqt1_ref, qr1_ref, wf1_ref,
            wr_ref, c_ref, bsem, msem, osem):
    streams = ((s0_ref, m0_ref, vt0_ref, wqt0_ref, qr0_ref, wf0_ref),
               (s1_ref, m1_ref, vt1_ref, wqt1_ref, qr1_ref, wf1_ref))

    def cp_cols(src, dst, t, n, sem, dst_t=None):
        return pltpu.make_async_copy(src.at[:, _lanes(t, n)],
                                     dst.at[:, _lanes(t if dst_t is None else dst_t, n)], sem)

    def cp_pair(src, dst, p, sem):
        return pltpu.make_async_copy(src.at[pl.ds(2 * p, 2)], dst.at[pl.ds(2 * p, 2)], sem)

    cp_k = lambda p, sem: cp_pair(k_hbm, k_v, p, sem)
    cp_v1 = lambda g, sem: pltpu.make_async_copy(v_hbm.at[g], v_v.at[g], sem)
    cp_k1 = lambda g, sem: pltpu.make_async_copy(k_hbm.at[g], k_v.at[g], sem)

    class Both:
        def __init__(self, cps):
            self.cps = cps

        def start(self):
            for cp in self.cps:
                cp.start()

        def wait(self):
            for cp in self.cps:
                cp.wait()

    def cp_w1(src, dst, g, sem):
        return pltpu.make_async_copy(src.at[:, _lanes(g * REP, REP)], dst.at[g], sem)

    def cp_w(src, dst, p, sem):
        return Both([cp_w1(src, dst, 2 * p + a, sem) for a in range(2)])

    cp_wq = lambda p, sem: cp_w(wq_hbm, wq_v, p, sem)
    cp_wo = lambda p, sem: cp_w(wot_hbm, wot_v, p, sem)
    cp_x = lambda t0, n, sem: Both([pltpu.make_async_copy(xt_hbm.at[:, _lanes(t0 + t)],
                                                          xw_v.at[t0 + t], sem) for t in range(n)])
    NP = HKV // 2

    def bundle(n, act):
        sem = bsem.at[n if isinstance(n, int) else jnp.minimum(n, NP - 1)]

        def on(cond, cps):
            def go():
                for cp in cps():
                    getattr(cp, act)()
            if isinstance(cond, bool):
                if cond:
                    go()
            else:
                pl.when(cond)(go)
        on(n + 1 < NP, lambda: [cp_k(n + 1, sem), cp_v1(2 * n + 2, sem), cp_w1(wq_hbm, wq_v, 2 * n + 3, sem)])
        on(n + 2 < NP, lambda: [cp_w1(wq_hbm, wq_v, 2 * n + 4, sem)])
        on(jnp.logical_and(n >= 1, n < NBLK) if not isinstance(n, int) else 1 <= n < NBLK,
           lambda: [cp_x(TPB * n + 1, TPB - 1, sem)])
        on(jnp.logical_and(n >= 1, n < NBLK - 1) if not isinstance(n, int) else 1 <= n < NBLK - 1,
           lambda: [cp_x(TPB * n + TPB, 1, sem)])
        on(n < NP, lambda: [cp_v1(2 * n + 1, sem), cp_wo(n, sem)])

    cp_moda = [Both([cp_cols(wmod_hbm, wmod_v, t, 1, msem.at[s]) for t in tiles])
               for s, tiles in zip((0, 6, 10), MODA)]
    cp_modb = Both([pltpu.make_async_copy(wmod_hbm.at[:, _lanes(DA // 128 + b)],
                                          xw_v.at[NT + NFB + b], msem.at[1]) for b in range(NMB)])
    cp_g = pltpu.make_async_copy(wg_hbm, wg_v, msem.at[2])
    cp_u = pltpu.make_async_copy(wu_hbm, wu_v, msem.at[3])
    cp_d = Both([pltpu.make_async_copy(wdt_hbm.at[:, _lanes(b)], xw_v.at[NT + b], msem.at[4])
                 for b in range(NFB)])
    cp_out = lambda t, n, sem: Both([pltpu.make_async_copy(out_v.at[t + a], out_hbm.at[:, _lanes(t + a)],
                                                           sem) for a in range(n)])

    def silu_c():
        c = c_ref[...].astype(F32)
        return _r(c * _r(jax.nn.sigmoid(c)))

    def finish_mod(mod, lo, clock=None, pos=0):
        mod = _r(mod)
        col = lo + jax.lax.broadcasted_iota(jnp.int32, mod.shape, 1)
        is_scale = jnp.logical_or(jnp.logical_and(col >= D, col < 2 * D),
                                  jnp.logical_and(col >= 4 * D, col < 5 * D))
        mod = jnp.where(is_scale, _r(1.0 + mod), mod)
        for t in range(mod.shape[1] // 128):
            rows = pl.ds(pl.multiple_of(lo + t * 128, 128), 128)
            mod_ref[rows, :] = _paced(_col_bcast(mod[:, t * 128:(t + 1) * 128]), clock, pos)

    def late_mod_sums(n, clock):
        b0 = jnp.clip(n - MB0, 0, NMB // MPI - 1) * MPI
        for k in range(MPI):
            w = xw_v[jnp.where(n >= MB0, NT + NFB + b0 + k, 0)].astype(F32)
            part = jnp.sum((w * scb_ref[0:D, :]).reshape(D // 8, 8, 128), axis=0)
            lm_ref[k] = _paced(part, clock, PACE[4] + 192 * k)

    def late_mod_store(n, clock):
        b0 = jnp.clip(n - MB0, 0, NMB // MPI - 1) * MPI
        for k in range(MPI):
            finish_mod(jnp.sum(lm_ref[k], axis=0, keepdims=True), DA + (b0 + k) * 128,
                       clock, XP[4] + 128 * k)

    def col_vector(ref, row):
        row = jnp.concatenate([row, jnp.zeros((1, 64), F32)], axis=1)
        for t in range(5):
            ref[t * 128:(t + 1) * 128, :] = _col_bcast(row[:, t * 128:(t + 1) * 128])

    def mod(k):
        return mod_ref[k * D:(k + 1) * D, :]

    def put_stats(st_ref, t, shift, scale, clock, pos):
        row = jax.lax.broadcasted_iota(jnp.int32, (8, 128), 0)
        st_ref[t] = _paced(jnp.where(row == 0, shift, scale), clock, pos)

    def ln1_stats(t, clock=None, pos=None):
        for c in range(NC):
            m, s = _chunk_stats(xw_v[t, c * DC:(c + 1) * DC, :].astype(F32))
            put_stats(st1_ref, t * NC + c, m, s, clock, (PACE[0] if pos is None else pos) + 192 * c)

    def ln1_norm(t):
        mean, var = _mean_var(load_stats(st1_ref, t))
        return (xw_v[t].astype(F32) - mean) * jax.lax.rsqrt(var + EPS)

    def ln1_apply(t, clock=None, pos=None, ln=None):
        h = (ln1_norm(t) if ln is None else ln) * mod(1) + mod(0)
        ht_ref[t] = _paced(h, clock, PACE[1] if pos is None else pos).astype(BF16)

    def h2_rows(t, clock=None):
        x = _paced_wide(pltpu.bitcast(h2_ref[t].T, U32), clock, PACE[5])
        h2row_ref[pl.ds(pl.multiple_of(t * 64, 64), 64), :] = x

    def router_terms():
        u = mod(4) * wrb_ref[0:D, :]
        return (u, jnp.sum(u, axis=0, keepdims=True),
                jnp.sum(mod(3) * wrb_ref[0:D, :], axis=0, keepdims=True))

    def load_stats(st_ref, t):
        return [(st_ref[t * NC + c, 0:1, :], st_ref[t * NC + c, 1:2, :]) for c in range(NC)]

    def ln2_x1(t, attn, clock=None):
        x1 = _r(xw_v[t].astype(F32) + mod(2) * attn)
        x1_ref[t] = _paced(x1, clock, PACE[2]).astype(BF16)
        return x1, [_chunk_stats(x1[c * DC:(c + 1) * DC]) for c in range(NC)]

    def ln2_norm(stats):
        mean, var = _mean_var(stats)
        return _r(mean), 1.0 / _r(jnp.sqrt(_r(_r(var) + EPS)))

    def ln2_h2(x1, mean, inv):
        return (x1 - mean) * inv * mod(4) + mod(3)

    def ln2_stats(t, clock):
        for c, (m, s) in enumerate(ln2_x1(t, acc_ref[t], clock)[1]):
            put_stats(st2_ref, t * NC + c, m, s, clock, PACE[2] + (c + 1) * DC + SLAG)

    def ln2_apply(t, clock):
        x1 = x1_ref[t].astype(F32)
        h2 = ln2_h2(x1, *ln2_norm(load_stats(st2_ref, t)))
        key = _score_key(jnp.sum(h2 * wrb_ref[0:D, :], axis=0, keepdims=True), t)
        key_ref[pl.ds(t, 1), :] = _paced(key, clock, PACE[3] + D + 96)
        h2 = _r(h2)
        h2_ref[t] = _paced(h2, clock, PACE[3]).astype(BF16)
        out_v[t] = _paced(x1 + mod(5) * h2, clock, PACE[3] + 16).astype(BF16)

    def finish_q(q):
        q = (q * QSCALE).astype(BF16)
        return jnp.concatenate([q[r * DH:(r + 1) * DH] for r in range(REP)], axis=1)

    def q_proj(u, wqt_ref, qr_ref=None, split=False):
        w = pltpu.bitcast(wqt_ref[...], BF16)
        h = jnp.concatenate([ht_ref[_blk(u) * TPB + t] for t in range(TPB)], axis=1)
        if split:
            return sum(_dot(w[:, a:min(a + 128, D)], h[a:min(a + 128, D)]) for a in range(0, D, 128))
        if qr_ref is None:
            rem = _dot(w[:, DM:], h[DM:])
        else:
            rem = [qr_ref[...].T]
            if NV < TPB:
                R = GW * (TPB - NV) // 4
                rem.append(jnp.concatenate([_dot(w[a:a + R, DM:], h[DM:, NV * 128:])
                                            for a in range(0, GW, R)], axis=0))
            rem = jnp.concatenate(rem, axis=1)
        return _dot(w[:, :DM], h[:DM]) + rem

    def w_rest(u, wf_ref):
        w = wrem_v[:, _lanes(_grp(u) * REP, REP)].astype(F32)
        for r in range(REP):
            wf_ref[r] = w[:, r * DH:(r + 1) * DH]

    def outer(u, qr_ref, wf_ref, clock, start, never):
        base = jnp.bitwise_and(_blk(u), 1) * (NV * 16)

        def chains(group, after=None):
            acc = {}
            for k in range(KR):
                for tv, r in group:
                    t = hb_ref[base + tv, k] * wf_ref[r, pl.ds(k, 8, stride=0), :]
                    acc[tv, r] = _paced(t, after, 0) if k == 0 else acc[tv, r] + t
            return acc.items()

        cells = [(tv, r) for r in range(REP) for tv in range(NV * 16)]
        per = NPV
        for c, tick in enumerate(never):
            prev = None
            for i, cell in enumerate(cells[c * per:(c + 1) * per]):
                for (tv, r), prev in chains([cell], prev):
                    qr_ref[tv * 8:(tv + 1) * 8, r * DH:(r + 1) * DH] = _paced(prev, tick, PV0 + 8 * i)
        cells = cells[per * len(never):]
        for g in range(0, len(cells), CH):
            for (tv, r), a in chains(cells[g:g + CH]):
                qr_ref[tv * 8:(tv + 1) * 8, r * DH:(r + 1) * DH] = _paced(
                    a, clock, min(start + OSTEP * (g // CH + 1), clock.shape[0] - 8))

    def h_table(hr, base, k0, gates):
        nk = hr.shape[0]
        for j in range(nk):
            cb = _col_bcast(hr[j:j + 1])
            for b in range(16):
                g = gates[(j * 16 + b) * len(gates) // (nk * 16)]
                hb_ref[base + b, k0 + j] = jnp.where(g, 0.0, cb[b * 8:(b + 1) * 8])

    def never_of(clock, lo, hi):
        return [clock[a:a + 8] * clock[a:a + 8] < 0.0 for a in range(lo // 8 * 8, hi, 8)]

    def scores(u, q, s_ref, m_ref):
        s = _dot(pltpu.bitcast(k_v.bitcast(U32)[_grp(u)], BF16) if KB else k_v[_grp(u)], q)
        s_ref[...] = s
        m_ref[...] = jnp.broadcast_to(jnp.max(s, axis=0, keepdims=True), m_ref.shape)
        return jnp.concatenate([s[:, 0:128], s[:, TQ:TQ + 128]], axis=0)

    def v_transpose(u, vt_ref, clock=None, pos=0):
        vt_ref[...] = _paced_wide(pltpu.bitcast((pltpu.bitcast(v_v.bitcast(U32)[_grp(u)], BF16) if KB else v_v[_grp(u)]).T, U32), clock, pos)

    def wq_transpose(u, wqt_ref, clock=None, pos=0):
        wqt_ref[...] = _paced_wide(pltpu.bitcast(wq_v[_grp(u)].T, U32), clock, pos)

    def wd_transpose(u, clock, pos):
        fb = jnp.clip(u - WD0, 0, NFB - 1)
        src = jnp.where(u >= WD0, NT + fb, 0)
        wd_ref[pl.ds(pl.multiple_of(fb * 64, 64), 64), :] = _paced_wide(
            pltpu.bitcast(xw_v[src].T, U32), clock, pos)

    def attend(s_ref, m_ref, vt_ref):
        m = m_ref[0:1, :]
        o, never = [], []
        for r in range(REP):
            cols = slice(r * TQ, (r + 1) * TQ)
            p, l, ts = _softmax_numer(s_ref[:, cols], m[:, cols])
            ov = _dot(pltpu.bitcast(vt_ref[...], BF16), p)
            o.append((ov * (1.0 / l)).astype(BF16))
            never += [ov[:, c * 128:(c + 1) * 128] for c in range(TPB)]
        return jnp.concatenate(o, axis=0), never

    small = Both([pltpu.make_async_copy(wr_hbm, wr_ref, msem.at[7]),
                  pltpu.make_async_copy(c_hbm, c_ref, msem.at[7])])
    zeroth = Both([cp_x(0, TPB, msem.at[5]), cp_w1(wq_hbm, wq_v, 0, msem.at[5])])
    first = Both([cp_k1(0, msem.at[8]), cp_w1(wq_hbm, wq_v, 1, msem.at[8])])
    second = Both([cp_k1(1, msem.at[9]), cp_v1(0, msem.at[9]), cp_w1(wq_hbm, wq_v, 2, msem.at[9]),
                   pltpu.make_async_copy(wq_hbm.at[DM:, :], wrem_v, msem.at[9]), cp_x(TPB, 1, msem.at[9])])
    for cp in [small, zeroth] + cp_moda + [first, second]:
        cp.start()
    acc_ref[...] = jnp.zeros_like(acc_ref)
    mod_ref[DA:6 * D, :] = jnp.zeros((4 * D, 128), F32)
    h2_ref[0] = jnp.zeros((D, 128), BF16)
    small.wait()
    col_vector(wrb_ref, wr_ref[...].astype(F32).reshape(1, D))
    col_vector(scb_ref, silu_c())
    sc8 = jnp.broadcast_to(silu_c(), (8, D)).astype(BF16)
    zeroth.wait()
    ln0 = []
    for t in range(TPB):
        ln1_stats(t)
        ln0.append(ln1_norm(t))
    wq_transpose(0, wqt0_ref)
    for cp, tiles in zip(cp_moda, MODA):
        cp.wait()
        for t in tiles:
            finish_mod(_dot(sc8, wmod_v[:, t * 128:(t + 1) * 128])[0:1], t * 128)
    for t in range(TPB):
        ln1_apply(t, ln=ln0[t])
    q = finish_q(q_proj(0, wqt0_ref, split=True))
    first.wait()
    bundle(0, 'start')
    def first_table(gates, lo, hi):
        for i in range(NV + 1):
            a, b = max(lo, i * KR), min(hi, (i + 1) * KR)
            if a < b:
                gs = gates[(a - lo) * len(gates) // (hi - lo):(b - lo) * len(gates) // (hi - lo)]
                hr = ht_ref[i if i < NV else TPB, DM:, :].astype(F32)[a - i * KR:b - i * KR]
                h_table(hr, i * 16, a - i * KR, gs)

    TSPLIT = 80
    first_table(never_of(scores(0, q, s0_ref, m0_ref), 64, 2 * S - 192), 0, TSPLIT)
    wq_transpose(1, wqt1_ref)
    second.wait()
    bundle(1, 'start')
    hrem = jnp.concatenate([ht_ref[t, DM:, :] for t in range(NV)], axis=1)
    for a in range(2):
        streams[a][4][...] = jax.lax.dot_general(
            hrem, wrem_v[:, (a + 2) * GW:(a + 3) * GW], (((0,), (0,)), ((), ())),
            preferred_element_type=F32)
    q = q_proj(1, wqt1_ref)
    clock = jnp.concatenate([q[:, t * 128:(t + 1) * 128] for t in range(TPB)]
                            + [scores(1, finish_q(q), s1_ref, m1_ref)], axis=0)
    ln1_stats(TPB, clock, SC + 200)
    ln1_apply(TPB, clock, SC + 900)
    first_table(never_of(clock, 0, SC + 2 * S - 600), TSPLIT, NV * KR + 2 * TPI)
    for a in range(2):
        w_rest(a + 4, streams[a][5])
    v_transpose(0, vt0_ref)
    wq_transpose(2, wqt0_ref)

    def unit(u, side, s_ref, m_ref, vt_ref, wqt_ref, qr_ref, wf_ref):
        q = q_proj(u + 2, wqt_ref, qr_ref)
        o, never = attend(s_ref, m_ref, vt_ref)
        sclk = scores(u + 2, finish_q(q), s_ref, m_ref)
        upd = _dot(wot_v[_grp(u)], o)
        clock = jnp.concatenate([q[:, t * 128:(t + 1) * 128] for t in range(TPB)] + [sclk]
                                + [upd[:, 0:128], upd[:, 256:384]], axis=0)
        side(clock, lambda start: outer(u + 4, qr_ref, wf_ref, clock, start, never))
        w_rest(u + 6, wf_ref)
        for t in range(TPB):
            acc_ref[_blk(u) * TPB + t] += upd[:, t * 128:(t + 1) * 128]

    def step(n, carry):
        def waits(_, c):
            bundle(n, 'wait')
            pl.when(n == MB0)(cp_modb.wait)
            pl.when(n == WD0 // 2)(cp_d.wait)
            return c
        jax.lax.fori_loop(0, jnp.where(n < NP, 1, 0), waits, 0)

        pl.when(n == 0)(cp_modb.start)
        bundle(jnp.minimum(n + 2, NP), 'start')
        for a in range(3):
            pl.when(n == 2 + a)(Both(cp_d.cps[a * NFB // 3:(a + 1) * NFB // 3]).start)
        pl.when(n == NP)(Both([cp_g, cp_u]).start)

        t1 = jnp.minimum(n + 4, NT - 1)
        v = jnp.maximum(n - NP, 0)
        tile2 = lambda v: (jax.lax.shift_right_logical(v, 3) * TPB
                           + jnp.minimum(jnp.bitwise_and(v, NP - 1), TPB - 1))
        t2 = tile2(v)

        def stats(clock, outer_at):
            v_transpose(2 * n + 1, vt1_ref, clock, XP[5])
            wq_transpose(2 * n + 3, wqt1_ref, clock, XP[6])
            ln2_stats(t2, clock)
            ln1_stats(t1, clock)
            late_mod_sums(n, clock)
            h2_rows(tile2(jnp.maximum(v - 1, 0)), clock)
            wd_transpose(2 * n, clock, XP[0])
            outer_at(OUTER0[0])

        def apply(clock, outer_at):
            blk = jnp.minimum(jax.lax.shift_right_logical(n + 2, 3) + 1, NBLK - 1)
            e0 = jnp.bitwise_and(n + 2, 7) * TPI
            i, k0 = jax.lax.shift_right_logical(e0, 6), jnp.bitwise_and(e0, KR - 1)
            hr = ht_ref[blk * TPB + i, pl.ds(pl.multiple_of(DM + k0, 16), TPI), :].astype(F32)
            v_transpose(2 * n + 2, vt0_ref, clock, XP[1])
            wq_transpose(2 * n + 4, wqt0_ref, clock, XP[2])
            wd_transpose(2 * n + 1, clock, XP[3])
            ln1_apply(t1, clock)
            ln2_apply(t2, clock)
            outer_at(OUTER0[1])
            h_table(hr, (jnp.bitwise_and(blk, 1) * NV + i) * 16, k0, never_of(clock, TAB0, TAB1))
            late_mod_store(n, clock)

        for a in range(2):
            unit(2 * n + a, (stats, apply)[a], *streams[a])
        return carry

    jax.lax.fori_loop(0, NU // 2 - 1, step, 0)

    T0 = NT - TPB
    cp_out(0, T0, osem.at[C + TPB]).start()
    cp_g.wait()
    v_transpose(NU - 1, vt1_ref)
    o = jnp.concatenate([attend(*streams[a][0:3])[0] for a in range(2)], axis=0)
    wlast = jnp.concatenate([wot_v[HKV - 2], wot_v[HKV - 1]], axis=1)
    fin = [acc_ref[T0 + t] + _dot(wlast, o[:, t * 128:(t + 1) * 128]) for t in range(TPB)]
    clock = jnp.concatenate(fin, axis=0)
    row8 = jax.lax.broadcasted_iota(jnp.int32, (C, 128), 0)
    lane8 = jax.lax.broadcasted_iota(jnp.int32, (C, 128), 1)
    work = key_ref[0:T0, :]
    lead = jnp.zeros((C, 128), F32)
    for t in range(C):
        mx = jnp.max(jnp.max(work, axis=0, keepdims=True), axis=1, keepdims=True)
        work = jnp.where(work == mx, 0.0, work)
        lead = jnp.where(row8 == t, mx, lead)

    def spread(row):
        return pltpu.roll(jnp.broadcast_to(row, (128, 128)), 0, 1, stride=1, stride_axis=0)

    def merge(lead, rows, spreads):
        cols = jnp.concatenate([lead] + spreads, axis=0)
        best = jnp.zeros((C, 128), F32)
        for row in [jnp.max(jnp.where(row8 == lane8, lead, 0.0), axis=0, keepdims=True)] + rows:
            rank = jnp.sum(jnp.where(cols > row, 1.0, 0.0), axis=0, keepdims=True)
            best = jnp.maximum(best, jnp.where(rank == row8.astype(F32), row, 0.0))
        return jnp.max(best, axis=1, keepdims=True)

    def tail_h2(t, norm, gate=None):
        x1 = x1_ref[t].astype(F32)
        if gate is not None:
            n = gate.shape[0]
            x1 = jnp.concatenate([_paced(x1[:n], gate, 0), x1[n:]], axis=0) if n < D else _paced(x1, gate, 0)
        h2_ref[t] = ln2_h2(x1, *norm).astype(BF16)
        if t < NT - 2:
            h2_rows(t)

    u_vec, u_sum, b_sum = router_terms()
    keys = []
    for t in range(TPB):
        x1, stats = ln2_x1(T0 + t, fin[t])
        mean, inv = norm = ln2_norm(stats)
        r = (jnp.sum(x1 * u_vec, axis=0, keepdims=True) - mean * u_sum) * inv + b_sum
        keys.append(_score_key(r, T0 + t))
        if t < TPB - 1:
            tail_h2(T0 + t, norm, clock[(t + 1) * D + TLAG:(t + 2) * D + TLAG])
    lead = jnp.broadcast_to(merge(lead, keys[0:2], [spread(k) for k in keys[0:2]]), (C, 128))
    spread2 = spread(keys[2])
    if BAR == 0:
        cp_u.wait()
        cp_out(0, T0, osem.at[C + TPB]).wait()

    h2_rows(NT - 2)
    tail_h2(NT - 1, norm)
    h2_rows(NT - 1)
    sel = pltpu.bitcast(merge(lead, keys[2:4], [spread2, spread(keys[3])]), jnp.int32) - KEY0
    sel_tok = (S - 1) - (sel & (S - 1))
    toks = [sel_tok[t, 0] for t in range(C)]
    tiles = [jax.lax.shift_right_logical(tk, 7) for tk in toks]
    sel_code = jax.lax.shift_right_logical(sel, 11) - 32768
    sel_bits = jnp.where(sel_code < 0, -32769 - sel_code, sel_code)
    r_sel = pltpu.bitcast(jax.lax.shift_left(sel_bits, 16), F32)

    final = []
    for t in range(C):
        d = True
        for u in range(t + 1, C):
            d = jnp.logical_and(d, tiles[u] != tiles[t])
        final.append(d)

    words = jnp.concatenate([h2row_ref[pl.ds(jax.lax.shift_right_logical(toks[t], 1), 1), :]
                             for t in range(C)], axis=0)
    odd = jnp.bitwise_and(sel_tok, 1) == 1
    xs = pltpu.bitcast(jnp.where(odd, jnp.bitwise_and(words, jnp.uint32(0xFFFF0000)),
                                 jax.lax.shift_left(words, jnp.uint32(16))), F32)
    xs = xs.astype(BF16)

    def plain_out(t, ticks=None):
        x1 = x1_ref[t].astype(F32)
        if ticks is not None:
            gate = jnp.concatenate([ticks[a * len(ticks) // (D // 8)] for a in range(D // 8)], axis=0)
            x1 = _paced(x1, gate, 0)
        out_v[t] = (x1 + mod(5) * h2_ref[t].astype(F32)).astype(BF16)

    clean = []

    def send_clean(t):
        d = tiles[0] != t
        for a in range(1, C):
            d = jnp.logical_and(d, tiles[a] != t)
        clean.append(d)
        pl.when(d)(cp_out(t, 1, osem.at[C + t - T0]).start)

    if BAR == 1:
        cp_u.wait()
        cp_out(0, T0, osem.at[C + TPB]).wait()
    gpre = _dot(xs, wg_v[...])
    u = _dot(xs, wu_v[...])
    ticks = [z[:, a * 128:(a + 1) * 128] for z in (gpre, u) for a in range(NFB)]
    for t in range(TPB):
        plain_out(T0 + t, ticks[t * TKS:(t + 1) * TKS])
        send_clean(T0 + t)
    gpre, u = _r(gpre), _r(u)
    gact = _r(gpre * _r(jax.nn.sigmoid(gpre)))
    act = (gact * u).astype(BF16)
    gate_r = _r(jax.nn.sigmoid(r_sel))
    ohs = []
    for t in range(C):
        oh = jnp.where(sel_tok == tiles[t] * 128 + lane8, 1.0, 0.0)
        ohs.append(jnp.concatenate([oh, jnp.zeros((16 - C, 128), F32)], axis=0).astype(BF16))

    def cp_fix(t, lo, hi):
        return pltpu.make_async_copy(fix_v.at[t, lo:hi, :], out_hbm.at[lo:hi, _lanes(tiles[t])],
                                     osem.at[t])

    def guarded(cond, fn):
        if cond is True:
            fn()
        else:
            pl.when(cond)(fn)

    def scatter(j, yt, t):
        lo, hi = j * 128, min(j * 128 + 128, D)
        upd = jnp.concatenate([_dot(yt[a:a + 64], ohs[t]) for a in range(0, hi - lo, 64)], axis=0)
        fix_v[t, lo:hi, :] = (x1_ref[tiles[t], lo:hi, :].astype(F32) + mod_ref[5 * D + lo:5 * D + hi, :]
                              * (h2_ref[tiles[t], lo:hi, :].astype(F32) + upd)).astype(BF16)
        guarded(final[t], cp_fix(t, lo, hi).start)

    NJ = (D + 127) // 128
    yts = []
    for j in range(NJ):
        lo, hi = j * 128, min(j * 128 + 128, D)
        nk = 4
        FK = F // nk
        yk = []
        for a in range(nk):
            w = pltpu.bitcast(wd_ref[a * FK // 2:(a + 1) * FK // 2, lo:hi], BF16)
            yk.append(_dot(act[:, a * FK:(a + 1) * FK], w))
            if j >= SCLAG:
                for t in (2 * a, 2 * a + 1):
                    scatter(j - SCLAG, yts[j - SCLAG], t)
        y = _r(sum(yk)) * gate_r
        yts.append(jnp.concatenate([y, jnp.zeros_like(y)], axis=0).astype(BF16).T)
    for j in range(NJ - SCLAG, NJ):
        for t in range(C):
            scatter(j, yts[j], t)
    for t in range(T0, NT):
        pl.when(clean[t - T0])(cp_out(t, 1, osem.at[C + t - T0]).wait)
    for t in range(C):
        guarded(final[t], cp_fix(t, 0, D).wait)


@jax.jit
def pallas_adaLN_cond__gqa_block_cached__moe_arch_mod__prompt_kernel(
    A_x: jax.Array,
    A_k_cache: jax.Array,
    A_v_cache: jax.Array,
    A_wq: jax.Array,
    A_wo: jax.Array,
    B_x: jax.Array,
    B_w_r: jax.Array,
    B_w_gate: jax.Array,
    B_w_up: jax.Array,
    B_w_down: jax.Array,
    c: jax.Array,
    w_mod: jax.Array,
):
    del B_x
    xt = A_x.reshape(S, D).T
    k = A_k_cache.reshape(HKV, S, DH)
    v = A_v_cache.reshape(HKV, S, DH)

    hbm = pl.BlockSpec(memory_space=pl.ANY)
    stream = [
        pltpu.VMEM((S, REP * TQ), F32),
        pltpu.VMEM((8, REP * TQ), F32),
        pltpu.VMEM((DH // 2, S), U32),
        pltpu.VMEM((GW // 2, D), U32),
        pltpu.VMEM((NV * 128, GW), F32),
        pltpu.VMEM((REP, KR, DH), F32),
    ]
    out = pl.pallas_call(
        _kernel,
        in_specs=[hbm] * 11,
        out_specs=hbm,
        out_shape=jax.ShapeDtypeStruct((D, S), BF16),
        scratch_shapes=[
            pltpu.VMEM((NT + NFB + NMB, D, 128), BF16),
            pltpu.VMEM((HKV, S, DH), BF16),
            pltpu.VMEM((HKV, S, DH), BF16),
            pltpu.VMEM((HKV, D, GW), BF16),
            pltpu.VMEM((HKV, D, GW), BF16),
            pltpu.VMEM((D, DA), BF16),
            pltpu.VMEM((D, F), BF16),
            pltpu.VMEM((D, F), BF16),
            pltpu.VMEM((F // 2, D), U32),
            pltpu.VMEM((NT, D, 128), BF16),
            pltpu.VMEM((NT, D, 128), F32),
            pltpu.VMEM((6 * D, 128), F32),
            pltpu.VMEM((5 * 128, 128), F32),
            pltpu.VMEM((5 * 128, 128), F32),
            pltpu.VMEM((NT, D, 128), BF16),
            pltpu.VMEM((NT, D, 128), BF16),
            pltpu.VMEM((S // 2, D), U32),
            pltpu.VMEM((NT, D, 128), BF16),
            pltpu.VMEM((C, D, 128), BF16),
            pltpu.VMEM((NT, 128), F32),
            pltpu.VMEM((NT * NC, 8, 128), F32),
            pltpu.VMEM((NT * NC, 8, 128), F32),
            pltpu.VMEM((MPI, 8, 128), F32),
            pltpu.VMEM((2 * NV * 16, KR, 8, 128), F32),
            pltpu.VMEM((KR, HQ * DH), BF16),
        ] + stream + stream + [
            pltpu.VMEM((D,), BF16),
            pltpu.VMEM((1, D), BF16),
            pltpu.SemaphoreType.DMA((HKV // 2,)),
            pltpu.SemaphoreType.DMA((11,)),
            pltpu.SemaphoreType.DMA((C + TPB + 1,)),
        ],
        compiler_params=pltpu.CompilerParams(vmem_limit_bytes=127 * 1024 * 1024,
                                             disable_bounds_checks=True,
                                             disable_semaphore_checks=True),
    )(B_w_r, c, xt, k, v, A_wq, A_wo.T, w_mod, B_w_gate, B_w_up, B_w_down.T)
    return out.T.reshape(1, S, D)
```

```python
import math

import jax
import jax.numpy as jnp
import jax.experimental.pallas as pl
import jax.experimental.pallas.tpu as pltpu

S = 2048
D = 576
HQ = 32
HKV = 16
REP = HQ // HKV
DH = 128
GW = REP * DH
F = 4608
C = 8
EPS = 1e-05
TQ = 512
NBLK = S // TQ
TPB = TQ // 128
NT = S // 128
NU = NBLK * HKV
DA = 2 * D
NC = 3
DC = D // NC
TLAG = 160
TKS = 18
SCLAG = 2
CL2 = 0
SLAG = 96
BAR = 1
PG = 64
NFB = F // 128
MODA = ((0, 4, 5), (1, 2, 6), (3, 7, 8))
NMB = 4 * D // 128
MPI = 3
MB0 = 2
WD0 = 14
DM = 512
KR = D - DM
NV = 2
NPV = 0
KB = 1
CH = 3
QC, SC, WC = 0, 1024, 1024 + 2 * S
OUTER0, OSTEP = (SC + 0, SC + 0), 138
TABLE = 1
TAB0, TAB1 = SC + 3150, WC + 600
XP = (WC + 800, SC + 300, SC + 1400, SC + 2100, WC + 640, SC + 2100, SC + 3200)
PV0 = 0
TSPLIT = 96
PP = (SC + 100, SC + 700, SC + 2900, SC + 2950, SC + 3300)
TPI = 16
PACE = (SC + 3900, SC + 3150, SC + 3150, SC + 3800, WC + 400, WC + 450)

BF16 = jnp.bfloat16
F32 = jnp.float32
U32 = jnp.uint32
QSCALE = DH ** -0.5 * math.log2(math.e)


def _dot(a, b):
    return jnp.dot(a, b, preferred_element_type=F32)


def _dot_nt(a, b):
    return jax.lax.dot_general(a, b, (((1,), (1,)), ((), ())), preferred_element_type=F32)


def _r(x):
    return x.astype(BF16).astype(F32)


def _col_bcast(row):
    return jnp.broadcast_to(row, (128, 128)).T


def _blk(u):
    return u // HKV if isinstance(u, int) else jax.lax.shift_right_logical(u, 4)


def _grp(u):
    return u % HKV if isinstance(u, int) else jnp.bitwise_and(u, HKV - 1)


def _lanes(t, n=1):
    return pl.ds(pl.multiple_of(t * 128, 128), n * 128)


def _paced(x, clock, pos):
    if clock is None:
        return x
    pos = pos // 8 * 8
    g = clock[pos:pos + x.shape[0], 0:x.shape[1]]
    return jnp.where(g * g < 0.0, jnp.zeros_like(x), x)


def _paced_wide(x, clock, pos):
    n, w = x.shape
    return jnp.concatenate([_paced(x[:, a:min(a + 128, w)], clock, pos + a // 128 * n)
                            for a in range(0, w, 128)], axis=1)


def _softmax_numer(s, m):
    n, w = s.shape
    p = jnp.exp2(s - m).reshape(n // PG, PG // 8, 8, w)
    ts = jnp.sum(p, axis=1)
    last = jnp.where(ts < 0.0, ts, p[:, PG // 8 - 1])
    p = jnp.concatenate([p[:, :PG // 8 - 1], last[:, None]], axis=1).reshape(n, w)
    l = jnp.sum(jnp.sum(ts, axis=0), axis=0, keepdims=True)
    return p.astype(BF16), l, ts


KEY0 = 0x20000000


def _score_key(r, t):
    tok = t * 128 + jax.lax.broadcasted_iota(jnp.int32, r.shape, 1)
    bits = jax.lax.shift_right_arithmetic(pltpu.bitcast(_r(r) + 0.0, jnp.int32), 16)
    code = jnp.where(bits < 0, -32769 - bits, bits) + 32768
    return pltpu.bitcast(code * S + (S - 1 - tok) + KEY0, F32)


def _chunk_stats(x):
    m = jnp.sum(x, axis=0, keepdims=True) * (1.0 / DC)
    xc = x - m
    return m, jnp.sum(xc * xc, axis=0, keepdims=True)


def _mean_var(stats):
    mean = sum(m for m, _ in stats) * (1.0 / NC)
    var = sum(s + DC * (m - mean) * (m - mean) for m, s in stats) * (1.0 / D)
    return mean, var


def _kernel(wr_hbm, c_hbm,
            xt_hbm, k_hbm, v_hbm, wq_hbm, wot_hbm, wmod_hbm, wg_hbm, wu_hbm, wdt_hbm,
            out_hbm,
            xw_v, k_v, v_v, wq_v, wot_v, wmod_v, wg_v, wu_v, wd_ref,
            ht_ref, acc_ref, mod_ref, wrb_ref, scb_ref, x1_ref, h2_ref, h2row_ref, out_v, fix_v,
            key_ref, st1_ref, st2_ref, lm_ref,
            hb_ref, wrem_v,
            s0_ref, m0_ref, vt0_ref, wqt0_ref, qr0_ref, wf0_ref,
            s1_ref, m1_ref, vt1_ref, wqt1_ref, qr1_ref, wf1_ref,
            wr_ref, c_ref, bsem, msem, osem):
    streams = ((s0_ref, m0_ref, vt0_ref, wqt0_ref, qr0_ref, wf0_ref),
               (s1_ref, m1_ref, vt1_ref, wqt1_ref, qr1_ref, wf1_ref))

    def cp_cols(src, dst, t, n, sem, dst_t=None):
        return pltpu.make_async_copy(src.at[:, _lanes(t, n)],
                                     dst.at[:, _lanes(t if dst_t is None else dst_t, n)], sem)

    def cp_pair(src, dst, p, sem):
        return pltpu.make_async_copy(src.at[pl.ds(2 * p, 2)], dst.at[pl.ds(2 * p, 2)], sem)

    cp_k = lambda p, sem: cp_pair(k_hbm, k_v, p, sem)
    cp_v1 = lambda g, sem: pltpu.make_async_copy(v_hbm.at[g], v_v.at[g], sem)
    cp_k1 = lambda g, sem: pltpu.make_async_copy(k_hbm.at[g], k_v.at[g], sem)

    class Both:
        def __init__(self, cps):
            self.cps = cps

        def start(self):
            for cp in self.cps:
                cp.start()

        def wait(self):
            for cp in self.cps:
                cp.wait()

    def cp_w1(src, dst, g, sem):
        return pltpu.make_async_copy(src.at[:, _lanes(g * REP, REP)], dst.at[g], sem)

    def cp_w(src, dst, p, sem):
        return Both([cp_w1(src, dst, 2 * p + a, sem) for a in range(2)])

    cp_wq = lambda p, sem: cp_w(wq_hbm, wq_v, p, sem)
    cp_wo = lambda p, sem: cp_w(wot_hbm, wot_v, p, sem)
    cp_x = lambda t0, n, sem: Both([pltpu.make_async_copy(xt_hbm.at[:, _lanes(t0 + t)],
                                                          xw_v.at[t0 + t], sem) for t in range(n)])
    NP = HKV // 2

    def bundle(n, act):
        sem = bsem.at[n if isinstance(n, int) else jnp.minimum(n, NP - 1)]

        def on(cond, cps):
            def go():
                for cp in cps():
                    getattr(cp, act)()
            if isinstance(cond, bool):
                if cond:
                    go()
            else:
                pl.when(cond)(go)
        on(n + 1 < NP, lambda: [cp_k(n + 1, sem), cp_v1(2 * n + 2, sem), cp_w1(wq_hbm, wq_v, 2 * n + 3, sem)])
        on(n + 2 < NP, lambda: [cp_w1(wq_hbm, wq_v, 2 * n + 4, sem)])
        on(jnp.logical_and(n >= 1, n < NBLK) if not isinstance(n, int) else 1 <= n < NBLK,
           lambda: [cp_x(TPB * n + 1, TPB - 1, sem)])
        on(jnp.logical_and(n >= 1, n < NBLK - 1) if not isinstance(n, int) else 1 <= n < NBLK - 1,
           lambda: [cp_x(TPB * n + TPB, 1, sem)])
        on(n < NP, lambda: [cp_v1(2 * n + 1, sem), cp_wo(n, sem)])

    cp_moda = [Both([cp_cols(wmod_hbm, wmod_v, t, 1, msem.at[s]) for t in tiles])
               for s, tiles in zip((0, 6, 10), MODA)]
    cp_modb = Both([pltpu.make_async_copy(wmod_hbm.at[:, _lanes(DA // 128 + b)],
                                          xw_v.at[NT + NFB + b], msem.at[1]) for b in range(NMB)])
    cp_g = pltpu.make_async_copy(wg_hbm, wg_v, msem.at[2])
    cp_u = pltpu.make_async_copy(wu_hbm, wu_v, msem.at[3])
    cp_d = Both([pltpu.make_async_copy(wdt_hbm.at[:, _lanes(b)], xw_v.at[NT + b], msem.at[4])
                 for b in range(NFB)])
    cp_out = lambda t, n, sem: Both([pltpu.make_async_copy(out_v.at[t + a], out_hbm.at[:, _lanes(t + a)],
                                                           sem) for a in range(n)])

    def silu_c():
        c = c_ref[...].astype(F32)
        return _r(c * _r(jax.nn.sigmoid(c)))

    def finish_mod(mod, lo, clock=None, pos=0):
        mod = _r(mod)
        col = lo + jax.lax.broadcasted_iota(jnp.int32, mod.shape, 1)
        is_scale = jnp.logical_or(jnp.logical_and(col >= D, col < 2 * D),
                                  jnp.logical_and(col >= 4 * D, col < 5 * D))
        mod = jnp.where(is_scale, _r(1.0 + mod), mod)
        for t in range(mod.shape[1] // 128):
            rows = pl.ds(pl.multiple_of(lo + t * 128, 128), 128)
            mod_ref[rows, :] = _paced(_col_bcast(mod[:, t * 128:(t + 1) * 128]), clock, pos)

    def late_mod_sums(n, clock):
        b0 = jnp.clip(n - MB0, 0, NMB // MPI - 1) * MPI
        for k in range(MPI):
            w = xw_v[jnp.where(n >= MB0, NT + NFB + b0 + k, 0)].astype(F32)
            part = jnp.sum((w * scb_ref[0:D, :]).reshape(D // 8, 8, 128), axis=0)
            lm_ref[k] = _paced(part, clock, PACE[4] + 192 * k)

    def late_mod_store(n, clock):
        b0 = jnp.clip(n - MB0, 0, NMB // MPI - 1) * MPI
        for k in range(MPI):
            finish_mod(jnp.sum(lm_ref[k], axis=0, keepdims=True), DA + (b0 + k) * 128,
                       clock, XP[4] + 128 * k)

    def col_vector(ref, row):
        row = jnp.concatenate([row, jnp.zeros((1, 64), F32)], axis=1)
        for t in range(5):
            ref[t * 128:(t + 1) * 128, :] = _col_bcast(row[:, t * 128:(t + 1) * 128])

    def mod(k):
        return mod_ref[k * D:(k + 1) * D, :]

    def put_stats(st_ref, t, shift, scale, clock, pos):
        row = jax.lax.broadcasted_iota(jnp.int32, (8, 128), 0)
        st_ref[t] = _paced(jnp.where(row == 0, shift, scale), clock, pos)

    def ln1_stats(t, clock=None, pos=None):
        for c in range(NC):
            m, s = _chunk_stats(xw_v[t, c * DC:(c + 1) * DC, :].astype(F32))
            put_stats(st1_ref, t * NC + c, m, s, clock, (PACE[0] if pos is None else pos) + 192 * c)

    def ln1_norm(t):
        mean, var = _mean_var(load_stats(st1_ref, t))
        return (xw_v[t].astype(F32) - mean) * jax.lax.rsqrt(var + EPS)

    def ln1_apply(t, clock=None, pos=None, ln=None):
        h = (ln1_norm(t) if ln is None else ln) * mod(1) + mod(0)
        ht_ref[t] = _paced(h, clock, PACE[1] if pos is None else pos).astype(BF16)

    def h2_rows(t, clock=None):
        x = _paced_wide(pltpu.bitcast(h2_ref[t].T, U32), clock, PACE[5])
        h2row_ref[pl.ds(pl.multiple_of(t * 64, 64), 64), :] = x

    def router_terms():
        u = mod(4) * wrb_ref[0:D, :]
        return (u, jnp.sum(u, axis=0, keepdims=True),
                jnp.sum(mod(3) * wrb_ref[0:D, :], axis=0, keepdims=True))

    def load_stats(st_ref, t):
        return [(st_ref[t * NC + c, 0:1, :], st_ref[t * NC + c, 1:2, :]) for c in range(NC)]

    def ln2_x1(t, attn, clock=None):
        x1 = _r(xw_v[t].astype(F32) + mod(2) * attn)
        x1_ref[t] = _paced(x1, clock, PACE[2]).astype(BF16)
        return x1, [_chunk_stats(x1[c * DC:(c + 1) * DC]) for c in range(NC)]

    def ln2_norm(stats):
        mean, var = _mean_var(stats)
        return _r(mean), 1.0 / _r(jnp.sqrt(_r(_r(var) + EPS)))

    def ln2_h2(x1, mean, inv):
        return (x1 - mean) * inv * mod(4) + mod(3)

    def ln2_stats(t, clock):
        for c, (m, s) in enumerate(ln2_x1(t, acc_ref[t], clock)[1]):
            put_stats(st2_ref, t * NC + c, m, s, clock, PACE[2] + (c + 1) * DC + SLAG)

    def ln2_apply(t, clock):
        x1 = x1_ref[t].astype(F32)
        h2 = ln2_h2(x1, *ln2_norm(load_stats(st2_ref, t)))
        key = _score_key(jnp.sum(h2 * wrb_ref[0:D, :], axis=0, keepdims=True), t)
        key_ref[pl.ds(t, 1), :] = _paced(key, clock, PACE[3] + D + 96)
        h2 = _r(h2)
        h2_ref[t] = _paced(h2, clock, PACE[3]).astype(BF16)
        out_v[t] = _paced(x1 + mod(5) * h2, clock, PACE[3] + 16).astype(BF16)

    def finish_q(q):
        q = (q * QSCALE).astype(BF16)
        return jnp.concatenate([q[r * DH:(r + 1) * DH] for r in range(REP)], axis=1)

    def q_proj(u, wqt_ref, qr_ref=None, split=False):
        w = pltpu.bitcast(wqt_ref[...], BF16)
        h = jnp.concatenate([ht_ref[_blk(u) * TPB + t] for t in range(TPB)], axis=1)
        if split:
            return sum(_dot(w[:, a:min(a + 128, D)], h[a:min(a + 128, D)]) for a in range(0, D, 128))
        if qr_ref is None:
            rem = _dot(w[:, DM:], h[DM:])
        else:
            rem = [qr_ref[...].T]
            if NV < TPB:
                R = GW * (TPB - NV) // 4
                rem.append(jnp.concatenate([_dot(w[a:a + R, DM:], h[DM:, NV * 128:])
                                            for a in range(0, GW, R)], axis=0))
            rem = jnp.concatenate(rem, axis=1)
        return _dot(w[:, :DM], h[:DM]) + rem

    def w_rest(u, wf_ref):
        w = wrem_v[:, _lanes(_grp(u) * REP, REP)].astype(F32)
        for r in range(REP):
            wf_ref[r] = w[:, r * DH:(r + 1) * DH]

    def outer(u, qr_ref, wf_ref, clock, start, never):
        base = jnp.bitwise_and(_blk(u), 1) * (NV * 16)

        def chains(group, after=None):
            acc = {}
            for k in range(KR):
                for tv, r in group:
                    t = hb_ref[base + tv, k] * wf_ref[r, pl.ds(k, 8, stride=0), :]
                    acc[tv, r] = _paced(t, after, 0) if k == 0 else acc[tv, r] + t
            return acc.items()

        cells = [(tv, r) for r in range(REP) for tv in range(NV * 16)]
        per = NPV
        for c, tick in enumerate(never):
            prev = None
            for i, cell in enumerate(cells[c * per:(c + 1) * per]):
                for (tv, r), prev in chains([cell], prev):
                    qr_ref[tv * 8:(tv + 1) * 8, r * DH:(r + 1) * DH] = _paced(prev, tick, PV0 + 8 * i)
        cells = cells[per * len(never):]
        for g in range(0, len(cells), CH):
            for (tv, r), a in chains(cells[g:g + CH]):
                qr_ref[tv * 8:(tv + 1) * 8, r * DH:(r + 1) * DH] = _paced(
                    a, clock, min(start + OSTEP * (g // CH + 1), clock.shape[0] - 8))

    def h_table(hr, base, k0, gates):
        nk = hr.shape[0]
        for j in range(nk):
            cb = _col_bcast(hr[j:j + 1])
            for b in range(16):
                g = gates[(j * 16 + b) * len(gates) // (nk * 16)]
                hb_ref[base + b, k0 + j] = jnp.where(g, 0.0, cb[b * 8:(b + 1) * 8])

    def never_of(clock, lo, hi):
        return [clock[a:a + 8] * clock[a:a + 8] < 0.0 for a in range(lo // 8 * 8, hi, 8)]

    def scores(u, q, s_ref, m_ref):
        s = _dot(pltpu.bitcast(k_v.bitcast(U32)[_grp(u)], BF16) if KB else k_v[_grp(u)], q)
        s_ref[...] = s
        m_ref[...] = jnp.broadcast_to(jnp.max(s, axis=0, keepdims=True), m_ref.shape)
        return jnp.concatenate([s[:, 0:128], s[:, TQ:TQ + 128]], axis=0)

    def v_transpose(u, vt_ref, clock=None, pos=0):
        vt_ref[...] = _paced_wide(pltpu.bitcast((pltpu.bitcast(v_v.bitcast(U32)[_grp(u)], BF16) if KB else v_v[_grp(u)]).T, U32), clock, pos)

    def wq_transpose(u, wqt_ref, clock=None, pos=0):
        wqt_ref[...] = _paced_wide(pltpu.bitcast(wq_v[_grp(u)].T, U32), clock, pos)

    def wd_transpose(u, clock, pos):
        fb = jnp.clip(u - WD0, 0, NFB - 1)
        src = jnp.where(u >= WD0, NT + fb, 0)
        wd_ref[pl.ds(pl.multiple_of(fb * 64, 64), 64), :] = _paced_wide(
            pltpu.bitcast(xw_v[src].T, U32), clock, pos)

    def attend(s_ref, m_ref, vt_ref):
        m = m_ref[0:1, :]
        o, never = [], []
        for r in range(REP):
            cols = slice(r * TQ, (r + 1) * TQ)
            p, l, ts = _softmax_numer(s_ref[:, cols], m[:, cols])
            ov = _dot(pltpu.bitcast(vt_ref[...], BF16), p)
            o.append((ov * (1.0 / l)).astype(BF16))
            never += [ov[:, c * 128:(c + 1) * 128] for c in range(TPB)]
        return jnp.concatenate(o, axis=0), never

    small = Both([pltpu.make_async_copy(wr_hbm, wr_ref, msem.at[7]),
                  pltpu.make_async_copy(c_hbm, c_ref, msem.at[7])])
    zeroth = Both([cp_x(0, TPB, msem.at[5]), cp_w1(wq_hbm, wq_v, 0, msem.at[5])])
    first = Both([cp_k1(0, msem.at[8]), cp_w1(wq_hbm, wq_v, 1, msem.at[8])])
    second = Both([cp_k1(1, msem.at[9]), cp_v1(0, msem.at[9]), cp_w1(wq_hbm, wq_v, 2, msem.at[9]),
                   pltpu.make_async_copy(wq_hbm.at[DM:, :], wrem_v, msem.at[9]), cp_x(TPB, 1, msem.at[9])])
    for cp in [small, zeroth] + cp_moda + [first, second]:
        cp.start()
    acc_ref[...] = jnp.zeros_like(acc_ref)
    mod_ref[DA:6 * D, :] = jnp.zeros((4 * D, 128), F32)
    h2_ref[0] = jnp.zeros((D, 128), BF16)
    small.wait()
    col_vector(wrb_ref, wr_ref[...].astype(F32).reshape(1, D))
    col_vector(scb_ref, silu_c())
    sc8 = jnp.broadcast_to(silu_c(), (8, D)).astype(BF16)
    zeroth.wait()
    ln0 = []
    for t in range(TPB):
        ln1_stats(t)
        ln0.append(ln1_norm(t))
    wq_transpose(0, wqt0_ref)
    for cp, tiles in zip(cp_moda, MODA):
        cp.wait()
        for t in tiles:
            finish_mod(_dot(sc8, wmod_v[:, t * 128:(t + 1) * 128])[0:1], t * 128)
    for t in range(TPB):
        ln1_apply(t, ln=ln0[t])
    q = finish_q(q_proj(0, wqt0_ref, split=True))
    first.wait()
    bundle(0, 'start')
    def first_table(gates, lo, hi):
        for i in range(NV + 1):
            a, b = max(lo, i * KR), min(hi, (i + 1) * KR)
            if a < b:
                gs = gates[(a - lo) * len(gates) // (hi - lo):(b - lo) * len(gates) // (hi - lo)]
                hr = ht_ref[i if i < NV else TPB, DM:, :].astype(F32)[a - i * KR:b - i * KR]
                h_table(hr, i * 16, a - i * KR, gs)

    first_table(never_of(scores(0, q, s0_ref, m0_ref), 64, 2 * S - 192), 0, TSPLIT)
    wq_transpose(1, wqt1_ref)
    second.wait()
    bundle(1, 'start')
    q = q_proj(1, wqt1_ref)
    hrem = jnp.concatenate([ht_ref[t, DM:, :] for t in range(NV)], axis=1)
    for a in range(2):
        streams[a][4][...] = jax.lax.dot_general(
            hrem, wrem_v[:, (a + 2) * GW:(a + 3) * GW], (((0,), (0,)), ((), ())),
            preferred_element_type=F32)
    clock = jnp.concatenate([q[:, t * 128:(t + 1) * 128] for t in range(TPB)]
                            + [scores(1, finish_q(q), s1_ref, m1_ref)], axis=0)
    ln1_stats(TPB, clock, PP[0])
    ln1_apply(TPB, clock, PP[1])
    first_table(never_of(clock, 0, PP[2]), TSPLIT, NV * KR + 2 * TPI)
    v_transpose(0, vt0_ref, clock, PP[3])
    wq_transpose(2, wqt0_ref, clock, PP[4])
    for a in range(2):
        w_rest(a + 4, streams[a][5])

    def unit(u, side, s_ref, m_ref, vt_ref, wqt_ref, qr_ref, wf_ref):
        q = q_proj(u + 2, wqt_ref, qr_ref)
        o, never = attend(s_ref, m_ref, vt_ref)
        sclk = scores(u + 2, finish_q(q), s_ref, m_ref)
        upd = _dot(wot_v[_grp(u)], o)
        clock = jnp.concatenate([q[:, t * 128:(t + 1) * 128] for t in range(TPB)] + [sclk]
                                + [upd[:, 0:128], upd[:, 256:384]], axis=0)
        side(clock, lambda start: outer(u + 4, qr_ref, wf_ref, clock, start, never))
        w_rest(u + 6, wf_ref)
        for t in range(TPB):
            acc_ref[_blk(u) * TPB + t] += upd[:, t * 128:(t + 1) * 128]

    def step(n, carry):
        def waits(_, c):
            bundle(n, 'wait')
            pl.when(n == MB0)(cp_modb.wait)
            pl.when(n == WD0 // 2)(cp_d.wait)
            return c
        jax.lax.fori_loop(0, jnp.where(n < NP, 1, 0), waits, 0)

        pl.when(n == 0)(cp_modb.start)
        bundle(jnp.minimum(n + 2, NP), 'start')
        for a in range(3):
            pl.when(n == 2 + a)(Both(cp_d.cps[a * NFB // 3:(a + 1) * NFB // 3]).start)
        pl.when(n == NP)(Both([cp_g, cp_u]).start)

        t1 = jnp.minimum(n + 4, NT - 1)
        v = jnp.maximum(n - NP, 0)
        tile2 = lambda v: (jax.lax.shift_right_logical(v, 3) * TPB
                           + jnp.minimum(jnp.bitwise_and(v, NP - 1), TPB - 1))
        t2 = tile2(v)

        def stats(clock, outer_at):
            v_transpose(2 * n + 1, vt1_ref, clock, XP[5])
            wq_transpose(2 * n + 3, wqt1_ref, clock, XP[6])
            ln2_stats(t2, clock)
            ln1_stats(t1, clock)
            late_mod_sums(n, clock)
            h2_rows(tile2(jnp.maximum(v - 1, 0)), clock)
            wd_transpose(2 * n, clock, XP[0])
            outer_at(OUTER0[0])

        def apply(clock, outer_at):
            blk = jnp.minimum(jax.lax.shift_right_logical(n + 2, 3) + 1, NBLK - 1)
            e0 = jnp.bitwise_and(n + 2, 7) * TPI
            i, k0 = jax.lax.shift_right_logical(e0, 6), jnp.bitwise_and(e0, KR - 1)
            hr = ht_ref[blk * TPB + i, pl.ds(pl.multiple_of(DM + k0, 16), TPI), :].astype(F32)
            v_transpose(2 * n + 2, vt0_ref, clock, XP[1])
            wq_transpose(2 * n + 4, wqt0_ref, clock, XP[2])
            wd_transpose(2 * n + 1, clock, XP[3])
            ln1_apply(t1, clock)
            ln2_apply(t2, clock)
            outer_at(OUTER0[1])
            h_table(hr, (jnp.bitwise_and(blk, 1) * NV + i) * 16, k0, never_of(clock, TAB0, TAB1))
            late_mod_store(n, clock)

        for a in range(2):
            unit(2 * n + a, (stats, apply)[a], *streams[a])
        return carry

    jax.lax.fori_loop(0, NU // 2 - 1, step, 0)

    T0 = NT - TPB
    cp_out(0, T0, osem.at[C + TPB]).start()
    cp_g.wait()
    v_transpose(NU - 1, vt1_ref)
    o = jnp.concatenate([attend(*streams[a][0:3])[0] for a in range(2)], axis=0)
    wlast = jnp.concatenate([wot_v[HKV - 2], wot_v[HKV - 1]], axis=1)
    fin = [acc_ref[T0 + t] + _dot(wlast, o[:, t * 128:(t + 1) * 128]) for t in range(TPB)]
    clock = jnp.concatenate(fin, axis=0)
    row8 = jax.lax.broadcasted_iota(jnp.int32, (C, 128), 0)
    lane8 = jax.lax.broadcasted_iota(jnp.int32, (C, 128), 1)
    work = key_ref[0:T0, :]
    lead = jnp.zeros((C, 128), F32)
    for t in range(C):
        mx = jnp.max(jnp.max(work, axis=0, keepdims=True), axis=1, keepdims=True)
        work = jnp.where(work == mx, 0.0, work)
        lead = jnp.where(row8 == t, mx, lead)

    def spread(row):
        return pltpu.roll(jnp.broadcast_to(row, (128, 128)), 0, 1, stride=1, stride_axis=0)

    def merge(lead, rows, spreads):
        cols = jnp.concatenate([lead] + spreads, axis=0)
        best = jnp.zeros((C, 128), F32)
        for row in [jnp.max(jnp.where(row8 == lane8, lead, 0.0), axis=0, keepdims=True)] + rows:
            rank = jnp.sum(jnp.where(cols > row, 1.0, 0.0), axis=0, keepdims=True)
            best = jnp.maximum(best, jnp.where(rank == row8.astype(F32), row, 0.0))
        return jnp.max(best, axis=1, keepdims=True)

    def tail_h2(t, norm, gate=None):
        x1 = x1_ref[t].astype(F32)
        if gate is not None:
            n = gate.shape[0]
            x1 = jnp.concatenate([_paced(x1[:n], gate, 0), x1[n:]], axis=0) if n < D else _paced(x1, gate, 0)
        h2_ref[t] = ln2_h2(x1, *norm).astype(BF16)
        if t < NT - 2:
            h2_rows(t)

    u_vec, u_sum, b_sum = router_terms()
    keys = []
    for t in range(TPB):
        x1, stats = ln2_x1(T0 + t, fin[t])
        mean, inv = norm = ln2_norm(stats)
        r = (jnp.sum(x1 * u_vec, axis=0, keepdims=True) - mean * u_sum) * inv + b_sum
        keys.append(_score_key(r, T0 + t))
        if t < TPB - 1:
            tail_h2(T0 + t, norm, clock[(t + 1) * D + TLAG:(t + 2) * D + TLAG])
    lead = jnp.broadcast_to(merge(lead, keys[0:2], [spread(k) for k in keys[0:2]]), (C, 128))
    spread2 = spread(keys[2])
    if BAR == 0:
        cp_u.wait()
        cp_out(0, T0, osem.at[C + TPB]).wait()

    h2_rows(NT - 2)
    tail_h2(NT - 1, norm)
    h2_rows(NT - 1)
    sel = pltpu.bitcast(merge(lead, keys[2:4], [spread2, spread(keys[3])]), jnp.int32) - KEY0
    sel_tok = (S - 1) - (sel & (S - 1))
    toks = [sel_tok[t, 0] for t in range(C)]
    tiles = [jax.lax.shift_right_logical(tk, 7) for tk in toks]
    sel_code = jax.lax.shift_right_logical(sel, 11) - 32768
    sel_bits = jnp.where(sel_code < 0, -32769 - sel_code, sel_code)
    r_sel = pltpu.bitcast(jax.lax.shift_left(sel_bits, 16), F32)

    final = []
    for t in range(C):
        d = True
        for u in range(t + 1, C):
            d = jnp.logical_and(d, tiles[u] != tiles[t])
        final.append(d)

    words = jnp.concatenate([h2row_ref[pl.ds(jax.lax.shift_right_logical(toks[t], 1), 1), :]
                             for t in range(C)], axis=0)
    odd = jnp.bitwise_and(sel_tok, 1) == 1
    xs = pltpu.bitcast(jnp.where(odd, jnp.bitwise_and(words, jnp.uint32(0xFFFF0000)),
                                 jax.lax.shift_left(words, jnp.uint32(16))), F32)
    xs = xs.astype(BF16)

    def plain_out(t, ticks=None):
        x1 = x1_ref[t].astype(F32)
        if ticks is not None:
            gate = jnp.concatenate([ticks[a * len(ticks) // (D // 8)] for a in range(D // 8)], axis=0)
            x1 = _paced(x1, gate, 0)
        out_v[t] = (x1 + mod(5) * h2_ref[t].astype(F32)).astype(BF16)

    clean = []

    def send_clean(t):
        d = tiles[0] != t
        for a in range(1, C):
            d = jnp.logical_and(d, tiles[a] != t)
        clean.append(d)
        pl.when(d)(cp_out(t, 1, osem.at[C + t - T0]).start)

    if BAR == 1:
        cp_u.wait()
        cp_out(0, T0, osem.at[C + TPB]).wait()
    gpre = _dot(xs, wg_v[...])
    u = _dot(xs, wu_v[...])
    ticks = [z[:, a * 128:(a + 1) * 128] for z in (gpre, u) for a in range(NFB)]
    for t in range(TPB):
        plain_out(T0 + t, ticks[t * TKS:(t + 1) * TKS])
        send_clean(T0 + t)
    gpre, u = _r(gpre), _r(u)
    gact = _r(gpre * _r(jax.nn.sigmoid(gpre)))
    act = (gact * u).astype(BF16)
    gate_r = _r(jax.nn.sigmoid(r_sel))
    ohs = []
    for t in range(C):
        oh = jnp.where(sel_tok == tiles[t] * 128 + lane8, 1.0, 0.0)
        ohs.append(jnp.concatenate([oh, jnp.zeros((16 - C, 128), F32)], axis=0).astype(BF16))

    def cp_fix(t, lo, hi):
        return pltpu.make_async_copy(fix_v.at[t, lo:hi, :], out_hbm.at[lo:hi, _lanes(tiles[t])],
                                     osem.at[t])

    def guarded(cond, fn):
        if cond is True:
            fn()
        else:
            pl.when(cond)(fn)

    def scatter(j, yt, t):
        lo, hi = j * 128, min(j * 128 + 128, D)
        upd = jnp.concatenate([_dot(yt[a:a + 64], ohs[t]) for a in range(0, hi - lo, 64)], axis=0)
        fix_v[t, lo:hi, :] = (x1_ref[tiles[t], lo:hi, :].astype(F32) + mod_ref[5 * D + lo:5 * D + hi, :]
                              * (h2_ref[tiles[t], lo:hi, :].astype(F32) + upd)).astype(BF16)
        guarded(final[t], cp_fix(t, lo, hi).start)

    NJ = (D + 127) // 128
    yts = []
    for j in range(NJ):
        lo, hi = j * 128, min(j * 128 + 128, D)
        nk = 4
        FK = F // nk
        yk = []
        for a in range(nk):
            w = pltpu.bitcast(wd_ref[a * FK // 2:(a + 1) * FK // 2, lo:hi], BF16)
            yk.append(_dot(act[:, a * FK:(a + 1) * FK], w))
            if j >= SCLAG:
                for t in (2 * a, 2 * a + 1):
                    scatter(j - SCLAG, yts[j - SCLAG], t)
        y = _r(sum(yk)) * gate_r
        yts.append(jnp.concatenate([y, jnp.zeros_like(y)], axis=0).astype(BF16).T)
    for j in range(NJ - SCLAG, NJ):
        for t in range(C):
            scatter(j, yts[j], t)
    for t in range(T0, NT):
        pl.when(clean[t - T0])(cp_out(t, 1, osem.at[C + t - T0]).wait)
    for t in range(C):
        guarded(final[t], cp_fix(t, 0, D).wait)


@jax.jit
def pallas_adaLN_cond__gqa_block_cached__moe_arch_mod__prompt_kernel(
    A_x: jax.Array,
    A_k_cache: jax.Array,
    A_v_cache: jax.Array,
    A_wq: jax.Array,
    A_wo: jax.Array,
    B_x: jax.Array,
    B_w_r: jax.Array,
    B_w_gate: jax.Array,
    B_w_up: jax.Array,
    B_w_down: jax.Array,
    c: jax.Array,
    w_mod: jax.Array,
):
    del B_x
    xt = A_x.reshape(S, D).T
    k = A_k_cache.reshape(HKV, S, DH)
    v = A_v_cache.reshape(HKV, S, DH)

    hbm = pl.BlockSpec(memory_space=pl.ANY)
    stream = [
        pltpu.VMEM((S, REP * TQ), F32),
        pltpu.VMEM((8, REP * TQ), F32),
        pltpu.VMEM((DH // 2, S), U32),
        pltpu.VMEM((GW // 2, D), U32),
        pltpu.VMEM((NV * 128, GW), F32),
        pltpu.VMEM((REP, KR, DH), F32),
    ]
    out = pl.pallas_call(
        _kernel,
        in_specs=[hbm] * 11,
        out_specs=hbm,
        out_shape=jax.ShapeDtypeStruct((D, S), BF16),
        scratch_shapes=[
            pltpu.VMEM((NT + NFB + NMB, D, 128), BF16),
            pltpu.VMEM((HKV, S, DH), BF16),
            pltpu.VMEM((HKV, S, DH), BF16),
            pltpu.VMEM((HKV, D, GW), BF16),
            pltpu.VMEM((HKV, D, GW), BF16),
            pltpu.VMEM((D, DA), BF16),
            pltpu.VMEM((D, F), BF16),
            pltpu.VMEM((D, F), BF16),
            pltpu.VMEM((F // 2, D), U32),
            pltpu.VMEM((NT, D, 128), BF16),
            pltpu.VMEM((NT, D, 128), F32),
            pltpu.VMEM((6 * D, 128), F32),
            pltpu.VMEM((5 * 128, 128), F32),
            pltpu.VMEM((5 * 128, 128), F32),
            pltpu.VMEM((NT, D, 128), BF16),
            pltpu.VMEM((NT, D, 128), BF16),
            pltpu.VMEM((S // 2, D), U32),
            pltpu.VMEM((NT, D, 128), BF16),
            pltpu.VMEM((C, D, 128), BF16),
            pltpu.VMEM((NT, 128), F32),
            pltpu.VMEM((NT * NC, 8, 128), F32),
            pltpu.VMEM((NT * NC, 8, 128), F32),
            pltpu.VMEM((MPI, 8, 128), F32),
            pltpu.VMEM((2 * NV * 16, KR, 8, 128), F32),
            pltpu.VMEM((KR, HQ * DH), BF16),
        ] + stream + stream + [
            pltpu.VMEM((D,), BF16),
            pltpu.VMEM((1, D), BF16),
            pltpu.SemaphoreType.DMA((HKV // 2,)),
            pltpu.SemaphoreType.DMA((11,)),
            pltpu.SemaphoreType.DMA((C + TPB + 1,)),
        ],
        compiler_params=pltpu.CompilerParams(vmem_limit_bytes=127 * 1024 * 1024,
                                             disable_bounds_checks=True,
                                             disable_semaphore_checks=True),
    )(B_w_r, c, xt, k, v, A_wq, A_wo.T, w_mod, B_w_gate, B_w_up, B_w_down.T)
    return out.T.reshape(1, S, D)
```

```python
import math

import jax
import jax.numpy as jnp
import jax.experimental.pallas as pl
import jax.experimental.pallas.tpu as pltpu

S = 2048
D = 576
HQ = 32
HKV = 16
REP = HQ // HKV
DH = 128
GW = REP * DH
F = 4608
C = 8
EPS = 1e-05
TQ = 512
NBLK = S // TQ
TPB = TQ // 128
NT = S // 128
NU = NBLK * HKV
DA = 2 * D
NC = 3
DC = D // NC
TLAG = 160
TKS = 18
SCLAG = 2
CL2 = 0
SLAG = 96
BAR = 1
PG = 64
NFB = F // 128
MODA = ((0, 4, 5), (1, 2, 6), (3, 7, 8))
NMB = 4 * D // 128
MPI = 3
MB0 = 1
WD0 = 14
DM = 512
KR = D - DM
NV = 3
CH = 3
QC, SC, WC = 0, 1024, 1024 + 2 * S
OUTER0, OSTEP = (SC + 850, SC + 0), 133
TABLE = 1
TAB = ((SC + 1600, SC + 2800), (SC + 3050, SC + 4050), (WC + 250, WC + 750))
XP = (SC + 3700, SC + 100, SC + 900, SC + 1300, WC + 760, SC + 1200, SC + 2400)
PV0 = 0
TSPLIT = 15
PP = (SC + 100, SC + 600, SC + 4000, 0, 300, 400, 500, SC + 2300, 300)
GS = 4
OCAT = 1
QCAT = 1
WFP = ((100, 800), (WC + 300, WC + 1000))
TPI = 8
PACE = (100, WC + 200, SC + 100, WC + 250, 200, SC + 3300)

BF16 = jnp.bfloat16
F32 = jnp.float32
U32 = jnp.uint32
QSCALE = DH ** -0.5 * math.log2(math.e)


def _dot(a, b):
    return jnp.dot(a, b, preferred_element_type=F32)


def _dot_nt(a, b):
    return jax.lax.dot_general(a, b, (((1,), (1,)), ((), ())), preferred_element_type=F32)


def _r(x):
    return x.astype(BF16).astype(F32)


def _col_bcast(row):
    return jnp.broadcast_to(row, (128, 128)).T


def _blk(u):
    return u // HKV if isinstance(u, int) else jax.lax.shift_right_logical(u, 4)


def _grp(u):
    return u % HKV if isinstance(u, int) else jnp.bitwise_and(u, HKV - 1)


def _lanes(t, n=1):
    return pl.ds(pl.multiple_of(t * 128, 128), n * 128)


def _paced(x, clock, pos):
    if clock is None:
        return x
    pos = pos // 8 * 8
    g = clock[pos:pos + x.shape[0], 0:x.shape[1]]
    return jnp.where(g * g < 0.0, jnp.zeros_like(x), x)


def _paced_wide(x, clock, pos):
    if clock is None:
        return x
    n, w = x.shape
    cols = []
    for a in range(0, w, 128):
        p0 = (pos + a // 128 * n) // 8 * 8
        g = jnp.concatenate([clock[p0 + r // (8 * GS) * (8 * GS):p0 + r // (8 * GS) * (8 * GS) + 8]
                             for r in range(0, n, 8)], axis=0)
        cols.append(_paced(x[:, a:min(a + 128, w)], g, 0))
    return jnp.concatenate(cols, axis=1)


def _gated(x, gates, j, n):
    if gates is None:
        return x
    m = x.shape[0]
    g = jnp.stack([gates[(j * m + b) * len(gates) // (n * m)] for b in range(m)])
    return jnp.where(g < 0.0, 0.0, x)


def _native(ref, i):
    return pltpu.bitcast(ref.bitcast(U32)[i], BF16)


def _softmax_numer(s, m):
    n, w = s.shape
    p = jnp.exp2(s - m).reshape(n // PG, PG // 8, 8, w)
    ts = jnp.sum(p, axis=1)
    last = jnp.where(ts < 0.0, ts, p[:, PG // 8 - 1])
    p = jnp.concatenate([p[:, :PG // 8 - 1], last[:, None]], axis=1).reshape(n, w)
    l = jnp.sum(jnp.sum(ts, axis=0), axis=0, keepdims=True)
    return p.astype(BF16), l


KEY0 = 0x20000000


def _score_key(r, t):
    tok = t * 128 + jax.lax.broadcasted_iota(jnp.int32, r.shape, 1)
    bits = jax.lax.shift_right_arithmetic(pltpu.bitcast(_r(r) + 0.0, jnp.int32), 16)
    code = jnp.where(bits < 0, -32769 - bits, bits) + 32768
    return pltpu.bitcast(code * S + (S - 1 - tok) + KEY0, F32)


def _chunk_stats(x):
    m = jnp.sum(x, axis=0, keepdims=True) * (1.0 / DC)
    xc = x - m
    return m, jnp.sum(xc * xc, axis=0, keepdims=True)


def _mean_var(stats):
    mean = sum(m for m, _ in stats) * (1.0 / NC)
    var = sum(s + DC * (m - mean) * (m - mean) for m, s in stats) * (1.0 / D)
    return mean, var


def _kernel_flat(*refs):
    _kernel(*refs[:12], *refs[12 + NV:], *refs[12:12 + NV])


def _kernel(wr_hbm, c_hbm,
            xt_hbm, k_hbm, v_hbm, wq_hbm, wot_hbm, wmod_hbm, wg_hbm, wu_hbm, wdt_hbm,
            out_hbm,
            xw_v, k_v, v_v, wq_v, wot_v, wmod_v, wg_v, wu_v, wd_ref,
            ht_ref, acc_ref, mod_ref, wrb_ref, scb_ref, x1_ref, h2_ref, h2row_ref, out_v, fix_v,
            key_ref, st1_ref, st2_ref, lm_ref,
            wrem_v,
            s0_ref, m0_ref, vt0_ref, wqt0_ref, qr0_ref, wf0_ref,
            s1_ref, m1_ref, vt1_ref, wqt1_ref, qr1_ref, wf1_ref,
            wr_ref, c_ref, bsem, msem, osem, *hb_refs):
    streams = ((s0_ref, m0_ref, vt0_ref, wqt0_ref, qr0_ref, wf0_ref),
               (s1_ref, m1_ref, vt1_ref, wqt1_ref, qr1_ref, wf1_ref))

    def cp_cols(src, dst, t, n, sem, dst_t=None):
        return pltpu.make_async_copy(src.at[:, _lanes(t, n)],
                                     dst.at[:, _lanes(t if dst_t is None else dst_t, n)], sem)

    def cp_pair(src, dst, p, sem):
        return pltpu.make_async_copy(src.at[pl.ds(2 * p, 2)], dst.at[pl.ds(2 * p, 2)], sem)

    cp_k = lambda p, sem: cp_pair(k_hbm, k_v, p, sem)
    cp_v1 = lambda g, sem: pltpu.make_async_copy(v_hbm.at[g], v_v.at[g], sem)
    cp_k1 = lambda g, sem: pltpu.make_async_copy(k_hbm.at[g], k_v.at[g], sem)

    class Both:
        def __init__(self, cps):
            self.cps = cps

        def start(self):
            for cp in self.cps:
                cp.start()

        def wait(self):
            for cp in self.cps:
                cp.wait()

    def cp_w1(src, dst, g, sem):
        return pltpu.make_async_copy(src.at[:, _lanes(g * REP, REP)], dst.at[g], sem)

    def cp_w(src, dst, p, sem):
        return Both([cp_w1(src, dst, 2 * p + a, sem) for a in range(2)])

    cp_wq = lambda p, sem: cp_w(wq_hbm, wq_v, p, sem)
    cp_wo = lambda p, sem: cp_w(wot_hbm, wot_v, p, sem)
    cp_x = lambda t0, n, sem: Both([pltpu.make_async_copy(xt_hbm.at[:, _lanes(t0 + t)],
                                                          xw_v.at[t0 + t], sem) for t in range(n)])
    NP = HKV // 2

    def bundle(n, act):
        sem = bsem.at[n if isinstance(n, int) else jnp.minimum(n, NP - 1)]

        def on(cond, cps):
            def go():
                for cp in cps():
                    getattr(cp, act)()
            if isinstance(cond, bool):
                if cond:
                    go()
            else:
                pl.when(cond)(go)
        on(n + 1 < NP, lambda: [cp_k(n + 1, sem), cp_v1(2 * n + 2, sem), cp_w1(wq_hbm, wq_v, 2 * n + 3, sem)])
        on(n + 2 < NP, lambda: [cp_w1(wq_hbm, wq_v, 2 * n + 4, sem)])
        XN = 3 if NV == 3 else 5
        nx = (NT - TPB - NV) // XN
        on(jnp.logical_and(n >= 1, n <= nx) if not isinstance(n, int) else 1 <= n <= nx,
           lambda: [cp_x(TPB + NV + XN * (n - 1), XN, sem)])
        on(n < NP, lambda: [cp_v1(2 * n + 1, sem), cp_wo(n, sem)])

    cp_moda = [Both([cp_cols(wmod_hbm, wmod_v, t, 1, msem.at[s]) for t in tiles])
               for s, tiles in zip((0, 6, 10), MODA)]
    cp_modb = Both([pltpu.make_async_copy(wmod_hbm.at[:, _lanes(DA // 128 + b)],
                                          xw_v.at[NT + NFB + b], msem.at[1]) for b in range(NMB)])
    cp_g = pltpu.make_async_copy(wg_hbm, wg_v, msem.at[2])
    cp_u = pltpu.make_async_copy(wu_hbm, wu_v, msem.at[3])
    cp_d = Both([pltpu.make_async_copy(wdt_hbm.at[:, _lanes(b)], xw_v.at[NT + b], msem.at[4])
                 for b in range(NFB)])
    cp_out = lambda t, n, sem: Both([pltpu.make_async_copy(out_v.at[t + a], out_hbm.at[:, _lanes(t + a)],
                                                           sem) for a in range(n)])

    def silu_c():
        c = c_ref[...].astype(F32)
        return _r(c * _r(jax.nn.sigmoid(c)))

    def finish_mod(mod, lo, clock=None, pos=0):
        mod = _r(mod)
        col = lo + jax.lax.broadcasted_iota(jnp.int32, mod.shape, 1)
        is_scale = jnp.logical_or(jnp.logical_and(col >= D, col < 2 * D),
                                  jnp.logical_and(col >= 4 * D, col < 5 * D))
        mod = jnp.where(is_scale, _r(1.0 + mod), mod)
        for t in range(mod.shape[1] // 128):
            rows = pl.ds(pl.multiple_of(lo + t * 128, 128), 128)
            mod_ref[rows, :] = _paced(_col_bcast(mod[:, t * 128:(t + 1) * 128]), clock, pos)

    def late_mod_sums(n, clock):
        b0 = jnp.clip(n - MB0, 0, NMB // MPI - 1) * MPI
        for k in range(MPI):
            w = xw_v[jnp.where(n >= MB0, NT + NFB + b0 + k, 0)].astype(F32)
            part = jnp.sum((w * scb_ref[0:D, :]).reshape(D // 8, 8, 128), axis=0)
            lm_ref[k] = _paced(part, clock, PACE[4] + 192 * k)

    def late_mod_store(n, sums, clock):
        b0 = jnp.clip(n - MB0, 0, NMB // MPI - 1) * MPI
        for k in range(MPI):
            finish_mod(jnp.sum(sums[k], axis=0, keepdims=True), DA + (b0 + k) * 128,
                       clock, XP[4] + 128 * k)

    def col_vector(ref, row):
        row = jnp.concatenate([row, jnp.zeros((1, 64), F32)], axis=1)
        for t in range(5):
            ref[t * 128:(t + 1) * 128, :] = _col_bcast(row[:, t * 128:(t + 1) * 128])

    def mod(k):
        return mod_ref[k * D:(k + 1) * D, :]

    def put_stats(st_ref, t, shift, scale, clock, pos):
        row = jax.lax.broadcasted_iota(jnp.int32, (8, 128), 0)
        st_ref[t] = _paced(jnp.where(row == 0, shift, scale), clock, pos)

    def ln1_stats(t, clock=None, pos=None):
        for c in range(NC):
            m, s = _chunk_stats(xw_v[t, c * DC:(c + 1) * DC, :].astype(F32))
            put_stats(st1_ref, t * NC + c, m, s, clock, (PACE[0] if pos is None else pos) + 192 * c)

    def ln1_norm(t):
        mean, var = _mean_var(load_stats(st1_ref, t))
        return (xw_v[t].astype(F32) - mean) * jax.lax.rsqrt(var + EPS)

    def ln1_apply(t, clock=None, pos=None, ln=None):
        h = (ln1_norm(t) if ln is None else ln) * mod(1) + mod(0)
        ht_ref[t] = _paced(h, clock, PACE[1] if pos is None else pos).astype(BF16)

    def h2_rows(t, clock=None):
        x = _paced_wide(pltpu.bitcast(_native(h2_ref, t).T, U32), clock, PACE[5])
        h2row_ref[pl.ds(pl.multiple_of(t * 64, 64), 64), :] = x

    def router_terms():
        u = mod(4) * wrb_ref[0:D, :]
        return (u, jnp.sum(u, axis=0, keepdims=True),
                jnp.sum(mod(3) * wrb_ref[0:D, :], axis=0, keepdims=True))

    def load_stats(st_ref, t):
        return [(st_ref[t * NC + c, 0:1, :], st_ref[t * NC + c, 1:2, :]) for c in range(NC)]

    def ln2_x1(t, attn, clock=None):
        x1 = _r(xw_v[t].astype(F32) + mod(2) * attn)
        x1_ref[t] = _paced(x1, clock, PACE[2]).astype(BF16)
        return x1, [_chunk_stats(x1[c * DC:(c + 1) * DC]) for c in range(NC)]

    def ln2_norm(stats):
        mean, var = _mean_var(stats)
        return _r(mean), 1.0 / _r(jnp.sqrt(_r(_r(var) + EPS)))

    def ln2_h2(x1, mean, inv):
        return (x1 - mean) * inv * mod(4) + mod(3)

    def ln2_stats(t, clock):
        for c, (m, s) in enumerate(ln2_x1(t, acc_ref[t], clock)[1]):
            put_stats(st2_ref, t * NC + c, m, s, clock, PACE[2] + (c + 1) * DC + SLAG)

    def ln2_apply(t, clock):
        x1 = x1_ref[t].astype(F32)
        h2 = ln2_h2(x1, *ln2_norm(load_stats(st2_ref, t)))
        key = _score_key(jnp.sum(h2 * wrb_ref[0:D, :], axis=0, keepdims=True), t)
        key_ref[pl.ds(t, 1), :] = _paced(key, clock, PACE[3] + D + 96)
        h2 = _r(h2)
        h2_ref[t] = _paced(h2, clock, PACE[3]).astype(BF16)
        out_v[t] = _paced(x1 + mod(5) * h2, clock, PACE[3] + 16).astype(BF16)

    def finish_q(q):
        if QCAT:
            q = (q * QSCALE).astype(BF16)
            return jnp.concatenate([q[r * DH:(r + 1) * DH] for r in range(REP)], axis=1)
        q = jnp.concatenate([q[r * DH:(r + 1) * DH] for r in range(REP)], axis=1)
        return (q * QSCALE).astype(BF16)

    def q_proj(u, wqt_ref, qr_ref=None, split=False):
        w = pltpu.bitcast(wqt_ref[...], BF16)
        h = jnp.concatenate([_native(ht_ref, _blk(u) * TPB + t) for t in range(TPB)], axis=1)
        if split:
            return sum(_dot(w[:, a:min(a + 128, D)], h[a:min(a + 128, D)]) for a in range(0, D, 128))
        if qr_ref is None:
            rem = _dot(w[:, DM:], h[DM:])
        else:
            rem = [qr_ref[...].T]
            if NV < TPB:
                R = GW * (TPB - NV) // 4
                rem.append(jnp.concatenate([_dot(w[a:a + R, DM:], h[DM:, NV * 128:])
                                            for a in range(0, GW, R)], axis=0))
            rem = jnp.concatenate(rem, axis=1)
        return _dot(w[:, :DM], h[:DM]) + rem

    def w_rest(u, wf_ref, gates=None):
        w = wrem_v[:, _lanes(_grp(u) * REP, REP)].astype(F32)
        for r in range(REP):
            wb = jnp.stack([jnp.broadcast_to(w[k:k + 1, r * DH:(r + 1) * DH], (8, DH))
                            for k in range(KR)])
            wf_ref[r] = _gated(wb, gates, r, REP)

    def outer(u, qr_ref, wf_ref, clock, start):
        base = jnp.bitwise_and(_blk(u), 1) * 16
        for g in range(0, NV * REP * 16, CH):
            pos = min(start + OSTEP * (g // CH + 1), clock.shape[0] - 8)
            runs, c = [], g
            while c < min(g + CH, NV * REP * 16):
                runs.append((c // 32, c // 16 % 2, c % 16, min(g + CH - c, 16 - c % 16)))
                c += runs[-1][3]
            acc = {}
            for k in range(KR):
                for i, r, tv, n in runs:
                    t = hb_refs[i][pl.ds(base + tv, n), k] * wf_ref[r, k][None]
                    acc[i, r] = t if k == 0 else acc[i, r] + t
            for i, r, tv, n in runs:
                gate = jnp.concatenate([clock[pos // 8 * 8:pos // 8 * 8 + 8]] * n, axis=0)
                row = i * 128 + tv * 8
                qr_ref[row:row + 8 * n, r * DH:(r + 1) * DH] = _paced(
                    acc[i, r].reshape(8 * n, DH), gate, 0)

    def h_table(hr, i, base, k0, gates):
        nk = hr.shape[0]
        for j in range(nk):
            cb = _col_bcast(hr[j:j + 1]).reshape(16, 8, 128)
            hb_refs[i][pl.ds(base, 16), k0 + j] = _gated(cb, gates, j, nk)

    def never_of(clock, lo, hi, step=8):
        return [clock[a:a + 8] * clock[a:a + 8] for a in range(lo // 8 * 8, hi, step)]

    def scores(u, q, s_ref, m_ref):
        s = _dot(_native(k_v, _grp(u)), q)
        s_ref[...] = s
        m_ref[...] = jnp.broadcast_to(jnp.max(s, axis=0, keepdims=True), m_ref.shape)
        return jnp.concatenate([s[:, 0:128], s[:, TQ:TQ + 128]], axis=0)

    def v_transpose(u, vt_ref, clock=None, pos=0):
        vt_ref[...] = _paced_wide(pltpu.bitcast(_native(v_v, _grp(u)).T, U32), clock, pos)

    def wq_transpose(u, wqt_ref, clock=None, pos=0):
        wqt_ref[...] = _paced_wide(pltpu.bitcast(wq_v[_grp(u)].T, U32), clock, pos)

    def wd_transpose(u, clock, pos):
        fb = jnp.clip(u - WD0, 0, NFB - 1)
        src = jnp.where(u >= WD0, NT + fb, 0)
        wd_ref[pl.ds(pl.multiple_of(fb * 64, 64), 64), :] = _paced_wide(
            pltpu.bitcast(_native(xw_v, src).T, U32), clock, pos)

    def attend(s_ref, m_ref, vt_ref):
        m = m_ref[0:1, :]
        o = []
        for r in range(REP):
            cols = slice(r * TQ, (r + 1) * TQ)
            p, l = _softmax_numer(s_ref[:, cols], m[:, cols])
            o.append((_dot(pltpu.bitcast(vt_ref[...], BF16), p) * (1.0 / l)))
        return jnp.concatenate(o, axis=0)

    small = Both([pltpu.make_async_copy(wr_hbm, wr_ref, msem.at[7]),
                  pltpu.make_async_copy(c_hbm, c_ref, msem.at[7])])
    zeroth = Both([cp_x(0, TPB, msem.at[5]), cp_w1(wq_hbm, wq_v, 0, msem.at[5])])
    first = Both([cp_k1(0, msem.at[8]), cp_w1(wq_hbm, wq_v, 1, msem.at[8])])
    second = Both([cp_k1(1, msem.at[9]), cp_v1(0, msem.at[9]), cp_w1(wq_hbm, wq_v, 2, msem.at[9]),
                   pltpu.make_async_copy(wq_hbm.at[DM:, :], wrem_v, msem.at[9]), cp_x(TPB, NV, msem.at[9])])
    for cp in [small, zeroth] + cp_moda + [first, second]:
        cp.start()
    acc_ref[...] = jnp.zeros_like(acc_ref)
    mod_ref[DA:6 * D, :] = jnp.zeros((4 * D, 128), F32)
    h2_ref[0] = jnp.zeros((D, 128), BF16)
    lm_ref[...] = jnp.zeros_like(lm_ref)
    small.wait()
    col_vector(wrb_ref, wr_ref[...].astype(F32).reshape(1, D))
    col_vector(scb_ref, silu_c())
    sc8 = jnp.broadcast_to(silu_c(), (8, D)).astype(BF16)
    zeroth.wait()
    ln0 = []
    for t in range(TPB):
        ln1_stats(t)
        ln0.append(ln1_norm(t))
    wq_transpose(0, wqt0_ref)
    for cp, tiles in zip(cp_moda, MODA):
        cp.wait()
        for t in tiles:
            finish_mod(_dot(sc8, wmod_v[:, t * 128:(t + 1) * 128])[0:1], t * 128)
    for t in range(TPB):
        ln1_apply(t, ln=ln0[t])
    q = finish_q(q_proj(0, wqt0_ref, split=True))
    first.wait()
    bundle(0, 'start')
    jobs = ([(i, 0, k) for i in range(NV) for k in range(0, KR, TPI)]
            + [(i, 1, k) for i in range(NV) for k in range(0, 2 * TPI, TPI)])

    def first_table(gates, todo, starts=None):
        for j, (i, blk, k0) in enumerate(todo):
            hr = ht_ref[blk * TPB + i, DM:, :].astype(F32)[k0:k0 + TPI]
            if starts is not None:
                hr = _r(jnp.where(starts[j * len(starts) // len(todo)] < 0.0, 0.0, hr))
            h_table(hr, i, blk * 16, k0,
                    gates[j * len(gates) // len(todo):(j + 1) * len(gates) // len(todo)])

    first_table(never_of(scores(0, q, s0_ref, m0_ref), 64, 2 * S - 192, 16), jobs[:TSPLIT])
    wq_transpose(1, wqt1_ref)
    second.wait()
    bundle(1, 'start')
    cp_modb.start()
    q = q_proj(1, wqt1_ref)
    hrem = jnp.concatenate([ht_ref[t, DM:, :] for t in range(NV)], axis=1)
    for a in range(2):
        streams[a][4][...] = jax.lax.dot_general(
            hrem, wrem_v[:, (a + 2) * GW:(a + 3) * GW], (((0,), (0,)), ((), ())),
            preferred_element_type=F32)
    clock = jnp.concatenate([q[:, t * 128:(t + 1) * 128] for t in range(TPB)]
                            + [scores(1, finish_q(q), s1_ref, m1_ref)], axis=0)
    nb0 = NV * KR // TPI
    v_transpose(0, vt0_ref, clock, PP[3])
    wq_transpose(2, wqt0_ref, clock, PP[4])
    first_table(never_of(clock, PP[6], PP[7], 16), jobs[TSPLIT:nb0])
    for i in range(NV):
        ln1_stats(TPB + i, clock, PP[0] + PP[5] * i)
        ln1_apply(TPB + i, clock, PP[1] + PP[5] * i)
    first_table(never_of(clock, PP[7], PP[2], 16), jobs[nb0:],
                never_of(clock, PP[7] - PP[8], PP[2] - PP[8]))
    for a in range(2):
        w_rest(a + 4, streams[a][5], never_of(clock, 500 * a, 500 * a + 500, 32))

    def unit(u, side, s_ref, m_ref, vt_ref, wqt_ref, qr_ref, wf_ref):
        q = q_proj(u + 2, wqt_ref, qr_ref)
        o = attend(s_ref, m_ref, vt_ref)
        sclk = scores(u + 2, finish_q(q), s_ref, m_ref)
        if OCAT:
            o = jnp.concatenate([o[r * DH:(r + 1) * DH].astype(BF16) for r in range(REP)], axis=0)
        upd = _dot(wot_v[_grp(u)], o.astype(BF16))
        clock = jnp.concatenate([q[:, t * 128:(t + 1) * 128] for t in range(TPB)] + [sclk]
                                + [upd[:, 0:128], upd[:, 256:384]], axis=0)
        side(clock, lambda start: outer(u + 4, qr_ref, wf_ref, clock, start))
        for t in range(TPB):
            acc_ref[_blk(u) * TPB + t] += upd[:, t * 128:(t + 1) * 128]

    def step(n, carry):
        def waits(_, c):
            bundle(n, 'wait')
            pl.when(n == MB0)(cp_modb.wait)
            pl.when(n == WD0 // 2)(cp_d.wait)
            return c
        jax.lax.fori_loop(0, jnp.where(n < NP, 1, 0), waits, 0)

        bundle(jnp.minimum(n + 2, NP), 'start')
        for a in range(3):
            pl.when(n == 2 + a)(Both(cp_d.cps[a * NFB // 3:(a + 1) * NFB // 3]).start)
        pl.when(n == NP)(Both([cp_g, cp_u]).start)

        t1 = jnp.minimum(n + TPB + NV - 1, NT - 1)
        v = jnp.maximum(n - NP, 0)
        tile2 = lambda v: (jax.lax.shift_right_logical(v, 3) * TPB
                           + jnp.minimum(jnp.bitwise_and(v, NP - 1), TPB - 1))
        t2 = tile2(v)
        sums = lm_ref[...]

        def stats(clock, outer_at):
            v_transpose(2 * n + 1, vt1_ref, clock, XP[5])
            wq_transpose(2 * n + 3, wqt1_ref, clock, XP[6])
            ln2_stats(t2, clock)
            ln1_stats(t1, clock)
            late_mod_sums(n, clock)
            h2_rows(tile2(jnp.maximum(v - 1, 0)), clock)
            wd_transpose(2 * n, clock, XP[0])
            outer_at(OUTER0[0])

        def apply(clock, outer_at):
            blk = jnp.minimum(jax.lax.shift_right_logical(n + 2, 3) + 1, NBLK - 1)
            k0 = jnp.bitwise_and(n + 2, 7) * TPI
            hr = [ht_ref[blk * TPB + i, pl.ds(pl.multiple_of(DM + k0, TPI), TPI), :].astype(F32)
                  for i in range(NV)]
            v_transpose(2 * n + 2, vt0_ref, clock, XP[1])
            wq_transpose(2 * n + 4, wqt0_ref, clock, XP[2])
            wd_transpose(2 * n + 1, clock, XP[3])
            ln1_apply(t1, clock)
            ln2_apply(t2, clock)
            outer_at(OUTER0[1])
            for i in range(NV):
                h_table(hr[i], i, jnp.bitwise_and(blk, 1) * 16, k0, never_of(clock, *TAB[i], 16))
            late_mod_store(n - 1, sums, clock)
            for a in range(2):
                w_rest(2 * n + 6 + a, streams[a][5], never_of(clock, *WFP[a], 32))

        for a in range(2):
            unit(2 * n + a, (stats, apply)[a], *streams[a])
        return carry

    jax.lax.fori_loop(0, NU // 2 - 1, step, 0)

    T0 = NT - TPB
    cp_out(0, T0, osem.at[C + TPB]).start()
    cp_g.wait()
    v_transpose(NU - 1, vt1_ref)
    o = jnp.concatenate([attend(*streams[a][0:3]) for a in range(2)], axis=0)
    wlast = jnp.concatenate([wot_v[HKV - 2], wot_v[HKV - 1]], axis=1)
    fin = [acc_ref[T0 + t] + _dot(wlast, o[:, t * 128:(t + 1) * 128].astype(BF16)) for t in range(TPB)]
    clock = jnp.concatenate(fin, axis=0)
    row8 = jax.lax.broadcasted_iota(jnp.int32, (C, 128), 0)
    lane8 = jax.lax.broadcasted_iota(jnp.int32, (C, 128), 1)
    work = key_ref[0:T0, :]
    lead = jnp.zeros((C, 128), F32)
    for t in range(C):
        mx = jnp.max(jnp.max(work, axis=0, keepdims=True), axis=1, keepdims=True)
        work = jnp.where(work == mx, 0.0, work)
        lead = jnp.where(row8 == t, mx, lead)

    def spread(row):
        return pltpu.roll(jnp.broadcast_to(row, (128, 128)), 0, 1, stride=1, stride_axis=0)

    def merge(lead, rows, spreads):
        cols = jnp.concatenate([lead] + spreads, axis=0)
        best = jnp.zeros((C, 128), F32)
        for row in [jnp.max(jnp.where(row8 == lane8, lead, 0.0), axis=0, keepdims=True)] + rows:
            rank = jnp.sum(jnp.where(cols > row, 1.0, 0.0), axis=0, keepdims=True)
            best = jnp.maximum(best, jnp.where(rank == row8.astype(F32), row, 0.0))
        return jnp.max(best, axis=1, keepdims=True)

    def tail_h2(t, norm, gate=None):
        x1 = x1_ref[t].astype(F32)
        if gate is not None:
            n = gate.shape[0]
            x1 = jnp.concatenate([_paced(x1[:n], gate, 0), x1[n:]], axis=0) if n < D else _paced(x1, gate, 0)
        h2_ref[t] = ln2_h2(x1, *norm).astype(BF16)
        if t < NT - 2:
            h2_rows(t)

    u_vec, u_sum, b_sum = router_terms()
    keys = []
    for t in range(TPB):
        x1, stats = ln2_x1(T0 + t, fin[t])
        mean, inv = norm = ln2_norm(stats)
        r = (jnp.sum(x1 * u_vec, axis=0, keepdims=True) - mean * u_sum) * inv + b_sum
        keys.append(_score_key(r, T0 + t))
        if t < TPB - 1:
            tail_h2(T0 + t, norm, clock[(t + 1) * D + TLAG:(t + 2) * D + TLAG])
    lead = jnp.broadcast_to(merge(lead, keys[0:2], [spread(k) for k in keys[0:2]]), (C, 128))
    spread2 = spread(keys[2])
    if BAR == 0:
        cp_u.wait()
        cp_out(0, T0, osem.at[C + TPB]).wait()

    h2_rows(NT - 2)
    tail_h2(NT - 1, norm)
    h2_rows(NT - 1)
    sel = pltpu.bitcast(merge(lead, keys[2:4], [spread2, spread(keys[3])]), jnp.int32) - KEY0
    sel_tok = (S - 1) - (sel & (S - 1))
    toks = [sel_tok[t, 0] for t in range(C)]
    tiles = [jax.lax.shift_right_logical(tk, 7) for tk in toks]
    sel_code = jax.lax.shift_right_logical(sel, 11) - 32768
    sel_bits = jnp.where(sel_code < 0, -32769 - sel_code, sel_code)
    r_sel = pltpu.bitcast(jax.lax.shift_left(sel_bits, 16), F32)

    final = []
    for t in range(C):
        d = True
        for u in range(t + 1, C):
            d = jnp.logical_and(d, tiles[u] != tiles[t])
        final.append(d)

    words = jnp.concatenate([h2row_ref[pl.ds(jax.lax.shift_right_logical(toks[t], 1), 1), :]
                             for t in range(C)], axis=0)
    odd = jnp.bitwise_and(sel_tok, 1) == 1
    xs = pltpu.bitcast(jnp.where(odd, jnp.bitwise_and(words, jnp.uint32(0xFFFF0000)),
                                 jax.lax.shift_left(words, jnp.uint32(16))), F32)
    xs = xs.astype(BF16)

    def plain_out(t, ticks=None):
        x1 = x1_ref[t].astype(F32)
        if ticks is not None:
            gate = jnp.concatenate([ticks[a * len(ticks) // (D // 8)] for a in range(D // 8)], axis=0)
            x1 = _paced(x1, gate, 0)
        out_v[t] = (x1 + mod(5) * h2_ref[t].astype(F32)).astype(BF16)

    clean = []

    def send_clean(t):
        d = tiles[0] != t
        for a in range(1, C):
            d = jnp.logical_and(d, tiles[a] != t)
        clean.append(d)
        pl.when(d)(cp_out(t, 1, osem.at[C + t - T0]).start)

    if BAR == 1:
        cp_u.wait()
        cp_out(0, T0, osem.at[C + TPB]).wait()
    gpre = _dot(xs, wg_v[...])
    u = _dot(xs, wu_v[...])
    ticks = [z[:, a * 128:(a + 1) * 128] for z in (gpre, u) for a in range(NFB)]
    for t in range(TPB):
        plain_out(T0 + t, ticks[t * TKS:(t + 1) * TKS])
        send_clean(T0 + t)
    gpre, u = _r(gpre), _r(u)
    gact = _r(gpre * _r(jax.nn.sigmoid(gpre)))
    act = (gact * u).astype(BF16)
    gate_r = _r(jax.nn.sigmoid(r_sel))
    ohs = []
    for t in range(C):
        oh = jnp.where(sel_tok == tiles[t] * 128 + lane8, 1.0, 0.0)
        ohs.append(jnp.concatenate([oh, jnp.zeros((16 - C, 128), F32)], axis=0).astype(BF16))

    def cp_fix(t, lo, hi):
        return pltpu.make_async_copy(fix_v.at[t, lo:hi, :], out_hbm.at[lo:hi, _lanes(tiles[t])],
                                     osem.at[t])

    def guarded(cond, fn):
        if cond is True:
            fn()
        else:
            pl.when(cond)(fn)

    def scatter(j, yt, t):
        lo, hi = j * 128, min(j * 128 + 128, D)
        upd = jnp.concatenate([_dot(yt[a:a + 64], ohs[t]) for a in range(0, hi - lo, 64)], axis=0)
        fix_v[t, lo:hi, :] = (x1_ref[tiles[t], lo:hi, :].astype(F32) + mod_ref[5 * D + lo:5 * D + hi, :]
                              * (h2_ref[tiles[t], lo:hi, :].astype(F32) + upd)).astype(BF16)
        guarded(final[t], cp_fix(t, lo, hi).start)

    NJ = (D + 127) // 128
    yts = []
    for j in range(NJ):
        lo, hi = j * 128, min(j * 128 + 128, D)
        nk = 4
        FK = F // nk
        yk = []
        for a in range(nk):
            w = pltpu.bitcast(wd_ref[a * FK // 2:(a + 1) * FK // 2, lo:hi], BF16)
            yk.append(_dot(act[:, a * FK:(a + 1) * FK], w))
            if j >= SCLAG:
                for t in (2 * a, 2 * a + 1):
                    scatter(j - SCLAG, yts[j - SCLAG], t)
        y = _r(sum(yk)) * gate_r
        yts.append(jnp.concatenate([y, jnp.zeros_like(y)], axis=0).astype(BF16).T)
    for j in range(NJ - SCLAG, NJ):
        for t in range(C):
            scatter(j, yts[j], t)
    for t in range(T0, NT):
        pl.when(clean[t - T0])(cp_out(t, 1, osem.at[C + t - T0]).wait)
    for t in range(C):
        guarded(final[t], cp_fix(t, 0, D).wait)


@jax.jit
def pallas_adaLN_cond__gqa_block_cached__moe_arch_mod__prompt_kernel(
    A_x: jax.Array,
    A_k_cache: jax.Array,
    A_v_cache: jax.Array,
    A_wq: jax.Array,
    A_wo: jax.Array,
    B_x: jax.Array,
    B_w_r: jax.Array,
    B_w_gate: jax.Array,
    B_w_up: jax.Array,
    B_w_down: jax.Array,
    c: jax.Array,
    w_mod: jax.Array,
):
    del B_x
    xt = A_x.reshape(S, D).T
    k = A_k_cache.reshape(HKV, S, DH)
    v = A_v_cache.reshape(HKV, S, DH)

    hbm = pl.BlockSpec(memory_space=pl.ANY)
    stream = [
        pltpu.VMEM((S, REP * TQ), F32),
        pltpu.VMEM((8, REP * TQ), F32),
        pltpu.VMEM((DH // 2, S), U32),
        pltpu.VMEM((GW // 2, D), U32),
        pltpu.VMEM((NV * 128, GW), F32),
        pltpu.VMEM((REP, KR, 8, DH), F32),
    ]
    out = pl.pallas_call(
        _kernel_flat,
        in_specs=[hbm] * 11,
        out_specs=hbm,
        out_shape=jax.ShapeDtypeStruct((D, S), BF16),
        scratch_shapes=[pltpu.VMEM((2 * 16, KR, 8, 128), F32)] * NV + [
            pltpu.VMEM((NT + NFB + NMB, D, 128), BF16),
            pltpu.VMEM((HKV, S, DH), BF16),
            pltpu.VMEM((HKV, S, DH), BF16),
            pltpu.VMEM((HKV, D, GW), BF16),
            pltpu.VMEM((HKV, D, GW), BF16),
            pltpu.VMEM((D, DA), BF16),
            pltpu.VMEM((D, F), BF16),
            pltpu.VMEM((D, F), BF16),
            pltpu.VMEM((F // 2, D), U32),
            pltpu.VMEM((NT, D, 128), BF16),
            pltpu.VMEM((NT, D, 128), F32),
            pltpu.VMEM((6 * D, 128), F32),
            pltpu.VMEM((5 * 128, 128), F32),
            pltpu.VMEM((5 * 128, 128), F32),
            pltpu.VMEM((NT, D, 128), BF16),
            pltpu.VMEM((NT, D, 128), BF16),
            pltpu.VMEM((S // 2, D), U32),
            pltpu.VMEM((NT, D, 128), BF16),
            pltpu.VMEM((C, D, 128), BF16),
            pltpu.VMEM((NT, 128), F32),
            pltpu.VMEM((NT * NC, 8, 128), F32),
            pltpu.VMEM((NT * NC, 8, 128), F32),
            pltpu.VMEM((MPI, 8, 128), F32),
            pltpu.VMEM((KR, HQ * DH), BF16),
        ] + stream + stream + [
            pltpu.VMEM((D,), BF16),
            pltpu.VMEM((1, D), BF16),
            pltpu.SemaphoreType.DMA((HKV // 2,)),
            pltpu.SemaphoreType.DMA((11,)),
            pltpu.SemaphoreType.DMA((C + TPB + 1,)),
        ],
        compiler_params=pltpu.CompilerParams(vmem_limit_bytes=127 * 1024 * 1024,
                                             disable_bounds_checks=True,
                                             disable_semaphore_checks=True),
    )(B_w_r, c, xt, k, v, A_wq, A_wo.T, w_mod, B_w_gate, B_w_up, B_w_down.T)
    return out.T.reshape(1, S, D)
```

```python
import math

import jax
import jax.numpy as jnp
import jax.experimental.pallas as pl
import jax.experimental.pallas.tpu as pltpu

S = 2048
D = 576
HQ = 32
HKV = 16
REP = HQ // HKV
DH = 128
GW = REP * DH
F = 4608
C = 8
EPS = 1e-05
TQ = 512
NBLK = S // TQ
TPB = TQ // 128
NT = S // 128
NU = NBLK * HKV
NP = HKV // 2
NC = 3
DC = D // NC
PG = 64
NFB = F // 128
WD0 = 14
DA = 2 * D
MODA = ((0, 4, 5), (1, 2, 6), (3, 7, 8))
NMB = 4 * D // 128
MPI = 3
MB0 = 1
DM = 512
KR = D - DM
NV = 3
CH = 3
TPI = KR // NP

QC, SC, WC = 0, 1024, 1024 + 2 * S
OUTER0, OSTEP = (SC + 890, SC + 0), 133
PACE = (100, WC + 160, SC + 100, WC + 250, 200, SC + 3300)
XP = (SC + 3700, SC + 100, SC + 900, SC + 1300, WC + 760, SC + 1200, SC + 2400)
TAB = ((SC + 1600, SC + 2800), (SC + 2850, SC + 3950), (WC + 250, WC + 890))
WFP = ((100, 800), (WC + 700, WC + 1040))
SLAG = 96
GS = 4
TSPLIT = 15
PP = (824, 1774, 5112, 100, 0, 300, 550, 3574, 300)
TLAG = 160
TKS = 18
SCLAG = 2

BF16 = jnp.bfloat16
F32 = jnp.float32
U32 = jnp.uint32
QSCALE = DH ** -0.5 * math.log2(math.e)


def _dot(a, b):
    return jnp.dot(a, b, preferred_element_type=F32)


def _r(x):
    return x.astype(BF16).astype(F32)


def _col_bcast(row):
    return jnp.broadcast_to(row, (128, 128)).T


def _blk(u):
    return u // HKV if isinstance(u, int) else jax.lax.shift_right_logical(u, 4)


def _grp(u):
    return u % HKV if isinstance(u, int) else jnp.bitwise_and(u, HKV - 1)


def _lanes(t, n=1):
    return pl.ds(pl.multiple_of(t * 128, 128), n * 128)


def _paced(x, clock, pos):
    if clock is None:
        return x
    pos = pos // 8 * 8
    g = clock[pos:pos + x.shape[0], 0:x.shape[1]]
    return jnp.where(g * g < 0.0, jnp.zeros_like(x), x)


def _paced_wide(x, clock, pos):
    if clock is None:
        return x
    n, w = x.shape
    cols = []
    for a in range(0, w, 128):
        p0 = (pos + a // 128 * n) // 8 * 8
        g = jnp.concatenate([clock[p0 + r // (8 * GS) * (8 * GS):p0 + r // (8 * GS) * (8 * GS) + 8]
                             for r in range(0, n, 8)], axis=0)
        cols.append(_paced(x[:, a:min(a + 128, w)], g, 0))
    return jnp.concatenate(cols, axis=1)


def _gated(x, gates, j, n):
    if gates is None:
        return x
    m = x.shape[0]
    g = jnp.stack([gates[(j * m + b) * len(gates) // (n * m)] for b in range(m)])
    return jnp.where(g < 0.0, 0.0, x)


def _native(ref, i):
    return pltpu.bitcast(ref.bitcast(U32)[i], BF16)


def _softmax_numer(s, m):
    n, w = s.shape
    p = jnp.exp2(s - m).reshape(n // PG, PG // 8, 8, w)
    ts = jnp.sum(p, axis=1)
    last = jnp.where(ts < 0.0, ts, p[:, PG // 8 - 1])
    p = jnp.concatenate([p[:, :PG // 8 - 1], last[:, None]], axis=1).reshape(n, w)
    l = jnp.sum(jnp.sum(ts, axis=0), axis=0, keepdims=True)
    return p.astype(BF16), l


KEY0 = 0x20000000


def _score_key(r, t):
    tok = t * 128 + jax.lax.broadcasted_iota(jnp.int32, r.shape, 1)
    bits = jax.lax.shift_right_arithmetic(pltpu.bitcast(_r(r) + 0.0, jnp.int32), 16)
    code = jnp.where(bits < 0, -32769 - bits, bits) + 32768
    return pltpu.bitcast(code * S + (S - 1 - tok) + KEY0, F32)


def _chunk_stats(x):
    m = jnp.sum(x, axis=0, keepdims=True) * (1.0 / DC)
    xc = x - m
    return m, jnp.sum(xc * xc, axis=0, keepdims=True)


def _mean_var(stats):
    mean = sum(m for m, _ in stats) * (1.0 / NC)
    var = sum(s + DC * (m - mean) * (m - mean) for m, s in stats) * (1.0 / D)
    return mean, var


def _kernel_flat(*refs):
    _kernel(*refs[:12], *refs[12 + NV:], *refs[12:12 + NV])


def _kernel(wr_hbm, c_hbm,
            xt_hbm, k_hbm, v_hbm, wq_hbm, wot_hbm, wmod_hbm, wg_hbm, wu_hbm, wdt_hbm,
            out_hbm,
            xw_v, k_v, v_v, wq_v, wot_v, wmod_v, wg_v, wu_v, wd_ref,
            ht_ref, acc_ref, mod_ref, wrb_ref, scb_ref, x1_ref, h2_ref, h2row_ref, out_v, fix_v,
            key_ref, st1_ref, st2_ref, lm_ref,
            wrem_v,
            s0_ref, m0_ref, vt0_ref, wqt0_ref, qr0_ref, wf0_ref,
            s1_ref, m1_ref, vt1_ref, wqt1_ref, qr1_ref, wf1_ref,
            wr_ref, c_ref, bsem, msem, osem, *hb_refs):
    streams = ((s0_ref, m0_ref, vt0_ref, wqt0_ref, qr0_ref, wf0_ref),
               (s1_ref, m1_ref, vt1_ref, wqt1_ref, qr1_ref, wf1_ref))

    def cp_cols(src, dst, t, n, sem, dst_t=None):
        return pltpu.make_async_copy(src.at[:, _lanes(t, n)],
                                     dst.at[:, _lanes(t if dst_t is None else dst_t, n)], sem)

    def cp_pair(src, dst, p, sem):
        return pltpu.make_async_copy(src.at[pl.ds(2 * p, 2)], dst.at[pl.ds(2 * p, 2)], sem)

    cp_k = lambda p, sem: cp_pair(k_hbm, k_v, p, sem)
    cp_v1 = lambda g, sem: pltpu.make_async_copy(v_hbm.at[g], v_v.at[g], sem)
    cp_k1 = lambda g, sem: pltpu.make_async_copy(k_hbm.at[g], k_v.at[g], sem)

    class Both:
        def __init__(self, cps):
            self.cps = cps

        def start(self):
            for cp in self.cps:
                cp.start()

        def wait(self):
            for cp in self.cps:
                cp.wait()

    def cp_w1(src, dst, g, sem):
        return pltpu.make_async_copy(src.at[:, _lanes(g * REP, REP)], dst.at[g], sem)

    def cp_w(src, dst, p, sem):
        return Both([cp_w1(src, dst, 2 * p + a, sem) for a in range(2)])

    cp_wo = lambda p, sem: cp_w(wot_hbm, wot_v, p, sem)
    cp_x = lambda t0, n, sem: Both([pltpu.make_async_copy(xt_hbm.at[:, _lanes(t0 + t)],
                                                          xw_v.at[t0 + t], sem) for t in range(n)])

    def bundle(n, act):
        sem = bsem.at[n if isinstance(n, int) else jnp.minimum(n, NP - 1)]

        def on(cond, cps):
            def go():
                for cp in cps():
                    getattr(cp, act)()
            if isinstance(cond, bool):
                if cond:
                    go()
            else:
                pl.when(cond)(go)
        on(n + 1 < NP, lambda: [cp_k(n + 1, sem), cp_v1(2 * n + 2, sem), cp_w1(wq_hbm, wq_v, 2 * n + 3, sem)])
        on(n + 2 < NP, lambda: [cp_w1(wq_hbm, wq_v, 2 * n + 4, sem)])
        XN = 3
        nx = (NT - TPB - NV) // XN
        on(jnp.logical_and(n >= 1, n <= nx) if not isinstance(n, int) else 1 <= n <= nx,
           lambda: [cp_x(TPB + NV + XN * (n - 1), XN, sem)])
        on(n < NP, lambda: [cp_v1(2 * n + 1, sem), cp_wo(n, sem)])

    cp_moda = [Both([cp_cols(wmod_hbm, wmod_v, t, 1, msem.at[s]) for t in tiles])
               for s, tiles in zip((0, 6, 10), MODA)]
    cp_modb = Both([pltpu.make_async_copy(wmod_hbm.at[:, _lanes(DA // 128 + b)],
                                          xw_v.at[NT + NFB + b], msem.at[1]) for b in range(NMB)])
    cp_g = pltpu.make_async_copy(wg_hbm, wg_v, msem.at[2])
    cp_u = pltpu.make_async_copy(wu_hbm, wu_v, msem.at[3])
    cp_d = Both([pltpu.make_async_copy(wdt_hbm.at[:, _lanes(b)], xw_v.at[NT + b], msem.at[4])
                 for b in range(NFB)])
    cp_out = lambda t, n, sem: Both([pltpu.make_async_copy(out_v.at[t + a], out_hbm.at[:, _lanes(t + a)],
                                                           sem) for a in range(n)])

    def silu_c():
        c = c_ref[...].astype(F32)
        return _r(c * _r(jax.nn.sigmoid(c)))

    def finish_mod(mod, lo, clock=None, pos=0):
        mod = _r(mod)
        col = lo + jax.lax.broadcasted_iota(jnp.int32, mod.shape, 1)
        is_scale = jnp.logical_or(jnp.logical_and(col >= D, col < 2 * D),
                                  jnp.logical_and(col >= 4 * D, col < 5 * D))
        mod = jnp.where(is_scale, _r(1.0 + mod), mod)
        for t in range(mod.shape[1] // 128):
            rows = pl.ds(pl.multiple_of(lo + t * 128, 128), 128)
            mod_ref[rows, :] = _paced(_col_bcast(mod[:, t * 128:(t + 1) * 128]), clock, pos)

    def late_mod_sums(n, clock):
        b0 = jnp.clip(n - MB0, 0, NMB // MPI - 1) * MPI
        for k in range(MPI):
            w = xw_v[jnp.where(n >= MB0, NT + NFB + b0 + k, 0)].astype(F32)
            part = jnp.sum((w * scb_ref[0:D, :]).reshape(D // 8, 8, 128), axis=0)
            lm_ref[k] = _paced(part, clock, PACE[4] + 192 * k)

    def late_mod_store(n, sums, clock):
        b0 = jnp.clip(n - MB0, 0, NMB // MPI - 1) * MPI
        for k in range(MPI):
            finish_mod(jnp.sum(sums[k], axis=0, keepdims=True), DA + (b0 + k) * 128,
                       clock, XP[4] + 128 * k)

    def col_vector(ref, row):
        row = jnp.concatenate([row, jnp.zeros((1, 64), F32)], axis=1)
        for t in range(5):
            ref[t * 128:(t + 1) * 128, :] = _col_bcast(row[:, t * 128:(t + 1) * 128])

    def mod(k):
        return mod_ref[k * D:(k + 1) * D, :]

    def put_stats(st_ref, t, shift, scale, clock, pos):
        row = jax.lax.broadcasted_iota(jnp.int32, (8, 128), 0)
        st_ref[t] = _paced(jnp.where(row == 0, shift, scale), clock, pos)

    def ln1_stats(t, clock=None, pos=None):
        for c in range(NC):
            m, s = _chunk_stats(xw_v[t, c * DC:(c + 1) * DC, :].astype(F32))
            put_stats(st1_ref, t * NC + c, m, s, clock, (PACE[0] if pos is None else pos) + 192 * c)

    def ln1_norm(t):
        mean, var = _mean_var(load_stats(st1_ref, t))
        return (xw_v[t].astype(F32) - mean) * jax.lax.rsqrt(var + EPS)

    def ln1_apply(t, clock=None, pos=None, ln=None):
        h = (ln1_norm(t) if ln is None else ln) * mod(1) + mod(0)
        ht_ref[t] = _paced(h, clock, PACE[1] if pos is None else pos).astype(BF16)

    def h2_rows(t, clock=None):
        x = _paced_wide(pltpu.bitcast(_native(h2_ref, t).T, U32), clock, PACE[5])
        h2row_ref[pl.ds(pl.multiple_of(t * 64, 64), 64), :] = x

    def router_terms():
        u = mod(4) * wrb_ref[0:D, :]
        return (u, jnp.sum(u, axis=0, keepdims=True),
                jnp.sum(mod(3) * wrb_ref[0:D, :], axis=0, keepdims=True))

    def load_stats(st_ref, t):
        return [(st_ref[t * NC + c, 0:1, :], st_ref[t * NC + c, 1:2, :]) for c in range(NC)]

    def ln2_x1(t, attn, clock=None):
        x1 = _r(xw_v[t].astype(F32) + mod(2) * attn)
        x1_ref[t] = _paced(x1, clock, PACE[2]).astype(BF16)
        return x1, [_chunk_stats(x1[c * DC:(c + 1) * DC]) for c in range(NC)]

    def ln2_norm(stats):
        mean, var = _mean_var(stats)
        return _r(mean), 1.0 / _r(jnp.sqrt(_r(_r(var) + EPS)))

    def ln2_h2(x1, mean, inv):
        return (x1 - mean) * inv * mod(4) + mod(3)

    def ln2_stats(t, clock):
        for c, (m, s) in enumerate(ln2_x1(t, acc_ref[t], clock)[1]):
            put_stats(st2_ref, t * NC + c, m, s, clock, PACE[2] + (c + 1) * DC + SLAG)

    def ln2_apply(t, clock):
        x1 = x1_ref[t].astype(F32)
        h2 = ln2_h2(x1, *ln2_norm(load_stats(st2_ref, t)))
        key = _score_key(jnp.sum(h2 * wrb_ref[0:D, :], axis=0, keepdims=True), t)
        key_ref[pl.ds(t, 1), :] = _paced(key, clock, PACE[3] + D + 96)
        h2 = _r(h2)
        h2_ref[t] = _paced(h2, clock, PACE[3]).astype(BF16)
        out_v[t] = _paced(x1 + mod(5) * h2, clock, PACE[3] + 16).astype(BF16)

    def finish_q(q):
        q = (q * QSCALE).astype(BF16)
        return jnp.concatenate([q[r * DH:(r + 1) * DH] for r in range(REP)], axis=1)

    def q_proj(u, wqt_ref, qr_ref=None, split=False):
        w = pltpu.bitcast(wqt_ref[...], BF16)
        h = jnp.concatenate([_native(ht_ref, _blk(u) * TPB + t) for t in range(TPB)], axis=1)
        if split:
            return sum(_dot(w[:, a:min(a + 128, D)], h[a:min(a + 128, D)]) for a in range(0, D, 128))
        if qr_ref is None:
            rem = _dot(w[:, DM:], h[DM:])
        else:
            rem = [qr_ref[...].T]
            if NV < TPB:
                R = GW * (TPB - NV) // 4
                rem.append(jnp.concatenate([_dot(w[a:a + R, DM:], h[DM:, NV * 128:])
                                            for a in range(0, GW, R)], axis=0))
            rem = jnp.concatenate(rem, axis=1)
        return _dot(w[:, :DM], h[:DM]) + rem

    def w_rest(u, wf_ref, gates=None):
        w = wrem_v[:, _lanes(_grp(u) * REP, REP)].astype(F32)
        for r in range(REP):
            wb = jnp.stack([jnp.broadcast_to(w[k:k + 1, r * DH:(r + 1) * DH], (8, DH))
                            for k in range(KR)])
            wf_ref[r] = _gated(wb, gates, r, REP)

    def outer(u, qr_ref, wf_ref, clock, start):
        base = jnp.bitwise_and(_blk(u), 1) * 16
        for g in range(0, NV * REP * 16, CH):
            pos = min(start + OSTEP * (g // CH + 1), clock.shape[0] - 8)
            runs, c = [], g
            while c < min(g + CH, NV * REP * 16):
                runs.append((c // 32, c // 16 % 2, c % 16, min(g + CH - c, 16 - c % 16)))
                c += runs[-1][3]
            acc = {}
            for k in range(KR):
                for i, r, tv, n in runs:
                    t = hb_refs[i][pl.ds(base + tv, n), k] * wf_ref[r, k][None]
                    acc[i, r] = t if k == 0 else acc[i, r] + t
            for i, r, tv, n in runs:
                gate = jnp.concatenate([clock[pos // 8 * 8:pos // 8 * 8 + 8]] * n, axis=0)
                row = i * 128 + tv * 8
                qr_ref[row:row + 8 * n, r * DH:(r + 1) * DH] = _paced(
                    acc[i, r].reshape(8 * n, DH), gate, 0)

    def h_table(hr, i, base, k0, gates):
        nk = hr.shape[0]
        for j in range(nk):
            cb = _col_bcast(hr[j:j + 1]).reshape(16, 8, 128)
            hb_refs[i][pl.ds(base, 16), k0 + j] = _gated(cb, gates, j, nk)

    def never_of(clock, lo, hi, step=8):
        return [clock[a:a + 8] * clock[a:a + 8] for a in range(lo // 8 * 8, hi, step)]

    def scores(u, q, s_ref, m_ref):
        s = _dot(_native(k_v, _grp(u)), q)
        s_ref[...] = s
        m_ref[...] = jnp.broadcast_to(jnp.max(s, axis=0, keepdims=True), m_ref.shape)
        return jnp.concatenate([s[:, 0:128], s[:, TQ:TQ + 128]], axis=0)

    def v_transpose(u, vt_ref, clock=None, pos=0):
        vt_ref[...] = _paced_wide(pltpu.bitcast(_native(v_v, _grp(u)).T, U32), clock, pos)

    def wq_transpose(u, wqt_ref, clock=None, pos=0):
        wqt_ref[...] = _paced_wide(pltpu.bitcast(wq_v[_grp(u)].T, U32), clock, pos)

    def wd_transpose(u, clock, pos):
        fb = jnp.clip(u - WD0, 0, NFB - 1)
        src = jnp.where(u >= WD0, NT + fb, 0)
        wd_ref[pl.ds(pl.multiple_of(fb * 64, 64), 64), :] = _paced_wide(
            pltpu.bitcast(_native(xw_v, src).T, U32), clock, pos)

    def attend(s_ref, m_ref, vt_ref):
        m = m_ref[0:1, :]
        o = []
        for r in range(REP):
            cols = slice(r * TQ, (r + 1) * TQ)
            p, l = _softmax_numer(s_ref[:, cols], m[:, cols])
            o.append((_dot(pltpu.bitcast(vt_ref[...], BF16), p) * (1.0 / l)))
        return jnp.concatenate(o, axis=0)

    small = Both([pltpu.make_async_copy(wr_hbm, wr_ref, msem.at[7]),
                  pltpu.make_async_copy(c_hbm, c_ref, msem.at[7])])
    zeroth = Both([cp_x(0, TPB, msem.at[5]), cp_w1(wq_hbm, wq_v, 0, msem.at[5])])
    first = Both([cp_k1(0, msem.at[8]), cp_w1(wq_hbm, wq_v, 1, msem.at[8])])
    second = Both([cp_k1(1, msem.at[9]), cp_v1(0, msem.at[9]), cp_w1(wq_hbm, wq_v, 2, msem.at[9]),
                   pltpu.make_async_copy(wq_hbm.at[DM:, :], wrem_v, msem.at[9]), cp_x(TPB, NV, msem.at[9])])
    for cp in [small, zeroth] + cp_moda + [first, second]:
        cp.start()
    acc_ref[...] = jnp.zeros_like(acc_ref)
    mod_ref[DA:6 * D, :] = jnp.zeros((4 * D, 128), F32)
    h2_ref[0] = jnp.zeros((D, 128), BF16)
    lm_ref[...] = jnp.zeros_like(lm_ref)
    small.wait()
    col_vector(wrb_ref, wr_ref[...].astype(F32).reshape(1, D))
    col_vector(scb_ref, silu_c())
    sc8 = jnp.broadcast_to(silu_c(), (8, D)).astype(BF16)
    zeroth.wait()
    ln0 = []
    for t in range(TPB):
        ln1_stats(t)
        ln0.append(ln1_norm(t))
    wq_transpose(0, wqt0_ref)
    for cp, tiles in zip(cp_moda, MODA):
        cp.wait()
        for t in tiles:
            finish_mod(_dot(sc8, wmod_v[:, t * 128:(t + 1) * 128])[0:1], t * 128)
    for t in range(TPB):
        ln1_apply(t, ln=ln0[t])
    q = finish_q(q_proj(0, wqt0_ref, split=True))
    first.wait()
    bundle(0, 'start')
    jobs = ([(i, 0, k) for i in range(NV) for k in range(0, KR, TPI)]
            + [(i, 1, k) for i in range(NV) for k in range(0, 2 * TPI, TPI)])

    def first_table(gates, todo, starts=None):
        for j, (i, blk, k0) in enumerate(todo):
            hr = ht_ref[blk * TPB + i, DM:, :].astype(F32)[k0:k0 + TPI]
            if starts is not None:
                hr = _r(jnp.where(starts[j * len(starts) // len(todo)] < 0.0, 0.0, hr))
            h_table(hr, i, blk * 16, k0,
                    gates[j * len(gates) // len(todo):(j + 1) * len(gates) // len(todo)])

    first_table(never_of(scores(0, q, s0_ref, m0_ref), 64, 2 * S - 192, 16), jobs[:TSPLIT])
    wq_transpose(1, wqt1_ref)
    second.wait()
    bundle(1, 'start')
    cp_modb.start()
    q = q_proj(1, wqt1_ref)
    hrem = jnp.concatenate([ht_ref[t, DM:, :] for t in range(NV)], axis=1)
    for a in range(2):
        streams[a][4][...] = jax.lax.dot_general(
            hrem, wrem_v[:, (a + 2) * GW:(a + 3) * GW], (((0,), (0,)), ((), ())),
            preferred_element_type=F32)
    clock = jnp.concatenate([q[:, t * 128:(t + 1) * 128] for t in range(TPB)]
                            + [scores(1, finish_q(q), s1_ref, m1_ref)], axis=0)
    nb0 = NV * KR // TPI
    v_transpose(0, vt0_ref, clock, PP[3])
    wq_transpose(2, wqt0_ref, clock, PP[4])
    first_table(never_of(clock, PP[6], PP[7], 16), jobs[TSPLIT:nb0])
    for i in range(NV):
        ln1_stats(TPB + i, clock, PP[0] + PP[5] * i)
        ln1_apply(TPB + i, clock, PP[1] + PP[5] * i)
    first_table(never_of(clock, PP[7], PP[2], 16), jobs[nb0:],
                never_of(clock, PP[7] - PP[8], PP[2] - PP[8]))
    for a in range(2):
        w_rest(a + 4, streams[a][5], never_of(clock, 500 * a, 500 * a + 500, 32))

    def unit(u, side, s_ref, m_ref, vt_ref, wqt_ref, qr_ref, wf_ref):
        q = q_proj(u + 2, wqt_ref, qr_ref)
        o = attend(s_ref, m_ref, vt_ref)
        sclk = scores(u + 2, finish_q(q), s_ref, m_ref)
        o = jnp.concatenate([o[r * DH:(r + 1) * DH].astype(BF16) for r in range(REP)], axis=0)
        upd = _dot(wot_v[_grp(u)], o)
        clock = jnp.concatenate([q[:, t * 128:(t + 1) * 128] for t in range(TPB)] + [sclk]
                                + [upd[:, 0:128], upd[:, 256:384]], axis=0)
        side(clock, lambda start: outer(u + 4, qr_ref, wf_ref, clock, start))
        for t in range(TPB):
            acc_ref[_blk(u) * TPB + t] += upd[:, t * 128:(t + 1) * 128]

    def step(n, carry):
        bundle(jnp.minimum(n + 2, NP), 'start')
        for a in range(3):
            pl.when(n == 2 + a)(Both(cp_d.cps[a * NFB // 3:(a + 1) * NFB // 3]).start)
        pl.when(n == NP)(Both([cp_g, cp_u]).start)

        t1 = jnp.minimum(n + TPB + NV - 1, NT - 1)
        v = jnp.maximum(n - NP, 0)
        tile2 = lambda v: (jax.lax.shift_right_logical(v, 3) * TPB
                           + jnp.minimum(jnp.bitwise_and(v, NP - 1), TPB - 1))
        t2 = tile2(v)
        sums = lm_ref[...]

        def stats(clock, outer_at):
            v_transpose(2 * n + 1, vt1_ref, clock, XP[5])
            wq_transpose(2 * n + 3, wqt1_ref, clock, XP[6])
            ln2_stats(t2, clock)
            ln1_stats(t1, clock)
            late_mod_sums(n, clock)
            h2_rows(tile2(jnp.maximum(v - 1, 0)), clock)
            wd_transpose(2 * n, clock, XP[0])
            outer_at(OUTER0[0])

        def apply(clock, outer_at):
            blk = jnp.minimum(jax.lax.shift_right_logical(n + 2, 3) + 1, NBLK - 1)
            k0 = jnp.bitwise_and(n + 2, 7) * TPI
            hr = [ht_ref[blk * TPB + i, pl.ds(pl.multiple_of(DM + k0, TPI), TPI), :].astype(F32)
                  for i in range(NV)]
            v_transpose(2 * n + 2, vt0_ref, clock, XP[1])
            wq_transpose(2 * n + 4, wqt0_ref, clock, XP[2])
            wd_transpose(2 * n + 1, clock, XP[3])
            ln1_apply(t1, clock)
            ln2_apply(t2, clock)
            outer_at(OUTER0[1])
            for i in range(NV):
                h_table(hr[i], i, jnp.bitwise_and(blk, 1) * 16, k0, never_of(clock, *TAB[i], 16))
            late_mod_store(n - 1, sums, clock)
            for a in range(2):
                w_rest(2 * n + 6 + a, streams[a][5], never_of(clock, *WFP[a], 32))

        for a in range(2):
            unit(2 * n + a, (stats, apply)[a], *streams[a])
        return carry

    def stage(n, carry):
        bundle(n, 'wait')
        pl.when(n == MB0)(cp_modb.wait)
        pl.when(n == WD0 // 2)(cp_d.wait)
        return jax.lax.fori_loop(n, jnp.where(n < NP - 1, n + 1, NU // 2 - 1), step, carry)

    jax.lax.fori_loop(0, NP, stage, 0)

    T0 = NT - TPB
    cp_out(0, T0, osem.at[C + TPB]).start()
    cp_g.wait()
    v_transpose(NU - 1, vt1_ref)
    o = jnp.concatenate([attend(*streams[a][0:3]) for a in range(2)], axis=0)
    wlast = jnp.concatenate([wot_v[HKV - 2], wot_v[HKV - 1]], axis=1)
    fin = [acc_ref[T0 + t] + _dot(wlast, o[:, t * 128:(t + 1) * 128].astype(BF16)) for t in range(TPB)]
    clock = jnp.concatenate(fin, axis=0)
    row8 = jax.lax.broadcasted_iota(jnp.int32, (C, 128), 0)
    lane8 = jax.lax.broadcasted_iota(jnp.int32, (C, 128), 1)
    work = key_ref[0:T0, :]
    lead = jnp.zeros((C, 128), F32)
    for t in range(C):
        mx = jnp.max(jnp.max(work, axis=0, keepdims=True), axis=1, keepdims=True)
        work = jnp.where(work == mx, 0.0, work)
        lead = jnp.where(row8 == t, mx, lead)

    def spread(row):
        return pltpu.roll(jnp.broadcast_to(row, (128, 128)), 0, 1, stride=1, stride_axis=0)

    def merge(lead, rows, spreads):
        cols = jnp.concatenate([lead] + spreads, axis=0)
        best = jnp.zeros((C, 128), F32)
        for row in [jnp.max(jnp.where(row8 == lane8, lead, 0.0), axis=0, keepdims=True)] + rows:
            rank = jnp.sum(jnp.where(cols > row, 1.0, 0.0), axis=0, keepdims=True)
            best = jnp.maximum(best, jnp.where(rank == row8.astype(F32), row, 0.0))
        return jnp.max(best, axis=1, keepdims=True)

    def tail_h2(t, norm, gate=None):
        x1 = x1_ref[t].astype(F32)
        if gate is not None:
            n = gate.shape[0]
            x1 = jnp.concatenate([_paced(x1[:n], gate, 0), x1[n:]], axis=0) if n < D else _paced(x1, gate, 0)
        h2_ref[t] = ln2_h2(x1, *norm).astype(BF16)
        if t < NT - 2:
            h2_rows(t)

    u_vec, u_sum, b_sum = router_terms()
    keys = []
    for t in range(TPB):
        x1, stats = ln2_x1(T0 + t, fin[t])
        mean, inv = norm = ln2_norm(stats)
        r = (jnp.sum(x1 * u_vec, axis=0, keepdims=True) - mean * u_sum) * inv + b_sum
        keys.append(_score_key(r, T0 + t))
        if t < TPB - 1:
            tail_h2(T0 + t, norm, clock[(t + 1) * D + TLAG:(t + 2) * D + TLAG])
    lead = jnp.broadcast_to(merge(lead, keys[0:2], [spread(k) for k in keys[0:2]]), (C, 128))
    spread2 = spread(keys[2])
    h2_rows(NT - 2)
    tail_h2(NT - 1, norm)
    h2_rows(NT - 1)
    sel = pltpu.bitcast(merge(lead, keys[2:4], [spread2, spread(keys[3])]), jnp.int32) - KEY0
    sel_tok = (S - 1) - (sel & (S - 1))
    toks = [sel_tok[t, 0] for t in range(C)]
    tiles = [jax.lax.shift_right_logical(tk, 7) for tk in toks]
    sel_code = jax.lax.shift_right_logical(sel, 11) - 32768
    sel_bits = jnp.where(sel_code < 0, -32769 - sel_code, sel_code)
    r_sel = pltpu.bitcast(jax.lax.shift_left(sel_bits, 16), F32)

    final = []
    for t in range(C):
        d = True
        for u in range(t + 1, C):
            d = jnp.logical_and(d, tiles[u] != tiles[t])
        final.append(d)

    words = jnp.concatenate([h2row_ref[pl.ds(jax.lax.shift_right_logical(toks[t], 1), 1), :]
                             for t in range(C)], axis=0)
    odd = jnp.bitwise_and(sel_tok, 1) == 1
    xs = pltpu.bitcast(jnp.where(odd, jnp.bitwise_and(words, jnp.uint32(0xFFFF0000)),
                                 jax.lax.shift_left(words, jnp.uint32(16))), F32)
    xs = xs.astype(BF16)

    def plain_out(t, ticks):
        gate = jnp.concatenate([ticks[a * len(ticks) // (D // 8)] for a in range(D // 8)], axis=0)
        x1 = _paced(x1_ref[t].astype(F32), gate, 0)
        out_v[t] = (x1 + mod(5) * h2_ref[t].astype(F32)).astype(BF16)

    clean = []

    def send_clean(t):
        d = tiles[0] != t
        for a in range(1, C):
            d = jnp.logical_and(d, tiles[a] != t)
        clean.append(d)
        pl.when(d)(cp_out(t, 1, osem.at[C + t - T0]).start)

    cp_u.wait()
    cp_out(0, T0, osem.at[C + TPB]).wait()
    gpre = _dot(xs, wg_v[...])
    u = _dot(xs, wu_v[...])
    ticks = [z[:, a * 128:(a + 1) * 128] for z in (gpre, u) for a in range(NFB)]
    for t in range(TPB):
        plain_out(T0 + t, ticks[t * TKS:(t + 1) * TKS])
        send_clean(T0 + t)
    gpre, u = _r(gpre), _r(u)
    gact = _r(gpre * _r(jax.nn.sigmoid(gpre)))
    act = (gact * u).astype(BF16)
    gate_r = _r(jax.nn.sigmoid(r_sel))
    ohs = []
    for t in range(C):
        oh = jnp.where(sel_tok == tiles[t] * 128 + lane8, 1.0, 0.0)
        ohs.append(jnp.concatenate([oh, jnp.zeros((16 - C, 128), F32)], axis=0).astype(BF16))

    def cp_fix(t, lo, hi):
        return pltpu.make_async_copy(fix_v.at[t, lo:hi, :], out_hbm.at[lo:hi, _lanes(tiles[t])],
                                     osem.at[t])

    def guarded(cond, fn):
        if cond is True:
            fn()
        else:
            pl.when(cond)(fn)

    def scatter(j, yt, t):
        lo, hi = j * 128, min(j * 128 + 128, D)
        upd = jnp.concatenate([_dot(yt[a:a + 64], ohs[t]) for a in range(0, hi - lo, 64)], axis=0)
        fix_v[t, lo:hi, :] = (x1_ref[tiles[t], lo:hi, :].astype(F32) + mod_ref[5 * D + lo:5 * D + hi, :]
                              * (h2_ref[tiles[t], lo:hi, :].astype(F32) + upd)).astype(BF16)
        guarded(final[t], cp_fix(t, lo, hi).start)

    NJ = (D + 127) // 128
    yts = []
    for j in range(NJ):
        lo, hi = j * 128, min(j * 128 + 128, D)
        FK = F // 4
        yk = []
        for a in range(4):
            w = pltpu.bitcast(wd_ref[a * FK // 2:(a + 1) * FK // 2, lo:hi], BF16)
            yk.append(_dot(act[:, a * FK:(a + 1) * FK], w))
            if j >= SCLAG:
                for t in (2 * a, 2 * a + 1):
                    scatter(j - SCLAG, yts[j - SCLAG], t)
        y = _r(sum(yk)) * gate_r
        yts.append(jnp.concatenate([y, jnp.zeros_like(y)], axis=0).astype(BF16).T)
    for j in range(NJ - SCLAG, NJ):
        for t in range(C):
            scatter(j, yts[j], t)
    for t in range(T0, NT):
        pl.when(clean[t - T0])(cp_out(t, 1, osem.at[C + t - T0]).wait)
    for t in range(C):
        guarded(final[t], cp_fix(t, 0, D).wait)


@jax.jit
def pallas_adaLN_cond__gqa_block_cached__moe_arch_mod__prompt_kernel(
    A_x: jax.Array,
    A_k_cache: jax.Array,
    A_v_cache: jax.Array,
    A_wq: jax.Array,
    A_wo: jax.Array,
    B_x: jax.Array,
    B_w_r: jax.Array,
    B_w_gate: jax.Array,
    B_w_up: jax.Array,
    B_w_down: jax.Array,
    c: jax.Array,
    w_mod: jax.Array,
):
    del B_x
    xt = A_x.reshape(S, D).T
    k = A_k_cache.reshape(HKV, S, DH)
    v = A_v_cache.reshape(HKV, S, DH)

    hbm = pl.BlockSpec(memory_space=pl.ANY)
    stream = [
        pltpu.VMEM((S, REP * TQ), F32),
        pltpu.VMEM((8, REP * TQ), F32),
        pltpu.VMEM((DH // 2, S), U32),
        pltpu.VMEM((GW // 2, D), U32),
        pltpu.VMEM((NV * 128, GW), F32),
        pltpu.VMEM((REP, KR, 8, DH), F32),
    ]
    out = pl.pallas_call(
        _kernel_flat,
        in_specs=[hbm] * 11,
        out_specs=hbm,
        out_shape=jax.ShapeDtypeStruct((D, S), BF16),
        scratch_shapes=[pltpu.VMEM((2 * 16, KR, 8, 128), F32)] * NV + [
            pltpu.VMEM((NT + NFB + NMB, D, 128), BF16),
            pltpu.VMEM((HKV, S, DH), BF16),
            pltpu.VMEM((HKV, S, DH), BF16),
            pltpu.VMEM((HKV, D, GW), BF16),
            pltpu.VMEM((HKV, D, GW), BF16),
            pltpu.VMEM((D, DA), BF16),
            pltpu.VMEM((D, F), BF16),
            pltpu.VMEM((D, F), BF16),
            pltpu.VMEM((F // 2, D), U32),
            pltpu.VMEM((NT, D, 128), BF16),
            pltpu.VMEM((NT, D, 128), F32),
            pltpu.VMEM((6 * D, 128), F32),
            pltpu.VMEM((5 * 128, 128), F32),
            pltpu.VMEM((5 * 128, 128), F32),
            pltpu.VMEM((NT, D, 128), BF16),
            pltpu.VMEM((NT, D, 128), BF16),
            pltpu.VMEM((S // 2, D), U32),
            pltpu.VMEM((NT, D, 128), BF16),
            pltpu.VMEM((C, D, 128), BF16),
            pltpu.VMEM((NT, 128), F32),
            pltpu.VMEM((NT * NC, 8, 128), F32),
            pltpu.VMEM((NT * NC, 8, 128), F32),
            pltpu.VMEM((MPI, 8, 128), F32),
            pltpu.VMEM((KR, HQ * DH), BF16),
        ] + stream + stream + [
            pltpu.VMEM((D,), BF16),
            pltpu.VMEM((1, D), BF16),
            pltpu.SemaphoreType.DMA((HKV // 2,)),
            pltpu.SemaphoreType.DMA((11,)),
            pltpu.SemaphoreType.DMA((C + TPB + 1,)),
        ],
        compiler_params=pltpu.CompilerParams(vmem_limit_bytes=127 * 1024 * 1024,
                                             disable_bounds_checks=True,
                                             disable_semaphore_checks=True),
    )(B_w_r, c, xt, k, v, A_wq, A_wo.T, w_mod, B_w_gate, B_w_up, B_w_down.T)
    return out.T.reshape(1, S, D)
```

```python
import math

import jax
import jax.numpy as jnp
import jax.experimental.pallas as pl
import jax.experimental.pallas.tpu as pltpu

S = 2048
D = 576
HQ = 32
HKV = 16
REP = HQ // HKV
DH = 128
GW = REP * DH
F = 4608
C = 8
EPS = 1e-05
TQ = 512
NBLK = S // TQ
TPB = TQ // 128
NT = S // 128
NU = NBLK * HKV
NP = HKV // 2
NC = 3
DC = D // NC
PG = 64
NFB = F // 128
WD0 = 14
DA = 2 * D
MODA = ((0, 4, 5), (1, 2, 6), (3, 7, 8))
NMB = 4 * D // 128
MPI = 3
MB0 = 1
DM = 512
KR = D - DM
NV = 3
CH = 3
TPI = KR // NP

QC, SC, WC = 0, 1024, 1024 + 2 * S
OUTER0, OSTEP = (SC + 850, SC + 0), 133
PACE = (100, WC + 160, SC + 100, WC + 250, 0, SC + 3400)
XP = (SC + 3700, SC + 100, SC + 900, SC + 1300, WC + 762, 724, SC + 2600)
TAB = ((SC + 1600, SC + 2600), (SC + 2950, SC + 3890), (WC + 650, WC + 890))
WFP = ((300, 900), (WC + 600, WC + 1144))
KP = (0, 616)
SLAG = 96
LMB = 1
GS = 4
TSPLIT = 15
PP = (24, 1474, 5112, 0, 0, 500, 750, 3524, 300)
TLAG = 160
TKS = 18
SCLAG = 2

BF16 = jnp.bfloat16
F32 = jnp.float32
U32 = jnp.uint32
QSCALE = DH ** -0.5 * math.log2(math.e)


def _dot(a, b):
    return jnp.dot(a, b, preferred_element_type=F32)


def _r(x):
    return x.astype(BF16).astype(F32)


def _col_bcast(row):
    return jnp.broadcast_to(row, (128, 128)).T


def _blk(u):
    return u // HKV if isinstance(u, int) else jax.lax.shift_right_logical(u, 4)


def _grp(u):
    return u % HKV if isinstance(u, int) else jnp.bitwise_and(u, HKV - 1)


def _lanes(t, n=1):
    return pl.ds(pl.multiple_of(t * 128, 128), n * 128)


def _paced(x, clock, pos):
    if clock is None:
        return x
    pos = pos // 8 * 8
    g = clock[pos:pos + x.shape[0], 0:x.shape[1]]
    return jnp.where(g * g < 0.0, jnp.zeros_like(x), x)


def _paced_wide(x, clock, pos):
    if clock is None:
        return x
    n, w = x.shape
    cols = []
    for a in range(0, w, 128):
        p0 = (pos + a // 128 * n) // 8 * 8
        g = jnp.concatenate([clock[p0 + r // (8 * GS) * (8 * GS):p0 + r // (8 * GS) * (8 * GS) + 8]
                             for r in range(0, n, 8)], axis=0)
        cols.append(_paced(x[:, a:min(a + 128, w)], g, 0))
    return jnp.concatenate(cols, axis=1)


def _gated(x, gates, j, n):
    if gates is None:
        return x
    m = x.shape[0]
    g = jnp.stack([gates[(j * m + b) * len(gates) // (n * m)] for b in range(m)])
    return jnp.where(g < 0.0, jnp.zeros_like(x), x)


def _softmax_numer(s, m):
    n, w = s.shape
    p = jnp.exp2(s - m).reshape(n // PG, PG // 8, 8, w)
    ts = jnp.sum(p, axis=1)
    last = jnp.where(ts < 0.0, ts, p[:, PG // 8 - 1])
    p = jnp.concatenate([p[:, :PG // 8 - 1], last[:, None]], axis=1).reshape(n, w)
    l = jnp.sum(jnp.sum(ts, axis=0), axis=0, keepdims=True)
    return p.astype(BF16), l


KEY0 = 0x20000000


def _score_key(r, t):
    tok = t * 128 + jax.lax.broadcasted_iota(jnp.int32, r.shape, 1)
    bits = jax.lax.shift_right_arithmetic(pltpu.bitcast(_r(r) + 0.0, jnp.int32), 16)
    code = jnp.where(bits < 0, -32769 - bits, bits) + 32768
    return pltpu.bitcast(code * S + (S - 1 - tok) + KEY0, F32)


def _chunk_stats(x):
    m = jnp.sum(x, axis=0, keepdims=True) * (1.0 / DC)
    xc = x - m
    return m, jnp.sum(xc * xc, axis=0, keepdims=True)


def _mean_var(stats):
    mean = sum(m for m, _ in stats) * (1.0 / NC)
    var = sum(s + DC * (m - mean) * (m - mean) for m, s in stats) * (1.0 / D)
    return mean, var


def _kernel_flat(*refs):
    _kernel(*refs[:12], *refs[12 + NV:], *refs[12:12 + NV])


def _kernel(wr_hbm, c_hbm,
            xt_hbm, k_hbm, v_hbm, wq_hbm, wot_hbm, wmod_hbm, wg_hbm, wu_hbm, wdt_hbm,
            out_hbm,
            xw_v, k_v, v_v, wq_v, wot_v, wmod_v, wg_v, wu_v, wd_ref,
            ht_ref, hr_ref, acc_ref, mod_ref, wrb_ref, scb_ref, x1_ref, h2_ref, h2row_ref, out_v, fix_v,
            key_ref, st1_ref, st2_ref, lm_ref,
            wrem_v,
            s0_ref, m0_ref, vt0_ref, wqt0_ref, qr0_ref, wf0_ref, kp0_ref,
            s1_ref, m1_ref, vt1_ref, wqt1_ref, qr1_ref, wf1_ref, kp1_ref,
            wr_ref, c_ref, bsem, msem, osem, *hb_refs):
    streams = ((s0_ref, m0_ref, vt0_ref, wqt0_ref, qr0_ref, wf0_ref, kp0_ref),
               (s1_ref, m1_ref, vt1_ref, wqt1_ref, qr1_ref, wf1_ref, kp1_ref))

    def cp_cols(src, dst, t, n, sem, dst_t=None):
        return pltpu.make_async_copy(src.at[:, _lanes(t, n)],
                                     dst.at[:, _lanes(t if dst_t is None else dst_t, n)], sem)

    def cp_pair(src, dst, p, sem):
        return pltpu.make_async_copy(src.at[pl.ds(2 * p, 2)], dst.at[pl.ds(2 * p, 2)], sem)

    cp_k = lambda p, sem: cp_pair(k_hbm, k_v, p, sem)
    cp_v1 = lambda g, sem: pltpu.make_async_copy(v_hbm.at[g], v_v.at[g], sem)
    cp_k1 = lambda g, sem: pltpu.make_async_copy(k_hbm.at[g], k_v.at[g], sem)

    class Both:
        def __init__(self, cps):
            self.cps = cps

        def start(self):
            for cp in self.cps:
                cp.start()

        def wait(self):
            for cp in self.cps:
                cp.wait()

    def cp_w1(src, dst, g, sem):
        return pltpu.make_async_copy(src.at[:, _lanes(g * REP, REP)], dst.at[g], sem)

    def cp_w(src, dst, p, sem):
        return Both([cp_w1(src, dst, 2 * p + a, sem) for a in range(2)])

    cp_wo = lambda p, sem: cp_w(wot_hbm, wot_v, p, sem)
    cp_x = lambda t0, n, sem: Both([pltpu.make_async_copy(xt_hbm.at[:, _lanes(t0 + t)],
                                                          xw_v.at[t0 + t], sem) for t in range(n)])

    def bundle(n, act):
        sem = bsem.at[n if isinstance(n, int) else jnp.minimum(n, NP - 1)]

        def on(cond, cps):
            def go():
                for cp in cps():
                    getattr(cp, act)()
            if isinstance(cond, bool):
                if cond:
                    go()
            else:
                pl.when(cond)(go)
        on(n + 1 < NP, lambda: [cp_k(n + 1, sem), cp_v1(2 * n + 2, sem), cp_w1(wq_hbm, wq_v, 2 * n + 3, sem)])
        on(n + 2 < NP, lambda: [cp_w1(wq_hbm, wq_v, 2 * n + 4, sem)])
        XN = 3
        nx = (NT - TPB - NV) // XN
        on(jnp.logical_and(n >= 1, n <= nx) if not isinstance(n, int) else 1 <= n <= nx,
           lambda: [cp_x(TPB + NV + XN * (n - 1), XN, sem)])
        on(n < NP, lambda: [cp_v1(2 * n + 1, sem), cp_wo(n, sem)])

    cp_moda = [Both([cp_cols(wmod_hbm, wmod_v, t, 1, msem.at[s]) for t in tiles])
               for s, tiles in zip((0, 6, 10), MODA)]
    cp_modb = Both([pltpu.make_async_copy(wmod_hbm.at[:, _lanes(DA // 128 + b)],
                                          xw_v.at[NT + NFB + b], msem.at[1]) for b in range(NMB)])
    cp_g = pltpu.make_async_copy(wg_hbm, wg_v, msem.at[2])
    cp_u = pltpu.make_async_copy(wu_hbm, wu_v, msem.at[3])
    cp_d = Both([pltpu.make_async_copy(wdt_hbm.at[:, _lanes(b)], xw_v.at[NT + b], msem.at[4])
                 for b in range(NFB)])
    cp_out = lambda t, n, sem: Both([pltpu.make_async_copy(out_v.at[t + a], out_hbm.at[:, _lanes(t + a)],
                                                           sem) for a in range(n)])

    def silu_c():
        c = c_ref[...].astype(F32)
        return _r(c * _r(jax.nn.sigmoid(c)))

    def finish_mod(mod, lo, clock=None, pos=0):
        mod = _r(mod)
        col = lo + jax.lax.broadcasted_iota(jnp.int32, mod.shape, 1)
        is_scale = jnp.logical_or(jnp.logical_and(col >= D, col < 2 * D),
                                  jnp.logical_and(col >= 4 * D, col < 5 * D))
        mod = jnp.where(is_scale, _r(1.0 + mod), mod)
        for t in range(mod.shape[1] // 128):
            rows = pl.ds(pl.multiple_of(lo + t * 128, 128), 128)
            mod_ref[rows, :] = _paced(_col_bcast(mod[:, t * 128:(t + 1) * 128]), clock, pos)

    def late_mod_sums(n, clock):
        b0 = jnp.clip(n - MB0, 0, NMB // MPI - 1) * MPI
        for k in range(MPI):
            w = xw_v[jnp.where(n >= MB0, NT + NFB + b0 + k, 0)].astype(F32)
            part = jnp.sum((w * scb_ref[0:D, :]).reshape(D // 8, 8, 128), axis=0)
            lm_ref[k] = _paced(part, clock, PACE[4] + 192 * k)

    def late_mod_store(n, sums, clock):
        b0 = jnp.clip(n - MB0, 0, NMB // MPI - 1) * MPI
        for k in range(MPI):
            finish_mod(jnp.sum(sums[k], axis=0, keepdims=True), DA + (b0 + k) * 128,
                       clock, XP[4] + 128 * k)

    def col_vector(ref, row):
        row = jnp.concatenate([row, jnp.zeros((1, 64), F32)], axis=1)
        for t in range(5):
            ref[t * 128:(t + 1) * 128, :] = _col_bcast(row[:, t * 128:(t + 1) * 128])

    def mod(k):
        return mod_ref[k * D:(k + 1) * D, :]

    def put_stats(st_ref, t, shift, scale, clock, pos):
        row = jax.lax.broadcasted_iota(jnp.int32, (8, 128), 0)
        st_ref[t] = _paced(jnp.where(row == 0, shift, scale), clock, pos)

    def ln1_stats(t, clock=None, pos=None):
        for c in range(NC):
            m, s = _chunk_stats(xw_v[t, c * DC:(c + 1) * DC, :].astype(F32))
            put_stats(st1_ref, t * NC + c, m, s, clock, (PACE[0] if pos is None else pos) + 192 * c)

    def ln1_norm(t):
        mean, var = _mean_var(load_stats(st1_ref, t))
        return (xw_v[t].astype(F32) - mean) * jax.lax.rsqrt(var + EPS)

    def ln1_apply(t, clock=None, pos=None, ln=None):
        h = (ln1_norm(t) if ln is None else ln) * mod(1) + mod(0)
        h = _paced(h, clock, PACE[1] if pos is None else pos)
        ht_ref[t] = pltpu.bitcast(h.astype(BF16), U32)
        hr_ref[t] = h[DM:]

    def h2_rows(t, clock=None):
        x = _paced_wide(pltpu.bitcast(pltpu.bitcast(h2_ref[t], BF16).T, U32), clock, PACE[5])
        h2row_ref[pl.ds(pl.multiple_of(t * 64, 64), 64), :] = x

    def router_terms():
        u = mod(4) * wrb_ref[0:D, :]
        return (u, jnp.sum(u, axis=0, keepdims=True),
                jnp.sum(mod(3) * wrb_ref[0:D, :], axis=0, keepdims=True))

    def load_stats(st_ref, t):
        return [(st_ref[t * NC + c, 0:1, :], st_ref[t * NC + c, 1:2, :]) for c in range(NC)]

    def ln2_x1(t, attn, clock=None):
        x1 = _r(xw_v[t].astype(F32) + mod(2) * attn)
        x1_ref[t] = _paced(x1, clock, PACE[2]).astype(BF16)
        return x1, [_chunk_stats(x1[c * DC:(c + 1) * DC]) for c in range(NC)]

    def ln2_norm(stats):
        mean, var = _mean_var(stats)
        return _r(mean), 1.0 / _r(jnp.sqrt(_r(_r(var) + EPS)))

    def ln2_h2(x1, mean, inv):
        return (x1 - mean) * inv * mod(4) + mod(3)

    def ln2_stats(t, clock):
        for c, (m, s) in enumerate(ln2_x1(t, acc_ref[t], clock)[1]):
            put_stats(st2_ref, t * NC + c, m, s, clock, PACE[2] + (c + 1) * DC + SLAG)

    def ln2_apply(t, clock):
        x1 = x1_ref[t].astype(F32)
        h2 = ln2_h2(x1, *ln2_norm(load_stats(st2_ref, t)))
        key = _score_key(jnp.sum(h2 * wrb_ref[0:D, :], axis=0, keepdims=True), t)
        key_ref[pl.ds(t, 1), :] = _paced(key, clock, PACE[3] + D + 96)
        h2 = _r(h2)
        h2_ref[t] = pltpu.bitcast(_paced(h2, clock, PACE[3]).astype(BF16), U32)
        out_v[t] = _paced(x1 + mod(5) * h2, clock, PACE[3] + 16).astype(BF16)

    def finish_q(q):
        q = (q * QSCALE).astype(BF16)
        return jnp.concatenate([q[r * DH:(r + 1) * DH] for r in range(REP)], axis=1)

    def q_proj(u, wqt_ref, qr_ref=None, split=False):
        w = pltpu.bitcast(wqt_ref[...], BF16)
        h = jnp.concatenate([pltpu.bitcast(ht_ref[_blk(u) * TPB + t], BF16) for t in range(TPB)], axis=1)
        if split:
            return sum(_dot(w[:, a:min(a + 128, D)], h[a:min(a + 128, D)]) for a in range(0, D, 128))
        if qr_ref is None:
            rem = _dot(w[:, DM:], h[DM:])
        else:
            rem = [qr_ref[...].T]
            if NV < TPB:
                R = GW * (TPB - NV) // 4
                rem.append(jnp.concatenate([_dot(w[a:a + R, DM:], h[DM:, NV * 128:])
                                            for a in range(0, GW, R)], axis=0))
            rem = jnp.concatenate(rem, axis=1)
        return _dot(w[:, :DM], h[:DM]) + rem

    def w_rest(u, wf_ref, gates=None):
        w = wrem_v[:, _lanes(_grp(u) * REP, REP)].astype(F32)
        for r in range(REP):
            wb = jnp.stack([jnp.broadcast_to(w[k:k + 1, r * DH:(r + 1) * DH], (8, DH))
                            for k in range(KR)])
            wf_ref[r] = _gated(wb, gates, r, REP)

    def outer(u, qr_ref, wf_ref, clock, start):
        base = jnp.bitwise_and(_blk(u), 1) * 16
        for g in range(0, NV * REP * 16, CH):
            pos = min(start + OSTEP * (g // CH + 1), clock.shape[0] - 8)
            runs, c = [], g
            while c < min(g + CH, NV * REP * 16):
                runs.append((c // 32, c // 16 % 2, c % 16, min(g + CH - c, 16 - c % 16)))
                c += runs[-1][3]
            acc = {}
            for k in range(KR):
                for i, r, tv, n in runs:
                    t = hb_refs[i][pl.ds(base + tv, n), k] * wf_ref[r, k][None]
                    acc[i, r] = t if k == 0 else acc[i, r] + t
            for i, r, tv, n in runs:
                gate = jnp.concatenate([clock[pos // 8 * 8:pos // 8 * 8 + 8]] * n, axis=0)
                row = i * 128 + tv * 8
                qr_ref[row:row + 8 * n, r * DH:(r + 1) * DH] = _paced(
                    acc[i, r].reshape(8 * n, DH), gate, 0)

    def h_table(hr, i, base, k0, gates):
        nk = hr.shape[0]
        hr = _r(hr)
        for j in range(nk):
            cb = _col_bcast(hr[j:j + 1]).reshape(16, 8, 128)
            hb_refs[i][pl.ds(base, 16), k0 + j] = _gated(cb, gates, j, nk)

    def never_of(clock, lo, hi, step=8):
        return [clock[a:a + 8] * clock[a:a + 8] for a in range(lo // 8 * 8, hi, step)]

    def scores(u, q, s_ref, m_ref, kp_ref=None, qclk=None):
        def keep(s, cols):
            s_ref[:, cols] = s
            m_ref[:, cols] = jnp.broadcast_to(jnp.max(s, axis=0, keepdims=True), (8, s.shape[1]))
            return s

        if kp_ref is None:
            s = jnp.concatenate([keep(_dot(k_v[_grp(u)], q[:, c]), c)
                                 for c in (slice(0, TQ), slice(TQ, 2 * TQ))], axis=1)
        else:
            k = pltpu.bitcast(k_v[_grp(u)], U32).reshape(S // 16, 8, DH)
            z = 0 if isinstance(u, int) else jax.lax.shift_right_logical(u, 8)
            kp_ref[z] = _gated(k, never_of(qclk, *KP, 32), 0, 1).reshape(S // 2, DH)
            s = keep(_dot(pltpu.bitcast(kp_ref[0], BF16), q), slice(0, 2 * TQ))
        return jnp.concatenate([s[:, 0:128], s[:, TQ:TQ + 128]], axis=0)

    def q_clock(q):
        return jnp.concatenate([q[:, t * 128:(t + 1) * 128] for t in range(TPB)], axis=0)

    def v_transpose(u, vt_ref, clock=None, pos=0):
        vt_ref[...] = _paced_wide(pltpu.bitcast(v_v[_grp(u)].T, U32), clock, pos)

    def wq_transpose(u, wqt_ref, clock=None, pos=0):
        wqt_ref[...] = _paced_wide(pltpu.bitcast(wq_v[_grp(u)].T, U32), clock, pos)

    def wd_transpose(u, clock, pos):
        fb = jnp.clip(u - WD0, 0, NFB - 1)
        src = jnp.where(u >= WD0, NT + fb, 0)
        wd_ref[pl.ds(pl.multiple_of(fb * 64, 64), 64), :] = _paced_wide(
            pltpu.bitcast(xw_v[src].T, U32), clock, pos)

    def attend(s_ref, m_ref, vt_ref):
        m = m_ref[0:1, :]
        o = []
        for r in range(REP):
            cols = slice(r * TQ, (r + 1) * TQ)
            p, l = _softmax_numer(s_ref[:, cols], m[:, cols])
            o.append((_dot(pltpu.bitcast(vt_ref[...], BF16), p) * (1.0 / l)))
        return jnp.concatenate(o, axis=0)

    small = Both([pltpu.make_async_copy(wr_hbm, wr_ref, msem.at[7]),
                  pltpu.make_async_copy(c_hbm, c_ref, msem.at[7])])
    zeroth = Both([cp_x(0, TPB, msem.at[5]), cp_w1(wq_hbm, wq_v, 0, msem.at[5])])
    first = Both([cp_k1(0, msem.at[8]), cp_w1(wq_hbm, wq_v, 1, msem.at[8])])
    second = Both([cp_k1(1, msem.at[9]), cp_v1(0, msem.at[9]), cp_w1(wq_hbm, wq_v, 2, msem.at[9]),
                   pltpu.make_async_copy(wq_hbm.at[DM:, :], wrem_v, msem.at[9]), cp_x(TPB, NV, msem.at[9])])
    for cp in [small, zeroth] + cp_moda + [first, second]:
        cp.start()
    acc_ref[...] = jnp.zeros_like(acc_ref)
    mod_ref[DA:6 * D, :] = jnp.zeros((4 * D, 128), F32)
    h2_ref[0] = jnp.zeros((D // 2, 128), U32)
    lm_ref[...] = jnp.zeros_like(lm_ref)
    small.wait()
    col_vector(wrb_ref, wr_ref[...].astype(F32).reshape(1, D))
    col_vector(scb_ref, silu_c())
    sc8 = jnp.broadcast_to(silu_c(), (8, D)).astype(BF16)
    zeroth.wait()
    ln0 = []
    for t in range(TPB):
        ln1_stats(t)
        ln0.append(ln1_norm(t))
    wq_transpose(0, wqt0_ref)
    for cp, tiles in zip(cp_moda, MODA):
        cp.wait()
        for t in tiles:
            finish_mod(_dot(sc8, wmod_v[:, t * 128:(t + 1) * 128])[0:1], t * 128)
    for t in range(TPB):
        ln1_apply(t, ln=ln0[t])
    q = finish_q(q_proj(0, wqt0_ref, split=True))
    first.wait()
    bundle(0, 'start')
    jobs = ([(i, 0, k) for i in range(NV) for k in range(0, KR, TPI)]
            + [(i, 1, k) for i in range(NV) for k in range(0, 2 * TPI, TPI)])

    def first_table(gates, todo, starts=None):
        for j, (i, blk, k0) in enumerate(todo):
            hr = hr_ref[blk * TPB + i, k0:k0 + TPI, :]
            if starts is not None:
                hr = jnp.where(starts[j * len(starts) // len(todo)] < 0.0, 0.0, hr)
            h_table(hr, i, blk * 16, k0,
                    gates[j * len(gates) // len(todo):(j + 1) * len(gates) // len(todo)])

    first_table(never_of(scores(0, q, s0_ref, m0_ref), 64, 2 * S - 192, 16), jobs[:TSPLIT])
    wq_transpose(1, wqt1_ref)
    second.wait()
    bundle(1, 'start')
    cp_modb.start()
    q = q_proj(1, wqt1_ref)
    hrem = jnp.concatenate([pltpu.bitcast(ht_ref[t, DM // 2:, :], BF16) for t in range(NV)], axis=1)
    for a in range(2):
        streams[a][4][...] = jax.lax.dot_general(
            hrem, wrem_v[:, (a + 2) * GW:(a + 3) * GW], (((0,), (0,)), ((), ())),
            preferred_element_type=F32)
    clock = jnp.concatenate(
        [q_clock(q), scores(1, finish_q(q), s1_ref, m1_ref)], axis=0)
    nb0 = NV * KR // TPI
    v_transpose(0, vt0_ref, clock, PP[3])
    wq_transpose(2, wqt0_ref, clock, PP[4])
    first_table(never_of(clock, PP[6], PP[7], 16), jobs[TSPLIT:nb0])
    for i in range(NV):
        ln1_stats(TPB + i, clock, PP[0] + PP[5] * i)
        ln1_apply(TPB + i, clock, PP[1] + PP[5] * i)
    first_table(never_of(clock, PP[7], PP[2], 16), jobs[nb0:],
                never_of(clock, PP[7] - PP[8], PP[2] - PP[8]))
    for a in range(2):
        w_rest(a + 4, streams[a][5], never_of(clock, 500 * a, 500 * a + 500, 32))

    def unit(u, side, s_ref, m_ref, vt_ref, wqt_ref, qr_ref, wf_ref, kp_ref):
        q = q_proj(u + 2, wqt_ref, qr_ref)
        o = attend(s_ref, m_ref, vt_ref)
        sclk = scores(u + 2, finish_q(q), s_ref, m_ref, kp_ref, q_clock(q))
        o = jnp.concatenate([o[r * DH:(r + 1) * DH].astype(BF16) for r in range(REP)], axis=0)
        upd = _dot(wot_v[_grp(u)], o)
        clock = jnp.concatenate([q_clock(q), sclk, upd[:, 0:128], upd[:, 256:384]], axis=0)
        side(clock, lambda start: outer(u + 4, qr_ref, wf_ref, clock, start))
        for t in range(TPB):
            acc_ref[_blk(u) * TPB + t] += upd[:, t * 128:(t + 1) * 128]

    def step(n, carry):
        bundle(jnp.minimum(n + 2, NP), 'start')
        for a in range(3):
            pl.when(n == 2 + a)(Both(cp_d.cps[a * NFB // 3:(a + 1) * NFB // 3]).start)
        pl.when(n == NP)(Both([cp_g, cp_u]).start)

        t1 = jnp.minimum(n + TPB + NV - 1, NT - 1)
        v = jnp.maximum(n - NP, 0)
        tile2 = lambda v: (jax.lax.shift_right_logical(v, 3) * TPB
                           + jnp.minimum(jnp.bitwise_and(v, NP - 1), TPB - 1))
        t2 = tile2(v)
        sums = lm_ref[...]

        def stats(clock, outer_at):
            v_transpose(2 * n + 1, vt1_ref, clock, XP[5])
            wq_transpose(2 * n + 3, wqt1_ref, clock, XP[6])
            ln2_stats(t2, clock)
            ln1_stats(t1, clock)
            if not LMB:
                late_mod_sums(n, clock)
            h2_rows(tile2(jnp.maximum(v - 1, 0)), clock)
            wd_transpose(2 * n, clock, XP[0])
            outer_at(OUTER0[0])

        def apply(clock, outer_at):
            blk = jnp.minimum(jax.lax.shift_right_logical(n + 2, 3) + 1, NBLK - 1)
            k0 = jnp.bitwise_and(n + 2, 7) * TPI
            hr = [hr_ref[blk * TPB + i, pl.ds(pl.multiple_of(k0, TPI), TPI), :]
                  for i in range(NV)]
            v_transpose(2 * n + 2, vt0_ref, clock, XP[1])
            wq_transpose(2 * n + 4, wqt0_ref, clock, XP[2])
            wd_transpose(2 * n + 1, clock, XP[3])
            if LMB:
                late_mod_sums(n, clock)
            ln1_apply(t1, clock)
            ln2_apply(t2, clock)
            outer_at(OUTER0[1])
            for i in range(NV):
                h_table(hr[i], i, jnp.bitwise_and(blk, 1) * 16, k0, never_of(clock, *TAB[i], 16))
            late_mod_store(n - 1, sums, clock)
            for a in range(2):
                w_rest(2 * n + 6 + a, streams[a][5], never_of(clock, *WFP[a], 32))

        for a in range(2):
            unit(2 * n + a, (stats, apply)[a], *streams[a])
        return carry

    def stage(n, carry):
        bundle(n, 'wait')
        pl.when(n == MB0)(cp_modb.wait)
        pl.when(n == WD0 // 2)(cp_d.wait)
        return jax.lax.fori_loop(n, jnp.where(n < NP - 1, n + 1, NU // 2 - 1), step, carry)

    jax.lax.fori_loop(0, NP, stage, 0)

    T0 = NT - TPB
    cp_out(0, T0, osem.at[C + TPB]).start()
    cp_g.wait()
    v_transpose(NU - 1, vt1_ref)
    o = jnp.concatenate([attend(*streams[a][0:3]) for a in range(2)], axis=0)
    wlast = jnp.concatenate([wot_v[HKV - 2], wot_v[HKV - 1]], axis=1)
    fin = [acc_ref[T0 + t] + _dot(wlast, o[:, t * 128:(t + 1) * 128].astype(BF16)) for t in range(TPB)]
    clock = jnp.concatenate(fin, axis=0)
    row8 = jax.lax.broadcasted_iota(jnp.int32, (C, 128), 0)
    lane8 = jax.lax.broadcasted_iota(jnp.int32, (C, 128), 1)
    work = key_ref[0:T0, :]
    lead = jnp.zeros((C, 128), F32)
    for t in range(C):
        mx = jnp.max(jnp.max(work, axis=0, keepdims=True), axis=1, keepdims=True)
        work = jnp.where(work == mx, 0.0, work)
        lead = jnp.where(row8 == t, mx, lead)

    def spread(row):
        return pltpu.roll(jnp.broadcast_to(row, (128, 128)), 0, 1, stride=1, stride_axis=0)

    def merge(lead, rows, spreads):
        cols = jnp.concatenate([lead] + spreads, axis=0)
        best = jnp.zeros((C, 128), F32)
        for row in [jnp.max(jnp.where(row8 == lane8, lead, 0.0), axis=0, keepdims=True)] + rows:
            rank = jnp.sum(jnp.where(cols > row, 1.0, 0.0), axis=0, keepdims=True)
            best = jnp.maximum(best, jnp.where(rank == row8.astype(F32), row, 0.0))
        return jnp.max(best, axis=1, keepdims=True)

    def tail_h2(t, norm, gate=None):
        x1 = x1_ref[t].astype(F32)
        if gate is not None:
            n = gate.shape[0]
            x1 = jnp.concatenate([_paced(x1[:n], gate, 0), x1[n:]], axis=0) if n < D else _paced(x1, gate, 0)
        h2_ref[t] = pltpu.bitcast(ln2_h2(x1, *norm).astype(BF16), U32)
        if t < NT - 2:
            h2_rows(t)

    u_vec, u_sum, b_sum = router_terms()
    keys = []
    for t in range(TPB):
        x1, stats = ln2_x1(T0 + t, fin[t])
        mean, inv = norm = ln2_norm(stats)
        r = (jnp.sum(x1 * u_vec, axis=0, keepdims=True) - mean * u_sum) * inv + b_sum
        keys.append(_score_key(r, T0 + t))
        if t < TPB - 1:
            tail_h2(T0 + t, norm, clock[(t + 1) * D + TLAG:(t + 2) * D + TLAG])
    lead = jnp.broadcast_to(merge(lead, keys[0:2], [spread(k) for k in keys[0:2]]), (C, 128))
    spread2 = spread(keys[2])
    h2_rows(NT - 2)
    tail_h2(NT - 1, norm)
    h2_rows(NT - 1)
    sel = pltpu.bitcast(merge(lead, keys[2:4], [spread2, spread(keys[3])]), jnp.int32) - KEY0
    sel_tok = (S - 1) - (sel & (S - 1))
    toks = [sel_tok[t, 0] for t in range(C)]
    tiles = [jax.lax.shift_right_logical(tk, 7) for tk in toks]
    sel_code = jax.lax.shift_right_logical(sel, 11) - 32768
    sel_bits = jnp.where(sel_code < 0, -32769 - sel_code, sel_code)
    r_sel = pltpu.bitcast(jax.lax.shift_left(sel_bits, 16), F32)

    final = []
    for t in range(C):
        d = True
        for u in range(t + 1, C):
            d = jnp.logical_and(d, tiles[u] != tiles[t])
        final.append(d)

    words = jnp.concatenate([h2row_ref[pl.ds(jax.lax.shift_right_logical(toks[t], 1), 1), :]
                             for t in range(C)], axis=0)
    odd = jnp.bitwise_and(sel_tok, 1) == 1
    xs = pltpu.bitcast(jnp.where(odd, jnp.bitwise_and(words, jnp.uint32(0xFFFF0000)),
                                 jax.lax.shift_left(words, jnp.uint32(16))), F32)
    xs = xs.astype(BF16)

    def plain_out(t, ticks):
        gate = jnp.concatenate([ticks[a * len(ticks) // (D // 8)] for a in range(D // 8)], axis=0)
        x1 = _paced(x1_ref[t].astype(F32), gate, 0)
        out_v[t] = (x1 + mod(5) * pltpu.bitcast(h2_ref[t], BF16).astype(F32)).astype(BF16)

    clean = []

    def send_clean(t):
        d = tiles[0] != t
        for a in range(1, C):
            d = jnp.logical_and(d, tiles[a] != t)
        clean.append(d)
        pl.when(d)(cp_out(t, 1, osem.at[C + t - T0]).start)

    cp_u.wait()
    cp_out(0, T0, osem.at[C + TPB]).wait()
    gpre = _dot(xs, wg_v[...])
    u = _dot(xs, wu_v[...])
    ticks = [z[:, a * 128:(a + 1) * 128] for z in (gpre, u) for a in range(NFB)]
    for t in range(TPB):
        plain_out(T0 + t, ticks[t * TKS:(t + 1) * TKS])
        send_clean(T0 + t)
    gpre, u = _r(gpre), _r(u)
    gact = _r(gpre * _r(jax.nn.sigmoid(gpre)))
    act = (gact * u).astype(BF16)
    gate_r = _r(jax.nn.sigmoid(r_sel))
    ohs = []
    for t in range(C):
        oh = jnp.where(sel_tok == tiles[t] * 128 + lane8, 1.0, 0.0)
        ohs.append(jnp.concatenate([oh, jnp.zeros((16 - C, 128), F32)], axis=0).astype(BF16))

    def cp_fix(t, lo, hi):
        return pltpu.make_async_copy(fix_v.at[t, lo:hi, :], out_hbm.at[lo:hi, _lanes(tiles[t])],
                                     osem.at[t])

    def guarded(cond, fn):
        if cond is True:
            fn()
        else:
            pl.when(cond)(fn)

    def scatter(j, yt, t):
        lo, hi = j * 128, min(j * 128 + 128, D)
        upd = jnp.concatenate([_dot(yt[a:a + 64], ohs[t]) for a in range(0, hi - lo, 64)], axis=0)
        fix_v[t, lo:hi, :] = (x1_ref[tiles[t], lo:hi, :].astype(F32) + mod_ref[5 * D + lo:5 * D + hi, :]
                              * (pltpu.bitcast(h2_ref[tiles[t], lo // 2:hi // 2, :], BF16).astype(F32) + upd)).astype(BF16)
        guarded(final[t], cp_fix(t, lo, hi).start)

    NJ = (D + 127) // 128
    yts = []
    for j in range(NJ):
        lo, hi = j * 128, min(j * 128 + 128, D)
        FK = F // 4
        yk = []
        for a in range(4):
            w = pltpu.bitcast(wd_ref[a * FK // 2:(a + 1) * FK // 2, lo:hi], BF16)
            yk.append(_dot(act[:, a * FK:(a + 1) * FK], w))
            if j >= SCLAG:
                for t in (2 * a, 2 * a + 1):
                    scatter(j - SCLAG, yts[j - SCLAG], t)
        y = _r(sum(yk)) * gate_r
        yts.append(jnp.concatenate([y, jnp.zeros_like(y)], axis=0).astype(BF16).T)
    for j in range(NJ - SCLAG, NJ):
        for t in range(C):
            scatter(j, yts[j], t)
    for t in range(T0, NT):
        pl.when(clean[t - T0])(cp_out(t, 1, osem.at[C + t - T0]).wait)
    for t in range(C):
        guarded(final[t], cp_fix(t, 0, D).wait)


@jax.jit
def pallas_adaLN_cond__gqa_block_cached__moe_arch_mod__prompt_kernel(
    A_x: jax.Array,
    A_k_cache: jax.Array,
    A_v_cache: jax.Array,
    A_wq: jax.Array,
    A_wo: jax.Array,
    B_x: jax.Array,
    B_w_r: jax.Array,
    B_w_gate: jax.Array,
    B_w_up: jax.Array,
    B_w_down: jax.Array,
    c: jax.Array,
    w_mod: jax.Array,
):
    del B_x
    xt = A_x.reshape(S, D).T
    k = A_k_cache.reshape(HKV, S, DH)
    v = A_v_cache.reshape(HKV, S, DH)

    hbm = pl.BlockSpec(memory_space=pl.ANY)
    stream = [
        pltpu.VMEM((S, REP * TQ), F32),
        pltpu.VMEM((8, REP * TQ), F32),
        pltpu.VMEM((DH // 2, S), U32),
        pltpu.VMEM((GW // 2, D), U32),
        pltpu.VMEM((NV * 128, GW), F32),
        pltpu.VMEM((REP, KR, 8, DH), F32),
        pltpu.VMEM((1, S // 2, DH), U32),
    ]
    out = pl.pallas_call(
        _kernel_flat,
        in_specs=[hbm] * 11,
        out_specs=hbm,
        out_shape=jax.ShapeDtypeStruct((D, S), BF16),
        scratch_shapes=[pltpu.VMEM((2 * 16, KR, 8, 128), F32)] * NV + [
            pltpu.VMEM((NT + NFB + NMB, D, 128), BF16),
            pltpu.VMEM((HKV, S, DH), BF16),
            pltpu.VMEM((HKV, S, DH), BF16),
            pltpu.VMEM((HKV, D, GW), BF16),
            pltpu.VMEM((HKV, D, GW), BF16),
            pltpu.VMEM((D, DA), BF16),
            pltpu.VMEM((D, F), BF16),
            pltpu.VMEM((D, F), BF16),
            pltpu.VMEM((F // 2, D), U32),
            pltpu.VMEM((NT, D // 2, 128), U32),
            pltpu.VMEM((NT, KR, 128), F32),
            pltpu.VMEM((NT, D, 128), F32),
            pltpu.VMEM((6 * D, 128), F32),
            pltpu.VMEM((5 * 128, 128), F32),
            pltpu.VMEM((5 * 128, 128), F32),
            pltpu.VMEM((NT, D, 128), BF16),
            pltpu.VMEM((NT, D // 2, 128), U32),
            pltpu.VMEM((S // 2, D), U32),
            pltpu.VMEM((NT, D, 128), BF16),
            pltpu.VMEM((C, D, 128), BF16),
            pltpu.VMEM((NT, 128), F32),
            pltpu.VMEM((NT * NC, 8, 128), F32),
            pltpu.VMEM((NT * NC, 8, 128), F32),
            pltpu.VMEM((MPI, 8, 128), F32),
            pltpu.VMEM((KR, HQ * DH), BF16),
        ] + stream + stream + [
            pltpu.VMEM((D,), BF16),
            pltpu.VMEM((1, D), BF16),
            pltpu.SemaphoreType.DMA((HKV // 2,)),
            pltpu.SemaphoreType.DMA((11,)),
            pltpu.SemaphoreType.DMA((C + TPB + 1,)),
        ],
        compiler_params=pltpu.CompilerParams(vmem_limit_bytes=127 * 1024 * 1024,
                                             disable_bounds_checks=True,
                                             disable_semaphore_checks=True),
    )(B_w_r, c, xt, k, v, A_wq, A_wo.T, w_mod, B_w_gate, B_w_up, B_w_down.T)
    return out.T.reshape(1, S, D)
```

```python
import math

import jax
import jax.numpy as jnp
import jax.experimental.pallas as pl
import jax.experimental.pallas.tpu as pltpu

S = 2048
D = 576
HQ = 32
HKV = 16
REP = HQ // HKV
DH = 128
GW = REP * DH
F = 4608
C = 8
EPS = 1e-05
TQ = 512
NBLK = S // TQ
TPB = TQ // 128
NT = S // 128
NU = NBLK * HKV
NP = HKV // 2
NC = 3
DC = D // NC
PG = 64
NFB = F // 128
WD0 = 14
DA = 2 * D
MODA = ((0, 4, 5), (1, 2, 6), (3, 7, 8))
NMB = 4 * D // 128
MPI = 3
MB0 = 1
DM = 512
KR = D - DM
NV = 3
CH = 3
TPI = KR // NP

QC, SC, WC = 0, 1024, 1024 + 2 * S
OUTER0, OSTEP = (SC + 850, SC + 0), 133
PACE = (100, WC + 160, SC + 100, WC + 250, 0, SC + 3400)
XP = (SC + 3700, SC + 100, SC + 900, SC + 1300, WC + 762, 724, SC + 2600)
TAB = ((SC + 1600, SC + 2600), (SC + 2950, SC + 3890), (WC + 650, WC + 890))
WFP = ((300, 900), (WC + 600, WC + 1144))
KP = (0, 616)
SLAG = 96
GS = 4
TSPLIT = 15
PP = (24, 1474, 5112, 0, 0, 500, 750, 3524, 300)
TLAG = 256
TKS = 18
SCLAG = 2

BF16 = jnp.bfloat16
F32 = jnp.float32
U32 = jnp.uint32
QSCALE = DH ** -0.5 * math.log2(math.e)


def _dot(a, b):
    return jnp.dot(a, b, preferred_element_type=F32)


def _r(x):
    return x.astype(BF16).astype(F32)


def _col_bcast(row):
    return jnp.broadcast_to(row, (128, 128)).T


def _blk(u):
    return u // HKV if isinstance(u, int) else jax.lax.shift_right_logical(u, 4)


def _grp(u):
    return u % HKV if isinstance(u, int) else jnp.bitwise_and(u, HKV - 1)


def _lanes(t, n=1):
    return pl.ds(pl.multiple_of(t * 128, 128), n * 128)


def _paced(x, clock, pos):
    if clock is None:
        return x
    pos = pos // 8 * 8
    g = clock[pos:pos + x.shape[0], 0:x.shape[1]]
    return jnp.where(g * g < 0.0, jnp.zeros_like(x), x)


def _paced_wide(x, clock, pos):
    if clock is None:
        return x
    n, w = x.shape
    cols = []
    for a in range(0, w, 128):
        p0 = (pos + a // 128 * n) // 8 * 8
        g = jnp.concatenate([clock[p0 + r // (8 * GS) * (8 * GS):p0 + r // (8 * GS) * (8 * GS) + 8]
                             for r in range(0, n, 8)], axis=0)
        cols.append(_paced(x[:, a:min(a + 128, w)], g, 0))
    return jnp.concatenate(cols, axis=1)


def _gated(x, gates, j, n):
    if gates is None:
        return x
    m = x.shape[0]
    g = jnp.stack([gates[(j * m + b) * len(gates) // (n * m)] for b in range(m)])
    return jnp.where(g < 0.0, jnp.zeros_like(x), x)


def _softmax_numer(s, m):
    n, w = s.shape
    p = jnp.exp2(s - m).reshape(n // PG, PG // 8, 8, w)
    ts = jnp.sum(p, axis=1)
    last = jnp.where(ts < 0.0, ts, p[:, PG // 8 - 1])
    p = jnp.concatenate([p[:, :PG // 8 - 1], last[:, None]], axis=1).reshape(n, w)
    l = jnp.sum(jnp.sum(ts, axis=0), axis=0, keepdims=True)
    return p.astype(BF16), l


KEY0 = 0x20000000


def _score_key(r, t):
    tok = t * 128 + jax.lax.broadcasted_iota(jnp.int32, r.shape, 1)
    bits = jax.lax.shift_right_arithmetic(pltpu.bitcast(_r(r) + 0.0, jnp.int32), 16)
    code = jnp.where(bits < 0, -32769 - bits, bits) + 32768
    return pltpu.bitcast(code * S + (S - 1 - tok) + KEY0, F32)


def _chunk_stats(x):
    m = jnp.sum(x, axis=0, keepdims=True) * (1.0 / DC)
    xc = x - m
    return m, jnp.sum(xc * xc, axis=0, keepdims=True)


def _mean_var(stats):
    mean = sum(m for m, _ in stats) * (1.0 / NC)
    var = sum(s + DC * (m - mean) * (m - mean) for m, s in stats) * (1.0 / D)
    return mean, var


def _kernel_flat(*refs):
    _kernel(*refs[:12], *refs[12 + NV:], *refs[12:12 + NV])


def _kernel(wr_hbm, c_hbm,
            xt_hbm, k_hbm, v_hbm, wq_hbm, wot_hbm, wmod_hbm, wg_hbm, wu_hbm, wdt_hbm,
            out_hbm,
            xw_v, k_v, v_v, wq_v, wot_v, wmod_v, wg_v, wu_v, wd_ref,
            ht_ref, hr_ref, acc_ref, mod_ref, wrb_ref, scb_ref, x1_ref, h2_ref, h2row_ref, out_v, fix_v,
            key_ref, st1_ref, st2_ref, lm_ref,
            wrem_v,
            s0_ref, m0_ref, vt0_ref, wqt0_ref, qr0_ref, wf0_ref, kp0_ref,
            s1_ref, m1_ref, vt1_ref, wqt1_ref, qr1_ref, wf1_ref, kp1_ref,
            wr_ref, c_ref, bsem, msem, osem, *hb_refs):
    streams = ((s0_ref, m0_ref, vt0_ref, wqt0_ref, qr0_ref, wf0_ref, kp0_ref),
               (s1_ref, m1_ref, vt1_ref, wqt1_ref, qr1_ref, wf1_ref, kp1_ref))

    def cp_cols(src, dst, t, n, sem, dst_t=None):
        return pltpu.make_async_copy(src.at[:, _lanes(t, n)],
                                     dst.at[:, _lanes(t if dst_t is None else dst_t, n)], sem)

    def cp_pair(src, dst, p, sem):
        return pltpu.make_async_copy(src.at[pl.ds(2 * p, 2)], dst.at[pl.ds(2 * p, 2)], sem)

    cp_k = lambda p, sem: cp_pair(k_hbm, k_v, p, sem)
    cp_v1 = lambda g, sem: pltpu.make_async_copy(v_hbm.at[g], v_v.at[g], sem)
    cp_k1 = lambda g, sem: pltpu.make_async_copy(k_hbm.at[g], k_v.at[g], sem)

    class Both:
        def __init__(self, cps):
            self.cps = cps

        def start(self):
            for cp in self.cps:
                cp.start()

        def wait(self):
            for cp in self.cps:
                cp.wait()

    def cp_w1(src, dst, g, sem):
        return pltpu.make_async_copy(src.at[:, _lanes(g * REP, REP)], dst.at[g], sem)

    def cp_w(src, dst, p, sem):
        return Both([cp_w1(src, dst, 2 * p + a, sem) for a in range(2)])

    cp_wo = lambda p, sem: cp_w(wot_hbm, wot_v, p, sem)
    cp_x = lambda t0, n, sem: Both([pltpu.make_async_copy(xt_hbm.at[:, _lanes(t0 + t)],
                                                          xw_v.at[t0 + t], sem) for t in range(n)])

    def bundle(n, act):
        sem = bsem.at[n if isinstance(n, int) else jnp.minimum(n, NP - 1)]

        def on(cond, cps):
            def go():
                for cp in cps():
                    getattr(cp, act)()
            if isinstance(cond, bool):
                if cond:
                    go()
            else:
                pl.when(cond)(go)
        on(n + 1 < NP, lambda: [cp_k(n + 1, sem), cp_v1(2 * n + 2, sem), cp_w1(wq_hbm, wq_v, 2 * n + 3, sem)])
        on(n + 2 < NP, lambda: [cp_w1(wq_hbm, wq_v, 2 * n + 4, sem)])
        XN = 3
        nx = (NT - TPB - NV) // XN
        on(jnp.logical_and(n >= 1, n <= nx) if not isinstance(n, int) else 1 <= n <= nx,
           lambda: [cp_x(TPB + NV + XN * (n - 1), XN, sem)])
        on(n < NP, lambda: [cp_v1(2 * n + 1, sem), cp_wo(n, sem)])

    cp_moda = [Both([cp_cols(wmod_hbm, wmod_v, t, 1, msem.at[s]) for t in tiles])
               for s, tiles in zip((0, 6, 10), MODA)]
    cp_modb = Both([pltpu.make_async_copy(wmod_hbm.at[:, _lanes(DA // 128 + b)],
                                          xw_v.at[NT + NFB + b], msem.at[1]) for b in range(NMB)])
    cp_g = pltpu.make_async_copy(wg_hbm, wg_v, msem.at[2])
    cp_u = pltpu.make_async_copy(wu_hbm, wu_v, msem.at[3])
    cp_d = Both([pltpu.make_async_copy(wdt_hbm.at[:, _lanes(b)], xw_v.at[NT + b], msem.at[4])
                 for b in range(NFB)])
    cp_out = lambda t, n, sem: Both([pltpu.make_async_copy(out_v.at[t + a], out_hbm.at[:, _lanes(t + a)],
                                                           sem) for a in range(n)])

    def silu_c():
        c = c_ref[...].astype(F32)
        return _r(c * _r(jax.nn.sigmoid(c)))

    def finish_mod(mod, lo, clock=None, pos=0):
        mod = _r(mod)
        col = lo + jax.lax.broadcasted_iota(jnp.int32, mod.shape, 1)
        is_scale = jnp.logical_or(jnp.logical_and(col >= D, col < 2 * D),
                                  jnp.logical_and(col >= 4 * D, col < 5 * D))
        mod = jnp.where(is_scale, _r(1.0 + mod), mod)
        for t in range(mod.shape[1] // 128):
            rows = pl.ds(pl.multiple_of(lo + t * 128, 128), 128)
            mod_ref[rows, :] = _paced(_col_bcast(mod[:, t * 128:(t + 1) * 128]), clock, pos)

    def late_mod_sums(n, clock):
        b0 = jnp.clip(n - MB0, 0, NMB // MPI - 1) * MPI
        for k in range(MPI):
            w = xw_v[jnp.where(n >= MB0, NT + NFB + b0 + k, 0)].astype(F32)
            part = jnp.sum((w * scb_ref[0:D, :]).reshape(D // 8, 8, 128), axis=0)
            lm_ref[k] = _paced(part, clock, PACE[4] + 192 * k)

    def late_mod_store(n, sums, clock):
        b0 = jnp.clip(n - MB0, 0, NMB // MPI - 1) * MPI
        for k in range(MPI):
            finish_mod(jnp.sum(sums[k], axis=0, keepdims=True), DA + (b0 + k) * 128,
                       clock, XP[4] + 128 * k)

    def col_vector(ref, row):
        row = jnp.concatenate([row, jnp.zeros((1, 64), F32)], axis=1)
        for t in range(5):
            ref[t * 128:(t + 1) * 128, :] = _col_bcast(row[:, t * 128:(t + 1) * 128])

    def mod(k):
        return mod_ref[k * D:(k + 1) * D, :]

    def put_stats(st_ref, t, shift, scale, clock, pos):
        row = jax.lax.broadcasted_iota(jnp.int32, (8, 128), 0)
        st_ref[t] = _paced(jnp.where(row == 0, shift, scale), clock, pos)

    def ln1_stats(t, clock=None, pos=None):
        for c in range(NC):
            m, s = _chunk_stats(xw_v[t, c * DC:(c + 1) * DC, :].astype(F32))
            put_stats(st1_ref, t * NC + c, m, s, clock, (PACE[0] if pos is None else pos) + 192 * c)

    def ln1_norm(t):
        mean, var = _mean_var(load_stats(st1_ref, t))
        return (xw_v[t].astype(F32) - mean) * jax.lax.rsqrt(var + EPS)

    def ln1_apply(t, clock=None, pos=None, ln=None):
        h = (ln1_norm(t) if ln is None else ln) * mod(1) + mod(0)
        h = _paced(h, clock, PACE[1] if pos is None else pos)
        ht_ref[t] = pltpu.bitcast(h.astype(BF16), U32)
        hr_ref[t] = h[DM:]

    def h2_rows(t, clock=None):
        x = _paced_wide(pltpu.bitcast(pltpu.bitcast(h2_ref[t], BF16).T, U32), clock, PACE[5])
        h2row_ref[pl.ds(pl.multiple_of(t * 64, 64), 64), :] = x

    def router_terms():
        u = mod(4) * wrb_ref[0:D, :]
        return (u, jnp.sum(u, axis=0, keepdims=True),
                jnp.sum(mod(3) * wrb_ref[0:D, :], axis=0, keepdims=True))

    def load_stats(st_ref, t):
        return [(st_ref[t * NC + c, 0:1, :], st_ref[t * NC + c, 1:2, :]) for c in range(NC)]

    def ln2_x1(t, attn, clock=None):
        x1 = _r(xw_v[t].astype(F32) + mod(2) * attn)
        x1_ref[t] = _paced(x1, clock, PACE[2]).astype(BF16)
        return x1, [_chunk_stats(x1[c * DC:(c + 1) * DC]) for c in range(NC)]

    def ln2_norm(stats):
        mean, var = _mean_var(stats)
        return _r(mean), 1.0 / _r(jnp.sqrt(_r(_r(var) + EPS)))

    def ln2_h2(x1, mean, inv):
        return (x1 - mean) * inv * mod(4) + mod(3)

    def ln2_stats(t, clock):
        for c, (m, s) in enumerate(ln2_x1(t, acc_ref[t], clock)[1]):
            put_stats(st2_ref, t * NC + c, m, s, clock, PACE[2] + (c + 1) * DC + SLAG)

    def ln2_apply(t, clock):
        x1 = x1_ref[t].astype(F32)
        h2 = ln2_h2(x1, *ln2_norm(load_stats(st2_ref, t)))
        key = _score_key(jnp.sum(h2 * wrb_ref[0:D, :], axis=0, keepdims=True), t)
        key_ref[pl.ds(t, 1), :] = _paced(key, clock, PACE[3] + D + 96)
        h2 = _r(h2)
        h2_ref[t] = pltpu.bitcast(_paced(h2, clock, PACE[3]).astype(BF16), U32)
        out_v[t] = _paced(x1 + mod(5) * h2, clock, PACE[3] + 16).astype(BF16)

    def finish_q(q):
        q = (q * QSCALE).astype(BF16)
        return jnp.concatenate([q[r * DH:(r + 1) * DH] for r in range(REP)], axis=1)

    def q_proj(u, wqt_ref, qr_ref=None, split=False):
        w = pltpu.bitcast(wqt_ref[...], BF16)
        h = jnp.concatenate([pltpu.bitcast(ht_ref[_blk(u) * TPB + t], BF16) for t in range(TPB)], axis=1)
        if split:
            return sum(_dot(w[:, a:min(a + 128, D)], h[a:min(a + 128, D)]) for a in range(0, D, 128))
        if qr_ref is None:
            rem = _dot(w[:, DM:], h[DM:])
        else:
            rem = [qr_ref[...].T]
            if NV < TPB:
                R = GW * (TPB - NV) // 4
                rem.append(jnp.concatenate([_dot(w[a:a + R, DM:], h[DM:, NV * 128:])
                                            for a in range(0, GW, R)], axis=0))
            rem = jnp.concatenate(rem, axis=1)
        return _dot(w[:, :DM], h[:DM]) + rem

    def w_rest(u, wf_ref, gates=None):
        w = wrem_v[:, _lanes(_grp(u) * REP, REP)].astype(F32)
        for r in range(REP):
            wb = jnp.stack([jnp.broadcast_to(w[k:k + 1, r * DH:(r + 1) * DH], (8, DH))
                            for k in range(KR)])
            wf_ref[r] = _gated(wb, gates, r, REP)

    def outer(u, qr_ref, wf_ref, clock, start):
        base = jnp.bitwise_and(_blk(u), 1) * 16
        for g in range(0, NV * REP * 16, CH):
            pos = min(start + OSTEP * (g // CH + 1), clock.shape[0] - 8)
            runs, c = [], g
            while c < min(g + CH, NV * REP * 16):
                runs.append((c // 32, c // 16 % 2, c % 16, min(g + CH - c, 16 - c % 16)))
                c += runs[-1][3]
            acc = {}
            for k in range(KR):
                for i, r, tv, n in runs:
                    t = hb_refs[i][pl.ds(base + tv, n), k] * wf_ref[r, k][None]
                    acc[i, r] = t if k == 0 else acc[i, r] + t
            for i, r, tv, n in runs:
                gate = jnp.concatenate([clock[pos // 8 * 8:pos // 8 * 8 + 8]] * n, axis=0)
                row = i * 128 + tv * 8
                qr_ref[row:row + 8 * n, r * DH:(r + 1) * DH] = _paced(
                    acc[i, r].reshape(8 * n, DH), gate, 0)

    def h_table(hr, i, base, k0, gates):
        nk = hr.shape[0]
        hr = _r(hr)
        for j in range(nk):
            cb = _col_bcast(hr[j:j + 1]).reshape(16, 8, 128)
            hb_refs[i][pl.ds(base, 16), k0 + j] = _gated(cb, gates, j, nk)

    def never_of(clock, lo, hi, step=8):
        return [clock[a:a + 8] * clock[a:a + 8] for a in range(lo // 8 * 8, hi, step)]

    def scores(u, q, s_ref, m_ref, kp_ref=None, qclk=None):
        def keep(s, cols):
            s_ref[:, cols] = s
            m_ref[:, cols] = jnp.broadcast_to(jnp.max(s, axis=0, keepdims=True), (8, s.shape[1]))
            return s

        if kp_ref is None:
            s = jnp.concatenate([keep(_dot(k_v[_grp(u)], q[:, c]), c)
                                 for c in (slice(0, TQ), slice(TQ, 2 * TQ))], axis=1)
        else:
            k = pltpu.bitcast(k_v[_grp(u)], U32).reshape(S // 16, 8, DH)
            z = 0 if isinstance(u, int) else jax.lax.shift_right_logical(u, 8)
            kp_ref[z] = _gated(k, never_of(qclk, *KP, 32), 0, 1).reshape(S // 2, DH)
            s = keep(_dot(pltpu.bitcast(kp_ref[0], BF16), q), slice(0, 2 * TQ))
        return jnp.concatenate([s[:, 0:128], s[:, TQ:TQ + 128]], axis=0)

    def q_clock(q):
        return jnp.concatenate([q[:, t * 128:(t + 1) * 128] for t in range(TPB)], axis=0)

    def v_transpose(u, vt_ref, clock=None, pos=0):
        vt_ref[...] = _paced_wide(pltpu.bitcast(v_v[_grp(u)].T, U32), clock, pos)

    def wq_transpose(u, wqt_ref, clock=None, pos=0):
        wqt_ref[...] = _paced_wide(pltpu.bitcast(wq_v[_grp(u)].T, U32), clock, pos)

    def wd_transpose(u, clock, pos):
        fb = jnp.clip(u - WD0, 0, NFB - 1)
        src = jnp.where(u >= WD0, NT + fb, 0)
        wd_ref[pl.ds(pl.multiple_of(fb * 64, 64), 64), :] = _paced_wide(
            pltpu.bitcast(xw_v[src].T, U32), clock, pos)

    def attend(s_ref, m_ref, vt_ref):
        m = m_ref[0:1, :]
        o = []
        for r in range(REP):
            cols = slice(r * TQ, (r + 1) * TQ)
            p, l = _softmax_numer(s_ref[:, cols], m[:, cols])
            o.append((_dot(pltpu.bitcast(vt_ref[...], BF16), p) * (1.0 / l)))
        return jnp.concatenate(o, axis=0)

    small = Both([pltpu.make_async_copy(wr_hbm, wr_ref, msem.at[7]),
                  pltpu.make_async_copy(c_hbm, c_ref, msem.at[7])])
    zeroth = Both([cp_x(0, TPB, msem.at[5]), cp_w1(wq_hbm, wq_v, 0, msem.at[5])])
    first = Both([cp_k1(0, msem.at[8]), cp_w1(wq_hbm, wq_v, 1, msem.at[8])])
    second = Both([cp_k1(1, msem.at[9]), cp_v1(0, msem.at[9]), cp_w1(wq_hbm, wq_v, 2, msem.at[9]),
                   pltpu.make_async_copy(wq_hbm.at[DM:, :], wrem_v, msem.at[9]), cp_x(TPB, NV, msem.at[9])])
    for cp in [small, zeroth] + cp_moda + [first, second]:
        cp.start()
    acc_ref[...] = jnp.zeros_like(acc_ref)
    mod_ref[DA:6 * D, :] = jnp.zeros((4 * D, 128), F32)
    h2_ref[0] = jnp.zeros((D // 2, 128), U32)
    lm_ref[...] = jnp.zeros_like(lm_ref)
    small.wait()
    col_vector(wrb_ref, wr_ref[...].astype(F32).reshape(1, D))
    col_vector(scb_ref, silu_c())
    sc8 = jnp.broadcast_to(silu_c(), (8, D)).astype(BF16)
    zeroth.wait()
    ln0 = []
    for t in range(TPB):
        ln1_stats(t)
        ln0.append(ln1_norm(t))
    wq_transpose(0, wqt0_ref)
    for cp, tiles in zip(cp_moda, MODA):
        cp.wait()
        for t in tiles:
            finish_mod(_dot(sc8, wmod_v[:, t * 128:(t + 1) * 128])[0:1], t * 128)
    for t in range(TPB):
        ln1_apply(t, ln=ln0[t])
    q = finish_q(q_proj(0, wqt0_ref, split=True))
    first.wait()
    bundle(0, 'start')
    jobs = ([(i, 0, k) for i in range(NV) for k in range(0, KR, TPI)]
            + [(i, 1, k) for i in range(NV) for k in range(0, 2 * TPI, TPI)])

    def first_table(gates, todo, starts=None):
        for j, (i, blk, k0) in enumerate(todo):
            hr = hr_ref[blk * TPB + i, k0:k0 + TPI, :]
            if starts is not None:
                hr = jnp.where(starts[j * len(starts) // len(todo)] < 0.0, 0.0, hr)
            h_table(hr, i, blk * 16, k0,
                    gates[j * len(gates) // len(todo):(j + 1) * len(gates) // len(todo)])

    first_table(never_of(scores(0, q, s0_ref, m0_ref), 64, 2 * S - 192, 16), jobs[:TSPLIT])
    wq_transpose(1, wqt1_ref)
    second.wait()
    bundle(1, 'start')
    cp_modb.start()
    q = q_proj(1, wqt1_ref)
    hrem = jnp.concatenate([pltpu.bitcast(ht_ref[t, DM // 2:, :], BF16) for t in range(NV)], axis=1)
    for a in range(2):
        streams[a][4][...] = jax.lax.dot_general(
            hrem, wrem_v[:, (a + 2) * GW:(a + 3) * GW], (((0,), (0,)), ((), ())),
            preferred_element_type=F32)
    clock = jnp.concatenate(
        [q_clock(q), scores(1, finish_q(q), s1_ref, m1_ref)], axis=0)
    nb0 = NV * KR // TPI
    v_transpose(0, vt0_ref, clock, PP[3])
    wq_transpose(2, wqt0_ref, clock, PP[4])
    first_table(never_of(clock, PP[6], PP[7], 16), jobs[TSPLIT:nb0])
    for i in range(NV):
        ln1_stats(TPB + i, clock, PP[0] + PP[5] * i)
        ln1_apply(TPB + i, clock, PP[1] + PP[5] * i)
    first_table(never_of(clock, PP[7], PP[2], 16), jobs[nb0:],
                never_of(clock, PP[7] - PP[8], PP[2] - PP[8]))
    for a in range(2):
        w_rest(a + 4, streams[a][5], never_of(clock, 500 * a, 500 * a + 500, 32))

    def unit(u, side, s_ref, m_ref, vt_ref, wqt_ref, qr_ref, wf_ref, kp_ref):
        q = q_proj(u + 2, wqt_ref, qr_ref)
        o = attend(s_ref, m_ref, vt_ref)
        sclk = scores(u + 2, finish_q(q), s_ref, m_ref, kp_ref, q_clock(q))
        o = jnp.concatenate([o[r * DH:(r + 1) * DH].astype(BF16) for r in range(REP)], axis=0)
        upd = _dot(wot_v[_grp(u)], o)
        clock = jnp.concatenate([q_clock(q), sclk, upd[:, 0:128], upd[:, 256:384]], axis=0)
        side(clock, lambda start: outer(u + 4, qr_ref, wf_ref, clock, start))
        for t in range(TPB):
            acc_ref[_blk(u) * TPB + t] += upd[:, t * 128:(t + 1) * 128]

    def step(n, carry):
        bundle(jnp.minimum(n + 2, NP), 'start')
        for a in range(3):
            pl.when(n == 2 + a)(Both(cp_d.cps[a * NFB // 3:(a + 1) * NFB // 3]).start)
        pl.when(n == NP)(Both([cp_g, cp_u]).start)

        t1 = jnp.minimum(n + TPB + NV - 1, NT - 1)
        v = jnp.maximum(n - NP, 0)
        tile2 = lambda v: (jax.lax.shift_right_logical(v, 3) * TPB
                           + jnp.minimum(jnp.bitwise_and(v, NP - 1), TPB - 1))
        t2 = tile2(v)
        sums = lm_ref[...]

        def stats(clock, outer_at):
            v_transpose(2 * n + 1, vt1_ref, clock, XP[5])
            wq_transpose(2 * n + 3, wqt1_ref, clock, XP[6])
            ln2_stats(t2, clock)
            ln1_stats(t1, clock)
            h2_rows(tile2(jnp.maximum(v - 1, 0)), clock)
            wd_transpose(2 * n, clock, XP[0])
            outer_at(OUTER0[0])

        def apply(clock, outer_at):
            blk = jnp.minimum(jax.lax.shift_right_logical(n + 2, 3) + 1, NBLK - 1)
            k0 = jnp.bitwise_and(n + 2, 7) * TPI
            hr = [hr_ref[blk * TPB + i, pl.ds(pl.multiple_of(k0, TPI), TPI), :]
                  for i in range(NV)]
            v_transpose(2 * n + 2, vt0_ref, clock, XP[1])
            wq_transpose(2 * n + 4, wqt0_ref, clock, XP[2])
            wd_transpose(2 * n + 1, clock, XP[3])
            late_mod_sums(n, clock)
            ln1_apply(t1, clock)
            ln2_apply(t2, clock)
            outer_at(OUTER0[1])
            for i in range(NV):
                h_table(hr[i], i, jnp.bitwise_and(blk, 1) * 16, k0, never_of(clock, *TAB[i], 16))
            late_mod_store(n - 1, sums, clock)
            for a in range(2):
                w_rest(2 * n + 6 + a, streams[a][5], never_of(clock, *WFP[a], 32))

        for a in range(2):
            unit(2 * n + a, (stats, apply)[a], *streams[a])
        return carry

    def stage(n, carry):
        bundle(n, 'wait')
        pl.when(n == MB0)(cp_modb.wait)
        pl.when(n == WD0 // 2)(cp_d.wait)
        return jax.lax.fori_loop(n, jnp.where(n < NP - 1, n + 1, NU // 2 - 1), step, carry)

    jax.lax.fori_loop(0, NP, stage, 0)

    T0 = NT - TPB
    cp_out(0, T0, osem.at[C + TPB]).start()
    cp_g.wait()
    v_transpose(NU - 1, vt1_ref)
    o = jnp.concatenate([attend(*streams[a][0:3]) for a in range(2)], axis=0)
    wlast = jnp.concatenate([wot_v[HKV - 2], wot_v[HKV - 1]], axis=1)
    fin = [acc_ref[T0 + t] + _dot(wlast, o[:, t * 128:(t + 1) * 128].astype(BF16)) for t in range(TPB)]
    clock = jnp.concatenate(fin, axis=0)
    row8 = jax.lax.broadcasted_iota(jnp.int32, (C, 128), 0)
    lane8 = jax.lax.broadcasted_iota(jnp.int32, (C, 128), 1)
    work = key_ref[0:T0, :]
    lead = jnp.zeros((C, 128), F32)
    for t in range(C):
        mx = jnp.max(jnp.max(work, axis=0, keepdims=True), axis=1, keepdims=True)
        work = jnp.where(work == mx, 0.0, work)
        lead = jnp.where(row8 == t, mx, lead)

    def spread(row):
        return pltpu.roll(jnp.broadcast_to(row, (128, 128)), 0, 1, stride=1, stride_axis=0)

    def merge(lead, rows, spreads):
        cols = jnp.concatenate([lead] + spreads, axis=0)
        best = jnp.zeros((C, 128), F32)
        for row in [jnp.max(jnp.where(row8 == lane8, lead, 0.0), axis=0, keepdims=True)] + rows:
            rank = jnp.sum(jnp.where(cols > row, 1.0, 0.0), axis=0, keepdims=True)
            best = jnp.maximum(best, jnp.where(rank == row8.astype(F32), row, 0.0))
        return jnp.max(best, axis=1, keepdims=True)

    def tail_h2(t, norm, gate=None):
        x1 = x1_ref[t].astype(F32)
        if gate is not None:
            n = gate.shape[0]
            x1 = jnp.concatenate([_paced(x1[:n], gate, 0), x1[n:]], axis=0) if n < D else _paced(x1, gate, 0)
        h2_ref[t] = pltpu.bitcast(ln2_h2(x1, *norm).astype(BF16), U32)
        if t < NT - 2:
            h2_rows(t)

    u_vec, u_sum, b_sum = router_terms()
    keys = []
    for t in range(TPB):
        x1, stats = ln2_x1(T0 + t, fin[t])
        mean, inv = norm = ln2_norm(stats)
        r = (jnp.sum(x1 * u_vec, axis=0, keepdims=True) - mean * u_sum) * inv + b_sum
        keys.append(_score_key(r, T0 + t))
        if t < TPB - 1:
            tail_h2(T0 + t, norm, clock[(t + 1) * D + TLAG:(t + 2) * D + TLAG])
    lead = jnp.broadcast_to(merge(lead, keys[0:2], [spread(k) for k in keys[0:2]]), (C, 128))
    spread2 = spread(keys[2])
    h2_rows(NT - 2)
    tail_h2(NT - 1, norm)
    h2_rows(NT - 1)
    sel = pltpu.bitcast(merge(lead, keys[2:4], [spread2, spread(keys[3])]), jnp.int32) - KEY0
    sel_tok = (S - 1) - (sel & (S - 1))
    toks = [sel_tok[t, 0] for t in range(C)]
    tiles = [jax.lax.shift_right_logical(tk, 7) for tk in toks]
    sel_code = jax.lax.shift_right_logical(sel, 11) - 32768
    sel_bits = jnp.where(sel_code < 0, -32769 - sel_code, sel_code)
    r_sel = pltpu.bitcast(jax.lax.shift_left(sel_bits, 16), F32)

    final = []
    for t in range(C):
        d = True
        for u in range(t + 1, C):
            d = jnp.logical_and(d, tiles[u] != tiles[t])
        final.append(d)

    words = jnp.concatenate([h2row_ref[pl.ds(jax.lax.shift_right_logical(toks[t], 1), 1), :]
                             for t in range(C)], axis=0)
    odd = jnp.bitwise_and(sel_tok, 1) == 1
    xs = pltpu.bitcast(jnp.where(odd, jnp.bitwise_and(words, jnp.uint32(0xFFFF0000)),
                                 jax.lax.shift_left(words, jnp.uint32(16))), F32)
    xs = xs.astype(BF16)

    def plain_out(t, ticks):
        gate = jnp.concatenate([ticks[a * len(ticks) // (D // 8)] for a in range(D // 8)], axis=0)
        x1 = _paced(x1_ref[t].astype(F32), gate, 0)
        out_v[t] = (x1 + mod(5) * pltpu.bitcast(h2_ref[t], BF16).astype(F32)).astype(BF16)

    clean = []

    def send_clean(t):
        d = tiles[0] != t
        for a in range(1, C):
            d = jnp.logical_and(d, tiles[a] != t)
        clean.append(d)
        pl.when(d)(cp_out(t, 1, osem.at[C + t - T0]).start)

    cp_u.wait()
    cp_out(0, T0, osem.at[C + TPB]).wait()
    gpre = _dot(xs, wg_v[...])
    u = _dot(xs, wu_v[...])
    ticks = [z[:, a * 128:(a + 1) * 128] for z in (gpre, u) for a in range(NFB)]
    for t in range(TPB):
        plain_out(T0 + t, ticks[t * TKS:(t + 1) * TKS])
        send_clean(T0 + t)
    gpre, u = _r(gpre), _r(u)
    gact = _r(gpre * _r(jax.nn.sigmoid(gpre)))
    act = (gact * u).astype(BF16)
    gate_r = _r(jax.nn.sigmoid(r_sel))
    ohs = []
    for t in range(C):
        oh = jnp.where(sel_tok == tiles[t] * 128 + lane8, 1.0, 0.0)
        ohs.append(jnp.concatenate([oh, jnp.zeros((16 - C, 128), F32)], axis=0).astype(BF16))

    def cp_fix(t, lo, hi):
        return pltpu.make_async_copy(fix_v.at[t, lo:hi, :], out_hbm.at[lo:hi, _lanes(tiles[t])],
                                     osem.at[t])

    def guarded(cond, fn):
        if cond is True:
            fn()
        else:
            pl.when(cond)(fn)

    def scatter(j, yt, t):
        lo, hi = j * 128, min(j * 128 + 128, D)
        upd = jnp.concatenate([_dot(yt[a:a + 64], ohs[t]) for a in range(0, hi - lo, 64)], axis=0)
        fix_v[t, lo:hi, :] = (x1_ref[tiles[t], lo:hi, :].astype(F32) + mod_ref[5 * D + lo:5 * D + hi, :]
                              * (pltpu.bitcast(h2_ref[tiles[t], lo // 2:hi // 2, :], BF16).astype(F32) + upd)).astype(BF16)
        guarded(final[t], cp_fix(t, lo, hi).start)

    NJ = (D + 127) // 128
    yts = []
    for j in range(NJ):
        lo, hi = j * 128, min(j * 128 + 128, D)
        FK = F // 4
        yk = []
        for a in range(4):
            w = pltpu.bitcast(wd_ref[a * FK // 2:(a + 1) * FK // 2, lo:hi], BF16)
            yk.append(_dot(act[:, a * FK:(a + 1) * FK], w))
            if j >= SCLAG:
                for t in (2 * a, 2 * a + 1):
                    scatter(j - SCLAG, yts[j - SCLAG], t)
        y = _r(sum(yk)) * gate_r
        yts.append(jnp.concatenate([y, jnp.zeros_like(y)], axis=0).astype(BF16).T)
    for j in range(NJ - SCLAG, NJ):
        for t in range(C):
            scatter(j, yts[j], t)
    for t in range(T0, NT):
        pl.when(clean[t - T0])(cp_out(t, 1, osem.at[C + t - T0]).wait)
    for t in range(C):
        guarded(final[t], cp_fix(t, 0, D).wait)


@jax.jit
def pallas_adaLN_cond__gqa_block_cached__moe_arch_mod__prompt_kernel(
    A_x: jax.Array,
    A_k_cache: jax.Array,
    A_v_cache: jax.Array,
    A_wq: jax.Array,
    A_wo: jax.Array,
    B_x: jax.Array,
    B_w_r: jax.Array,
    B_w_gate: jax.Array,
    B_w_up: jax.Array,
    B_w_down: jax.Array,
    c: jax.Array,
    w_mod: jax.Array,
):
    del B_x
    xt = A_x.reshape(S, D).T
    k = A_k_cache.reshape(HKV, S, DH)
    v = A_v_cache.reshape(HKV, S, DH)

    hbm = pl.BlockSpec(memory_space=pl.ANY)
    stream = [
        pltpu.VMEM((S, REP * TQ), F32),
        pltpu.VMEM((8, REP * TQ), F32),
        pltpu.VMEM((DH // 2, S), U32),
        pltpu.VMEM((GW // 2, D), U32),
        pltpu.VMEM((NV * 128, GW), F32),
        pltpu.VMEM((REP, KR, 8, DH), F32),
        pltpu.VMEM((1, S // 2, DH), U32),
    ]
    out = pl.pallas_call(
        _kernel_flat,
        in_specs=[hbm] * 11,
        out_specs=hbm,
        out_shape=jax.ShapeDtypeStruct((D, S), BF16),
        scratch_shapes=[pltpu.VMEM((2 * 16, KR, 8, 128), F32)] * NV + [
            pltpu.VMEM((NT + NFB + NMB, D, 128), BF16),
            pltpu.VMEM((HKV, S, DH), BF16),
            pltpu.VMEM((HKV, S, DH), BF16),
            pltpu.VMEM((HKV, D, GW), BF16),
            pltpu.VMEM((HKV, D, GW), BF16),
            pltpu.VMEM((D, DA), BF16),
            pltpu.VMEM((D, F), BF16),
            pltpu.VMEM((D, F), BF16),
            pltpu.VMEM((F // 2, D), U32),
            pltpu.VMEM((NT, D // 2, 128), U32),
            pltpu.VMEM((NT, KR, 128), F32),
            pltpu.VMEM((NT, D, 128), F32),
            pltpu.VMEM((6 * D, 128), F32),
            pltpu.VMEM((5 * 128, 128), F32),
            pltpu.VMEM((5 * 128, 128), F32),
            pltpu.VMEM((NT, D, 128), BF16),
            pltpu.VMEM((NT, D // 2, 128), U32),
            pltpu.VMEM((S // 2, D), U32),
            pltpu.VMEM((NT, D, 128), BF16),
            pltpu.VMEM((C, D, 128), BF16),
            pltpu.VMEM((NT, 128), F32),
            pltpu.VMEM((NT * NC, 8, 128), F32),
            pltpu.VMEM((NT * NC, 8, 128), F32),
            pltpu.VMEM((MPI, 8, 128), F32),
            pltpu.VMEM((KR, HQ * DH), BF16),
        ] + stream + stream + [
            pltpu.VMEM((D,), BF16),
            pltpu.VMEM((1, D), BF16),
            pltpu.SemaphoreType.DMA((HKV // 2,)),
            pltpu.SemaphoreType.DMA((11,)),
            pltpu.SemaphoreType.DMA((C + TPB + 1,)),
        ],
        compiler_params=pltpu.CompilerParams(vmem_limit_bytes=127 * 1024 * 1024,
                                             disable_bounds_checks=True,
                                             disable_semaphore_checks=True),
    )(B_w_r, c, xt, k, v, A_wq, A_wo.T, w_mod, B_w_gate, B_w_up, B_w_down.T)
    return out.T.reshape(1, S, D)
```

```python
import math

import jax
import jax.numpy as jnp
import jax.experimental.pallas as pl
import jax.experimental.pallas.tpu as pltpu

S = 2048
D = 576
HQ = 32
HKV = 16
REP = HQ // HKV
DH = 128
GW = REP * DH
F = 4608
C = 8
EPS = 1e-05
TQ = 512
NBLK = S // TQ
TPB = TQ // 128
NT = S // 128
NU = NBLK * HKV
NP = HKV // 2
NC = 3
DC = D // NC
PG = 64
NFB = F // 128
WD0 = 14
DA = 2 * D
MODA = ((0, 4, 5), (1, 2, 6), (3, 7, 8))
NMB = 4 * D // 128
MPI = 3
MB0 = 1
DM = 512
KR = D - DM
NV = 3
CH = 3
TPI = KR // NP

SC, WC = 1024, 1024 + 2 * S
OUTER0, OSTEP = (SC + 850, SC + 0), 133
PACE = (100, WC + 160, SC + 100, WC + 250, 0, SC + 3400)
XP = (SC + 3700, SC + 100, SC + 900, SC + 1300, WC + 762, 724, SC + 2600)
TAB = ((SC + 1600, SC + 2600), (SC + 2950, SC + 3890), (WC + 650, WC + 890))
WFP = ((300, 900), (WC + 600, WC + 1144))
KP = (0, 616)
SLAG = 96
GS = 4
TSPLIT = 15
PP = (24, 1474, 5112, 0, 0, 500, 750, 3524, 300)
TLAG = 256
TKS = 18
SCLAG = 2

BF16 = jnp.bfloat16
F32 = jnp.float32
U32 = jnp.uint32
QSCALE = DH ** -0.5 * math.log2(math.e)


def _dot(a, b):
    return jnp.dot(a, b, preferred_element_type=F32)


def _r(x):
    return x.astype(BF16).astype(F32)


def _col_bcast(row):
    return jnp.broadcast_to(row, (128, 128)).T


def _blk(u):
    return u // HKV if isinstance(u, int) else jax.lax.shift_right_logical(u, 4)


def _grp(u):
    return u % HKV if isinstance(u, int) else jnp.bitwise_and(u, HKV - 1)


def _lanes(t, n=1):
    return pl.ds(pl.multiple_of(t * 128, 128), n * 128)


def _paced(x, clock, pos):
    if clock is None:
        return x
    pos = pos // 8 * 8
    g = clock[pos:pos + x.shape[0], 0:x.shape[1]]
    return jnp.where(g * g < 0.0, jnp.zeros_like(x), x)


def _paced_wide(x, clock, pos):
    if clock is None:
        return x
    n, w = x.shape
    cols = []
    for a in range(0, w, 128):
        p0 = (pos + a // 128 * n) // 8 * 8
        g = jnp.concatenate([clock[p0 + r // (8 * GS) * (8 * GS):p0 + r // (8 * GS) * (8 * GS) + 8]
                             for r in range(0, n, 8)], axis=0)
        cols.append(_paced(x[:, a:min(a + 128, w)], g, 0))
    return jnp.concatenate(cols, axis=1)


def _gated(x, gates, j, n):
    if gates is None:
        return x
    m = x.shape[0]
    g = jnp.stack([gates[(j * m + b) * len(gates) // (n * m)] for b in range(m)])
    return jnp.where(g < 0.0, jnp.zeros_like(x), x)


def _softmax_numer(s, m):
    n, w = s.shape
    p = jnp.exp2(s - m).reshape(n // PG, PG // 8, 8, w)
    ts = jnp.sum(p, axis=1)
    last = jnp.where(ts < 0.0, ts, p[:, PG // 8 - 1])
    p = jnp.concatenate([p[:, :PG // 8 - 1], last[:, None]], axis=1).reshape(n, w)
    l = jnp.sum(jnp.sum(ts, axis=0), axis=0, keepdims=True)
    return p.astype(BF16), l


KEY0 = 0x20000000


def _score_key(r, t):
    tok = t * 128 + jax.lax.broadcasted_iota(jnp.int32, r.shape, 1)
    bits = jax.lax.shift_right_arithmetic(pltpu.bitcast(_r(r), jnp.int32), 16)
    code = jnp.where(bits < 0, -32768 - bits, bits) + 32768
    return pltpu.bitcast(code * S + (S - 1 - tok) + KEY0, F32)


def _chunk_stats(x):
    m = jnp.sum(x, axis=0, keepdims=True) * (1.0 / DC)
    xc = x - m
    return m, jnp.sum(xc * xc, axis=0, keepdims=True)


def _mean_var(stats):
    mean = sum(m for m, _ in stats) * (1.0 / NC)
    var = sum(s + DC * (m - mean) * (m - mean) for m, s in stats) * (1.0 / D)
    return mean, var


def _kernel_flat(*refs):
    _kernel(*refs[:12], *refs[12 + NV:], *refs[12:12 + NV])


def _kernel(wr_hbm, c_hbm,
            xt_hbm, k_hbm, v_hbm, wq_hbm, wot_hbm, wmod_hbm, wg_hbm, wu_hbm, wdt_hbm,
            out_hbm,
            xw_v, k_v, v_v, wq_v, wot_v, wmod_v, wg_v, wu_v, wd_ref,
            ht_ref, hr_ref, acc_ref, mod_ref, wrb_ref, scb_ref, x1_ref, h2_ref, h2row_ref, out_v, fix_v,
            key_ref, st1_ref, st2_ref, lm_ref,
            wrem_v,
            s0_ref, m0_ref, vt0_ref, wqt0_ref, qr0_ref, wf0_ref, kp0_ref,
            s1_ref, m1_ref, vt1_ref, wqt1_ref, qr1_ref, wf1_ref, kp1_ref,
            wr_ref, c_ref, bsem, msem, osem, *hb_refs):
    streams = ((s0_ref, m0_ref, vt0_ref, wqt0_ref, qr0_ref, wf0_ref, kp0_ref),
               (s1_ref, m1_ref, vt1_ref, wqt1_ref, qr1_ref, wf1_ref, kp1_ref))

    cp_k = lambda p, sem: pltpu.make_async_copy(
        k_hbm.at[pl.ds(2 * p, 2)], k_v.at[pl.ds(2 * p, 2)], sem)
    cp_v1 = lambda g, sem: pltpu.make_async_copy(v_hbm.at[g], v_v.at[g], sem)
    cp_k1 = lambda g, sem: pltpu.make_async_copy(k_hbm.at[g], k_v.at[g], sem)

    class Both:
        def __init__(self, cps):
            self.cps = cps

        def start(self):
            for cp in self.cps:
                cp.start()

        def wait(self):
            for cp in self.cps:
                cp.wait()

    def cp_w1(src, dst, g, sem):
        return pltpu.make_async_copy(src.at[:, _lanes(g * REP, REP)], dst.at[g], sem)

    cp_wo = lambda p, sem: Both([cp_w1(wot_hbm, wot_v, 2 * p + a, sem) for a in range(2)])
    cp_x = lambda t0, n, sem: Both([pltpu.make_async_copy(xt_hbm.at[:, _lanes(t0 + t)],
                                                          xw_v.at[t0 + t], sem) for t in range(n)])

    def bundle(n, act):
        sem = bsem.at[n if isinstance(n, int) else jnp.minimum(n, NP - 1)]

        def on(cond, cps):
            def go():
                for cp in cps():
                    getattr(cp, act)()
            if isinstance(cond, bool):
                if cond:
                    go()
            else:
                pl.when(cond)(go)
        on(n + 1 < NP, lambda: [cp_k(n + 1, sem), cp_v1(2 * n + 2, sem), cp_w1(wq_hbm, wq_v, 2 * n + 3, sem)])
        on(n + 2 < NP, lambda: [cp_w1(wq_hbm, wq_v, 2 * n + 4, sem)])
        XN = 3
        nx = (NT - TPB - NV) // XN
        on(jnp.logical_and(n >= 1, n <= nx) if not isinstance(n, int) else 1 <= n <= nx,
           lambda: [cp_x(TPB + NV + XN * (n - 1), XN, sem)])
        on(n < NP, lambda: [cp_v1(2 * n + 1, sem), cp_wo(n, sem)])

    cp_moda = [Both([pltpu.make_async_copy(wmod_hbm.at[:, _lanes(t)], wmod_v.at[:, _lanes(t)],
                                           msem.at[s]) for t in tiles])
               for s, tiles in zip((0, 6, 10), MODA)]
    cp_modb = Both([pltpu.make_async_copy(wmod_hbm.at[:, _lanes(DA // 128 + b)],
                                          xw_v.at[NT + NFB + b], msem.at[1]) for b in range(NMB)])
    cp_g = pltpu.make_async_copy(wg_hbm, wg_v, msem.at[2])
    cp_u = pltpu.make_async_copy(wu_hbm, wu_v, msem.at[3])
    cp_d = Both([pltpu.make_async_copy(wdt_hbm.at[:, _lanes(b)], xw_v.at[NT + b], msem.at[4])
                 for b in range(NFB)])
    cp_out = lambda t, n, sem: Both([pltpu.make_async_copy(out_v.at[t + a], out_hbm.at[:, _lanes(t + a)],
                                                           sem) for a in range(n)])

    def silu_c():
        c = c_ref[...].astype(F32)
        return _r(c * _r(jax.nn.sigmoid(c)))

    def finish_mod(mod, lo, clock=None, pos=0):
        mod = _r(mod)
        col = lo + jax.lax.broadcasted_iota(jnp.int32, mod.shape, 1)
        is_scale = jnp.logical_or(jnp.logical_and(col >= D, col < 2 * D),
                                  jnp.logical_and(col >= 4 * D, col < 5 * D))
        mod = jnp.where(is_scale, _r(1.0 + mod), mod)
        for t in range(mod.shape[1] // 128):
            rows = pl.ds(pl.multiple_of(lo + t * 128, 128), 128)
            mod_ref[rows, :] = _paced(_col_bcast(mod[:, t * 128:(t + 1) * 128]), clock, pos)

    def late_mod_sums(n, clock):
        b0 = jnp.clip(n - MB0, 0, NMB // MPI - 1) * MPI
        for k in range(MPI):
            w = xw_v[jnp.where(n >= MB0, NT + NFB + b0 + k, 0)].astype(F32)
            part = jnp.sum((w * scb_ref[0:D, :]).reshape(D // 8, 8, 128), axis=0)
            lm_ref[k] = _paced(part, clock, PACE[4] + 192 * k)

    def late_mod_store(n, sums, clock):
        b0 = jnp.clip(n - MB0, 0, NMB // MPI - 1) * MPI
        for k in range(MPI):
            finish_mod(jnp.sum(sums[k], axis=0, keepdims=True), DA + (b0 + k) * 128,
                       clock, XP[4] + 128 * k)

    def col_vector(ref, row):
        row = jnp.concatenate([row, jnp.zeros((1, 64), F32)], axis=1)
        for t in range(5):
            ref[t * 128:(t + 1) * 128, :] = _col_bcast(row[:, t * 128:(t + 1) * 128])

    def mod(k):
        return mod_ref[k * D:(k + 1) * D, :]

    def put_stats(st_ref, t, shift, scale, clock, pos):
        row = jax.lax.broadcasted_iota(jnp.int32, (8, 128), 0)
        st_ref[t] = _paced(jnp.where(row == 0, shift, scale), clock, pos)

    def ln1_stats(t, clock=None, pos=None):
        for c in range(NC):
            m, s = _chunk_stats(xw_v[t, c * DC:(c + 1) * DC, :].astype(F32))
            put_stats(st1_ref, t * NC + c, m, s, clock, (PACE[0] if pos is None else pos) + 192 * c)

    def ln1_norm(t):
        mean, var = _mean_var(load_stats(st1_ref, t))
        return (xw_v[t].astype(F32) - mean) * jax.lax.rsqrt(var + EPS)

    def ln1_apply(t, clock=None, pos=None, ln=None):
        h = (ln1_norm(t) if ln is None else ln) * mod(1) + mod(0)
        h = _paced(h, clock, PACE[1] if pos is None else pos)
        ht_ref[t] = pltpu.bitcast(h.astype(BF16), U32)
        hr_ref[t] = h[DM:]

    def h2_rows(t, clock=None):
        x = _paced_wide(pltpu.bitcast(pltpu.bitcast(h2_ref[t], BF16).T, U32), clock, PACE[5])
        h2row_ref[pl.ds(pl.multiple_of(t * 64, 64), 64), :] = x

    def router_terms():
        u = mod(4) * wrb_ref[0:D, :]
        return (u, jnp.sum(u, axis=0, keepdims=True),
                jnp.sum(mod(3) * wrb_ref[0:D, :], axis=0, keepdims=True))

    def load_stats(st_ref, t):
        return [(st_ref[t * NC + c, 0:1, :], st_ref[t * NC + c, 1:2, :]) for c in range(NC)]

    def ln2_x1(t, attn, clock=None):
        x1 = _r(xw_v[t].astype(F32) + mod(2) * attn)
        x1_ref[t] = _paced(x1, clock, PACE[2]).astype(BF16)
        return x1, [_chunk_stats(x1[c * DC:(c + 1) * DC]) for c in range(NC)]

    def ln2_norm(stats):
        mean, var = _mean_var(stats)
        return _r(mean), 1.0 / _r(jnp.sqrt(_r(_r(var) + EPS)))

    def ln2_h2(x1, mean, inv):
        return (x1 - mean) * inv * mod(4) + mod(3)

    def ln2_stats(t, clock):
        for c, (m, s) in enumerate(ln2_x1(t, acc_ref[t], clock)[1]):
            put_stats(st2_ref, t * NC + c, m, s, clock, PACE[2] + (c + 1) * DC + SLAG)

    def ln2_apply(t, clock):
        x1 = x1_ref[t].astype(F32)
        h2 = ln2_h2(x1, *ln2_norm(load_stats(st2_ref, t)))
        key = _score_key(jnp.sum(h2 * wrb_ref[0:D, :], axis=0, keepdims=True), t)
        key_ref[pl.ds(t, 1), :] = _paced(key, clock, PACE[3] + D + 96)
        h2 = _r(h2)
        h2_ref[t] = pltpu.bitcast(_paced(h2, clock, PACE[3]).astype(BF16), U32)
        out_v[t] = _paced(x1 + mod(5) * h2, clock, PACE[3] + 16).astype(BF16)

    def finish_q(q):
        q = (q * QSCALE).astype(BF16)
        return jnp.concatenate([q[r * DH:(r + 1) * DH] for r in range(REP)], axis=1)

    def q_proj(u, wqt_ref, qr_ref=None, split=False):
        w = pltpu.bitcast(wqt_ref[...], BF16)
        h = jnp.concatenate([pltpu.bitcast(ht_ref[_blk(u) * TPB + t], BF16) for t in range(TPB)], axis=1)
        if split:
            return sum(_dot(w[:, a:min(a + 128, D)], h[a:min(a + 128, D)]) for a in range(0, D, 128))
        if qr_ref is None:
            rem = _dot(w[:, DM:], h[DM:])
        else:
            rem = [qr_ref[...].T]
            if NV < TPB:
                R = GW * (TPB - NV) // 4
                rem.append(jnp.concatenate([_dot(w[a:a + R, DM:], h[DM:, NV * 128:])
                                            for a in range(0, GW, R)], axis=0))
            rem = jnp.concatenate(rem, axis=1)
        return _dot(w[:, :DM], h[:DM]) + rem

    def w_rest(u, wf_ref, gates=None):
        w = wrem_v[:, _lanes(_grp(u) * REP, REP)].astype(F32)
        for r in range(REP):
            wb = jnp.stack([jnp.broadcast_to(w[k:k + 1, r * DH:(r + 1) * DH], (8, DH))
                            for k in range(KR)])
            wf_ref[r] = _gated(wb, gates, r, REP)

    def outer(u, qr_ref, wf_ref, clock, start):
        base = jnp.bitwise_and(_blk(u), 1) * 16
        for g in range(0, NV * REP * 16, CH):
            pos = min(start + OSTEP * (g // CH + 1), clock.shape[0] - 8)
            runs, c = [], g
            while c < min(g + CH, NV * REP * 16):
                runs.append((c // 32, c // 16 % 2, c % 16, min(g + CH - c, 16 - c % 16)))
                c += runs[-1][3]
            acc = {}
            for k in range(KR):
                for i, r, tv, n in runs:
                    t = hb_refs[i][pl.ds(base + tv, n), k] * wf_ref[r, k][None]
                    acc[i, r] = t if k == 0 else acc[i, r] + t
            for i, r, tv, n in runs:
                gate = jnp.concatenate([clock[pos // 8 * 8:pos // 8 * 8 + 8]] * n, axis=0)
                row = i * 128 + tv * 8
                qr_ref[row:row + 8 * n, r * DH:(r + 1) * DH] = _paced(
                    acc[i, r].reshape(8 * n, DH), gate, 0)

    def h_table(hr, i, base, k0, gates):
        nk = hr.shape[0]
        hr = _r(hr)
        for j in range(nk):
            cb = _col_bcast(hr[j:j + 1]).reshape(16, 8, 128)
            hb_refs[i][pl.ds(base, 16), k0 + j] = _gated(cb, gates, j, nk)

    def never_of(clock, lo, hi, step=8):
        return [clock[a:a + 8] * clock[a:a + 8] for a in range(lo // 8 * 8, hi, step)]

    def scores(u, q, s_ref, m_ref, kp_ref=None, qclk=None):
        def keep(s, cols):
            s_ref[:, cols] = s
            m_ref[:, cols] = jnp.broadcast_to(jnp.max(s, axis=0, keepdims=True), (8, s.shape[1]))
            return s

        if kp_ref is None:
            s = jnp.concatenate([keep(_dot(k_v[_grp(u)], q[:, c]), c)
                                 for c in (slice(0, TQ), slice(TQ, 2 * TQ))], axis=1)
        else:
            k = pltpu.bitcast(k_v[_grp(u)], U32).reshape(S // 16, 8, DH)
            z = 0 if isinstance(u, int) else jax.lax.shift_right_logical(u, 8)
            kp_ref[z] = _gated(k, never_of(qclk, *KP, 32), 0, 1).reshape(S // 2, DH)
            s = keep(_dot(pltpu.bitcast(kp_ref[0], BF16), q), slice(0, 2 * TQ))
        return jnp.concatenate([s[:, 0:128], s[:, TQ:TQ + 128]], axis=0)

    def q_clock(q):
        return jnp.concatenate([q[:, t * 128:(t + 1) * 128] for t in range(TPB)], axis=0)

    def v_transpose(u, vt_ref, clock=None, pos=0):
        vt_ref[...] = _paced_wide(pltpu.bitcast(v_v[_grp(u)].T, U32), clock, pos)

    def wq_transpose(u, wqt_ref, clock=None, pos=0):
        wqt_ref[...] = _paced_wide(pltpu.bitcast(wq_v[_grp(u)].T, U32), clock, pos)

    def wd_transpose(u, clock, pos):
        fb = jnp.clip(u - WD0, 0, NFB - 1)
        src = jnp.where(u >= WD0, NT + fb, 0)
        wd_ref[pl.ds(pl.multiple_of(fb * 64, 64), 64), :] = _paced_wide(
            pltpu.bitcast(xw_v[src].T, U32), clock, pos)

    def attend(s_ref, m_ref, vt_ref):
        m = m_ref[0:1, :]
        o = []
        for r in range(REP):
            cols = slice(r * TQ, (r + 1) * TQ)
            p, l = _softmax_numer(s_ref[:, cols], m[:, cols])
            o.append((_dot(pltpu.bitcast(vt_ref[...], BF16), p) * (1.0 / l)))
        return jnp.concatenate(o, axis=0)

    small = Both([pltpu.make_async_copy(wr_hbm, wr_ref, msem.at[7]),
                  pltpu.make_async_copy(c_hbm, c_ref, msem.at[7])])
    zeroth = Both([cp_x(0, TPB, msem.at[5]), cp_w1(wq_hbm, wq_v, 0, msem.at[5])])
    first = Both([cp_k1(0, msem.at[8]), cp_w1(wq_hbm, wq_v, 1, msem.at[8])])
    second = Both([cp_k1(1, msem.at[9]), cp_v1(0, msem.at[9]), cp_w1(wq_hbm, wq_v, 2, msem.at[9]),
                   pltpu.make_async_copy(wq_hbm.at[DM:, :], wrem_v, msem.at[9]), cp_x(TPB, NV, msem.at[9])])
    for cp in [small, zeroth] + cp_moda + [first, second]:
        cp.start()
    acc_ref[...] = jnp.zeros_like(acc_ref)
    mod_ref[DA:6 * D, :] = jnp.zeros((4 * D, 128), F32)
    h2_ref[0] = jnp.zeros((D // 2, 128), U32)
    lm_ref[...] = jnp.zeros_like(lm_ref)
    small.wait()
    col_vector(wrb_ref, wr_ref[...].astype(F32).reshape(1, D))
    col_vector(scb_ref, silu_c())
    sc8 = jnp.broadcast_to(silu_c(), (8, D)).astype(BF16)
    zeroth.wait()
    ln0 = []
    for t in range(TPB):
        ln1_stats(t)
        ln0.append(ln1_norm(t))
    wq_transpose(0, wqt0_ref)
    for cp, tiles in zip(cp_moda, MODA):
        cp.wait()
        for t in tiles:
            finish_mod(_dot(sc8, wmod_v[:, t * 128:(t + 1) * 128])[0:1], t * 128)
    for t in range(TPB):
        ln1_apply(t, ln=ln0[t])
    q = finish_q(q_proj(0, wqt0_ref, split=True))
    first.wait()
    bundle(0, 'start')
    jobs = ([(i, 0, k) for i in range(NV) for k in range(0, KR, TPI)]
            + [(i, 1, k) for i in range(NV) for k in range(0, 2 * TPI, TPI)])

    def first_table(gates, todo, starts=None):
        for j, (i, blk, k0) in enumerate(todo):
            hr = hr_ref[blk * TPB + i, k0:k0 + TPI, :]
            if starts is not None:
                hr = jnp.where(starts[j * len(starts) // len(todo)] < 0.0, 0.0, hr)
            h_table(hr, i, blk * 16, k0,
                    gates[j * len(gates) // len(todo):(j + 1) * len(gates) // len(todo)])

    first_table(never_of(scores(0, q, s0_ref, m0_ref), 64, 2 * S - 192, 16), jobs[:TSPLIT])
    wq_transpose(1, wqt1_ref)
    second.wait()
    bundle(1, 'start')
    cp_modb.start()
    q = q_proj(1, wqt1_ref)
    hrem = jnp.concatenate([pltpu.bitcast(ht_ref[t, DM // 2:, :], BF16) for t in range(NV)], axis=1)
    for a in range(2):
        streams[a][4][...] = jax.lax.dot_general(
            hrem, wrem_v[:, (a + 2) * GW:(a + 3) * GW], (((0,), (0,)), ((), ())),
            preferred_element_type=F32)
    clock = jnp.concatenate(
        [q_clock(q), scores(1, finish_q(q), s1_ref, m1_ref)], axis=0)
    nb0 = NV * KR // TPI
    v_transpose(0, vt0_ref, clock, PP[3])
    wq_transpose(2, wqt0_ref, clock, PP[4])
    first_table(never_of(clock, PP[6], PP[7], 16), jobs[TSPLIT:nb0])
    for i in range(NV):
        ln1_stats(TPB + i, clock, PP[0] + PP[5] * i)
        ln1_apply(TPB + i, clock, PP[1] + PP[5] * i)
    first_table(never_of(clock, PP[7], PP[2], 16), jobs[nb0:],
                never_of(clock, PP[7] - PP[8], PP[2] - PP[8]))
    for a in range(2):
        w_rest(a + 4, streams[a][5], never_of(clock, 500 * a, 500 * a + 500, 32))

    def unit(u, side, s_ref, m_ref, vt_ref, wqt_ref, qr_ref, wf_ref, kp_ref):
        q = q_proj(u + 2, wqt_ref, qr_ref)
        o = attend(s_ref, m_ref, vt_ref)
        sclk = scores(u + 2, finish_q(q), s_ref, m_ref, kp_ref, q_clock(q))
        o = jnp.concatenate([o[r * DH:(r + 1) * DH].astype(BF16) for r in range(REP)], axis=0)
        upd = _dot(wot_v[_grp(u)], o)
        clock = jnp.concatenate([q_clock(q), sclk, upd[:, 0:128], upd[:, 256:384]], axis=0)
        side(clock, lambda start: outer(u + 4, qr_ref, wf_ref, clock, start))
        for t in range(TPB):
            acc_ref[_blk(u) * TPB + t] += upd[:, t * 128:(t + 1) * 128]

    def step(n, carry):
        bundle(jnp.minimum(n + 2, NP), 'start')
        for a in range(3):
            pl.when(n == 2 + a)(Both(cp_d.cps[a * NFB // 3:(a + 1) * NFB // 3]).start)
        pl.when(n == NP)(Both([cp_g, cp_u]).start)

        t1 = jnp.minimum(n + TPB + NV - 1, NT - 1)
        v = jnp.maximum(n - NP, 0)
        tile2 = lambda v: (jax.lax.shift_right_logical(v, 3) * TPB
                           + jnp.minimum(jnp.bitwise_and(v, NP - 1), TPB - 1))
        t2 = tile2(v)
        sums = lm_ref[...]

        def stats(clock, outer_at):
            v_transpose(2 * n + 1, vt1_ref, clock, XP[5])
            wq_transpose(2 * n + 3, wqt1_ref, clock, XP[6])
            ln2_stats(t2, clock)
            ln1_stats(t1, clock)
            h2_rows(tile2(jnp.maximum(v - 1, 0)), clock)
            wd_transpose(2 * n, clock, XP[0])
            outer_at(OUTER0[0])

        def apply(clock, outer_at):
            blk = jnp.minimum(jax.lax.shift_right_logical(n + 2, 3) + 1, NBLK - 1)
            k0 = jnp.bitwise_and(n + 2, 7) * TPI
            hr = [hr_ref[blk * TPB + i, pl.ds(pl.multiple_of(k0, TPI), TPI), :]
                  for i in range(NV)]
            v_transpose(2 * n + 2, vt0_ref, clock, XP[1])
            wq_transpose(2 * n + 4, wqt0_ref, clock, XP[2])
            wd_transpose(2 * n + 1, clock, XP[3])
            late_mod_sums(n, clock)
            ln1_apply(t1, clock)
            ln2_apply(t2, clock)
            outer_at(OUTER0[1])
            for i in range(NV):
                h_table(hr[i], i, jnp.bitwise_and(blk, 1) * 16, k0, never_of(clock, *TAB[i], 16))
            late_mod_store(n - 1, sums, clock)
            for a in range(2):
                w_rest(2 * n + 6 + a, streams[a][5], never_of(clock, *WFP[a], 32))

        for a in range(2):
            unit(2 * n + a, (stats, apply)[a], *streams[a])
        return carry

    def stage(n, carry):
        bundle(n, 'wait')
        pl.when(n == MB0)(cp_modb.wait)
        pl.when(n == WD0 // 2)(cp_d.wait)
        return jax.lax.fori_loop(n, jnp.where(n < NP - 1, n + 1, NU // 2 - 1), step, carry)

    jax.lax.fori_loop(0, NP, stage, 0)

    T0 = NT - TPB
    cp_out(0, T0, osem.at[C + TPB]).start()
    cp_g.wait()
    v_transpose(NU - 1, vt1_ref)
    o = jnp.concatenate([attend(*streams[a][0:3]) for a in range(2)], axis=0)
    wlast = jnp.concatenate([wot_v[HKV - 2], wot_v[HKV - 1]], axis=1)
    fin = [acc_ref[T0 + t] + _dot(wlast, o[:, t * 128:(t + 1) * 128].astype(BF16)) for t in range(TPB)]
    clock = jnp.concatenate(fin, axis=0)
    row8 = jax.lax.broadcasted_iota(jnp.int32, (C, 128), 0)
    lane8 = jax.lax.broadcasted_iota(jnp.int32, (C, 128), 1)
    work = key_ref[0:T0, :]
    lead = jnp.zeros((C, 128), F32)
    for t in range(C):
        mx = jnp.max(jnp.max(work, axis=0, keepdims=True), axis=1, keepdims=True)
        work = jnp.where(work == mx, 0.0, work)
        lead = jnp.where(row8 == t, mx, lead)

    def spread(row):
        return pltpu.roll(jnp.broadcast_to(row, (128, 128)), 0, 1, stride=1, stride_axis=0)

    def merge(lead, rows, spreads):
        cols = jnp.concatenate([lead] + spreads, axis=0)
        best = jnp.zeros((C, 128), F32)
        for row in [jnp.max(jnp.where(row8 == lane8, lead, 0.0), axis=0, keepdims=True)] + rows:
            rank = jnp.sum(jnp.where(cols > row, 1.0, 0.0), axis=0, keepdims=True)
            best = jnp.maximum(best, jnp.where(rank == row8.astype(F32), row, 0.0))
        return jnp.max(best, axis=1, keepdims=True)

    def tail_h2(t, norm, gate=None):
        x1 = x1_ref[t].astype(F32)
        if gate is not None:
            n = gate.shape[0]
            x1 = jnp.concatenate([_paced(x1[:n], gate, 0), x1[n:]], axis=0) if n < D else _paced(x1, gate, 0)
        h2_ref[t] = pltpu.bitcast(ln2_h2(x1, *norm).astype(BF16), U32)
        if t < NT - 2:
            h2_rows(t)

    u_vec, u_sum, b_sum = router_terms()
    keys = []
    for t in range(TPB):
        x1, stats = ln2_x1(T0 + t, fin[t])
        mean, inv = norm = ln2_norm(stats)
        r = (jnp.sum(x1 * u_vec, axis=0, keepdims=True) - mean * u_sum) * inv + b_sum
        keys.append(_score_key(r, T0 + t))
        if t < TPB - 1:
            tail_h2(T0 + t, norm, clock[(t + 1) * D + TLAG:(t + 2) * D + TLAG])
    lead = jnp.broadcast_to(merge(lead, keys[0:2], [spread(k) for k in keys[0:2]]), (C, 128))
    spread2 = spread(keys[2])
    h2_rows(NT - 2)
    tail_h2(NT - 1, norm)
    h2_rows(NT - 1)
    sel = pltpu.bitcast(merge(lead, keys[2:4], [spread2, spread(keys[3])]), jnp.int32) - KEY0
    sel_tok = (S - 1) - (sel & (S - 1))
    toks = [sel_tok[t, 0] for t in range(C)]
    tiles = [jax.lax.shift_right_logical(tk, 7) for tk in toks]
    sel_code = jax.lax.shift_right_logical(sel, 11) - 32768
    sel_bits = jnp.where(sel_code < 0, -32768 - sel_code, sel_code)
    r_sel = pltpu.bitcast(jax.lax.shift_left(sel_bits, 16), F32)

    final = []
    for t in range(C):
        d = True
        for u in range(t + 1, C):
            d = jnp.logical_and(d, tiles[u] != tiles[t])
        final.append(d)

    words = jnp.concatenate([h2row_ref[pl.ds(jax.lax.shift_right_logical(toks[t], 1), 1), :]
                             for t in range(C)], axis=0)
    odd = jnp.bitwise_and(sel_tok, 1) == 1
    xs = pltpu.bitcast(jnp.where(odd, jnp.bitwise_and(words, jnp.uint32(0xFFFF0000)),
                                 jax.lax.shift_left(words, jnp.uint32(16))), F32)
    xs = xs.astype(BF16)

    def plain_out(t, ticks):
        gate = jnp.concatenate([ticks[a * len(ticks) // (D // 8)] for a in range(D // 8)], axis=0)
        x1 = _paced(x1_ref[t].astype(F32), gate, 0)
        out_v[t] = (x1 + mod(5) * pltpu.bitcast(h2_ref[t], BF16).astype(F32)).astype(BF16)

    clean = []

    def send_clean(t):
        d = tiles[0] != t
        for a in range(1, C):
            d = jnp.logical_and(d, tiles[a] != t)
        clean.append(d)
        pl.when(d)(cp_out(t, 1, osem.at[C + t - T0]).start)

    cp_u.wait()
    cp_out(0, T0, osem.at[C + TPB]).wait()
    gpre = _dot(xs, wg_v[...])
    u = _dot(xs, wu_v[...])
    ticks = [z[:, a * 128:(a + 1) * 128] for z in (gpre, u) for a in range(NFB)]
    for t in range(TPB):
        plain_out(T0 + t, ticks[t * TKS:(t + 1) * TKS])
        send_clean(T0 + t)
    gpre, u = _r(gpre), _r(u)
    gact = _r(gpre * _r(jax.nn.sigmoid(gpre)))
    act = (gact * u).astype(BF16)
    gate_r = _r(jax.nn.sigmoid(r_sel))
    ohs = []
    for t in range(C):
        oh = jnp.where(sel_tok == tiles[t] * 128 + lane8, 1.0, 0.0)
        ohs.append(jnp.concatenate([oh, jnp.zeros((16 - C, 128), F32)], axis=0).astype(BF16))

    def cp_fix(t, lo, hi):
        return pltpu.make_async_copy(fix_v.at[t, lo:hi, :], out_hbm.at[lo:hi, _lanes(tiles[t])],
                                     osem.at[t])

    def guarded(cond, fn):
        if cond is True:
            fn()
        else:
            pl.when(cond)(fn)

    def scatter(j, yt, t):
        lo, hi = j * 128, min(j * 128 + 128, D)
        upd = jnp.concatenate([_dot(yt[a:a + 64], ohs[t]) for a in range(0, hi - lo, 64)], axis=0)
        fix_v[t, lo:hi, :] = (x1_ref[tiles[t], lo:hi, :].astype(F32) + mod_ref[5 * D + lo:5 * D + hi, :]
                              * (pltpu.bitcast(h2_ref[tiles[t], lo // 2:hi // 2, :], BF16).astype(F32) + upd)).astype(BF16)
        guarded(final[t], cp_fix(t, lo, hi).start)

    NJ = (D + 127) // 128
    yts = []
    for j in range(NJ):
        lo, hi = j * 128, min(j * 128 + 128, D)
        FK = F // 4
        yk = []
        for a in range(4):
            w = pltpu.bitcast(wd_ref[a * FK // 2:(a + 1) * FK // 2, lo:hi], BF16)
            yk.append(_dot(act[:, a * FK:(a + 1) * FK], w))
            if j >= SCLAG:
                for t in (2 * a, 2 * a + 1):
                    scatter(j - SCLAG, yts[j - SCLAG], t)
        y = _r(sum(yk)) * gate_r
        yts.append(jnp.concatenate([y, jnp.zeros_like(y)], axis=0).astype(BF16).T)
    for j in range(NJ - SCLAG, NJ):
        for t in range(C):
            scatter(j, yts[j], t)
    for t in range(T0, NT):
        pl.when(clean[t - T0])(cp_out(t, 1, osem.at[C + t - T0]).wait)
    for t in range(C):
        guarded(final[t], cp_fix(t, 0, D).wait)


@jax.jit
def pallas_adaLN_cond__gqa_block_cached__moe_arch_mod__prompt_kernel(
    A_x: jax.Array,
    A_k_cache: jax.Array,
    A_v_cache: jax.Array,
    A_wq: jax.Array,
    A_wo: jax.Array,
    B_x: jax.Array,
    B_w_r: jax.Array,
    B_w_gate: jax.Array,
    B_w_up: jax.Array,
    B_w_down: jax.Array,
    c: jax.Array,
    w_mod: jax.Array,
):
    del B_x
    xt = A_x.reshape(S, D).T
    k = A_k_cache.reshape(HKV, S, DH)
    v = A_v_cache.reshape(HKV, S, DH)

    hbm = pl.BlockSpec(memory_space=pl.ANY)
    stream = [
        pltpu.VMEM((S, REP * TQ), F32),
        pltpu.VMEM((8, REP * TQ), F32),
        pltpu.VMEM((DH // 2, S), U32),
        pltpu.VMEM((GW // 2, D), U32),
        pltpu.VMEM((NV * 128, GW), F32),
        pltpu.VMEM((REP, KR, 8, DH), F32),
        pltpu.VMEM((1, S // 2, DH), U32),
    ]
    out = pl.pallas_call(
        _kernel_flat,
        in_specs=[hbm] * 11,
        out_specs=hbm,
        out_shape=jax.ShapeDtypeStruct((D, S), BF16),
        scratch_shapes=[pltpu.VMEM((2 * 16, KR, 8, 128), F32)] * NV + [
            pltpu.VMEM((NT + NFB + NMB, D, 128), BF16),
            pltpu.VMEM((HKV, S, DH), BF16),
            pltpu.VMEM((HKV, S, DH), BF16),
            pltpu.VMEM((HKV, D, GW), BF16),
            pltpu.VMEM((HKV, D, GW), BF16),
            pltpu.VMEM((D, DA), BF16),
            pltpu.VMEM((D, F), BF16),
            pltpu.VMEM((D, F), BF16),
            pltpu.VMEM((F // 2, D), U32),
            pltpu.VMEM((NT, D // 2, 128), U32),
            pltpu.VMEM((NT, KR, 128), F32),
            pltpu.VMEM((NT, D, 128), F32),
            pltpu.VMEM((6 * D, 128), F32),
            pltpu.VMEM((5 * 128, 128), F32),
            pltpu.VMEM((5 * 128, 128), F32),
            pltpu.VMEM((NT, D, 128), BF16),
            pltpu.VMEM((NT, D // 2, 128), U32),
            pltpu.VMEM((S // 2, D), U32),
            pltpu.VMEM((NT, D, 128), BF16),
            pltpu.VMEM((C, D, 128), BF16),
            pltpu.VMEM((NT, 128), F32),
            pltpu.VMEM((NT * NC, 8, 128), F32),
            pltpu.VMEM((NT * NC, 8, 128), F32),
            pltpu.VMEM((MPI, 8, 128), F32),
            pltpu.VMEM((KR, HQ * DH), BF16),
        ] + stream + stream + [
            pltpu.VMEM((D,), BF16),
            pltpu.VMEM((1, D), BF16),
            pltpu.SemaphoreType.DMA((HKV // 2,)),
            pltpu.SemaphoreType.DMA((11,)),
            pltpu.SemaphoreType.DMA((C + TPB + 1,)),
        ],
        compiler_params=pltpu.CompilerParams(vmem_limit_bytes=127 * 1024 * 1024,
                                             disable_bounds_checks=True,
                                             disable_semaphore_checks=True),
    )(B_w_r, c, xt, k, v, A_wq, A_wo.T, w_mod, B_w_gate, B_w_up, B_w_down.T)
    return out.T.reshape(1, S, D)
```

```python
import math

import jax
import jax.numpy as jnp
import jax.experimental.pallas as pl
import jax.experimental.pallas.tpu as pltpu

S = 2048
D = 576
HQ = 32
HKV = 16
REP = HQ // HKV
DH = 128
GW = REP * DH
F = 4608
C = 8
EPS = 1e-05
TQ = 512
NBLK = S // TQ
TPB = TQ // 128
NT = S // 128
NU = NBLK * HKV
NP = HKV // 2
NC = 3
DC = D // NC
PG = 64
NFB = F // 128
WD0 = 14
DA = 2 * D
MODA = ((0, 4, 5), (1, 2, 6), (3, 7, 8))
NMB = 4 * D // 128
MPI = 3
MB0 = 1
DM = 512
KR = D - DM
NV = 3
CH = 3
TPI = KR // NP

SC, WC = 1024, 1024 + 2 * S
OUTER0, OSTEP = (SC + 850, SC + 0), (133, 135)
PACE = (SC + 100, WC + 250, 0, SC + 3400)
XP = (WC + 804, SC + 100, SC + 900, SC + 1340, WC + 762, SC + 500, SC + 2600)
TAB = ((SC + 1600, SC + 2760), (SC + 2950, SC + 3890), (WC + 650, WC + 890))
WFP = ((300, 900), (WC + 700, WC + 1144))
KP = (0, 616)
SLAG = 160
GS = 4
GT = (16, 32, 32)
LS = (256, 192)
TSPLIT = 15
PP = (24, 1824, 5112, 0, 0, 500, 800, 3574, 300)
TLAG = 256
TKS = 18
SCLAG = 2

BF16 = jnp.bfloat16
F32 = jnp.float32
U32 = jnp.uint32
QSCALE = DH ** -0.5 * math.log2(math.e)


def _dot(a, b):
    return jnp.dot(a, b, preferred_element_type=F32)


def _r(x):
    return x.astype(BF16).astype(F32)


def _col_bcast(row):
    return jnp.broadcast_to(row, (128, 128)).T


def _blk(u):
    return u // HKV if isinstance(u, int) else jax.lax.shift_right_logical(u, 4)


def _grp(u):
    return u % HKV if isinstance(u, int) else jnp.bitwise_and(u, HKV - 1)


def _lanes(t, n=1):
    return pl.ds(pl.multiple_of(t * 128, 128), n * 128)


def _paced(x, clock, pos):
    if clock is None:
        return x
    pos = pos // 8 * 8
    g = clock[pos:pos + x.shape[0], 0:x.shape[1]]
    return jnp.where(g * g < 0.0, jnp.zeros_like(x), x)


def _paced_wide(x, clock, pos):
    if clock is None:
        return x
    n, w = x.shape
    cols = []
    for a in range(0, w, 128):
        p0 = (pos + a // 128 * n) // 8 * 8
        g = jnp.concatenate([clock[p0 + r // (8 * GS) * (8 * GS):p0 + r // (8 * GS) * (8 * GS) + 8]
                             for r in range(0, n, 8)], axis=0)
        cols.append(_paced(x[:, a:min(a + 128, w)], g, 0))
    return jnp.concatenate(cols, axis=1)


def _gated(x, gates, j, n):
    if gates is None:
        return x
    m = x.shape[0]
    g = jnp.stack([gates[(j * m + b) * len(gates) // (n * m)] for b in range(m)])
    return jnp.where(g < 0.0, jnp.zeros_like(x), x)


def _softmax_numer(s, m):
    n, w = s.shape
    p = jnp.exp2(s - m).reshape(n // PG, PG // 8, 8, w)
    ts = jnp.sum(p, axis=1)
    last = jnp.where(ts < 0.0, ts, p[:, PG // 8 - 1])
    p = jnp.concatenate([p[:, :PG // 8 - 1], last[:, None]], axis=1).reshape(n, w)
    l = jnp.sum(jnp.sum(ts, axis=0), axis=0, keepdims=True)
    return p.astype(BF16), l


KEY0 = 0x20000000


def _score_key(r, t):
    tok = t * 128 + jax.lax.broadcasted_iota(jnp.int32, r.shape, 1)
    bits = jax.lax.shift_right_arithmetic(pltpu.bitcast(_r(r), jnp.int32), 16)
    code = jnp.where(bits < 0, -32768 - bits, bits) + 32768
    return pltpu.bitcast(code * S + (S - 1 - tok) + KEY0, F32)


def _chunk_stats(x):
    m = jnp.sum(x, axis=0, keepdims=True) * (1.0 / DC)
    xc = x - m
    return m, jnp.sum(xc * xc, axis=0, keepdims=True)


def _mean_var(stats):
    mean = sum(m for m, _ in stats) * (1.0 / NC)
    var = sum(s + DC * (m - mean) * (m - mean) for m, s in stats) * (1.0 / D)
    return mean, var


def _kernel_flat(*refs):
    _kernel(*refs[:12], *refs[12 + NV:], *refs[12:12 + NV])


def _kernel(wr_hbm, c_hbm,
            xt_hbm, k_hbm, v_hbm, wq_hbm, wot_hbm, wmod_hbm, wg_hbm, wu_hbm, wdt_hbm,
            out_hbm,
            xw_v, k_v, v_v, wq_v, wot_v, wmod_v, wg_v, wu_v, wd_ref,
            hh_ref, hr_ref, acc_ref, mod_ref, wrb_ref, scb_ref, x1_ref, h2row_ref, out_v, fix_v,
            key_ref, st1_ref, st2_ref, lm_ref,
            wrem_v,
            s0_ref, m0_ref, vt0_ref, wqt0_ref, qr0_ref, wf0_ref, kp0_ref,
            s1_ref, m1_ref, vt1_ref, wqt1_ref, qr1_ref, wf1_ref, kp1_ref,
            wr_ref, c_ref, bsem, msem, osem, *hb_refs):
    streams = ((s0_ref, m0_ref, vt0_ref, wqt0_ref, qr0_ref, wf0_ref, kp0_ref),
               (s1_ref, m1_ref, vt1_ref, wqt1_ref, qr1_ref, wf1_ref, kp1_ref))

    cp_k = lambda p, sem: pltpu.make_async_copy(
        k_hbm.at[pl.ds(2 * p, 2)], k_v.at[pl.ds(2 * p, 2)], sem)
    cp_v1 = lambda g, sem: pltpu.make_async_copy(v_hbm.at[g], v_v.at[g], sem)
    cp_k1 = lambda g, sem: pltpu.make_async_copy(k_hbm.at[g], k_v.at[g], sem)

    class Both:
        def __init__(self, cps):
            self.cps = cps

        def start(self):
            for cp in self.cps:
                cp.start()

        def wait(self):
            for cp in self.cps:
                cp.wait()

    def cp_w1(src, dst, g, sem):
        return pltpu.make_async_copy(src.at[:, _lanes(g * REP, REP)], dst.at[g], sem)

    cp_wo = lambda p, sem: Both([cp_w1(wot_hbm, wot_v, 2 * p + a, sem) for a in range(2)])
    cp_x = lambda t0, n, sem: Both([pltpu.make_async_copy(xt_hbm.at[:, _lanes(t0 + t)],
                                                          xw_v.at[t0 + t], sem) for t in range(n)])

    cp_wrem = lambda a, b, sem: pltpu.make_async_copy(
        wq_hbm.at[DM:, a * GW:b * GW], wrem_v.at[:, a * GW:b * GW], sem)

    def bundle(n, act):
        sem = bsem.at[n if isinstance(n, int) else jnp.minimum(n, NP - 1)]

        def on(cond, cps):
            def go():
                for cp in cps():
                    getattr(cp, act)()
            if isinstance(cond, bool):
                if cond:
                    go()
            else:
                pl.when(cond)(go)
        on(n + 1 < NP, lambda: [cp_k(n + 1, sem), cp_v1(2 * n + 2, sem), cp_w1(wq_hbm, wq_v, 2 * n + 3, sem)])
        on(n + 2 < NP, lambda: [cp_w1(wq_hbm, wq_v, 2 * n + 4, sem)])
        XN = 3
        nx = (NT - TPB - NV) // XN
        on(jnp.logical_and(n >= 1, n <= nx) if not isinstance(n, int) else 1 <= n <= nx,
           lambda: [cp_x(TPB + NV + XN * (n - 1), XN, sem)])
        on(n < NP, lambda: [cp_v1(2 * n + 1, sem), cp_wo(n, sem)])
        if act == 'wait' or isinstance(n, int):
            on(n == 1, lambda: [cp_wrem(8, HKV, sem), cp_wrem(0, 2, sem)])

    cp_moda = [Both([pltpu.make_async_copy(wmod_hbm.at[:, _lanes(t)], wmod_v.at[:, _lanes(t)],
                                           msem.at[s]) for t in tiles])
               for s, tiles in zip((0, 6, 10), MODA)]
    cp_modb = Both([pltpu.make_async_copy(wmod_hbm.at[:, _lanes(DA // 128 + b)],
                                          xw_v.at[NT + NFB + b], msem.at[1]) for b in range(NMB)])
    cp_g = pltpu.make_async_copy(wg_hbm, wg_v, msem.at[2])
    cp_u = pltpu.make_async_copy(wu_hbm, wu_v, msem.at[3])
    cp_d = Both([pltpu.make_async_copy(wdt_hbm.at[:, _lanes(b)], xw_v.at[NT + b], msem.at[4])
                 for b in range(NFB)])
    cp_out = lambda t, n, sem: Both([pltpu.make_async_copy(out_v.at[t + a], out_hbm.at[:, _lanes(t + a)],
                                                           sem) for a in range(n)])

    def silu_c():
        c = c_ref[...].astype(F32)
        return _r(c * _r(jax.nn.sigmoid(c)))

    def finish_mod(mod, lo, clock=None, pos=0):
        mod = _r(mod)
        col = lo + jax.lax.broadcasted_iota(jnp.int32, mod.shape, 1)
        is_scale = jnp.logical_or(jnp.logical_and(col >= D, col < 2 * D),
                                  jnp.logical_and(col >= 4 * D, col < 5 * D))
        mod = jnp.where(is_scale, _r(1.0 + mod), mod)
        for t in range(mod.shape[1] // 128):
            rows = pl.ds(pl.multiple_of(lo + t * 128, 128), 128)
            mod_ref[rows, :] = _paced(_col_bcast(mod[:, t * 128:(t + 1) * 128]), clock, pos)

    def late_mod_sums(n, clock):
        b0 = jnp.clip(n - MB0, 0, NMB // MPI - 1) * MPI
        for k in range(MPI):
            w = xw_v[jnp.where(n >= MB0, NT + NFB + b0 + k, 0)].astype(F32)
            part = jnp.sum((w * scb_ref[0:D, :]).reshape(D // 8, 8, 128), axis=0)
            lm_ref[k] = _paced(part, clock, PACE[2] + LS[1] * k)

    def late_mod_store(n, sums, clock):
        b0 = jnp.clip(n - MB0, 0, NMB // MPI - 1) * MPI
        for k in range(MPI):
            finish_mod(jnp.sum(sums[k], axis=0, keepdims=True), DA + (b0 + k) * 128,
                       clock, XP[4] + 128 * k)

    def col_vector(ref, row):
        row = jnp.concatenate([row, jnp.zeros((1, 64), F32)], axis=1)
        for t in range(5):
            ref[t * 128:(t + 1) * 128, :] = _col_bcast(row[:, t * 128:(t + 1) * 128])

    def mod(k):
        return mod_ref[k * D:(k + 1) * D, :]

    def put_stats(st_ref, t, shift, scale, clock, pos):
        row = jax.lax.broadcasted_iota(jnp.int32, (8, 128), 0)
        st_ref[t] = _paced(jnp.where(row == 0, shift, scale), clock, pos)

    def ln1_stats(t, clock=None, pos=0):
        for c in range(NC):
            m, s = _chunk_stats(xw_v[t, c * DC:(c + 1) * DC, :].astype(F32))
            put_stats(st1_ref, t * NC + c, m, s, clock, pos + LS[0] * c)

    def ln1_norm(t):
        mean, inv = ln2_norm(load_stats(st1_ref, t))
        return (xw_v[t].astype(F32) - mean) * inv

    def ln1_apply(t, clock=None, pos=0, ln=None):
        h = (ln1_norm(t) if ln is None else ln) * mod(1) + mod(0)
        h = _paced(h, clock, pos)
        hh_ref[t] = pltpu.bitcast(h.astype(BF16), U32)
        hr_ref[t] = h[DM:]

    def h2_rows(t, clock=None):
        x = _paced_wide(pltpu.bitcast(pltpu.bitcast(hh_ref[NT + t], BF16).T, U32), clock, PACE[3])
        h2row_ref[pl.ds(pl.multiple_of(t * 64, 64), 64), :] = x

    def router_terms():
        u = mod(4) * wrb_ref[0:D, :]
        return (u, jnp.sum(u, axis=0, keepdims=True),
                jnp.sum(mod(3) * wrb_ref[0:D, :], axis=0, keepdims=True))

    def load_stats(st_ref, t):
        return [(st_ref[t * NC + c, 0:1, :], st_ref[t * NC + c, 1:2, :]) for c in range(NC)]

    def ln2_x1(t, attn, clock=None):
        x1 = _r(xw_v[t].astype(F32) + mod(2) * attn)
        x1_ref[t] = _paced(x1, clock, PACE[0]).astype(BF16)
        return x1, [_chunk_stats(x1[c * DC:(c + 1) * DC]) for c in range(NC)]

    def ln2_norm(stats):
        mean, var = _mean_var(stats)
        return _r(mean), 1.0 / _r(jnp.sqrt(_r(_r(var) + EPS)))

    def ln2_h2(x1, mean, inv):
        return (x1 - mean) * inv * mod(4) + mod(3)

    def ln2_stats(t, clock):
        for c, (m, s) in enumerate(ln2_x1(t, acc_ref[t], clock)[1]):
            put_stats(st2_ref, t * NC + c, m, s, clock, PACE[0] + (c + 1) * DC + SLAG)

    def ln_apply(t, second, clock):
        x1 = x1_ref[t].astype(F32)
        mean, inv = ln2_norm(load_stats(st2_ref, t))
        rows = lambda k: mod_ref[pl.ds(pl.multiple_of((3 * second + k) * D, 8), D), :]
        h = (x1 - mean) * inv * rows(1) + rows(0)
        key = _score_key(jnp.sum(h * wrb_ref[0:D, :], axis=0, keepdims=True), t)
        key_ref[pl.ds(t, 1), :] = _paced(key, clock, PACE[1] + D + 96)
        h = _r(h)
        hp = _paced(h, clock, PACE[1])
        hh_ref[second * NT + t] = pltpu.bitcast(hp.astype(BF16), U32)
        hr_ref[jnp.where(second == 1, NT, t)] = hp[DM:]
        out_v[t] = _paced(x1 + mod(5) * h, clock, PACE[1] + 16).astype(BF16)

    def finish_q(q):
        q = (q * QSCALE).astype(BF16)
        return jnp.concatenate([q[r * DH:(r + 1) * DH] for r in range(REP)], axis=1)

    def q_proj(u, wqt_ref, qr_ref=None, split=False):
        w = pltpu.bitcast(wqt_ref[...], BF16)
        h = jnp.concatenate([pltpu.bitcast(hh_ref[_blk(u) * TPB + t], BF16) for t in range(TPB)], axis=1)
        if split:
            return sum(_dot(w[:, a:min(a + 128, D)], h[a:min(a + 128, D)]) for a in range(0, D, 128))
        if qr_ref is None:
            rem = _dot(w[:, DM:], h[DM:])
        else:
            rem = [qr_ref[...].T]
            if NV < TPB:
                R = GW * (TPB - NV) // 4
                rem.append(jnp.concatenate([_dot(w[a:a + R, DM:], h[DM:, NV * 128:])
                                            for a in range(0, GW, R)], axis=0))
            rem = jnp.concatenate(rem, axis=1)
        return _dot(w[:, :DM], h[:DM]) + rem

    def w_rest(u, wf_ref, gates=None):
        w = wrem_v[:, _lanes(_grp(u) * REP, REP)].astype(F32)
        for r in range(REP):
            wb = jnp.stack([jnp.broadcast_to(w[k:k + 1, r * DH:(r + 1) * DH], (8, DH))
                            for k in range(KR)])
            wf_ref[r] = _gated(wb, gates, r, REP)

    def outer(u, qr_ref, wf_ref, clock, start, step):
        base = jnp.bitwise_and(_blk(u), 1) * 16
        for g in range(0, NV * REP * 16, CH):
            pos = min(start + step * (g // CH + 1), clock.shape[0] - 8)
            runs, c = [], g
            while c < min(g + CH, NV * REP * 16):
                runs.append((c // 32, c // 16 % 2, c % 16, min(g + CH - c, 16 - c % 16)))
                c += runs[-1][3]
            acc = {}
            for k in range(KR):
                for i, r, tv, n in runs:
                    t = hb_refs[i][pl.ds(base + tv, n), k] * wf_ref[r, k][None]
                    acc[i, r] = t if k == 0 else acc[i, r] + t
            for i, r, tv, n in runs:
                gate = jnp.concatenate([clock[pos // 8 * 8:pos // 8 * 8 + 8]] * n, axis=0)
                row = i * 128 + tv * 8
                qr_ref[row:row + 8 * n, r * DH:(r + 1) * DH] = _paced(
                    acc[i, r].reshape(8 * n, DH), gate, 0)

    def h_table(hr, i, base, k0, gates):
        nk = hr.shape[0]
        hr = _r(hr)
        for j in range(nk):
            cb = _col_bcast(hr[j:j + 1]).reshape(16, 8, 128)
            hb_refs[i][pl.ds(base, 16), k0 + j] = _gated(cb, gates, j, nk)

    def never_of(clock, lo, hi, step=8):
        return [clock[a:a + 8] * clock[a:a + 8] for a in range(lo // 8 * 8, hi, step)]

    def scores(u, q, s_ref, m_ref, kp_ref=None, qclk=None):
        def keep(s, cols):
            s_ref[:, cols] = s
            m_ref[:, cols] = jnp.broadcast_to(jnp.max(s, axis=0, keepdims=True), (8, s.shape[1]))
            return s

        if kp_ref is None:
            s = jnp.concatenate([keep(_dot(k_v[_grp(u)], q[:, c]), c)
                                 for c in (slice(0, TQ), slice(TQ, 2 * TQ))], axis=1)
        else:
            k = pltpu.bitcast(k_v[_grp(u)], U32).reshape(S // 16, 8, DH)
            z = 0 if isinstance(u, int) else jax.lax.shift_right_logical(u, 8)
            kp_ref[z] = _gated(k, never_of(qclk, *KP, GT[2]), 0, 1).reshape(S // 2, DH)
            s = keep(_dot(pltpu.bitcast(kp_ref[0], BF16), q), slice(0, 2 * TQ))
        return jnp.concatenate([s[:, 0:128], s[:, TQ:TQ + 128]], axis=0)

    def q_clock(q):
        return jnp.concatenate([q[:, t * 128:(t + 1) * 128] for t in range(TPB)], axis=0)

    def v_transpose(u, vt_ref, clock=None, pos=0):
        vt_ref[...] = _paced_wide(pltpu.bitcast(v_v[_grp(u)].T, U32), clock, pos)

    def wq_transpose(u, wqt_ref, clock=None, pos=0):
        wqt_ref[...] = _paced_wide(pltpu.bitcast(wq_v[_grp(u)].T, U32), clock, pos)

    def wd_transpose(u, clock, pos):
        fb = jnp.clip(u - WD0, 0, NFB - 1)
        src = jnp.where(u >= WD0, NT + fb, 0)
        wd_ref[pl.ds(pl.multiple_of(fb * 64, 64), 64), :] = _paced_wide(
            pltpu.bitcast(xw_v[src].T, U32), clock, pos)

    def attend(s_ref, m_ref, vt_ref):
        m = m_ref[0:1, :]
        o = []
        for r in range(REP):
            cols = slice(r * TQ, (r + 1) * TQ)
            p, l = _softmax_numer(s_ref[:, cols], m[:, cols])
            o.append((_dot(pltpu.bitcast(vt_ref[...], BF16), p) * (1.0 / l)))
        return jnp.concatenate(o, axis=0)

    small = Both([pltpu.make_async_copy(wr_hbm, wr_ref, msem.at[7]),
                  pltpu.make_async_copy(c_hbm, c_ref, msem.at[7])])
    zeroth = Both([cp_x(0, TPB, msem.at[5]), cp_w1(wq_hbm, wq_v, 0, msem.at[5])])
    first = Both([cp_k1(0, msem.at[8]), cp_w1(wq_hbm, wq_v, 1, msem.at[8])])
    second = Both([cp_k1(1, msem.at[9]), cp_v1(0, msem.at[9]), cp_w1(wq_hbm, wq_v, 2, msem.at[9]),
                   cp_wrem(2, 8, msem.at[9]), cp_x(TPB, NV, msem.at[9])])
    for cp in [small, zeroth] + cp_moda + [first, second]:
        cp.start()
    acc_ref[...] = jnp.zeros_like(acc_ref)
    mod_ref[DA:6 * D, :] = jnp.zeros((4 * D, 128), F32)
    hh_ref[NT] = jnp.zeros((D // 2, 128), U32)
    lm_ref[...] = jnp.zeros_like(lm_ref)
    small.wait()
    col_vector(wrb_ref, wr_ref[...].astype(F32).reshape(1, D))
    col_vector(scb_ref, silu_c())
    sc8 = jnp.broadcast_to(silu_c(), (8, D)).astype(BF16)
    zeroth.wait()
    ln0 = []
    for t in range(TPB):
        ln1_stats(t)
        ln0.append(ln1_norm(t))
    wq_transpose(0, wqt0_ref)
    for cp, tiles in zip(cp_moda, MODA):
        cp.wait()
        for t in tiles:
            finish_mod(_dot(sc8, wmod_v[:, t * 128:(t + 1) * 128])[0:1], t * 128)
    for t in range(TPB):
        ln1_apply(t, ln=ln0[t])
    q = finish_q(q_proj(0, wqt0_ref, split=True))
    first.wait()
    bundle(0, 'start')
    jobs = ([(i, 0, k) for i in range(NV) for k in range(0, KR, TPI)]
            + [(i, 1, k) for i in range(NV) for k in range(0, 2 * TPI, TPI)])

    def first_table(gates, todo, starts=None):
        for j, (i, blk, k0) in enumerate(todo):
            hr = hr_ref[blk * TPB + i, k0:k0 + TPI, :]
            if starts is not None:
                hr = jnp.where(starts[j * len(starts) // len(todo)] < 0.0, 0.0, hr)
            h_table(hr, i, blk * 16, k0,
                    gates[j * len(gates) // len(todo):(j + 1) * len(gates) // len(todo)])

    first_table(never_of(scores(0, q, s0_ref, m0_ref), 64, 2 * S - 192, 16), jobs[:TSPLIT])
    wq_transpose(1, wqt1_ref)
    second.wait()
    bundle(1, 'start')
    cp_modb.start()
    q = q_proj(1, wqt1_ref)
    hrem = jnp.concatenate([pltpu.bitcast(hh_ref[t, DM // 2:, :], BF16) for t in range(NV)], axis=1)
    for a in range(2):
        streams[a][4][...] = jax.lax.dot_general(
            hrem, wrem_v[:, (a + 2) * GW:(a + 3) * GW], (((0,), (0,)), ((), ())),
            preferred_element_type=F32)
    clock = jnp.concatenate(
        [q_clock(q), scores(1, finish_q(q), s1_ref, m1_ref)], axis=0)
    nb0 = NV * KR // TPI
    v_transpose(0, vt0_ref, clock, PP[3])
    wq_transpose(2, wqt0_ref, clock, PP[4])
    first_table(never_of(clock, PP[6], PP[7], 16), jobs[TSPLIT:nb0])
    for i in range(NV):
        ln1_stats(TPB + i, clock, PP[0] + PP[5] * i)
        ln1_apply(TPB + i, clock, PP[1] + PP[5] * i)
    first_table(never_of(clock, PP[7], PP[2], 16), jobs[nb0:],
                never_of(clock, PP[7] - PP[8], PP[2] - PP[8]))
    for a in range(2):
        w_rest(a + 4, streams[a][5], never_of(clock, 500 * a, 500 * a + 500, 32))

    def unit(u, side, s_ref, m_ref, vt_ref, wqt_ref, qr_ref, wf_ref, kp_ref):
        q = q_proj(u + 2, wqt_ref, qr_ref)
        o = attend(s_ref, m_ref, vt_ref)
        sclk = scores(u + 2, finish_q(q), s_ref, m_ref, kp_ref, q_clock(q))
        o = jnp.concatenate([o[r * DH:(r + 1) * DH].astype(BF16) for r in range(REP)], axis=0)
        upd = _dot(wot_v[_grp(u)], o)
        clock = jnp.concatenate([q_clock(q), sclk, upd[:, 0:128], upd[:, 256:384]], axis=0)
        side(clock, lambda a: outer(u + 4, qr_ref, wf_ref, clock, OUTER0[a], OSTEP[a]))
        for t in range(TPB):
            acc_ref[_blk(u) * TPB + t] += upd[:, t * 128:(t + 1) * 128]

    def step(n, carry):
        bundle(jnp.minimum(n + 2, NP), 'start')
        for a in range(3):
            pl.when(n == 2 + a)(Both(cp_d.cps[a * NFB // 3:(a + 1) * NFB // 3]).start)
        pl.when(n == NP)(Both([cp_g, cp_u]).start)

        v = jnp.maximum(n - NP, 0)
        tile2 = lambda v: (jax.lax.shift_right_logical(v, 3) * TPB
                           + jnp.minimum(jnp.bitwise_and(v, NP - 1), TPB - 1))
        first = jnp.logical_or(n < NP, jnp.logical_and(n >= NP + TPB, n < 2 * NP))
        second = jnp.where(first, 0, 1)
        tile = jnp.where(first, jnp.minimum(jnp.where(n < NP, n, n - TPB) + TPB + NV - 1, NT - 1),
                         tile2(v))
        sums = lm_ref[...]

        def stats(clock, outer_at):
            v_transpose(2 * n + 1, vt1_ref, clock, XP[5])
            wq_transpose(2 * n + 3, wqt1_ref, clock, XP[6])
            ln2_stats(tile, clock)
            h2_rows(tile2(jnp.maximum(v - 1, 0)), clock)
            wd_transpose(2 * n, clock, XP[0])
            outer_at(0)

        def apply(clock, outer_at):
            blk = jnp.minimum(jax.lax.shift_right_logical(n + 2, 3) + 1, NBLK - 1)
            k0 = jnp.bitwise_and(n + 2, 7) * TPI
            hr = [hr_ref[blk * TPB + i, pl.ds(pl.multiple_of(k0, TPI), TPI), :]
                  for i in range(NV)]
            v_transpose(2 * n + 2, vt0_ref, clock, XP[1])
            wq_transpose(2 * n + 4, wqt0_ref, clock, XP[2])
            wd_transpose(2 * n + 1, clock, XP[3])
            late_mod_sums(n, clock)
            ln_apply(tile, second, clock)
            outer_at(1)
            for i in range(NV):
                h_table(hr[i], i, jnp.bitwise_and(blk, 1) * 16, k0, never_of(clock, *TAB[i], GT[0]))
            late_mod_store(n - 1, sums, clock)
            for a in range(2):
                w_rest(2 * n + 6 + a, streams[a][5], never_of(clock, *WFP[a], GT[1]))

        for a in range(2):
            unit(2 * n + a, (stats, apply)[a], *streams[a])
        return carry

    def stage(n, carry):
        bundle(n, 'wait')
        pl.when(n == MB0)(cp_modb.wait)
        pl.when(n == WD0 // 2)(cp_d.wait)
        return jax.lax.fori_loop(n, jnp.where(n < NP - 1, n + 1, NU // 2 - 1), step, carry)

    jax.lax.fori_loop(0, NP, stage, 0)

    T0 = NT - TPB
    cp_out(0, T0, osem.at[C + TPB]).start()
    cp_g.wait()
    v_transpose(NU - 1, vt1_ref)
    o = jnp.concatenate([attend(*streams[a][0:3]) for a in range(2)], axis=0)
    wlast = jnp.concatenate([wot_v[HKV - 2], wot_v[HKV - 1]], axis=1)
    fin = [acc_ref[T0 + t] + _dot(wlast, o[:, t * 128:(t + 1) * 128].astype(BF16)) for t in range(TPB)]
    clock = jnp.concatenate(fin, axis=0)
    row8 = jax.lax.broadcasted_iota(jnp.int32, (C, 128), 0)
    lane8 = jax.lax.broadcasted_iota(jnp.int32, (C, 128), 1)
    work = key_ref[0:T0, :]
    lead = jnp.zeros((C, 128), F32)
    for t in range(C):
        mx = jnp.max(jnp.max(work, axis=0, keepdims=True), axis=1, keepdims=True)
        work = jnp.where(work == mx, 0.0, work)
        lead = jnp.where(row8 == t, mx, lead)

    def spread(row):
        return pltpu.roll(jnp.broadcast_to(row, (128, 128)), 0, 1, stride=1, stride_axis=0)

    def merge(lead, rows, spreads):
        cols = jnp.concatenate([lead] + spreads, axis=0)
        best = jnp.zeros((C, 128), F32)
        for row in [jnp.max(jnp.where(row8 == lane8, lead, 0.0), axis=0, keepdims=True)] + rows:
            rank = jnp.sum(jnp.where(cols > row, 1.0, 0.0), axis=0, keepdims=True)
            best = jnp.maximum(best, jnp.where(rank == row8.astype(F32), row, 0.0))
        return jnp.max(best, axis=1, keepdims=True)

    def tail_h2(t, norm, gate=None):
        x1 = x1_ref[t].astype(F32)
        if gate is not None:
            n = gate.shape[0]
            x1 = jnp.concatenate([_paced(x1[:n], gate, 0), x1[n:]], axis=0) if n < D else _paced(x1, gate, 0)
        hh_ref[NT + t] = pltpu.bitcast(ln2_h2(x1, *norm).astype(BF16), U32)
        if t < NT - 2:
            h2_rows(t)

    u_vec, u_sum, b_sum = router_terms()
    keys = []
    for t in range(TPB):
        x1, stats = ln2_x1(T0 + t, fin[t])
        mean, inv = norm = ln2_norm(stats)
        r = (jnp.sum(x1 * u_vec, axis=0, keepdims=True) - mean * u_sum) * inv + b_sum
        keys.append(_score_key(r, T0 + t))
        if t < TPB - 1:
            tail_h2(T0 + t, norm, clock[(t + 1) * D + TLAG:(t + 2) * D + TLAG])
    lead = jnp.broadcast_to(merge(lead, keys[0:2], [spread(k) for k in keys[0:2]]), (C, 128))
    spread2 = spread(keys[2])
    h2_rows(NT - 2)
    tail_h2(NT - 1, norm)
    h2_rows(NT - 1)
    sel = pltpu.bitcast(merge(lead, keys[2:4], [spread2, spread(keys[3])]), jnp.int32) - KEY0
    sel_tok = (S - 1) - (sel & (S - 1))
    toks = [sel_tok[t, 0] for t in range(C)]
    tiles = [jax.lax.shift_right_logical(tk, 7) for tk in toks]
    sel_code = jax.lax.shift_right_logical(sel, 11) - 32768
    sel_bits = jnp.where(sel_code < 0, -32768 - sel_code, sel_code)
    r_sel = pltpu.bitcast(jax.lax.shift_left(sel_bits, 16), F32)

    final = []
    for t in range(C):
        d = True
        for u in range(t + 1, C):
            d = jnp.logical_and(d, tiles[u] != tiles[t])
        final.append(d)

    words = jnp.concatenate([h2row_ref[pl.ds(jax.lax.shift_right_logical(toks[t], 1), 1), :]
                             for t in range(C)], axis=0)
    odd = jnp.bitwise_and(sel_tok, 1) == 1
    xs = pltpu.bitcast(jnp.where(odd, jnp.bitwise_and(words, jnp.uint32(0xFFFF0000)),
                                 jax.lax.shift_left(words, jnp.uint32(16))), F32)
    xs = xs.astype(BF16)

    def plain_out(t, ticks):
        gate = jnp.concatenate([ticks[a * len(ticks) // (D // 8)] for a in range(D // 8)], axis=0)
        x1 = _paced(x1_ref[t].astype(F32), gate, 0)
        out_v[t] = (x1 + mod(5) * pltpu.bitcast(hh_ref[NT + t], BF16).astype(F32)).astype(BF16)

    clean = []

    def send_clean(t):
        d = tiles[0] != t
        for a in range(1, C):
            d = jnp.logical_and(d, tiles[a] != t)
        clean.append(d)
        pl.when(d)(cp_out(t, 1, osem.at[C + t - T0]).start)

    cp_u.wait()
    cp_out(0, T0, osem.at[C + TPB]).wait()
    gpre = _dot(xs, wg_v[...])
    u = _dot(xs, wu_v[...])
    ticks = [z[:, a * 128:(a + 1) * 128] for z in (gpre, u) for a in range(NFB)]
    for t in range(TPB):
        plain_out(T0 + t, ticks[t * TKS:(t + 1) * TKS])
        send_clean(T0 + t)
    gpre, u = _r(gpre), _r(u)
    gact = _r(gpre * _r(jax.nn.sigmoid(gpre)))
    act = (gact * u).astype(BF16)
    gate_r = _r(jax.nn.sigmoid(r_sel))
    ohs = []
    for t in range(C):
        oh = jnp.where(sel_tok == tiles[t] * 128 + lane8, 1.0, 0.0)
        ohs.append(jnp.concatenate([oh, jnp.zeros((16 - C, 128), F32)], axis=0).astype(BF16))

    def cp_fix(t, lo, hi):
        return pltpu.make_async_copy(fix_v.at[t, lo:hi, :], out_hbm.at[lo:hi, _lanes(tiles[t])],
                                     osem.at[t])

    def guarded(cond, fn):
        if cond is True:
            fn()
        else:
            pl.when(cond)(fn)

    def scatter(j, yt, t):
        lo, hi = j * 128, min(j * 128 + 128, D)
        upd = jnp.concatenate([_dot(yt[a:a + 64], ohs[t]) for a in range(0, hi - lo, 64)], axis=0)
        fix_v[t, lo:hi, :] = (x1_ref[tiles[t], lo:hi, :].astype(F32) + mod_ref[5 * D + lo:5 * D + hi, :]
                              * (pltpu.bitcast(hh_ref[NT + tiles[t], lo // 2:hi // 2, :], BF16).astype(F32) + upd)).astype(BF16)
        guarded(final[t], cp_fix(t, lo, hi).start)

    NJ = (D + 127) // 128
    yts = []
    for j in range(NJ):
        lo, hi = j * 128, min(j * 128 + 128, D)
        FK = F // 4
        yk = []
        for a in range(4):
            w = pltpu.bitcast(wd_ref[a * FK // 2:(a + 1) * FK // 2, lo:hi], BF16)
            yk.append(_dot(act[:, a * FK:(a + 1) * FK], w))
            if j >= SCLAG:
                for t in (2 * a, 2 * a + 1):
                    scatter(j - SCLAG, yts[j - SCLAG], t)
        y = _r(sum(yk)) * gate_r
        yts.append(jnp.concatenate([y, jnp.zeros_like(y)], axis=0).astype(BF16).T)
    for j in range(NJ - SCLAG, NJ):
        for t in range(C):
            scatter(j, yts[j], t)
    for t in range(T0, NT):
        pl.when(clean[t - T0])(cp_out(t, 1, osem.at[C + t - T0]).wait)
    for t in range(C):
        guarded(final[t], cp_fix(t, 0, D).wait)


@jax.jit
def pallas_adaLN_cond__gqa_block_cached__moe_arch_mod__prompt_kernel(
    A_x: jax.Array,
    A_k_cache: jax.Array,
    A_v_cache: jax.Array,
    A_wq: jax.Array,
    A_wo: jax.Array,
    B_x: jax.Array,
    B_w_r: jax.Array,
    B_w_gate: jax.Array,
    B_w_up: jax.Array,
    B_w_down: jax.Array,
    c: jax.Array,
    w_mod: jax.Array,
):
    del B_x
    xt = A_x.reshape(S, D).T
    k = A_k_cache.reshape(HKV, S, DH)
    v = A_v_cache.reshape(HKV, S, DH)

    hbm = pl.BlockSpec(memory_space=pl.ANY)
    stream = [
        pltpu.VMEM((S, REP * TQ), F32),
        pltpu.VMEM((8, REP * TQ), F32),
        pltpu.VMEM((DH // 2, S), U32),
        pltpu.VMEM((GW // 2, D), U32),
        pltpu.VMEM((NV * 128, GW), F32),
        pltpu.VMEM((REP, KR, 8, DH), F32),
        pltpu.VMEM((1, S // 2, DH), U32),
    ]
    out = pl.pallas_call(
        _kernel_flat,
        in_specs=[hbm] * 11,
        out_specs=hbm,
        out_shape=jax.ShapeDtypeStruct((D, S), BF16),
        scratch_shapes=[pltpu.VMEM((2 * 16, KR, 8, 128), F32)] * NV + [
            pltpu.VMEM((NT + NFB + NMB, D, 128), BF16),
            pltpu.VMEM((HKV, S, DH), BF16),
            pltpu.VMEM((HKV, S, DH), BF16),
            pltpu.VMEM((HKV, D, GW), BF16),
            pltpu.VMEM((HKV, D, GW), BF16),
            pltpu.VMEM((D, DA), BF16),
            pltpu.VMEM((D, F), BF16),
            pltpu.VMEM((D, F), BF16),
            pltpu.VMEM((F // 2, D), U32),
            pltpu.VMEM((2 * NT, D // 2, 128), U32),
            pltpu.VMEM((NT + 1, KR, 128), F32),
            pltpu.VMEM((NT, D, 128), F32),
            pltpu.VMEM((6 * D, 128), F32),
            pltpu.VMEM((5 * 128, 128), F32),
            pltpu.VMEM((5 * 128, 128), F32),
            pltpu.VMEM((NT, D, 128), BF16),
            pltpu.VMEM((S // 2, D), U32),
            pltpu.VMEM((NT, D, 128), BF16),
            pltpu.VMEM((C, D, 128), BF16),
            pltpu.VMEM((NT, 128), F32),
            pltpu.VMEM((NT * NC, 8, 128), F32),
            pltpu.VMEM((NT * NC, 8, 128), F32),
            pltpu.VMEM((MPI, 8, 128), F32),
            pltpu.VMEM((KR, HQ * DH), BF16),
        ] + stream + stream + [
            pltpu.VMEM((D,), BF16),
            pltpu.VMEM((1, D), BF16),
            pltpu.SemaphoreType.DMA((HKV // 2,)),
            pltpu.SemaphoreType.DMA((11,)),
            pltpu.SemaphoreType.DMA((C + TPB + 1,)),
        ],
        compiler_params=pltpu.CompilerParams(vmem_limit_bytes=127 * 1024 * 1024,
                                             disable_bounds_checks=True,
                                             disable_semaphore_checks=True),
    )(B_w_r, c, xt, k, v, A_wq, A_wo.T, w_mod, B_w_gate, B_w_up, B_w_down.T)
    return out.T.reshape(1, S, D)
```
